```python
import jax
import jax.numpy as jnp

def _softmax(x, axis=-1):
    return jax.nn.softmax(x, axis=axis)

def _gelu(x):
    return jax.nn.gelu(x, approximate=True)

def _silu(x):
    return jax.nn.silu(x)

def _sigmoid(x):
    return jax.nn.sigmoid(x)

def _layernorm(x, axis=-1, eps=1e-05):
    m = jnp.mean(x, axis=axis, keepdims=True)
    v = jnp.var(x, axis=axis, keepdims=True)
    return (x - m) / jnp.sqrt(v + eps)

def _scatter_add(tgt, idx, src, axis=0):
    return tgt.at[idx].add(src)

def _segment_sum(src, seg, n):
    return jax.ops.segment_sum(src, seg, n)

class _Rng:

    def __init__(self, key):
        self._k = key

    def _next(self):
        self._k, sub = jax.random.split(self._k)
        return sub

    def normal(self, shape):
        return jax.random.normal(self._next(), shape, dtype=jnp.bfloat16)

    def randint(self, lo, hi, shape):
        return jax.random.randint(self._next(), shape, lo, hi, dtype=jnp.int32)

    def uniform(self, shape, lo=0.0, hi=1.0):
        return jax.random.uniform(self._next(), shape, jnp.bfloat16, lo, hi)

    def permutation(self, n):
        return jax.random.permutation(self._next(), n)
kernel_name = 'concat_heads__ssm_conv_h3__memory_aug_infini_attn__prompt'

def setup_inputs():
    _rng = _Rng(jax.random.key(int.from_bytes(__import__("os").urandom(4), "little")))
    _w = lambda a: (lambda t: t.astype(jnp.bfloat16) if jnp.issubdtype(t.dtype, jnp.floating) else t)(jnp.asarray(a))

    def _A_setup():
        B, S, D = (1, 2048, 640)
        ks = 4
        return {'q': _w((lambda *s: _rng.normal(s) * 0.05)(B, S, D)), 'k': _w((lambda *s: _rng.normal(s) * 0.05)(B, S, D)), 'v': _w((lambda *s: _rng.normal(s) * 0.05)(B, S, D)), 'shift_k': _w((lambda *s: _rng.normal(s) * 0.05)(D, ks) * 0.5), 'ssm_k': _w((lambda *s: _rng.normal(s) * 0.05)(D, S) * (1.0 / S ** 0.5)), 'ssm_D': _w((lambda *s: _rng.normal(s) * 0.05)(D))}
    _A_in = _A_setup()

    def _B_setup():
        B, S, D, H = (1, 2048, 640, 32)
        N = 4
        L = max(1, S // N)
        sc = D ** (-0.5)
        return {'x': _w((lambda *s: _rng.normal(s) * 0.05)(B, N * L, D)), 'wq': _w((lambda *s: _rng.normal(s) * 0.05)(D, D) * sc), 'wk': _w((lambda *s: _rng.normal(s) * 0.05)(D, D) * sc), 'wv': _w((lambda *s: _rng.normal(s) * 0.05)(D, D) * sc), 'wo': _w((lambda *s: _rng.normal(s) * 0.05)(D, D) * sc), 'beta': _w((lambda *s: _rng.normal(s) * 0.05)(H))}
    _B_in = _B_setup()
    return {'A_q': _A_in['q'], 'A_k': _A_in['k'], 'A_v': _A_in['v'], 'A_shift_k': _A_in['shift_k'], 'A_ssm_k': _A_in['ssm_k'], 'A_ssm_D': _A_in['ssm_D'], 'B_x': _B_in['x'], 'B_wq': _B_in['wq'], 'B_wk': _B_in['wk'], 'B_wv': _B_in['wv'], 'B_wo': _B_in['wo'], 'B_beta': _B_in['beta']}

def reference(A_q, A_k, A_v, A_shift_k, A_ssm_k, A_ssm_D, B_x, B_wq, B_wk, B_wv, B_wo, B_beta):

    def _A_ref(q, k, v, shift_k, ssm_k, ssm_D):
        B, S, D = q.shape
        ks = shift_k.shape[-1]
        k_pad = jnp.pad(k, ((0, 0), (ks - 1, 0), (0, 0)))
        k_shift = jnp.zeros_like(k)
        for t in range(ks):
            k_shift = k_shift + k_pad[:, t:t + S, :] * shift_k[:, ks - 1 - t][None, None, :]
        kv = k_shift * v
        L = 2 * S
        kv_pad = jnp.pad(kv, ((0, 0), (0, S), (0, 0)))
        kf_pad = jnp.pad(ssm_k, ((0, 0), (0, S)))
        kv_f = (lambda x, axes=(-2, -1): jnp.fft.rfft2(x.astype(jnp.float32), axes=axes))(kv_pad[:, None, :, :], axes=(1, 2))
        kf_f = (lambda x, axes=(-2, -1): jnp.fft.rfft2(x.astype(jnp.float32), axes=axes))(kf_pad[:, None, :], axes=(1, 2))
        kf_f = (lambda x, *d: x.transpose(*d))(kf_f, 1, 2, 0)
        y_f = kv_f * kf_f[None, :, :, :]
        y = (lambda x, s, axes=(-2, -1): jnp.fft.irfft2(x, s=s, axes=axes).astype(jnp.bfloat16))(y_f, (1, L), axes=(1, 2))[:, 0, :S, :]
        y = y + kv * ssm_D[None, None, :]
        return q * y

    def _B_ref(x, wq, wk, wv, wo, beta):
        B, S, D = x.shape
        H = 32
        Dh = D // H
        N = 4
        L = S // N
        q = (lambda x, *d: x.transpose(*d))((x @ wq).reshape(B, S, H, Dh), 0, 2, 1, 3).reshape(B, H, N, L, Dh)
        k = (lambda x, *d: x.transpose(*d))((x @ wk).reshape(B, S, H, Dh), 0, 2, 1, 3).reshape(B, H, N, L, Dh)
        v = (lambda x, *d: x.transpose(*d))((x @ wv).reshape(B, S, H, Dh), 0, 2, 1, 3).reshape(B, H, N, L, Dh)
        phi = lambda t: jnp.where(t > 0, t + 1.0, jnp.exp(t))
        scale = Dh ** (-0.5)
        ar = jnp.arange(L)
        mask = (lambda x, dt: x.astype(dt))(ar[:, None] < ar[None, :], x.dtype) * -1000000000.0
        g = _sigmoid(beta).reshape(1, H, 1, 1)
        M = jnp.einsum('bhd,bhe->bhde', q[:, :, 0, 0, :] * 0.0, q[:, :, 0, 0, :] * 0.0)
        z = q[:, :, 0, 0, :] * 0.0
        outs = []
        for s in range(N):
            qs, ks, vs = (q[:, :, s].copy(), k[:, :, s].copy(), v[:, :, s].copy())
            logits = jnp.einsum('bhqd,bhkd->bhqk', qs, ks) * scale + mask
            p = _softmax(logits, axis=-1)
            a_dot = jnp.einsum('bhqk,bhkd->bhqd', p, vs)
            pq = phi(qs)
            num = jnp.einsum('bhld,bhde->bhle', pq, M)
            den = jnp.einsum('bhld,bhd->bhl', pq, z)[..., None] + 1e-06
            a_mem = num / den
            o = g * a_mem + (1.0 - g) * a_dot
            outs.append(o)
            pk = phi(ks)
            M = M + jnp.einsum('bhld,bhle->bhde', pk, vs)
            z = z + jnp.einsum('bhld->bhd', pk)
        o = (lambda x, *d: x.transpose(*d))(jnp.stack(outs, 2).reshape(B, H, S, Dh), 0, 2, 1, 3).reshape(B, S, D)
        return o @ wo
    a = _A_ref(A_q, A_k, A_v, A_shift_k, A_ssm_k, A_ssm_D)
    b = _B_ref(B_x, B_wq, B_wk, B_wv, B_wo, B_beta)
    return jnp.concatenate([a, b], axis=-1)
```

```python
import math

import jax
import jax.numpy as jnp
import numpy as np
from jax import lax
from jax.experimental import pallas as pl
from jax.experimental.pallas import tpu as pltpu

S = 2048
D = 640
NT = D // 128
H = 32
DH = D // H
NSEG = 4
L = S // NSEG
KS = 4
N1, N2 = 128, 16

F32 = jnp.float32
BF16 = jnp.bfloat16
U32 = jnp.uint32
NN_DIMS = (((1,), (0,)), ((), ()))
NT_DIMS = (((1,), (1,)), ((), ()))
NEG = -1e30
LOG2E = 1.4426950408889634


def _dft_tables():
    n1 = np.arange(N1)
    k1 = np.arange(N1)
    fwd = np.zeros((N2, 2 * N1, N1), np.float64)
    inv = np.zeros((N2, N1, 2 * N1), np.float64)
    pos_re = (k1 // 8) * 16 + k1 % 8
    for n2 in range(N2):
        ang = 2.0 * np.pi * np.outer(k1 + 0.25, N2 * n1 + n2) / S
        c, s = np.cos(ang), np.sin(ang)
        fwd[n2, :N1] = c
        fwd[n2, N1:] = s
        inv[n2][:, pos_re] = c.T / S
        inv[n2][:, pos_re + 8] = s.T / S
    return fwd.astype(np.float32).astype(BF16), inv.astype(np.float32).astype(BF16)


_FWD, _INV = _dft_tables()


def _dot(a, b, dims=NN_DIMS):
    return lax.dot_general(a, b, dims, preferred_element_type=F32)


def _u32(x):
    return pltpu.bitcast(x, U32)


def _bf(x):
    return pltpu.bitcast(x, BF16)


def _lo(w):
    return pltpu.unpack_elementwise(w, index=0, packed_dtype=BF16, unpacked_dtype=F32)


def _hi(w):
    return pltpu.unpack_elementwise(w, index=1, packed_dtype=BF16, unpacked_dtype=F32)


def _radix4(x0, x1, x2, x3, sign):
    ar, ai = x0[0] + x2[0], x0[1] + x2[1]
    br, bi = x0[0] - x2[0], x0[1] - x2[1]
    cr, ci = x1[0] + x3[0], x1[1] + x3[1]
    dr, di = x1[0] - x3[0], x1[1] - x3[1]
    y0 = (ar + cr, ai + ci)
    y2 = (ar - cr, ai - ci)
    yp = (br - di, bi + dr)
    ym = (br + di, bi - dr)
    return (y0, yp, y2, ym) if sign > 0 else (y0, ym, y2, yp)


def _twiddle(x, e, sign):
    xr, xi = x
    if e == 0:
        return x
    if e == 4:
        return (-xi, xr) if sign > 0 else (xi, -xr)
    r = math.sqrt(0.5)
    if e == 2:
        return ((xr - xi) * r, (xr + xi) * r) if sign > 0 else ((xr + xi) * r, (xi - xr) * r)
    if e == 6:
        return ((xr + xi) * -r, (xr - xi) * r) if sign > 0 else ((xi - xr) * r, (xr + xi) * -r)
    c, s = math.cos(math.pi * e / 8), sign * math.sin(math.pi * e / 8)
    return (xr * c - xi * s, xr * s + xi * c)


def _radix4_tw(x0, x1, x2, x3, sign, b):
    if b != 2:
        return _radix4(x0, _twiddle(x1, b, sign), _twiddle(x2, 2 * b, sign),
                       _twiddle(x3, 3 * b, sign), sign)
    x1, x3 = _twiddle(x1, 2, sign), _twiddle(x3, 6, sign)
    if sign > 0:
        ar, ai = x0[0] - x2[1], x0[1] + x2[0]
        br, bi = x0[0] + x2[1], x0[1] - x2[0]
    else:
        ar, ai = x0[0] + x2[1], x0[1] - x2[0]
        br, bi = x0[0] - x2[1], x0[1] + x2[0]
    cr, ci = x1[0] + x3[0], x1[1] + x3[1]
    dr, di = x1[0] - x3[0], x1[1] - x3[1]
    y0 = (ar + cr, ai + ci)
    y2 = (ar - cr, ai - ci)
    yp = (br - di, bi + dr)
    ym = (br + di, bi - dr)
    return (y0, yp, y2, ym) if sign > 0 else (y0, ym, y2, yp)


def _interleave(*streams):
    live = [[g, n, 0] for g, n in streams]
    while live:
        cur = min(live, key=lambda e: (e[2] + 0.5) / e[1])
        try:
            next(cur[0])
            cur[2] += 1
        except StopIteration:
            live.remove(cur)


def _kernel(aq_hbm, ak_hbm, av_hbm, shift_ref, h_hbm, ssmd_ref, x_hbm, wq_hbm, wk_hbm,
            wv_hbm, wo_hbm, beta_ref, fwd_hbm, inv_hbm, out_hbm,
            xb, wqb, wkb, wvb, wob, wvt, hb, ht, kb, vb, qb, fwd, inv,
            kvf, gx, gh, hf, yb, outa, outb, wtab, gtab, cmask,
            q0, q1, k0, k1, pq0, pq1, pk0, pk1, ot0, ot1, mst, sems):
    qs, ks, pqs, pks, ots = (q0, q1), (k0, k1), (pq0, pq1), (pk0, pk1), (ot0, ot1)

    def col_tiles(src, dst, sem, rows=None, lead=(0,), dst_off=0, tiles=range(NT)):
        r0, n = rows if rows is not None else (0, src.shape[-2])

        def one(t):
            return lambda: pltpu.make_async_copy(
                src.at[(*lead, pl.ds(r0, n), pl.ds(128 * t, 128))],
                dst.at[t, pl.ds(dst_off + r0, n), :], sems.at[sem])
        return [one(t) for t in tiles]

    cp_x = [col_tiles(x_hbm, xb, s, rows=(L * s, L)) for s in range(NSEG)]
    cp_wq = col_tiles(wq_hbm, wqb, 4, lead=())
    cp_wk = col_tiles(wk_hbm, wkb, 5, lead=())
    cp_wv = col_tiles(wv_hbm, wvb, 6, lead=())
    cp_wo = col_tiles(wo_hbm, wob, 7, lead=())
    cp_h = [col_tiles(h_hbm, hb, 8 + i, lead=(), tiles=range(4 * i, 4 * i + 4)) for i in range(4)]
    cp_k = col_tiles(ak_hbm.bitcast(U32), kb, 12, dst_off=8)
    cp_v = col_tiles(av_hbm.bitcast(U32), vb, 13)
    cp_q = col_tiles(aq_hbm.bitcast(U32), qb, 14)
    cp_fwd = [lambda: pltpu.make_async_copy(fwd_hbm, fwd, sems.at[15])]
    cp_inv = [lambda: pltpu.make_async_copy(inv_hbm, inv, sems.at[16])]

    def out_a(c):
        c0 = 128 * c if isinstance(c, int) else pl.multiple_of(128 * c, 128)
        return lambda: pltpu.make_async_copy(
            outa.at[c], out_hbm.bitcast(U32).at[0, :, pl.ds(c0, 128)], sems.at[17])

    def out_b(s, n):
        return lambda: pltpu.make_async_copy(
            outb.at[n, pl.ds(L * s, L), :],
            out_hbm.at[0, pl.ds(L * s, L), pl.ds(D + 128 * n, 128)], sems.at[18])

    cp_oa = [out_a(c) for c in range(NT)]
    cp_ob = [[out_b(s, n) for n in range(NT)] for s in range(NSEG)]

    def start(*groups):
        for g in groups:
            for cp in g:
                cp().start()

    def wait(*groups):
        for g in groups:
            for cp in g:
                cp().wait()

    def rows(i, n):
        return pl.ds(pl.multiple_of(i * n, n), n) if not isinstance(i, int) else pl.ds(i * n, n)

    lane = lax.broadcasted_iota(jnp.int32, (8, 128), 1)
    sub = lax.broadcasted_iota(jnp.int32, (8, 128), 0)

    def lanes(n):
        return lax.broadcasted_iota(jnp.int32, (n, 128), 1)

    def qk_proj(s, i, want_pq, want_pk):
        p = s % 2
        tok = rows(4 * s + i, 128)
        for w_ref, dst, fdst, want, scale in (
                (wqb, qs[p], pqs[p], want_pq, DH ** -0.5 * LOG2E),
                (wkb, ks[p], pks[p], want_pk, None)):
            for n in range(NT):
                xt = jnp.concatenate([xb[c, tok, :] for c in range(NT)], axis=1)
                t = _dot(xt, w_ref[n])
                dst[n, rows(i, 128), :] = (t if scale is None else t * scale).astype(BF16)
                if want:
                    fdst[n, rows(i, 128), :] = jnp.where(t > 0, t + 1.0, jnp.exp(t)).astype(BF16)
                yield

    def out_proj(s, i):
        ot = ots[s % 2]
        o = jnp.concatenate([ot[i, 128 * c:128 * c + 128, :].T for c in range(NT)], axis=1)
        yield
        for n in range(NT):
            outb[n, rows(4 * s + i, 128), :] = _dot(o, wob[n]).astype(BF16)
            yield

    def tile_rows(r, n):
        return jnp.broadcast_to(r[None], (n // 8, 8, 128)).reshape(n, 128)

    def attention(s, i):
        p = s % 2
        vt = []
        for j in range(4):
            acc = None
            for c in range(NT):
                wrow = wvt[c, pl.ds(pl.multiple_of(160 * i, 160), 160), :]
                t = _dot(wrow, xb[c, L * s + 128 * j:L * s + 128 * j + 128, :], NT_DIMS)
                acc = t if acc is None else acc + t
            vt.append(acc)
            yield
        ones8 = jnp.ones((8, 128), F32)
        ones16 = jnp.ones((16, 128), BF16)
        for gi in range(2):
            g = 2 * i + gi
            t0 = (80 * g) // 128
            off = 80 * g - 128 * t0
            t1 = jnp.minimum(t0 + 1, NT - 1)
            rel = (lane - off) & 127
            hl = ((rel >= DH).astype(jnp.int32) + (rel >= 2 * DH).astype(jnp.int32)
                  + (rel >= 3 * DH).astype(jnp.int32) + (rel >= 4 * DH).astype(jnp.int32))

            def window(ref, j):
                a = _u32(ref[t0, 128 * j:128 * j + 128, :])
                b = _u32(ref[t1, 128 * j:128 * j + 128, :])
                return jnp.where(lanes(64) >= off, a, b)

            kw = [_bf(window(ks[p], j)) for j in range(4)]
            v80 = [v[80 * gi:80 * gi + 80] for v in vt]
            gate = gtab[g]
            amem = [None] * 4
            if s > 0:
                mem = mst[g].astype(BF16)
                for j in range(4):
                    r = _dot(mem, _bf(window(pqs[p], j)), NT_DIMS)
                    coef = gate / (r[80:88] + 1e-6)
                    cb = [jnp.broadcast_to(coef[a:a + 1], (8, 128)) for a in range(4)]
                    cols = []
                    for pr in range(2):
                        ca, cb_ = cb[2 * pr], cb[2 * pr + 1]
                        cols += [ca, ca, jnp.where(sub < 4, ca, cb_), cb_, cb_]
                    amem[j] = r[0:80] * jnp.concatenate(cols, axis=0)
                yield
            if s < NSEG - 1:
                acc = None
                for j in range(4):
                    lhs = jnp.concatenate([v80[j].astype(BF16), ones16], axis=0)
                    t = _dot(lhs, _bf(window(pks[p], j)))
                    acc = t if acc is None else acc + t
                keep = []
                for r in range(12):
                    row = sub + 8 * r
                    if r < 10:
                        hr = ((row >= DH).astype(jnp.int32) + (row >= 2 * DH).astype(jnp.int32)
                              + (row >= 3 * DH).astype(jnp.int32))
                    else:
                        hr = row - 80
                    keep.append(jnp.where(hr == hl, acc[8 * r:8 * r + 8], 0.0))
                upd = jnp.concatenate(keep, axis=0)
                mst[g] = upd if s == 0 else mst[g] + upd
                yield
            odot = [[None, None] for _ in range(4)]
            for pr in range(2):
                ma = jnp.where(hl == 2 * pr, np.uint32(0xFFFFFFFF), np.uint32(0))
                mb = jnp.where(hl == 2 * pr + 1, np.uint32(0xFFFFFFFF), np.uint32(0))
                va, vbb = [], []
                for j in range(4):
                    v40 = v80[j][40 * pr:40 * pr + 40]
                    va.append(jnp.concatenate([v40[0:24], ones8], axis=0).astype(BF16))
                    vbb.append(jnp.concatenate([v40[16:40], ones8], axis=0).astype(BF16))
                keep_a = 1.0 - jnp.broadcast_to(gate[2 * pr:2 * pr + 1], (8, 128))
                keep_b = 1.0 - jnp.broadcast_to(gate[2 * pr + 1:2 * pr + 2], (8, 128))
                for j in range(4):
                    qw = window(qs[p], j)
                    qa = qw & tile_rows(ma, 64)
                    qh = qw & tile_rows(mb, 64)
                    w_a = _bf(qa)
                    w_b = _bf(jnp.concatenate([qh[32:64], qh[0:32]], axis=0))
                    w_t = _bf(jnp.concatenate([qh[32:64], qa[32:64]], axis=0))
                    klhs = jnp.concatenate(kw[:j] + [kw[j][0:64]], axis=0)
                    n = 128 * j
                    s_a = _dot(klhs, w_a, NT_DIMS)
                    s_b = _dot(klhs, w_b, NT_DIMS)
                    s_t = _dot(kw[j][64:128], w_t, NT_DIMS) + cmask[2]
                    d_a = s_a[n:] + cmask[0]
                    d_b = s_b[n:] + cmask[1]
                    yield

                    def vmax(x):
                        m = x[0:8]
                        for r in range(1, x.shape[0] // 8):
                            m = jnp.maximum(m, x[8 * r:8 * r + 8])
                        return m

                    m_a, m_b, m_t = vmax(d_a), vmax(d_b), vmax(s_t)
                    if j:
                        m_a = jnp.maximum(m_a, vmax(s_a[:n]))
                        m_b = jnp.maximum(m_b, vmax(s_b[:n]))
                    m_a = jnp.maximum(m_a, jnp.where(lane >= 64, m_t, NEG))
                    m_b = jnp.maximum(m_b, jnp.where(lane < 64, m_t, NEG))
                    m_a = jnp.broadcast_to(jnp.max(m_a, axis=0, keepdims=True), (8, 128))
                    m_b = jnp.broadcast_to(jnp.max(m_b, axis=0, keepdims=True), (8, 128))
                    m_t = jnp.where(lane < 64, m_b, m_a)

                    def prob(x, m):
                        return jnp.exp2(x - tile_rows(m, x.shape[0])).astype(BF16)

                    p_t = _u32(prob(s_t, m_t))
                    hi_half = lanes(32) >= 64
                    p_ta = _bf(jnp.where(hi_half, p_t, np.uint32(0)))
                    p_tb = _bf(jnp.where(hi_half, np.uint32(0), p_t))
                    res = []
                    for s_x, d_x, m_x, p_tx, v_x in ((s_a, d_a, m_a, p_ta, va),
                                                     (s_b, d_b, m_b, p_tb, vbb)):
                        acc = _dot(v_x[j], jnp.concatenate([prob(d_x, m_x), p_tx], axis=0))
                        for kt in range(j):
                            acc = acc + _dot(v_x[kt], prob(s_x[128 * kt:128 * kt + 128], m_x))
                        res.append(acc)
                        yield
                    r_a = res[0]
                    r_b = pltpu.roll(res[1], 64, 1)
                    o_a = r_a[0:24] * tile_rows(keep_a / r_a[24:32], 24)
                    o_b = r_b[0:24] * tile_rows(keep_b / r_b[24:32], 24)
                    odot[j][pr] = jnp.concatenate(
                        [o_a[0:16], jnp.where(sub < 4, o_a[16:24], o_b[0:8]), o_b[8:24]], axis=0)
            for j in range(4):
                o = jnp.concatenate(odot[j], axis=0)
                if s > 0:
                    o = o + amem[j]
                ots[p][j, pl.ds(pl.multiple_of(80 * g, 80), 80), :] = o.astype(BF16)

    ATT_STEPS = lambda s: 4 + 2 * (24 + (s > 0) + (s < NSEG - 1))

    def h_transpose(i):
        for t in range(4):
            for c in range(NT):
                ht[c, rows(4 * i + t, 64), :] = _u32(hb[4 * i + t, 128 * c:128 * c + 128, :].T)
                yield

    def fwd_h(i):
        for c in range(NT):
            for jp in range(2):
                w = ht[c, pl.ds(2 * i + jp, N1, stride=8), :]
                for e, part in enumerate((_lo, _hi)):
                    n2 = 4 * i + 2 * jp + e
                    gh[c, n2] = _dot(fwd[n2], part(w).astype(BF16))
                    yield

    def fwd_x(i):
        for c in range(NT):
            taps = [wtab[c, j] for j in range(KS)]
            planes = [[] for _ in range(4)]
            for r in range(0, N1, 16):
                kw = [kb[c, pl.ds(8 * r + 6 + 2 * i + d, 16, stride=8), :] for d in range(4)]
                vw = [vb[c, pl.ds(8 * r + 2 * i + d, 16, stride=8), :] for d in range(2)]
                kp = [None, _hi(kw[0])] + [f(w) for w in kw[1:] for f in (_lo, _hi)]
                vp = [f(w) for w in vw for f in (_lo, _hi)]
                for e in range(4):
                    acc = kp[4 + e] * tile_rows(taps[0], 16)
                    for j in range(1, KS):
                        acc = acc + kp[4 + e - j] * tile_rows(taps[j], 16)
                    kv = acc * vp[e]
                    kvf[c, 4 * i + e, r:r + 16, :] = kv
                    planes[e].append(kv.astype(BF16))
                if r % 32 == 16:
                    yield
            for e in range(4):
                n2 = 4 * i + e
                gx[c, n2] = _dot(fwd[n2], jnp.concatenate(planes[e], axis=0))
                yield

    def spectrum(c, kblk):
        re, im = rows(kblk, 8), rows(N1 // 8 + kblk, 8)

        def first_pass(ref):
            t = [None] * 4
            for b in range(4):
                t[b] = _radix4(*[(ref[c, 4 * a + b, re, :], ref[c, 4 * a + b, im, :])
                                 for a in range(4)], 1)
                yield
            return t

        t = yield from first_pass(gh)
        for cc in range(4):
            z = _radix4_tw(*[t[b][cc] for b in range(4)], 1, cc)
            for d in range(4):
                hf[c, kblk, 2 * (cc + 4 * d)] = z[d][0]
                hf[c, kblk, 2 * (cc + 4 * d) + 1] = z[d][1]
            yield
        t = yield from first_pass(gx)
        u = [None] * 4
        for cc in range(4):
            z = _radix4_tw(*[t[b][cc] for b in range(4)], 1, cc)
            y = []
            for d in range(4):
                hr = hf[c, kblk, 2 * (cc + 4 * d)]
                hi = hf[c, kblk, 2 * (cc + 4 * d) + 1]
                y.append((z[d][0] * hr - z[d][1] * hi, z[d][0] * hi + z[d][1] * hr))
            yield
            u[cc] = _radix4(*y, -1)
            yield
        for b in range(4):
            z = _radix4_tw(*[u[cc][b] for cc in range(4)], -1, b)
            for a in range(4):
                yb[c, 4 * a + b, rows(kblk, 16), :] = jnp.concatenate(z[a], axis=0).astype(BF16)
            yield

    SPEC_STEPS = 24

    def spectra(cs, kblks):
        for c in cs:
            for kblk in kblks:
                yield from spectrum(c, kblk)

    def inverse(c):
        dvec = tile_rows(wtab[c, KS], N1)
        for jp in range(8):
            w = qb[c, pl.ds(jp, N1, stride=8), :]
            res = []
            for e, part in enumerate((_lo, _hi)):
                n2 = 2 * jp + e
                y = _dot(inv[n2], yb[c, n2])
                res.append(part(w) * (y + kvf[c, n2] * dvec))
            outa[c, pl.ds(jp, N1, stride=8), :] = pltpu.pack_elementwise(
                res, packed_dtype=BF16).astype(U32)
            yield

    start(cp_x[0], cp_wq)
    taps_t = shift_ref[...].astype(F32).T
    skip = ssmd_ref[...].astype(F32)
    for c in range(NT):
        for j in range(KS):
            wtab[c, j] = jnp.broadcast_to(taps_t[j:j + 1, 128 * c:128 * c + 128], (8, 128))
        wtab[c, KS] = jnp.broadcast_to(skip[:, 128 * c:128 * c + 128], (8, 128))
        kb[c, 0:8, :] = jnp.zeros((8, 128), U32)
    gates = jax.nn.sigmoid(beta_ref[...].astype(F32))
    gcol = jnp.broadcast_to(gates, (8, H)).T
    gcol = jnp.broadcast_to(gcol[:, 0:1], (H, 128))
    for g in range(8):
        gtab[g] = jnp.concatenate([gcol[4 * g:4 * g + 4]] * 2, axis=0)
    kk = lax.broadcasted_iota(jnp.int32, (64, 128), 0)
    ll = lax.broadcasted_iota(jnp.int32, (64, 128), 1)
    cmask[0] = jnp.where(kk <= ll, 0.0, NEG)
    cmask[1] = jnp.where((ll < 64) | (kk <= ll - 64), 0.0, NEG)
    cmask[2] = jnp.where(kk <= (ll & 63), 0.0, NEG)

    wait(cp_x[0], cp_wq)
    start(cp_wk, cp_wv, cp_x[1])
    wait(cp_wk)
    start(*cp_h)

    def prologue(i, carry):
        _interleave((qk_proj(0, i, False, True), 10))
        return carry

    lax.fori_loop(0, 4, prologue, 0)
    wait(cp_wv)
    for c in range(NT):
        for n in range(NT):
            wvt[c, 128 * n:128 * n + 128, :] = wvb[n, 128 * c:128 * c + 128, :].T
    wait(cp_x[1])
    start(cp_fwd, cp_k, cp_v, cp_x[2])

    def seg0(i, carry):
        for j in range(4):
            @pl.when(i == j)
            def _():
                wait(cp_h[j])
        _interleave((attention(0, i), ATT_STEPS(0)), (qk_proj(1, i, True, True), 10),
                    (h_transpose(i), 20))
        return carry

    lax.fori_loop(0, 4, seg0, 0)
    wait(cp_fwd, cp_k, cp_v, cp_x[2])
    start(cp_wo, cp_x[3], cp_inv, cp_q)
    wait(cp_wo)

    def seg1(i, carry):
        _interleave((attention(1, i), ATT_STEPS(1)), (qk_proj(2, i, True, True), 10),
                    (out_proj(0, i), 6), (fwd_h(i), 20), (fwd_x(i), 40))
        return carry

    lax.fori_loop(0, 4, seg1, 0)
    start(cp_ob[0])
    wait(cp_x[3])

    def seg2(i, carry):
        _interleave((attention(2, i), ATT_STEPS(2)), (qk_proj(3, i, True, False), 10),
                    (out_proj(1, i), 6),
                    (spectra((0, 1), [4 * i + a for a in range(4)]), 8 * SPEC_STEPS))
        return carry

    lax.fori_loop(0, 4, seg2, 0)
    wait(cp_ob[0])
    start(cp_ob[1])

    def seg3(i, carry):
        _interleave((attention(3, i), ATT_STEPS(3)), (out_proj(2, i), 6),
                    (spectra((2, 3, 4), [4 * i + a for a in range(4)]), 12 * SPEC_STEPS))
        return carry

    lax.fori_loop(0, 4, seg3, 0)
    wait(cp_ob[1])
    start(cp_ob[2])
    wait(cp_inv, cp_q)

    def epilogue(i, carry):
        _interleave((out_proj(3, i), 6), (inverse(i), 8))
        start([out_a(i)])
        return carry

    lax.fori_loop(0, 4, epilogue, 0)
    wait(cp_ob[2])
    start(cp_ob[3])
    _interleave((inverse(4), 8))
    start(cp_oa[4:])
    wait(cp_ob[3], cp_oa)


@jax.jit
def pallas_concat_heads__ssm_conv_h3__memory_aug_infini_attn__prompt_kernel(
    A_q: jax.Array,
    A_k: jax.Array,
    A_v: jax.Array,
    A_shift_k: jax.Array,
    A_ssm_k: jax.Array,
    A_ssm_D: jax.Array,
    B_x: jax.Array,
    B_wq: jax.Array,
    B_wk: jax.Array,
    B_wv: jax.Array,
    B_wo: jax.Array,
    B_beta: jax.Array,
):
    hbm = pl.BlockSpec(memory_space=pltpu.HBM)
    vmem = pl.BlockSpec(memory_space=pltpu.VMEM)
    seg_tiles = pltpu.VMEM((NT, L, 128), BF16)
    scratch = [
        pltpu.VMEM((NT, S, 128), BF16),
        pltpu.VMEM((NT, D, 128), BF16),
        pltpu.VMEM((NT, D, 128), BF16),
        pltpu.VMEM((NT, D, 128), BF16),
        pltpu.VMEM((NT, D, 128), BF16),
        pltpu.VMEM((NT, D, 128), BF16),
        pltpu.VMEM((S // 128, D, 128), BF16),
        pltpu.VMEM((NT, S // 2, 128), U32),
        pltpu.VMEM((NT, S // 2 + 8, 128), U32),
        pltpu.VMEM((NT, S // 2, 128), U32),
        pltpu.VMEM((NT, S // 2, 128), U32),
        pltpu.VMEM((N2, 2 * N1, N1), BF16),
        pltpu.VMEM((N2, N1, 2 * N1), BF16),
        pltpu.VMEM((NT, N2, N1, 128), F32),
        pltpu.VMEM((NT, N2, 2 * N1, 128), F32),
        pltpu.VMEM((NT, N2, 2 * N1, 128), F32),
        pltpu.VMEM((NT, N1 // 8, 2 * N2, 8, 128), F32),
        pltpu.VMEM((NT, N2, 2 * N1, 128), BF16),
        pltpu.VMEM((NT, S // 2, 128), U32),
        pltpu.VMEM((NT, S, 128), BF16),
        pltpu.VMEM((NT, KS + 1, 8, 128), F32),
        pltpu.VMEM((8, 8, 128), F32),
        pltpu.VMEM((3, 64, 128), F32),
        seg_tiles, seg_tiles, seg_tiles, seg_tiles,
        seg_tiles, seg_tiles, seg_tiles, seg_tiles,
        pltpu.VMEM((4, D, 128), BF16),
        pltpu.VMEM((4, D, 128), BF16),
        pltpu.VMEM((8, 96, 128), F32),
        pltpu.SemaphoreType.DMA((19,)),
    ]
    return pl.pallas_call(
        _kernel,
        out_shape=jax.ShapeDtypeStruct((1, S, 2 * D), BF16),
        in_specs=[hbm, hbm, hbm, vmem, hbm, vmem, hbm, hbm, hbm, hbm, hbm, vmem, hbm, hbm],
        out_specs=hbm,
        scratch_shapes=scratch,
        compiler_params=pltpu.CompilerParams(vmem_limit_bytes=110 * 1024 * 1024),
        name="h3_infini",
    )(A_q, A_k, A_v, A_shift_k, A_ssm_k, A_ssm_D.reshape(1, D), B_x, B_wq, B_wk, B_wv, B_wo,
      B_beta.reshape(1, H), _FWD, _INV)
```

```python
import math

import jax
import jax.numpy as jnp
import numpy as np
from jax import lax
from jax.experimental import pallas as pl
from jax.experimental.pallas import tpu as pltpu

S = 2048
D = 640
NT = D // 128
H = 32
DH = D // H
NSEG = 4
L = S // NSEG
KS = 4
N1, N2 = 128, 16

F32 = jnp.float32
BF16 = jnp.bfloat16
U32 = jnp.uint32
NN_DIMS = (((1,), (0,)), ((), ()))
NT_DIMS = (((1,), (1,)), ((), ()))
NEG = -1e30
LOG2E = 1.4426950408889634


def _pack_rows(a):
    u = a.astype(np.float32).astype(BF16).view(np.uint16).astype(np.uint32)
    return u[..., 0::2, :] | (u[..., 1::2, :] << 16)


def _dft_tables():
    n1 = np.arange(N1)
    k1 = np.arange(N1)
    fwd = np.zeros((N2, 2 * N1, N1), np.float64)
    inv = np.zeros((N2, N1, 2 * N1), np.float64)
    pos_re = 2 * k1
    for n2 in range(N2):
        ang = 2.0 * np.pi * np.outer(k1 + 0.25, N2 * n1 + n2) / S
        c, s = np.cos(ang), np.sin(ang)
        fwd[n2, :N1] = c
        fwd[n2, N1:] = s
        inv[n2][:, pos_re] = c.T / S
        inv[n2][:, pos_re + 1] = s.T / S
    inv = inv.reshape(N2, N1, 2, N1).transpose(0, 2, 1, 3)
    return _pack_rows(fwd), _pack_rows(inv)


_FWD, _INV = _dft_tables()


def _dot(a, b, dims=NN_DIMS):
    return lax.dot_general(a, b, dims, preferred_element_type=F32)


def _u32(x):
    return pltpu.bitcast(x, U32)


def _bf(x):
    return pltpu.bitcast(x, BF16)


def _pack(x):
    return _u32(x.astype(BF16))


def _lo(w):
    return pltpu.unpack_elementwise(w, index=0, packed_dtype=BF16, unpacked_dtype=F32)


def _hi(w):
    return pltpu.unpack_elementwise(w, index=1, packed_dtype=BF16, unpacked_dtype=F32)


def _radix4(x0, x1, x2, x3, sign):
    ar, ai = x0[0] + x2[0], x0[1] + x2[1]
    br, bi = x0[0] - x2[0], x0[1] - x2[1]
    cr, ci = x1[0] + x3[0], x1[1] + x3[1]
    dr, di = x1[0] - x3[0], x1[1] - x3[1]
    y0 = (ar + cr, ai + ci)
    y2 = (ar - cr, ai - ci)
    yp = (br - di, bi + dr)
    ym = (br + di, bi - dr)
    return (y0, yp, y2, ym) if sign > 0 else (y0, ym, y2, yp)


def _twiddle(x, e, sign):
    xr, xi = x
    if e == 0:
        return x
    if e == 4:
        return (-xi, xr) if sign > 0 else (xi, -xr)
    r = math.sqrt(0.5)
    if e == 2:
        return ((xr - xi) * r, (xr + xi) * r) if sign > 0 else ((xr + xi) * r, (xi - xr) * r)
    if e == 6:
        return ((xr + xi) * -r, (xr - xi) * r) if sign > 0 else ((xi - xr) * r, (xr + xi) * -r)
    c, s = math.cos(math.pi * e / 8), sign * math.sin(math.pi * e / 8)
    return (xr * c - xi * s, xr * s + xi * c)


def _radix4_tw(x0, x1, x2, x3, sign, b):
    if b != 2:
        return _radix4(x0, _twiddle(x1, b, sign), _twiddle(x2, 2 * b, sign),
                       _twiddle(x3, 3 * b, sign), sign)
    x1, x3 = _twiddle(x1, 2, sign), _twiddle(x3, 6, sign)
    if sign > 0:
        ar, ai = x0[0] - x2[1], x0[1] + x2[0]
        br, bi = x0[0] + x2[1], x0[1] - x2[0]
    else:
        ar, ai = x0[0] + x2[1], x0[1] - x2[0]
        br, bi = x0[0] - x2[1], x0[1] + x2[0]
    cr, ci = x1[0] + x3[0], x1[1] + x3[1]
    dr, di = x1[0] - x3[0], x1[1] - x3[1]
    y0 = (ar + cr, ai + ci)
    y2 = (ar - cr, ai - ci)
    yp = (br - di, bi + dr)
    ym = (br + di, bi - dr)
    return (y0, yp, y2, ym) if sign > 0 else (y0, ym, y2, yp)


class _Paced:
    def __init__(self, streams, sequential=False):
        self.live = [[g, total, 0] for g, total in streams]
        self.total = sum(total for _, total in streams)
        self.done = 0
        self.sequential = sequential

    def advance(self, fraction):
        while self.live and self.done < fraction * self.total:
            cur = self.live[0] if self.sequential else min(self.live, key=lambda e: e[2] / e[1])
            cost = next(cur[0], None)
            if cost is None:
                self.live.remove(cur)
            else:
                cur[2] += cost
                self.done += cost

    def finish(self):
        self.advance(math.inf)


DEPTH = 2


def _kernel(aq_hbm, ak_hbm, av_hbm, shift_ref, h_hbm, ssmd_ref, x_hbm, wq_hbm, wk_hbm,
            wv_hbm, wo_hbm, beta_ref, fwd_hbm, inv_hbm, out_hbm,
            xb, wqb, wkb, wvb, wob, wvt, hb, ht, kb, vb, qb, fwd, inv,
            kvf, gx, gh, hf, yb, outa, outb, wtab, gtab, cmask,
            q0, q1, k0, k1, pq0, pq1, pk0, pk1, ot0, ot1, mst, sems):
    qs, ks, pqs, pks, ots = (q0, q1), (k0, k1), (pq0, pq1), (pk0, pk1), (ot0, ot1)

    def col_tiles(src, dst, sem, rows=None, lead=(0,), dst_off=0, tiles=range(NT)):
        r0, n = rows if rows is not None else (0, src.shape[-2])

        def one(t):
            return lambda: pltpu.make_async_copy(
                src.bitcast(U32).at[(*lead, pl.ds(r0 // 2, n // 2), pl.ds(128 * t, 128))],
                dst.at[t, pl.ds(dst_off + r0 // 2, n // 2), :], sems.at[sem])
        return [one(t) for t in tiles]

    cp_x = [col_tiles(x_hbm, xb, s, rows=(L * s, L)) for s in range(NSEG)]
    cp_wq = col_tiles(wq_hbm, wqb, 4, lead=())
    cp_wk = col_tiles(wk_hbm, wkb, 5, lead=())
    cp_wv = col_tiles(wv_hbm, wvb, 6, lead=())
    cp_wo = col_tiles(wo_hbm, wob, 7, lead=())
    cp_h = [col_tiles(h_hbm, hb, 8 + i, lead=(), tiles=range(4 * i, 4 * i + 4)) for i in range(4)]
    cp_k = col_tiles(ak_hbm, kb, 12, dst_off=8)
    cp_v = col_tiles(av_hbm, vb, 13)
    cp_q = col_tiles(aq_hbm, qb, 14)
    cp_fwd = [lambda: pltpu.make_async_copy(fwd_hbm, fwd, sems.at[15])]
    cp_inv = [lambda: pltpu.make_async_copy(inv_hbm, inv, sems.at[16])]

    def out_a(c):
        c0 = 128 * c if isinstance(c, int) else pl.multiple_of(128 * c, 128)
        return lambda: pltpu.make_async_copy(
            outa.at[c], out_hbm.bitcast(U32).at[0, :, pl.ds(c0, 128)], sems.at[17])

    def out_b(s, n):
        return lambda: pltpu.make_async_copy(
            outb.at[n, pl.ds(L // 2 * s, L // 2), :],
            out_hbm.bitcast(U32).at[0, pl.ds(L // 2 * s, L // 2), pl.ds(D + 128 * n, 128)],
            sems.at[18])

    cp_oa = [out_a(c) for c in range(NT)]
    cp_ob = [[out_b(s, n) for n in range(NT)] for s in range(NSEG)]

    def start(*groups):
        for g in groups:
            for cp in g:
                cp().start()

    def wait(*groups):
        for g in groups:
            for cp in g:
                cp().wait()

    def rows(i, n):
        return pl.ds(pl.multiple_of(i * n, n), n) if not isinstance(i, int) else pl.ds(i * n, n)

    lane = lax.broadcasted_iota(jnp.int32, (8, 128), 1)
    sub = lax.broadcasted_iota(jnp.int32, (8, 128), 0)

    def lanes(n):
        return lax.broadcasted_iota(jnp.int32, (n, 128), 1)

    def qk_proj(s, i, want_pq, want_pk):
        p = s % 2
        tok = rows(4 * s + i, 64)
        for w_ref, dst, fdst, want, scale in (
                (wqb, qs[p], pqs[p], want_pq, DH ** -0.5 * LOG2E),
                (wkb, ks[p], pks[p], want_pk, None)):
            for n in range(NT):
                xt = jnp.concatenate([_bf(xb[c, tok, :]) for c in range(NT)], axis=1)
                t = _dot(xt, _bf(w_ref[n]))
                dst[n, rows(i, 64), :] = _pack(t if scale is None else t * scale)
                if want:
                    fdst[n, rows(i, 64), :] = _pack(jnp.where(t > 0, t + 1.0, jnp.exp(t)))
                yield 160

    def out_proj(s, i):
        ot = ots[s % 2]
        o = jnp.concatenate([_bf(ot[i, 64 * c:64 * c + 64, :]).T for c in range(NT)], axis=1)
        yield 160
        for n in range(NT):
            outb[n, rows(4 * s + i, 64), :] = _pack(_dot(o, _bf(wob[n])))
            yield 160

    def tile_rows(r, n):
        return jnp.broadcast_to(r[None], (n // 8, 8, 128)).reshape(n, 128)

    def vmax(x):
        m = x[0:8]
        for r in range(1, x.shape[0] // 8):
            m = jnp.maximum(m, x[8 * r:8 * r + 8])
        return m

    def prob(x, m):
        return jnp.exp2(x - tile_rows(m, x.shape[0])).astype(BF16)

    class Group:
        def __init__(self, s, g, vt, row0):
            self.s, self.g, self.vt, self.row0 = s, g, vt, row0
            self.t0 = (80 * g) // 128
            self.off = 80 * g - 128 * self.t0
            self.t1 = jnp.minimum(self.t0 + 1, NT - 1)
            rel = (lane - self.off) & 127
            self.head = sum((rel >= a * DH).astype(jnp.int32) for a in range(1, 5))
            self.gate = gtab[g]
            self.kw, self.qw, self.vab = {}, {}, {}
            self.amem = [None] * 4
            self.odot = [[None, None] for _ in range(4)]

        def window(self, ref, j):
            return jnp.where(lanes(64) >= self.off,
                             ref[self.t0, 64 * j:64 * j + 64, :],
                             ref[self.t1, 64 * j:64 * j + 64, :])

        def keys(self, j):
            if j not in self.kw:
                self.kw[j] = _bf(self.window(ks[self.s % 2], j))
            return self.kw[j]

        def values(self, pr, j):
            if (pr, j) not in self.vab:
                r0 = self.row0 + 40 * pr
                v40 = self.vt[j][r0:r0 + 40]
                ones8 = jnp.ones((8, 128), F32)
                self.vab[pr, j] = (jnp.concatenate([v40[0:24], ones8], axis=0).astype(BF16),
                                   jnp.concatenate([v40[16:40], ones8], axis=0).astype(BF16))
            return self.vab[pr, j]

        def mem_read(self):
            mem = mst[self.g].astype(BF16)
            for j in range(4):
                r = _dot(mem, _bf(self.window(pqs[self.s % 2], j)), NT_DIMS)
                coef = self.gate / (r[80:88] + 1e-6)
                cb = [jnp.broadcast_to(coef[a:a + 1], (8, 128)) for a in range(4)]
                cols = []
                for pr in range(2):
                    ca, cc = cb[2 * pr], cb[2 * pr + 1]
                    cols += [ca, ca, jnp.where(sub < 4, ca, cc), cc, cc]
                self.amem[j] = r[0:80] * jnp.concatenate(cols, axis=0)
                yield 24

        def mem_update(self):
            acc = None
            for j in range(4):
                lhs = jnp.concatenate([self.vt[j][self.row0:self.row0 + 80].astype(BF16),
                                       jnp.ones((16, 128), BF16)], axis=0)
                t = _dot(lhs, _bf(self.window(pks[self.s % 2], j)))
                acc = t if acc is None else acc + t
                yield 24
            keep = []
            for r in range(12):
                row = sub + 8 * r
                if r < 10:
                    hr = sum((row >= a * DH).astype(jnp.int32) for a in range(1, 4))
                else:
                    hr = row - 80
                keep.append(jnp.where(hr == self.head, acc[8 * r:8 * r + 8], 0.0))
            upd = jnp.concatenate(keep, axis=0)
            mst[self.g] = upd if self.s == 0 else mst[self.g] + upd

        def logits(self, pr, j):
            ma = jnp.where(self.head == 2 * pr, np.uint32(0xFFFFFFFF), np.uint32(0))
            mb = jnp.where(self.head == 2 * pr + 1, np.uint32(0xFFFFFFFF), np.uint32(0))
            qw = self.window(qs[self.s % 2], j)
            qa = qw & tile_rows(ma, 64)
            qh = qw & tile_rows(mb, 64)
            w_a = _bf(qa)
            w_b = _bf(jnp.concatenate([qh[32:64], qh[0:32]], axis=0))
            w_t = _bf(jnp.concatenate([qh[32:64], qa[32:64]], axis=0))
            klhs = jnp.concatenate([self.keys(kt) for kt in range(j)] + [self.keys(j)[0:64]], axis=0)
            s_a = _dot(klhs, w_a, NT_DIMS)
            s_t = _dot(self.keys(j)[64:128], w_t, NT_DIMS)
            s_b = _dot(klhs, w_b, NT_DIMS)
            return s_a, s_b, s_t

        def softmax(self, j, logits):
            s_a, s_b, s_t = logits
            n = 128 * j
            s_t = s_t + cmask[2]
            d_a = s_a[n:] + cmask[0]
            d_b = s_b[n:] + cmask[1]
            m_a, m_b, m_t = vmax(d_a), vmax(d_b), vmax(s_t)
            if j:
                m_a = jnp.maximum(m_a, vmax(s_a[:n]))
                m_b = jnp.maximum(m_b, vmax(s_b[:n]))
            m_a = jnp.maximum(m_a, jnp.where(lane >= 64, m_t, NEG))
            m_b = jnp.maximum(m_b, jnp.where(lane < 64, m_t, NEG))
            m_a = jnp.broadcast_to(jnp.max(m_a, axis=0, keepdims=True), (8, 128))
            m_b = jnp.broadcast_to(jnp.max(m_b, axis=0, keepdims=True), (8, 128))
            m_t = jnp.where(lane < 64, m_b, m_a)
            p_t = _u32(prob(s_t, m_t))
            p_ta = _bf(jnp.where(lanes(32) >= 64, p_t, np.uint32(0)))
            p_tb = _bf(jnp.where(lanes(32) >= 64, np.uint32(0), p_t))
            out = []
            for s_x, d_x, m_x, p_tx in ((s_a, d_a, m_a, p_ta), (s_b, d_b, m_b, p_tb)):
                tiles = [prob(s_x[128 * kt:128 * kt + 128], m_x) for kt in range(j)]
                out.append(tiles + [jnp.concatenate([prob(d_x, m_x), p_tx], axis=0)])
            return out

        def attend(self, pr, j, probs):
            res = []
            for e in range(2):
                acc = None
                for kt in range(j + 1):
                    t = _dot(self.values(pr, kt)[e], probs[e][kt])
                    acc = t if acc is None else acc + t
                res.append(acc)
            r_a = res[0]
            r_b = pltpu.roll(res[1], 64, 1)
            keep_a = 1.0 - jnp.broadcast_to(self.gate[2 * pr:2 * pr + 1], (8, 128))
            keep_b = 1.0 - jnp.broadcast_to(self.gate[2 * pr + 1:2 * pr + 2], (8, 128))
            o_a = r_a[0:24] * tile_rows(keep_a / r_a[24:32], 24)
            o_b = r_b[0:24] * tile_rows(keep_b / r_b[24:32], 24)
            self.odot[j][pr] = jnp.concatenate(
                [o_a[0:16], jnp.where(sub < 4, o_a[16:24], o_b[0:8]), o_b[8:24]], axis=0)
            if pr == 1:
                o = jnp.concatenate(self.odot[j], axis=0)
                if self.s > 0:
                    o = o + self.amem[j]
                ots[self.s % 2][j, rows(self.g, 40), :] = _pack(o)

    def v_proj(s, i, vt):
        for j in range(4):
            acc = None
            for c in range(NT):
                t = _dot(_bf(wvt[c, rows(i, 80), :]), _bf(xb[c, rows(4 * s + j, 64), :]), NT_DIMS)
                acc = t if acc is None else acc + t
            vt.append(acc)
            yield 200

    def segment_step(s, i, mxu_fill, vpu_fill):
        vt = []
        vgen = v_proj(s, i, vt)
        groups = [Group(s, 2 * i + gi, vt, 80 * gi) for gi in range(2)]
        units = [(gi, pr, j if (gi, pr) != (1, 1) else 3 - j)
                 for gi in range(2) for pr in range(2) for j in range(4)]
        mem = []
        for grp in groups:
            if s > 0:
                mem.append((grp.mem_read(), 96))
        for grp in groups:
            if s < NSEG - 1:
                mem.append((grp.mem_update(), 96))
        fill = _Paced(mxu_fill)
        late = _Paced(mem, sequential=True)
        side = _Paced(vpu_fill)
        nstep = len(units) + DEPTH
        lg, pb = {}, {}
        for u in range(nstep):
            if u < len(units):
                gi, pr, j = units[u]
                lg[u] = groups[gi].logits(pr, j)
            side.advance((u + 0.33) / nstep)
            if u < 4:
                next(vgen)
            else:
                fill.advance((u - 3.5) / (nstep - 4))
                late.advance((u - 3) / 4)
            if 0 <= u - 1 < len(units):
                gi, pr, j = units[u - 1]
                pb[u - 1] = groups[gi].softmax(j, lg.pop(u - 1))
            side.advance((u + 0.66) / nstep)
            if u - DEPTH >= 0:
                gi, pr, j = units[u - DEPTH]
                groups[gi].attend(pr, j, pb.pop(u - DEPTH))
            side.advance((u + 1) / nstep)
        late.finish()
        fill.finish()
        side.finish()

    def h_transpose(i):
        for t in range(4):
            for c in range(NT):
                ht[c, rows(4 * i + t, 64), :] = _u32(_bf(hb[4 * i + t, 64 * c:64 * c + 64, :]).T)
                yield 1

    def fwd_h(i):
        for c in range(NT):
            for jp in range(2):
                w = ht[c, pl.ds(2 * i + jp, N1, stride=8), :]
                for e, part in enumerate((_lo, _hi)):
                    n2 = 4 * i + 2 * jp + e
                    gh[c, n2] = _dot(_bf(fwd[n2]), part(w).astype(BF16))
                    yield 64

    def fwd_x(i):
        for c in range(NT):
            taps = [wtab[c, j] for j in range(KS)]
            planes = [[] for _ in range(4)]
            for r in range(0, N1, 16):
                kw = [kb[c, pl.ds(8 * r + 6 + 2 * i + d, 16, stride=8), :] for d in range(4)]
                vw = [vb[c, pl.ds(8 * r + 2 * i + d, 16, stride=8), :] for d in range(2)]
                kp = [None, _hi(kw[0])] + [f(w) for w in kw[1:] for f in (_lo, _hi)]
                vp = [f(w) for w in vw for f in (_lo, _hi)]
                for e in range(4):
                    acc = kp[4 + e] * tile_rows(taps[0], 16)
                    for j in range(1, KS):
                        acc = acc + kp[4 + e - j] * tile_rows(taps[j], 16)
                    kv = acc * vp[e]
                    kvf[c, 4 * i + e, r:r + 16, :] = kv
                    planes[e].append(kv.astype(BF16))
                if r % 32 == 16:
                    yield 16
            for e in range(4):
                n2 = 4 * i + e
                gx[c, n2] = _dot(_bf(fwd[n2]), jnp.concatenate(planes[e], axis=0))
                yield 48

    def spectrum(c, kblk):
        re, im = rows(kblk, 8), rows(N1 // 8 + kblk, 8)

        def first_pass(ref):
            t = [None] * 4
            for b in range(4):
                t[b] = _radix4(*[(ref[c, 4 * a + b, re, :], ref[c, 4 * a + b, im, :])
                                 for a in range(4)], 1)
                yield 1
            return t

        t = yield from first_pass(gh)
        for cc in range(4):
            z = _radix4_tw(*[t[b][cc] for b in range(4)], 1, cc)
            for d in range(4):
                hf[c, kblk, 2 * (cc + 4 * d)] = z[d][0]
                hf[c, kblk, 2 * (cc + 4 * d) + 1] = z[d][1]
            yield 1
        t = yield from first_pass(gx)
        u = [None] * 4
        for cc in range(4):
            z = _radix4_tw(*[t[b][cc] for b in range(4)], 1, cc)
            y = []
            for d in range(4):
                hr = hf[c, kblk, 2 * (cc + 4 * d)]
                hi = hf[c, kblk, 2 * (cc + 4 * d) + 1]
                y.append((z[d][0] * hr - z[d][1] * hi, z[d][0] * hi + z[d][1] * hr))
            yield 1
            u[cc] = _radix4(*y, -1)
            yield 1
        for b in range(4):
            z = _radix4_tw(*[u[cc][b] for cc in range(4)], -1, b)
            for a in range(4):
                yb[c, 4 * a + b, rows(kblk, 8), :] = pltpu.pack_elementwise(
                    z[a], packed_dtype=BF16).astype(U32)
            yield 1

    SPEC_STEPS = 24

    def spectra(cs, kblks):
        for c in cs:
            for kblk in kblks:
                yield from spectrum(c, kblk)

    def inverse(c):
        dvec = tile_rows(wtab[c, KS], N1)
        for jp in range(8):
            w = qb[c, pl.ds(jp, N1, stride=8), :]
            res = []
            for e, part in enumerate((_lo, _hi)):
                n2 = 2 * jp + e
                y = (_dot(_bf(inv[n2, 0]), _bf(yb[c, n2, 0:64, :]))
                     + _dot(_bf(inv[n2, 1]), _bf(yb[c, n2, 64:128, :])))
                res.append(part(w) * (y + kvf[c, n2] * dvec))
            outa[c, pl.ds(jp, N1, stride=8), :] = pltpu.pack_elementwise(
                res, packed_dtype=BF16).astype(U32)
            yield 128

    start(cp_x[0], cp_wq)
    taps_t = shift_ref[...].astype(F32)
    skip = ssmd_ref[...].astype(F32)
    for c in range(NT):
        for j in range(KS):
            wtab[c, j] = jnp.broadcast_to(taps_t[j:j + 1, 128 * c:128 * c + 128], (8, 128))
        wtab[c, KS] = jnp.broadcast_to(skip[c:c + 1], (8, 128))
        kb[c, 0:8, :] = jnp.zeros((8, 128), U32)
    gates = jax.nn.sigmoid(beta_ref[...].astype(F32))
    gcol = jnp.broadcast_to(gates, (8, H)).T
    gcol = jnp.broadcast_to(gcol[:, 0:1], (H, 128))
    for g in range(8):
        gtab[g] = jnp.concatenate([gcol[4 * g:4 * g + 4]] * 2, axis=0)
    kk = lax.broadcasted_iota(jnp.int32, (64, 128), 0)
    ll = lax.broadcasted_iota(jnp.int32, (64, 128), 1)
    cmask[0] = jnp.where(kk <= ll, 0.0, NEG)
    cmask[1] = jnp.where((ll < 64) | (kk <= ll - 64), 0.0, NEG)
    cmask[2] = jnp.where(kk <= (ll & 63), 0.0, NEG)

    wait(cp_x[0], cp_wq)
    start(cp_wk, cp_wv, cp_x[1])
    wait(cp_wk)
    start(*cp_h)

    def prologue(i, carry):
        _Paced([(qk_proj(0, i, False, True), 1600)]).finish()
        return carry

    with jax.named_scope("prologue"):
        lax.fori_loop(0, 4, prologue, 0)
    wait(cp_wv)
    for c in range(NT):
        for n in range(NT):
            wvt[c, 64 * n:64 * n + 64, :] = _u32(_bf(wvb[n, 64 * c:64 * c + 64, :]).T)
    wait(cp_x[1])
    start(cp_fwd, cp_k, cp_v, cp_x[2])

    def seg0(i, carry):
        for j in range(4):
            @pl.when(i == j)
            def _():
                wait(cp_h[j])
        segment_step(0, i, [(qk_proj(1, i, True, True), 1600)], [(h_transpose(i), 20)])
        return carry

    with jax.named_scope("seg0"):
        lax.fori_loop(0, 4, seg0, 0)
    wait(cp_fwd, cp_k, cp_v, cp_x[2])
    start(cp_wo, cp_x[3], cp_inv, cp_q)
    wait(cp_wo)

    def seg1(i, carry):
        segment_step(1, i, [(qk_proj(2, i, True, True), 1600), (out_proj(0, i), 960),
                            (fwd_h(i), 1280), (fwd_x(i), 1280)], [])
        return carry

    with jax.named_scope("seg1"):
        lax.fori_loop(0, 4, seg1, 0)
    start(cp_ob[0])
    wait(cp_x[3])

    def seg2(i, carry):
        segment_step(2, i, [(qk_proj(3, i, True, False), 1600), (out_proj(1, i), 960)],
                     [(spectra((0, 1, 2), [4 * i + a for a in range(4)]), 12 * SPEC_STEPS)])
        return carry

    with jax.named_scope("seg2"):
        lax.fori_loop(0, 4, seg2, 0)
    wait(cp_ob[0])
    start(cp_ob[1])

    def seg3(i, carry):
        segment_step(3, i, [(out_proj(2, i), 960)],
                     [(spectra((3, 4), [4 * i + a for a in range(4)]), 8 * SPEC_STEPS)])
        return carry

    with jax.named_scope("seg3"):
        lax.fori_loop(0, 4, seg3, 0)
    wait(cp_ob[1])
    start(cp_ob[2])
    wait(cp_inv, cp_q)

    def epilogue(i, carry):
        _Paced([(out_proj(3, i), 960), (inverse(i), 1024)]).finish()
        start([out_a(i)])
        return carry

    with jax.named_scope("epilogue"):
        lax.fori_loop(0, 4, epilogue, 0)
    wait(cp_ob[2])
    start(cp_ob[3])
    _Paced([(inverse(4), 1024)]).finish()
    start(cp_oa[4:])
    wait(cp_ob[3], cp_oa)


@jax.jit
def pallas_concat_heads__ssm_conv_h3__memory_aug_infini_attn__prompt_kernel(
    A_q: jax.Array,
    A_k: jax.Array,
    A_v: jax.Array,
    A_shift_k: jax.Array,
    A_ssm_k: jax.Array,
    A_ssm_D: jax.Array,
    B_x: jax.Array,
    B_wq: jax.Array,
    B_wk: jax.Array,
    B_wv: jax.Array,
    B_wo: jax.Array,
    B_beta: jax.Array,
):
    hbm = pl.BlockSpec(memory_space=pltpu.HBM)
    vmem = pl.BlockSpec(memory_space=pltpu.VMEM)
    seg_tiles = pltpu.VMEM((NT, L // 2, 128), U32)
    seq_tiles = pltpu.VMEM((NT, S // 2, 128), U32)
    w_tiles = pltpu.VMEM((NT, D // 2, 128), U32)
    scratch = [
        seq_tiles,
        w_tiles, w_tiles, w_tiles, w_tiles, w_tiles,
        pltpu.VMEM((S // 128, D // 2, 128), U32),
        seq_tiles,
        pltpu.VMEM((NT, S // 2 + 8, 128), U32),
        seq_tiles, seq_tiles,
        pltpu.VMEM((N2, N1, 128), U32),
        pltpu.VMEM((N2, 2, N1 // 2, 128), U32),
        pltpu.VMEM((NT, N2, N1, 128), F32),
        pltpu.VMEM((NT, N2, 2 * N1, 128), F32),
        pltpu.VMEM((NT, N2, 2 * N1, 128), F32),
        pltpu.VMEM((NT, N1 // 8, 2 * N2, 8, 128), F32),
        pltpu.VMEM((NT, N2, N1, 128), U32),
        seq_tiles, seq_tiles,
        pltpu.VMEM((NT, KS + 1, 8, 128), F32),
        pltpu.VMEM((8, 8, 128), F32),
        pltpu.VMEM((3, 64, 128), F32),
        seg_tiles, seg_tiles, seg_tiles, seg_tiles,
        seg_tiles, seg_tiles, seg_tiles, seg_tiles,
        pltpu.VMEM((4, D // 2, 128), U32),
        pltpu.VMEM((4, D // 2, 128), U32),
        pltpu.VMEM((8, 96, 128), F32),
        pltpu.SemaphoreType.DMA((19,)),
    ]
    return pl.pallas_call(
        _kernel,
        out_shape=jax.ShapeDtypeStruct((1, S, 2 * D), BF16),
        in_specs=[hbm, hbm, hbm, vmem, hbm, vmem, hbm, hbm, hbm, hbm, hbm, vmem, hbm, hbm],
        out_specs=hbm,
        scratch_shapes=scratch,
        compiler_params=pltpu.CompilerParams(vmem_limit_bytes=110 * 1024 * 1024),
        name="h3_infini",
    )(A_q, A_k, A_v, A_shift_k.T, A_ssm_k, A_ssm_D.reshape(NT, 128), B_x, B_wq, B_wk, B_wv, B_wo,
      B_beta.reshape(1, H), _FWD, _INV)
```

```python
import math

import jax
import jax.numpy as jnp
import numpy as np
from jax import lax
from jax.experimental import pallas as pl
from jax.experimental.pallas import tpu as pltpu

S = 2048
D = 640
NT = D // 128
H = 32
DH = D // H
NSEG = 4
L = S // NSEG
KS = 4
N1, N2 = 128, 16

F32 = jnp.float32
BF16 = jnp.bfloat16
U32 = jnp.uint32
NN_DIMS = (((1,), (0,)), ((), ()))
NT_DIMS = (((1,), (1,)), ((), ()))
NEG = -1e30
LOG2E = 1.4426950408889634


def _pack_rows(a):
    u = a.astype(np.float32).astype(BF16).view(np.uint16).astype(np.uint32)
    return u[..., 0::2, :] | (u[..., 1::2, :] << 16)


def _dft_tables():
    k1 = np.arange(N1)
    fwd = np.zeros((N2, 2 * N1, N1), np.float64)
    inv = np.zeros((N2, N1, 2 * N1), np.float64)
    kappa = np.arange(N1)
    n1_in = 16 * (kappa // 16) + 8 * (kappa % 2) + (kappa % 16) // 2
    row_re = 16 * (k1 // 8) + k1 % 8
    for n2 in range(N2):
        ang = 2.0 * np.pi * np.outer(k1 + 0.25, N2 * n1_in + n2) / S
        fwd[n2, row_re] = np.cos(ang)
        fwd[n2, row_re + 8] = np.sin(ang)
        ang = 2.0 * np.pi * np.outer(N2 * np.arange(N1) + n2, k1 + 0.25) / S
        inv[n2][:, 2 * k1] = np.cos(ang) / S
        inv[n2][:, 2 * k1 + 1] = np.sin(ang) / S
    inv = inv.reshape(N2, N1, 2, N1).transpose(0, 2, 1, 3)
    return _pack_rows(fwd), _pack_rows(inv)


_FWD, _INV = _dft_tables()


def _dot(a, b, dims=NN_DIMS):
    return lax.dot_general(a, b, dims, preferred_element_type=F32)


def _u32(x):
    return pltpu.bitcast(x, U32)


def _bf(x):
    return pltpu.bitcast(x, BF16)


def _pack2(a, b):
    return pltpu.pack_elementwise([a, b], packed_dtype=BF16).astype(U32)


def _lo(w):
    return pltpu.unpack_elementwise(w, index=0, packed_dtype=BF16, unpacked_dtype=F32)


def _hi(w):
    return pltpu.unpack_elementwise(w, index=1, packed_dtype=BF16, unpacked_dtype=F32)


def _radix4(x0, x1, x2, x3, sign):
    ar, ai = x0[0] + x2[0], x0[1] + x2[1]
    br, bi = x0[0] - x2[0], x0[1] - x2[1]
    cr, ci = x1[0] + x3[0], x1[1] + x3[1]
    dr, di = x1[0] - x3[0], x1[1] - x3[1]
    y0 = (ar + cr, ai + ci)
    y2 = (ar - cr, ai - ci)
    yp = (br - di, bi + dr)
    ym = (br + di, bi - dr)
    return (y0, yp, y2, ym) if sign > 0 else (y0, ym, y2, yp)


def _twiddle(x, e, sign):
    xr, xi = x
    if e == 0:
        return x
    if e == 4:
        return (-xi, xr) if sign > 0 else (xi, -xr)
    r = math.sqrt(0.5)
    if e == 2:
        return ((xr - xi) * r, (xr + xi) * r) if sign > 0 else ((xr + xi) * r, (xi - xr) * r)
    if e == 6:
        return ((xr + xi) * -r, (xr - xi) * r) if sign > 0 else ((xi - xr) * r, (xr + xi) * -r)
    c, s = math.cos(math.pi * e / 8), sign * math.sin(math.pi * e / 8)
    return (xr * c - xi * s, xr * s + xi * c)


def _radix4_tw(x0, x1, x2, x3, sign, b):
    if b != 2:
        return _radix4(x0, _twiddle(x1, b, sign), _twiddle(x2, 2 * b, sign),
                       _twiddle(x3, 3 * b, sign), sign)
    x1, x3 = _twiddle(x1, 2, sign), _twiddle(x3, 6, sign)
    if sign > 0:
        ar, ai = x0[0] - x2[1], x0[1] + x2[0]
        br, bi = x0[0] + x2[1], x0[1] - x2[0]
    else:
        ar, ai = x0[0] + x2[1], x0[1] - x2[0]
        br, bi = x0[0] - x2[1], x0[1] + x2[0]
    cr, ci = x1[0] + x3[0], x1[1] + x3[1]
    dr, di = x1[0] - x3[0], x1[1] - x3[1]
    y0 = (ar + cr, ai + ci)
    y2 = (ar - cr, ai - ci)
    yp = (br - di, bi + dr)
    ym = (br + di, bi - dr)
    return (y0, yp, y2, ym) if sign > 0 else (y0, ym, y2, yp)


class _Paced:
    def __init__(self, streams, sequential=False):
        self.live = [[g, total, 0] for g, total in streams]
        self.total = sum(total for _, total in streams)
        self.done = 0
        self.sequential = sequential

    def step(self):
        cur = self.live[0] if self.sequential else min(self.live, key=lambda e: e[2] / e[1])
        cost = next(cur[0], None)
        if cost is None:
            self.live.remove(cur)
        else:
            cur[2] += cost
            self.done += cost

    def advance(self, fraction):
        while self.live and self.done < fraction * self.total:
            self.step()

    def finish(self):
        self.advance(math.inf)


DEPTH = 3
TAIL = 0.06
NSLOT = DEPTH + 1
QCH = 256


def _kernel(aq_hbm, ak_hbm, av_hbm, shift_ref, h_hbm, ssmd_ref, x_hbm, wq_hbm, wk_hbm,
            wv_hbm, wo_hbm, beta_ref, fwd_hbm, inv_hbm, out_hbm,
            xb, wqb, wkb, wvb, wob, wvt, hb, ht, kb, vb, qb, fwd, inv,
            kvf, xp, hp, tx, th, ub, yb, outa, outb, wtab, gtab, cmask,
            q0, q1, k0, k1, pq0, pq1, pk0, pk1, ot0, ot1, mst, sems, *slots):
    qs, ks, pqs, pks, ots = (q0, q1), (k0, k1), (pq0, pq1), (pk0, pk1), (ot0, ot1)

    def col_tiles(src, dst, sem, rows=None, lead=(0,), dst_off=0, tiles=range(NT)):
        r0, n = rows if rows is not None else (0, src.shape[-2])

        def one(t):
            return lambda: pltpu.make_async_copy(
                src.bitcast(U32).at[(*lead, pl.ds(r0 // 2, n // 2), pl.ds(128 * t, 128))],
                dst.at[t, pl.ds(dst_off + r0 // 2, n // 2), :], sems.at[sem])
        return [one(t) for t in tiles]

    cp_x = [col_tiles(x_hbm, xb, s, rows=(L * s, L)) for s in range(NSEG)]
    cp_wq = col_tiles(wq_hbm, wqb, 4, lead=())
    cp_wk = col_tiles(wk_hbm, wkb, 5, lead=())
    cp_wv = col_tiles(wv_hbm, wvb, 6, lead=())
    cp_wo = col_tiles(wo_hbm, wob, 7, lead=())
    cp_h = [col_tiles(h_hbm, hb, 8 + i, lead=(), tiles=range(4 * i, 4 * i + 4)) for i in range(4)]
    cp_kv = [col_tiles(ak_hbm, kb, 19 + i, rows=(L * i, L), dst_off=8)
             + col_tiles(av_hbm, vb, 19 + i, rows=(L * i, L)) for i in range(4)]
    cp_q = col_tiles(aq_hbm, qb, 14)
    cp_fwd = [lambda: pltpu.make_async_copy(fwd_hbm, fwd, sems.at[15])]
    cp_inv = [lambda: pltpu.make_async_copy(inv_hbm, inv, sems.at[16])]

    def out_a(c):
        c0 = 128 * c if isinstance(c, int) else pl.multiple_of(128 * c, 128)
        return lambda: pltpu.make_async_copy(
            outa.at[c], out_hbm.bitcast(U32).at[0, :, pl.ds(c0, 128)], sems.at[17])

    def out_b(s, n):
        return lambda: pltpu.make_async_copy(
            outb.at[n, pl.ds(L * s, L), :],
            out_hbm.at[0, pl.ds(L * s, L), pl.ds(D + 128 * n, 128)], sems.at[18])

    cp_oa = [out_a(c) for c in range(NT)]
    cp_ob = [[out_b(s, n) for n in range(NT)] for s in range(NSEG)]

    def start(*groups):
        for g in groups:
            for cp in g:
                cp().start()

    def wait(*groups):
        for g in groups:
            for cp in g:
                cp().wait()

    def rows(i, n):
        return pl.ds(pl.multiple_of(i * n, n), n) if not isinstance(i, int) else pl.ds(i * n, n)

    lane = lax.broadcasted_iota(jnp.int32, (8, 128), 1)
    sub = lax.broadcasted_iota(jnp.int32, (8, 128), 0)

    def lanes(n):
        return lax.broadcasted_iota(jnp.int32, (n, 128), 1)

    def qk_proj(s, i, want_pq, want_pk):
        p = s % 2
        tok = rows(4 * s + i, 64)
        for w_ref, dst, fdst, want, scale in (
                (wqb, qs[p], pqs[p], want_pq, DH ** -0.5 * LOG2E),
                (wkb, ks[p], pks[p], want_pk, None)):
            for n in range(NT):
                t = None
                for c in range(NT):
                    part = _dot(_bf(xb[c, tok, :]), _bf(w_ref[n, 64 * c:64 * c + 64, :]))
                    t = part if t is None else t + part
                    if c < NT - 1:
                        yield 32
                dst[n, rows(i, 128), :] = (t if scale is None else t * scale).astype(BF16)
                if want:
                    fdst[n, rows(i, 128), :] = jnp.where(t > 0, t + 1.0, jnp.exp(t)).astype(BF16)
                yield 32

    def out_proj(s, i):
        ot = ots[s % 2].bitcast(U32)
        o = [_bf(_u32(_bf(ot[i, 64 * c:64 * c + 64, :]).T)) for c in range(NT)]
        for n in range(NT):
            t = None
            for c in range(NT):
                part = _dot(o[c], _bf(wob[n, 64 * c:64 * c + 64, :]))
                t = part if t is None else t + part
                if c < NT - 1:
                    yield 32
            outb[n, rows(4 * s + i, 128), :] = t.astype(BF16)
            yield 32

    def tile_rows(r, n):
        return jnp.broadcast_to(r[None], (n // 8, 8, 128)).reshape(n, 128)

    class Group:
        def __init__(self, s, g, vt, row0):
            self.s, self.g, self.vt, self.row0 = s, g, vt, row0
            self.t0 = (80 * g) // 128
            self.off = 80 * g - 128 * self.t0
            self.t1 = jnp.minimum(self.t0 + 1, NT - 1)
            rel = (lane - self.off) & 127
            self.head = sum((rel >= a * DH).astype(jnp.int32) for a in range(1, 5))
            self.gate = gtab[g]
            self.kw, self.qw, self.vab = {}, {}, {}
            self.amem = [None] * 4
            self.odot = [[None, None] for _ in range(4)]

        def window(self, ref, j):
            ref = ref.bitcast(U32)
            return jnp.where(lanes(64) >= self.off,
                             ref[self.t0, 64 * j:64 * j + 64, :],
                             ref[self.t1, 64 * j:64 * j + 64, :])

        def keys(self, j):
            if j not in self.kw:
                self.kw[j] = _bf(self.window(ks[self.s % 2], j))
            return self.kw[j]

        def values(self, pr, j):
            if (pr, j) not in self.vab:
                r0 = self.row0 + 40 * pr
                v40 = self.vt[j][r0:r0 + 40]
                ones8 = jnp.ones((8, 128), F32)
                self.vab[pr, j] = (jnp.concatenate([v40[0:24], ones8], axis=0).astype(BF16),
                                   jnp.concatenate([v40[16:40], ones8], axis=0).astype(BF16))
            return self.vab[pr, j]

        def mem_read(self):
            mem = mst[self.g].astype(BF16)
            for j in range(4):
                r = _dot(mem, _bf(self.window(pqs[self.s % 2], j)), NT_DIMS)
                coef = self.gate / (r[80:88] + 1e-6)
                cb = [jnp.broadcast_to(coef[a:a + 1], (8, 128)) for a in range(4)]
                cols = []
                for pr in range(2):
                    ca, cc = cb[2 * pr], cb[2 * pr + 1]
                    cols += [ca, ca, jnp.where(sub < 4, ca, cc), cc, cc]
                self.amem[j] = r[0:80] * jnp.concatenate(cols, axis=0)
                yield 24

        def mem_update(self):
            acc = None
            for j in range(4):
                lhs = jnp.concatenate([self.vt[j][self.row0:self.row0 + 80].astype(BF16),
                                       jnp.ones((16, 128), BF16)], axis=0)
                t = _dot(lhs, _bf(self.window(pks[self.s % 2], j)))
                acc = t if acc is None else acc + t
                yield 24
            keep = []
            for r in range(12):
                row = sub + 8 * r
                if r < 10:
                    hr = sum((row >= a * DH).astype(jnp.int32) for a in range(1, 4))
                else:
                    hr = row - 80
                keep.append(jnp.where(hr == self.head, acc[8 * r:8 * r + 8], 0.0))
            upd = jnp.concatenate(keep, axis=0)
            mst[self.g] = upd if self.s == 0 else mst[self.g] + upd

        def logits(self, pr, j, slot, maxes):
            ma = jnp.where(self.head == 2 * pr, np.uint32(0xFFFFFFFF), np.uint32(0))
            mb = jnp.where(self.head == 2 * pr + 1, np.uint32(0xFFFFFFFF), np.uint32(0))
            qw = self.window(qs[self.s % 2], j)
            qa = qw & tile_rows(ma, 64)
            qh = qw & tile_rows(mb, 64)
            w_a = _bf(qa)
            w_b = _bf(jnp.concatenate([qh[32:64], qh[0:32]], axis=0))
            w_t = _bf(jnp.concatenate([qh[32:64], qa[32:64]], axis=0))
            klhs = jnp.concatenate([self.keys(kt) for kt in range(j)] + [self.keys(j)[0:64]], axis=0)
            n = 128 * j

            def park(t, e, r0, m):
                for r in range(0, t.shape[0], 8):
                    v = t[r:r + 8]
                    if e == 2:
                        v = v + cmask[2, r:r + 8, :]
                    elif r0 + r >= n:
                        v = v + cmask[e, r0 + r - n:r0 + r - n + 8, :]
                    slot[e % 2, 448 * (e // 2) + r0 + r:448 * (e // 2) + r0 + r + 8, :] = v
                    m = v if m is None else jnp.maximum(m, v)
                return m

            m_t = park(_dot(self.keys(j)[64:128], w_t, NT_DIMS), 2, 0, None)
            yield 16
            cuts = list(range(0, n, QCH)) or [0]
            m = [None, None]
            for r0, r1 in zip(cuts, cuts[1:] + [n + 64]):
                for e, w in enumerate((w_a, w_b)):
                    m[e] = park(_dot(klhs[r0:r1], w, NT_DIMS), e, r0, m[e])
                    if r1 == n + 64 and e == 1:
                        m_a = jnp.maximum(m[0], jnp.where(lane >= 64, m_t, NEG))
                        m_b = jnp.maximum(m[1], jnp.where(lane < 64, m_t, NEG))
                        m_a = jnp.broadcast_to(jnp.max(m_a, axis=0, keepdims=True), (8, 128))
                        m_b = jnp.broadcast_to(jnp.max(m_b, axis=0, keepdims=True), (8, 128))
                        maxes += [m_a, m_b, jnp.where(lane < 64, m_b, m_a)]
                    yield (r1 - r0) // 4

        def attend(self, pr, j, slot, maxes, need_values):
            def prob(e, r0, n, m):
                m2 = tile_rows(m, 16)
                return [jnp.exp2(slot[e, r:r + 16, :] - m2).astype(BF16)
                        for r in range(r0, r0 + n, 16)]

            p_t = _u32(jnp.concatenate(prob(0, 448, 64, maxes[2]), axis=0))
            tails = (_bf(jnp.where(lanes(32) >= 64, p_t, np.uint32(0))),
                     _bf(jnp.where(lanes(32) >= 64, np.uint32(0), p_t)))
            res = []
            for e in range(2):
                acc = None
                for kt in range(j + 1):
                    need_values(kt)
                    if kt < j:
                        p = prob(e, 128 * kt, 128, maxes[e])
                    else:
                        p = prob(e, 128 * kt, 64, maxes[e]) + [tails[e]]
                    t = _dot(self.values(pr, kt)[e], jnp.concatenate(p, axis=0))
                    acc = t if acc is None else acc + t
                    if (e, kt) != (1, j):
                        yield 8
                res.append(acc)
            r_a = res[0]
            r_b = pltpu.roll(res[1], 64, 1)
            keep_a = 1.0 - jnp.broadcast_to(self.gate[2 * pr:2 * pr + 1], (8, 128))
            keep_b = 1.0 - jnp.broadcast_to(self.gate[2 * pr + 1:2 * pr + 2], (8, 128))
            o_a = r_a[0:24] * tile_rows(keep_a / r_a[24:32], 24)
            o_b = r_b[0:24] * tile_rows(keep_b / r_b[24:32], 24)
            self.odot[j][pr] = jnp.concatenate(
                [o_a[0:16], jnp.where(sub < 4, o_a[16:24], o_b[0:8]), o_b[8:24]], axis=0)
            if pr == 1:
                o = jnp.concatenate(self.odot[j], axis=0)
                if self.s > 0:
                    o = o + self.amem[j]
                ots[self.s % 2][j, rows(self.g, 80), :] = o.astype(BF16)
            yield 8

    def v_proj(s, i, vt):
        for j in range(4):
            acc = None
            for c in range(NT):
                t = _dot(_bf(wvt[c, rows(i, 80), :]), _bf(xb[c, rows(4 * s + j, 64), :]), NT_DIMS)
                acc = t if acc is None else acc + t
                if c == NT - 1:
                    vt.append(acc)
                yield 40

    def chain(*gens):
        for g in gens:
            yield from g

    def segment_step(s, i, mxu_fill, vpu_fill):
        vt = []
        groups = [Group(s, 2 * i + gi, vt, 80 * gi) for gi in range(2)]
        units = [(gi, pr, j if (gi, pr) != (1, 1) else 3 - j)
                 for gi in range(2) for pr in range(2) for j in range(4)]
        mem = [grp.mem_read() for grp in groups if s > 0]
        mem += [grp.mem_update() for grp in groups if s < NSEG - 1]
        first = _Paced([(chain(v_proj(s, i, vt), *mem), 800 + 96 * len(mem))])
        fill = _Paced(mxu_fill)
        side = _Paced(vpu_fill)
        nstep = len(units) + DEPTH
        total = first.total + fill.total

        def need_values(kt):
            while len(vt) <= kt:
                first.step()

        def pad(fraction):
            target = total * fraction / (1 + TAIL)
            first.advance(target / first.total)
            if fill.total:
                fill.advance((target - first.done) / fill.total)
            side.advance(fraction)

        def cost(j):
            return 48 + 64 * j, 16 + 16 * j

        whole = sum(sum(cost(j)) for _, _, j in units)
        done = 0
        maxes = {}
        for u in range(nstep):
            streams = []
            if u < len(units):
                gi, pr, j = units[u]
                maxes[u] = []
                streams.append((groups[gi].logits(pr, j, slots[u % NSLOT], maxes[u]), cost(j)[0]))
            if u >= DEPTH:
                v = u - DEPTH
                gi, pr, j = units[v]
                if pr == 1 and s > 0:
                    while groups[gi].amem[j] is None:
                        first.step()
                streams.append((groups[gi].attend(pr, j, slots[v % NSLOT], maxes.pop(v), need_values),
                                cost(j)[1]))
            att = _Paced(streams)
            while att.live:
                att.step()
                pad((done + att.done) / whole)
            done += att.total
        first.finish()
        fill.finish()
        side.finish()

    def split_h(i):
        for c in range(NT):
            for t in range(4):
                ht[c, 64 * t:64 * t + 64, :] = _u32(_bf(hb[4 * i + t, 64 * c:64 * c + 64, :]).T)
                yield 16
            for q in range(2):
                for j in range(8):
                    wa = ht[c, pl.ds(128 * q + j, 8, stride=8), :]
                    wb = ht[c, pl.ds(128 * q + 64 + j, 8, stride=8), :]
                    hp[c, 2 * j, rows(2 * i + q, 8), :] = _pack2(_lo(wa), _lo(wb))
                    hp[c, 2 * j + 1, rows(2 * i + q, 8), :] = _pack2(_hi(wa), _hi(wb))
                    if j % 2:
                        yield 4

    def split_kv(i):
        for c in range(NT):
            taps = [wtab[c, j] for j in range(KS)]
            for q in range(2):
                blk = 2 * i + q
                base = [blk * 128 + 64 * e for e in range(2)]
                hist = []
                for e in range(2):
                    w2 = kb[c, pl.ds(base[e] + 6, 8, stride=8), :]
                    w1 = kb[c, pl.ds(base[e] + 7, 8, stride=8), :]
                    hist.append([_hi(w2), _lo(w1), _hi(w1)])
                for j in range(8):
                    kv = [[None, None], [None, None]]
                    for e in range(2):
                        kw = kb[c, pl.ds(base[e] + 8 + j, 8, stride=8), :]
                        vw = vb[c, pl.ds(base[e] + j, 8, stride=8), :]
                        kp = hist[e] + [_lo(kw), _hi(kw)]
                        for half, part in enumerate((_lo, _hi)):
                            acc = kp[3 + half] * taps[0]
                            for d in range(1, KS):
                                acc = acc + kp[3 + half - d] * taps[d]
                            kv[half][e] = acc * part(vw)
                            kvf[c, 2 * j + half, rows(2 * blk + e, 8), :] = kv[half][e]
                        hist[e] = kp[2:]
                    for half in range(2):
                        xp[c, 2 * j + half, rows(blk, 8), :] = _pack2(*kv[half])
                    yield 11

    def fwd_fft(i):
        for c in range(NT):
            for src, dst in ((hp, th), (xp, tx)):
                g = [_dot(_bf(fwd[4 * a + i]), _bf(src[c, 4 * a + i])) for a in range(4)]
                for m in range(N1 // 8):
                    z = _radix4(*[(g[a][16 * m:16 * m + 8], g[a][16 * m + 8:16 * m + 16])
                                  for a in range(4)], 1)
                    for cc in range(4):
                        dst[c, m, cc, i, 0] = z[cc][0]
                        dst[c, m, cc, i, 1] = z[cc][1]
                yield 256

    def spectrum(c, m, slot):
        for cc in range(4):
            zh = _radix4_tw(*[(th[c, m, cc, b, 0], th[c, m, cc, b, 1]) for b in range(4)], 1, cc)
            yield 1
            zx = _radix4_tw(*[(tx[c, m, cc, b, 0], tx[c, m, cc, b, 1]) for b in range(4)], 1, cc)
            yield 1
            y = [(x[0] * h[0] - x[1] * h[1], x[0] * h[1] + x[1] * h[0]) for x, h in zip(zx, zh)]
            yield 1
            u = _radix4(*y, -1)
            for b in range(4):
                ub[slot, b, cc, 0] = u[b][0]
                ub[slot, b, cc, 1] = u[b][1]
            yield 1
        for b in range(4):
            z = _radix4_tw(*[(ub[slot, b, cc, 0], ub[slot, b, cc, 1]) for cc in range(4)], -1, b)
            for a in range(4):
                yb[c, 4 * a + b, rows(m, 8), :] = _pack2(*z[a])
            yield 1

    SPEC_STEPS = 20

    def spectra(cs, ms):
        for slot, (c, m) in enumerate((c, m) for c in cs for m in ms):
            yield from spectrum(c, m, slot)

    def inverse(c):
        dvec = tile_rows(wtab[c, KS], N1)
        for jp in range(8):
            w = qb[c, pl.ds(jp, N1, stride=8), :]
            res = []
            for e, part in enumerate((_lo, _hi)):
                n2 = 2 * jp + e
                y = (_dot(_bf(inv[n2, 0]), _bf(yb[c, n2, 0:64, :]))
                     + _dot(_bf(inv[n2, 1]), _bf(yb[c, n2, 64:128, :])))
                res.append(part(w) * (y + kvf[c, n2] * dvec))
            outa[c, pl.ds(jp, N1, stride=8), :] = _pack2(*res)
            yield 128

    start(cp_x[0], cp_wq)
    taps_t = shift_ref[...].astype(F32)
    skip = ssmd_ref[...].astype(F32)
    for c in range(NT):
        for j in range(KS):
            wtab[c, j] = jnp.broadcast_to(taps_t[j:j + 1, 128 * c:128 * c + 128], (8, 128))
        wtab[c, KS] = jnp.broadcast_to(skip[c:c + 1], (8, 128))
        kb[c, 0:8, :] = jnp.zeros((8, 128), U32)
    gates = jax.nn.sigmoid(beta_ref[...].astype(F32))
    gcol = jnp.broadcast_to(gates, (8, H)).T
    gcol = jnp.broadcast_to(gcol[:, 0:1], (H, 128))
    for g in range(8):
        gtab[g] = jnp.concatenate([gcol[4 * g:4 * g + 4]] * 2, axis=0)
    kk = lax.broadcasted_iota(jnp.int32, (64, 128), 0)
    ll = lax.broadcasted_iota(jnp.int32, (64, 128), 1)
    cmask[0] = jnp.where(kk <= ll, 0.0, NEG)
    cmask[1] = jnp.where((ll < 64) | (kk <= ll - 64), 0.0, NEG)
    cmask[2] = jnp.where(kk <= (ll & 63), 0.0, NEG)

    wait(cp_x[0], cp_wq)
    start(cp_wk, cp_wv, cp_x[1])
    wait(cp_wk)
    start(cp_h[0], cp_kv[0])

    def prologue(i, carry):
        _Paced([(qk_proj(0, i, False, True), 1600)]).finish()
        return carry

    with jax.named_scope("prologue"):
        lax.fori_loop(0, 4, prologue, 0)
    wait(cp_wv)
    for c in range(NT):
        for n in range(NT):
            wvt[c, 64 * n:64 * n + 64, :] = _u32(_bf(wvb[n, 64 * c:64 * c + 64, :]).T)
    wait(cp_x[1])
    start(cp_h[1], cp_kv[1], cp_h[2], cp_kv[2], cp_h[3], cp_kv[3], cp_fwd, cp_x[2])

    def seg0(i, carry):
        for j in range(4):
            @pl.when(i == j)
            def _():
                wait(cp_h[j], cp_kv[j])
        segment_step(0, i, [(qk_proj(1, i, True, True), 1600)], [(split_h(i), 480), (split_kv(i), 880)])
        return carry

    with jax.named_scope("seg0"):
        lax.fori_loop(0, 4, seg0, 0)
    wait(cp_fwd, cp_x[2])
    start(cp_wo, cp_x[3], cp_inv, cp_q)
    wait(cp_wo)

    def seg1(i, carry):
        segment_step(1, i, [(qk_proj(2, i, True, True), 1600), (out_proj(0, i), 800),
                            (fwd_fft(i), 2560)], [])
        return carry

    with jax.named_scope("seg1"):
        lax.fori_loop(0, 4, seg1, 0)
    start(cp_ob[0])
    wait(cp_x[3])

    def seg2(i, carry):
        segment_step(2, i, [(qk_proj(3, i, True, False), 1600), (out_proj(1, i), 800)],
                     [(spectra((0, 1, 2), [4 * i + a for a in range(4)]), 12 * SPEC_STEPS)])
        return carry

    with jax.named_scope("seg2"):
        lax.fori_loop(0, 4, seg2, 0)
    wait(cp_ob[0])
    start(cp_ob[1])

    def seg3(i, carry):
        segment_step(3, i, [(out_proj(2, i), 800)],
                     [(spectra((3, 4), [4 * i + a for a in range(4)]), 8 * SPEC_STEPS)])
        return carry

    with jax.named_scope("seg3"):
        lax.fori_loop(0, 4, seg3, 0)
    wait(cp_ob[1])
    start(cp_ob[2])
    wait(cp_inv, cp_q)

    def epilogue(i, carry):
        _Paced([(out_proj(3, i), 800), (inverse(i), 1024)]).finish()
        start([out_a(i)])
        return carry

    with jax.named_scope("epilogue"):
        lax.fori_loop(0, 4, epilogue, 0)
    wait(cp_ob[2])
    start(cp_ob[3])
    _Paced([(inverse(4), 1024)]).finish()
    start(cp_oa[4:])
    wait(cp_ob[3], cp_oa)


@jax.jit
def pallas_concat_heads__ssm_conv_h3__memory_aug_infini_attn__prompt_kernel(
    A_q: jax.Array,
    A_k: jax.Array,
    A_v: jax.Array,
    A_shift_k: jax.Array,
    A_ssm_k: jax.Array,
    A_ssm_D: jax.Array,
    B_x: jax.Array,
    B_wq: jax.Array,
    B_wk: jax.Array,
    B_wv: jax.Array,
    B_wo: jax.Array,
    B_beta: jax.Array,
):
    hbm = pl.BlockSpec(memory_space=pltpu.HBM)
    vmem = pl.BlockSpec(memory_space=pltpu.VMEM)
    seg_tiles = pltpu.VMEM((NT, L, 128), BF16)
    seq_tiles = pltpu.VMEM((NT, S // 2, 128), U32)
    w_tiles = pltpu.VMEM((NT, D // 2, 128), U32)
    scratch = [
        seq_tiles,
        w_tiles, w_tiles, w_tiles, w_tiles, w_tiles,
        pltpu.VMEM((S // 128, D // 2, 128), U32),
        pltpu.VMEM((NT, 256, 128), U32),
        pltpu.VMEM((NT, S // 2 + 8, 128), U32),
        seq_tiles, seq_tiles,
        pltpu.VMEM((N2, N1, 128), U32),
        pltpu.VMEM((N2, 2, N1 // 2, 128), U32),
        pltpu.VMEM((NT, N2, N1, 128), F32),
        pltpu.VMEM((NT, N2, N1 // 2, 128), U32),
        pltpu.VMEM((NT, N2, N1 // 2, 128), U32),
        pltpu.VMEM((NT, N1 // 8, 4, 4, 2, 8, 128), F32),
        pltpu.VMEM((NT, N1 // 8, 4, 4, 2, 8, 128), F32),
        pltpu.VMEM((12, 4, 4, 2, 8, 128), F32),
        pltpu.VMEM((NT, N2, N1, 128), U32),
        seq_tiles,
        pltpu.VMEM((NT, S, 128), BF16),
        pltpu.VMEM((NT, KS + 1, 8, 128), F32),
        pltpu.VMEM((8, 8, 128), F32),
        pltpu.VMEM((3, 64, 128), F32),
        seg_tiles, seg_tiles, seg_tiles, seg_tiles,
        seg_tiles, seg_tiles, seg_tiles, seg_tiles,
        pltpu.VMEM((4, D, 128), BF16),
        pltpu.VMEM((4, D, 128), BF16),
        pltpu.VMEM((8, 96, 128), F32),
        pltpu.SemaphoreType.DMA((23,)),
    ] + [pltpu.VMEM((2, 512, 128), F32)] * NSLOT
    return pl.pallas_call(
        _kernel,
        out_shape=jax.ShapeDtypeStruct((1, S, 2 * D), BF16),
        in_specs=[hbm, hbm, hbm, vmem, hbm, vmem, hbm, hbm, hbm, hbm, hbm, vmem, hbm, hbm],
        out_specs=hbm,
        scratch_shapes=scratch,
        compiler_params=pltpu.CompilerParams(vmem_limit_bytes=110 * 1024 * 1024),
        name="h3_infini",
    )(A_q, A_k, A_v, A_shift_k.T, A_ssm_k, A_ssm_D.reshape(NT, 128), B_x, B_wq, B_wk, B_wv, B_wo,
      B_beta.reshape(1, H), _FWD, _INV)
```

```python
import math

import jax
import jax.numpy as jnp
import numpy as np
from jax import lax
from jax.experimental import pallas as pl
from jax.experimental.pallas import tpu as pltpu

S = 2048
D = 640
NT = D // 128
H = 32
DH = D // H
NSEG = 4
L = S // NSEG
KS = 4
N1, N2 = 128, 16

F32 = jnp.float32
BF16 = jnp.bfloat16
U32 = jnp.uint32
NN_DIMS = (((1,), (0,)), ((), ()))
NT_DIMS = (((1,), (1,)), ((), ()))
NEG = -1e30
LOG2E = 1.4426950408889634


def _pack_rows(a):
    u = a.astype(np.float32).astype(BF16).view(np.uint16).astype(np.uint32)
    return u[..., 0::2, :] | (u[..., 1::2, :] << 16)


def _dft_tables():
    k1 = np.arange(N1)
    fwd = np.zeros((N2, 2 * N1, N1), np.float64)
    inv = np.zeros((N2, N1, 2 * N1), np.float64)
    kappa = np.arange(N1)
    n1_in = 16 * (kappa // 16) + 8 * (kappa % 2) + (kappa % 16) // 2
    row_re = 16 * (k1 // 8) + k1 % 8
    for n2 in range(N2):
        ang = 2.0 * np.pi * np.outer(k1 + 0.25, N2 * n1_in + n2) / S
        fwd[n2, row_re] = np.cos(ang)
        fwd[n2, row_re + 8] = np.sin(ang)
        ang = 2.0 * np.pi * np.outer(N2 * np.arange(N1) + n2, k1 + 0.25) / S
        inv[n2][:, 2 * k1] = np.cos(ang) / S
        inv[n2][:, 2 * k1 + 1] = np.sin(ang) / S
    inv = inv.reshape(N2, N1, 2, N1).transpose(0, 2, 1, 3)
    return _pack_rows(fwd), _pack_rows(inv)


_FWD, _INV = _dft_tables()


def _dot(a, b, dims=NN_DIMS):
    return lax.dot_general(a, b, dims, preferred_element_type=F32)


def _u32(x):
    return pltpu.bitcast(x, U32)


def _bf(x):
    return pltpu.bitcast(x, BF16)


def _u32_word(x):
    return lax.bitcast_convert_type(x, U32)


def _pack2(a, b):
    return pltpu.pack_elementwise([a, b], packed_dtype=BF16).astype(U32)


def _lo(w):
    return pltpu.unpack_elementwise(w, index=0, packed_dtype=BF16, unpacked_dtype=F32)


def _hi(w):
    return pltpu.unpack_elementwise(w, index=1, packed_dtype=BF16, unpacked_dtype=F32)


def _radix4(x0, x1, x2, x3, sign):
    ar, ai = x0[0] + x2[0], x0[1] + x2[1]
    br, bi = x0[0] - x2[0], x0[1] - x2[1]
    cr, ci = x1[0] + x3[0], x1[1] + x3[1]
    dr, di = x1[0] - x3[0], x1[1] - x3[1]
    y0 = (ar + cr, ai + ci)
    y2 = (ar - cr, ai - ci)
    yp = (br - di, bi + dr)
    ym = (br + di, bi - dr)
    return (y0, yp, y2, ym) if sign > 0 else (y0, ym, y2, yp)


def _twiddle(x, e, sign):
    xr, xi = x
    if e == 0:
        return x
    if e == 4:
        return (-xi, xr) if sign > 0 else (xi, -xr)
    r = math.sqrt(0.5)
    if e == 2:
        return ((xr - xi) * r, (xr + xi) * r) if sign > 0 else ((xr + xi) * r, (xi - xr) * r)
    if e == 6:
        return ((xr + xi) * -r, (xr - xi) * r) if sign > 0 else ((xi - xr) * r, (xr + xi) * -r)
    c, s = math.cos(math.pi * e / 8), sign * math.sin(math.pi * e / 8)
    return (xr * c - xi * s, xr * s + xi * c)


def _radix4_tw(x0, x1, x2, x3, sign, b):
    if b != 2:
        return _radix4(x0, _twiddle(x1, b, sign), _twiddle(x2, 2 * b, sign),
                       _twiddle(x3, 3 * b, sign), sign)
    x1, x3 = _twiddle(x1, 2, sign), _twiddle(x3, 6, sign)
    if sign > 0:
        ar, ai = x0[0] - x2[1], x0[1] + x2[0]
        br, bi = x0[0] + x2[1], x0[1] - x2[0]
    else:
        ar, ai = x0[0] + x2[1], x0[1] - x2[0]
        br, bi = x0[0] - x2[1], x0[1] + x2[0]
    cr, ci = x1[0] + x3[0], x1[1] + x3[1]
    dr, di = x1[0] - x3[0], x1[1] - x3[1]
    y0 = (ar + cr, ai + ci)
    y2 = (ar - cr, ai - ci)
    yp = (br - di, bi + dr)
    ym = (br + di, bi - dr)
    return (y0, yp, y2, ym) if sign > 0 else (y0, ym, y2, yp)


class _Paced:
    def __init__(self, streams, sequential=False):
        self.live = [[g, total, 0] for g, total in streams]
        self.total = sum(total for _, total in streams)
        self.done = 0
        self.sequential = sequential

    def step(self):
        cur = self.live[0] if self.sequential else min(self.live, key=lambda e: e[2] / e[1])
        cost = next(cur[0], None)
        if cost is None:
            self.live.remove(cur)
        else:
            cur[2] += cost
            self.done += cost

    def advance(self, fraction):
        while self.live and self.done < fraction * self.total:
            self.step()

    def finish(self):
        self.advance(math.inf)


DEPTH = 3
TAIL = 0.06
EARLY = 1.0
PACE = True
LW = 1.0
AW = 5.0
NSLOT = DEPTH + 1
QCH = 256


def _kernel(aq_hbm, ak_hbm, av_hbm, shift_ref, h_hbm, ssmd_ref, x_hbm, wq_hbm, wk_hbm,
            wv_hbm, wo_hbm, beta_ref, fwd_hbm, inv_hbm, out_hbm,
            xb, wqb, wkb, wvb, wob, wvt, hb, ht, kb, vb, qb, fwd, inv,
            kvf, xp, hp, tx, th, ub, yb, outa, outb, wtab, gtab, cmask,
            q0, q1, k0, k1, pq0, pq1, pk0, pk1, ot0, ot1, mst,
            hmask, hsel, bmask, kwin, vall, vhead, opart, onat, sems, *slots):
    qs, ks, pqs, pks, ots = (q0, q1), (k0, k1), (pq0, pq1), (pk0, pk1), (ot0, ot1)

    def col_tiles(src, dst, sem, rows=None, lead=(0,), dst_off=0, tiles=range(NT)):
        r0, n = rows if rows is not None else (0, src.shape[-2])

        def one(t):
            return lambda: pltpu.make_async_copy(
                src.bitcast(U32).at[(*lead, pl.ds(r0 // 2, n // 2), pl.ds(128 * t, 128))],
                dst.at[t, pl.ds(dst_off + r0 // 2, n // 2), :], sems.at[sem])
        return [one(t) for t in tiles]

    cp_x = [col_tiles(x_hbm, xb, s, rows=(L * s, L)) for s in range(NSEG)]
    cp_wq = col_tiles(wq_hbm, wqb, 4, lead=())
    cp_wk = col_tiles(wk_hbm, wkb, 5, lead=())
    cp_wv = col_tiles(wv_hbm, wvb, 6, lead=())
    cp_wo = col_tiles(wo_hbm, wob, 7, lead=())
    cp_h = [col_tiles(h_hbm, hb, 8 + i, lead=(), tiles=range(4 * i, 4 * i + 4)) for i in range(4)]
    cp_kv = [col_tiles(ak_hbm, kb, 19 + i, rows=(L * i, L), dst_off=8)
             + col_tiles(av_hbm, vb, 19 + i, rows=(L * i, L)) for i in range(4)]
    cp_q = col_tiles(aq_hbm, qb, 14)
    cp_fwd = [lambda: pltpu.make_async_copy(fwd_hbm, fwd, sems.at[15])]
    cp_inv = [lambda: pltpu.make_async_copy(inv_hbm, inv, sems.at[16])]

    def out_a(c):
        c0 = 128 * c if isinstance(c, int) else pl.multiple_of(128 * c, 128)
        return lambda: pltpu.make_async_copy(
            outa.at[c], out_hbm.bitcast(U32).at[0, :, pl.ds(c0, 128)], sems.at[17])

    def out_b(s, n):
        return lambda: pltpu.make_async_copy(
            outb.at[n, pl.ds(L * s, L), :],
            out_hbm.at[0, pl.ds(L * s, L), pl.ds(D + 128 * n, 128)], sems.at[18])

    cp_oa = [out_a(c) for c in range(NT)]
    cp_ob = [[out_b(s, n) for n in range(NT)] for s in range(NSEG)]

    def start(*groups):
        for g in groups:
            for cp in g:
                cp().start()

    def wait(*groups):
        for g in groups:
            for cp in g:
                cp().wait()

    def rows(i, n):
        return pl.ds(pl.multiple_of(i * n, n), n) if not isinstance(i, int) else pl.ds(i * n, n)

    lane = lax.broadcasted_iota(jnp.int32, (8, 128), 1)
    sub = lax.broadcasted_iota(jnp.int32, (8, 128), 0)

    def lanes(n):
        return lax.broadcasted_iota(jnp.int32, (n, 128), 1)

    recent = [None]

    def dot(a, b, dims=NN_DIMS):
        recent[0] = _dot(a, b, dims)
        return recent[0]

    def pace(i, targets):
        if recent[0] is not None:
            for target in targets:
                target(jnp.minimum(i, 3), recent[0][-8:])
            recent[0] = None

    def qk_proj(s, i, want_pq, want_pk):
        p = s % 2
        tok = rows(4 * s + i, 64)
        for w_ref, dst, fdst, want, scale in (
                (wqb, qs[p], pqs[p], want_pq, DH ** -0.5 * LOG2E),
                (wkb, ks[p], pks[p], want_pk, None)):
            for n in range(NT):
                t = None
                for c in range(NT):
                    part = dot(_bf(xb[c, tok, :]), _bf(w_ref[n, 64 * c:64 * c + 64, :]))
                    t = part if t is None else t + part
                    if c < NT - 1:
                        yield 32
                dst[n, rows(i, 128), :] = (t if scale is None else t * scale).astype(BF16)
                if want:
                    fdst[n, rows(i, 128), :] = jnp.where(t > 0, t + 1.0, jnp.exp(t)).astype(BF16)
                yield 32

    def out_proj(s, i):
        ot = ots[s % 2].bitcast(U32)
        for n in range(NT):
            t = None
            for c in range(NT):
                if n == 0:
                    o = _u32(_bf(ot[i, 64 * c:64 * c + 64, :]).T)
                    onat[c] = o
                else:
                    o = onat[c]
                part = dot(_bf(o), _bf(wob[n, 64 * c:64 * c + 64, :]))
                t = part if t is None else t + part
                if c < NT - 1:
                    yield 32
            outb[n, rows(4 * s + i, 128), :] = t.astype(BF16)
            yield 32

    def tile_rows(r, n):
        return jnp.broadcast_to(r[None], (n // 8, 8, 128)).reshape(n, 128)

    class Group:
        def __init__(self, s, g, gi):
            self.s, self.g, self.gi = s, g, gi
            self.t0 = (80 * g) // 128
            self.off = 80 * g - 128 * self.t0
            self.t1 = jnp.minimum(self.t0 + 1, NT - 1)
            rel = (lane - self.off) & 127
            head = sum((rel >= a * DH).astype(jnp.int32) for a in range(1, 5))
            for a in range(4):
                hmask[gi, a] = jnp.where(head == a, np.uint32(0xFFFFFFFF), np.uint32(0))
            hsel[gi] = jnp.left_shift(1, head)
            self.have_keys, self.have_mem = set(), set()

        def window(self, ref, j, r0=0, n=64):
            ref = ref.bitcast(U32)
            at = pl.ds(64 * j + r0, n)
            return jnp.where(lanes(n) >= self.off, ref[self.t0, at, :], ref[self.t1, at, :])

        def keys(self, r0, r1):
            out = []
            for r in range(r0, r1, 64):
                at = pl.ds(r // 2, 32)
                if r in self.have_keys:
                    out.append(kwin[self.gi, at, :])
                else:
                    self.have_keys.add(r)
                    out.append(self.window(ks[self.s % 2], 0, r // 2, 32))
                    kwin[self.gi, at, :] = out[-1]
            return _bf(jnp.concatenate(out, axis=0))

        def park_values(self, j, v80):
            vall[self.gi, j, 0:80, :] = v80.astype(BF16)
            ones8 = jnp.ones((8, 128), F32)
            for pr in range(2):
                for e in range(2):
                    r0 = 40 * pr + 16 * e
                    vhead[self.gi, j, r0 // 8] = jnp.concatenate(
                        [v80[r0:r0 + 24], ones8], axis=0).astype(BF16)

        def mem_read(self):
            for j in range(4):
                r = dot(mst[self.g].astype(BF16), _bf(self.window(pqs[self.s % 2], j)), NT_DIMS)
                coef = gtab[self.g] / (r[80:88] + 1e-6)
                cb = [jnp.broadcast_to(coef[a:a + 1], (8, 128)) for a in range(4)]
                for pr in range(2):
                    ca, cc = cb[2 * pr], cb[2 * pr + 1]
                    for e, scale in enumerate((ca, ca, jnp.where(sub < 4, ca, cc), cc, cc)):
                        r0 = 40 * pr + 8 * e
                        opart[self.gi, j, r0:r0 + 8, :] = r[r0:r0 + 8] * scale
                self.have_mem.add(j)
                yield 24

        def mem_update(self):
            acc = None
            for j in range(4):
                t = dot(_bf(vall.bitcast(U32)[self.gi, j]), _bf(self.window(pks[self.s % 2], j)))
                acc = t if acc is None else acc + t
                if j < 3:
                    yield 24
            for r in range(12):
                new = jnp.where(bmask[r] & hsel[self.gi] != 0, acc[8 * r:8 * r + 8], 0.0)
                at = pl.ds(8 * r, 8)
                mst[self.g, at, :] = new if self.s == 0 else mst[self.g, at, :] + new
            yield 24

        def logits(self, pr, j, slot):
            qw = self.window(qs[self.s % 2], j)
            qa = qw & tile_rows(hmask[self.gi, 2 * pr], 64)
            qh = qw & tile_rows(hmask[self.gi, 2 * pr + 1], 64)
            w_a = _bf(qa)
            w_b = _bf(jnp.concatenate([qh[32:64], qh[0:32]], axis=0))
            w_t = _bf(jnp.concatenate([qh[32:64], qa[32:64]], axis=0))
            n = 128 * j

            def park(t, e, r0, m):
                for r in range(0, t.shape[0], 8):
                    v = t[r:r + 8]
                    if e == 2:
                        v = v + cmask[2, r:r + 8, :]
                    elif r0 + r >= n:
                        v = v + cmask[e, r0 + r - n:r0 + r - n + 8, :]
                    slot[e % 2, 448 * (e // 2) + r0 + r:448 * (e // 2) + r0 + r + 8, :] = v
                    m = v if m is None else jnp.maximum(m, v)
                return m

            m_t = park(dot(self.keys(n + 64, n + 128), w_t, NT_DIMS), 2, 0, None)
            yield 16 * LW
            cuts = list(range(0, n, QCH)) or [0]
            m = [None, None]
            for r0, r1 in zip(cuts, cuts[1:] + [n + 64]):
                for e, w in enumerate((w_a, w_b)):
                    m[e] = park(dot(self.keys(r0, r1), w, NT_DIMS), e, r0, m[e])
                    if r1 == n + 64 and e == 1:
                        m_a = jnp.maximum(m[0], jnp.where(lane >= 64, m_t, NEG))
                        m_b = jnp.maximum(m[1], jnp.where(lane < 64, m_t, NEG))
                        m_a = jnp.broadcast_to(jnp.max(m_a, axis=0, keepdims=True), (8, 128))
                        m_b = jnp.broadcast_to(jnp.max(m_b, axis=0, keepdims=True), (8, 128))
                        slot[1, 448:456, :] = m_a
                        slot[1, 456:464, :] = m_b
                        slot[1, 464:472, :] = jnp.where(lane < 64, m_b, m_a)
                    yield (r1 - r0) // 4 * LW

        def attend(self, pr, j, slot, need_values):
            def prob(e, r0, n, which):
                m2 = tile_rows(slot[1, 448 + 8 * which:456 + 8 * which, :], 16)
                return [jnp.exp2(slot[e, r:r + 16, :] - m2).astype(BF16)
                        for r in range(r0, r0 + n, 16)]

            p_t = _u32(jnp.concatenate(prob(0, 448, 64, 2), axis=0))
            tails = (_bf(jnp.where(lanes(32) >= 64, p_t, np.uint32(0))),
                     _bf(jnp.where(lanes(32) >= 64, np.uint32(0), p_t)))
            res = []
            for e in range(2):
                acc = None
                for kt in range(j + 1):
                    need_values(kt)
                    if kt < j:
                        p = prob(e, 128 * kt, 128, e)
                    else:
                        p = prob(e, 128 * kt, 64, e) + [tails[e]]
                    t = dot(_bf(vhead.bitcast(U32)[self.gi, kt, 5 * pr + 2 * e]),
                             jnp.concatenate(p, axis=0))
                    acc = t if acc is None else acc + t
                    if (e, kt) != (1, j):
                        yield 8 * AW
                res.append(acc)
            r_a = res[0]
            r_b = pltpu.roll(res[1], 64, 1)
            keep = 1.0 - gtab[self.g]
            keep_a = jnp.broadcast_to(keep[2 * pr:2 * pr + 1], (8, 128))
            keep_b = jnp.broadcast_to(keep[2 * pr + 1:2 * pr + 2], (8, 128))
            o_a = r_a[0:24] * tile_rows(keep_a / r_a[24:32], 24)
            o_b = r_b[0:24] * tile_rows(keep_b / r_b[24:32], 24)
            o = jnp.concatenate(
                [o_a[0:16], jnp.where(sub < 4, o_a[16:24], o_b[0:8]), o_b[8:24]], axis=0)
            if self.s > 0:
                o = o + opart[self.gi, j, 40 * pr:40 * pr + 40, :]
            if pr == 0:
                opart[self.gi, j, 0:40, :] = o
            else:
                o = jnp.concatenate([opart[self.gi, j, 0:40, :], o], axis=0)
                ots[self.s % 2][j, rows(self.g, 80), :] = o.astype(BF16)
            yield 8 * AW

    def v_proj(s, i, groups, have):
        for j in range(4):
            acc = None
            for c in range(NT):
                t = dot(_bf(wvt[c, rows(i, 80), :]), _bf(xb[c, rows(4 * s + j, 64), :]), NT_DIMS)
                acc = t if acc is None else acc + t
                if c == NT - 1:
                    for gi in range(2):
                        groups[gi].park_values(j, acc[80 * gi:80 * gi + 80])
                    have.append(j)
                yield 40

    def chain(*gens):
        for g in gens:
            yield from g

    def segment_step(s, i, mxu_fill, vpu_fill, targets):
        vt = []
        groups = [Group(s, 2 * i + gi, gi) for gi in range(2)]
        units = [(gi, pr, j if (gi, pr) != (1, 1) else 3 - j)
                 for gi in range(2) for pr in range(2) for j in range(4)]
        reads = [grp.mem_read() for grp in groups if s > 0]
        updates = [grp.mem_update() for grp in groups if s < NSEG - 1]
        first = _Paced([(chain(*reads[:1], v_proj(s, i, groups, vt), *reads[1:], *updates),
                         800 + 96 * (len(reads) + len(updates)))])
        fill = _Paced(mxu_fill)
        side = _Paced(vpu_fill)
        nstep = len(units) + DEPTH
        total = first.total + fill.total

        def need_values(kt):
            while len(vt) <= kt:
                first.step()

        def pad(fraction):
            target = total * fraction / (1 + TAIL)
            early = min(target * EARLY, first.total)
            first.advance(early / first.total)
            fill.advance((target - early) / fill.total)
            if side.live and side.done < fraction * side.total:
                if PACE:
                    pace(i, targets)
                side.advance(fraction)

        def cost(j):
            return (48 + 64 * j) * LW, (16 + 16 * j) * AW

        whole = sum(sum(cost(j)) for _, _, j in units)
        done = 0
        for u in range(nstep):
            streams = []
            if u < len(units):
                gi, pr, j = units[u]
                streams.append((groups[gi].logits(pr, j, slots[u % NSLOT]), cost(j)[0]))
            if u >= DEPTH:
                v = u - DEPTH
                gi, pr, j = units[v]
                while s > 0 and j not in groups[gi].have_mem:
                    first.step()
                streams.append((groups[gi].attend(pr, j, slots[v % NSLOT], need_values), cost(j)[1]))
            att = _Paced(streams)
            while att.live:
                att.step()
                pad((done + att.done) / whole)
            done += att.total
        first.finish()
        fill.finish()
        side.finish()

    def split_h(i):
        for c in range(NT):
            for t in range(4):
                ht[c, 64 * t:64 * t + 64, :] = _u32(_bf(hb[4 * i + t, 64 * c:64 * c + 64, :]).T)
                yield 16
            for q in range(2):
                for j in range(8):
                    wa = ht[c, pl.ds(128 * q + j, 8, stride=8), :]
                    wb = ht[c, pl.ds(128 * q + 64 + j, 8, stride=8), :]
                    hp[c, 2 * j, rows(2 * i + q, 8), :] = _pack2(_lo(wa), _lo(wb))
                    hp[c, 2 * j + 1, rows(2 * i + q, 8), :] = _pack2(_hi(wa), _hi(wb))
                    if j % 2:
                        yield 4

    def split_kv(i):
        for c in range(NT):
            taps = [wtab[c, j] for j in range(KS)]
            for q in range(2):
                blk = 2 * i + q
                base = [blk * 128 + 64 * e for e in range(2)]
                hist = []
                for e in range(2):
                    w2 = kb[c, pl.ds(base[e] + 6, 8, stride=8), :]
                    w1 = kb[c, pl.ds(base[e] + 7, 8, stride=8), :]
                    hist.append([_hi(w2), _lo(w1), _hi(w1)])
                for j in range(8):
                    kv = [[None, None], [None, None]]
                    for e in range(2):
                        kw = kb[c, pl.ds(base[e] + 8 + j, 8, stride=8), :]
                        vw = vb[c, pl.ds(base[e] + j, 8, stride=8), :]
                        kp = hist[e] + [_lo(kw), _hi(kw)]
                        for half, part in enumerate((_lo, _hi)):
                            acc = kp[3 + half] * taps[0]
                            for d in range(1, KS):
                                acc = acc + kp[3 + half - d] * taps[d]
                            kv[half][e] = acc * part(vw)
                            kvf[c, 2 * j + half, rows(2 * blk + e, 8), :] = kv[half][e]
                        hist[e] = kp[2:]
                    for half in range(2):
                        xp[c, 2 * j + half, rows(blk, 8), :] = _pack2(*kv[half])
                    yield 11

    def fwd_fft(i):
        for c in range(NT):
            for src, dst in ((hp, th), (xp, tx)):
                g = [dot(_bf(fwd[4 * a + i]), _bf(src[c, 4 * a + i])) for a in range(4)]
                for m in range(N1 // 8):
                    z = _radix4(*[(g[a][16 * m:16 * m + 8], g[a][16 * m + 8:16 * m + 16])
                                  for a in range(4)], 1)
                    for cc in range(4):
                        dst[c, m, cc, i, 0] = z[cc][0]
                        dst[c, m, cc, i, 1] = z[cc][1]
                yield 256

    def spectrum(c, m, slot):
        for cc in range(4):
            zh = _radix4_tw(*[(th[c, m, cc, b, 0], th[c, m, cc, b, 1]) for b in range(4)], 1, cc)
            yield 1
            zx = _radix4_tw(*[(tx[c, m, cc, b, 0], tx[c, m, cc, b, 1]) for b in range(4)], 1, cc)
            yield 1
            y = [(x[0] * h[0] - x[1] * h[1], x[0] * h[1] + x[1] * h[0]) for x, h in zip(zx, zh)]
            yield 1
            u = _radix4(*y, -1)
            for b in range(4):
                ub[slot, b, cc, 0] = u[b][0]
                ub[slot, b, cc, 1] = u[b][1]
            yield 1
        for b in range(4):
            z = _radix4_tw(*[(ub[slot, b, cc, 0], ub[slot, b, cc, 1]) for cc in range(4)], -1, b)
            for a in range(4):
                yb[c, 4 * a + b, rows(m, 8), :] = _pack2(*z[a])
            yield 1

    SPEC_STEPS = 20

    def spectra(cs, ms):
        for slot, (c, m) in enumerate((c, m) for c in cs for m in ms):
            yield from spectrum(c, m, slot)

    def spare_h(d, v):
        hb[S // 128, rows(d, 8), :] = _u32_word(v)

    def spare_k(d, v):
        kb[NT, rows(d, 8), :] = _u32_word(v)

    def spare_t(d, v):
        th[NT, d, 0, 0, 0] = v

    def inverse(c):
        dvec = tile_rows(wtab[c, KS], N1)
        for jp in range(8):
            w = qb[c, pl.ds(jp, N1, stride=8), :]
            res = []
            for e, part in enumerate((_lo, _hi)):
                n2 = 2 * jp + e
                y = (dot(_bf(inv[n2, 0]), _bf(yb[c, n2, 0:64, :]))
                     + dot(_bf(inv[n2, 1]), _bf(yb[c, n2, 64:128, :])))
                res.append(part(w) * (y + kvf[c, n2] * dvec))
            outa[c, pl.ds(jp, N1, stride=8), :] = _pack2(*res)
            yield 128

    start(cp_x[0], cp_wq)
    taps_t = shift_ref[...].astype(F32)
    skip = ssmd_ref[...].astype(F32)
    for c in range(NT):
        for j in range(KS):
            wtab[c, j] = jnp.broadcast_to(taps_t[j:j + 1, 128 * c:128 * c + 128], (8, 128))
        wtab[c, KS] = jnp.broadcast_to(skip[c:c + 1], (8, 128))
        kb[c, 0:8, :] = jnp.zeros((8, 128), U32)
    gates = jax.nn.sigmoid(beta_ref[...].astype(F32))
    gcol = jnp.broadcast_to(gates, (8, H)).T
    gcol = jnp.broadcast_to(gcol[:, 0:1], (H, 128))
    for g in range(8):
        gtab[g] = jnp.concatenate([gcol[4 * g:4 * g + 4]] * 2, axis=0)
    kk = lax.broadcasted_iota(jnp.int32, (64, 128), 0)
    ll = lax.broadcasted_iota(jnp.int32, (64, 128), 1)
    cmask[0] = jnp.where(kk <= ll, 0.0, NEG)
    cmask[1] = jnp.where((ll < 64) | (kk <= ll - 64), 0.0, NEG)
    cmask[2] = jnp.where(kk <= (ll & 63), 0.0, NEG)
    for r in range(12):
        row = sub + 8 * r
        hr = sum((row >= a * DH).astype(jnp.int32) for a in range(1, 4)) if r < 10 else row - 80
        bmask[r] = jnp.left_shift(1, hr)
    for gi in range(2):
        for j in range(4):
            vall[gi, j, 80:96, :] = jnp.ones((16, 128), BF16)

    wait(cp_x[0], cp_wq)
    start(cp_wk, cp_wv, cp_x[1])
    wait(cp_wk)
    start(cp_h[0], cp_kv[0])

    def prologue(i, carry):
        _Paced([(qk_proj(0, i, False, True), 1600)]).finish()
        return carry

    with jax.named_scope("prologue"):
        lax.fori_loop(0, 4, prologue, 0)
    wait(cp_wv)
    for c in range(NT):
        for n in range(NT):
            wvt[c, 64 * n:64 * n + 64, :] = _u32(_bf(wvb[n, 64 * c:64 * c + 64, :]).T)
    wait(cp_x[1])
    start(cp_h[1], cp_kv[1], cp_h[2], cp_kv[2], cp_h[3], cp_kv[3], cp_fwd, cp_x[2])

    def seg0(i, carry):
        for j in range(4):
            @pl.when(i == j)
            def _():
                wait(cp_h[j], cp_kv[j])
        segment_step(0, i, [(qk_proj(1, i, True, True), 1600)], [(split_h(i), 480), (split_kv(i), 880)], [spare_h, spare_k])
        return carry

    with jax.named_scope("seg0"):
        lax.fori_loop(0, 4, seg0, 0)
    wait(cp_fwd, cp_x[2])
    start(cp_wo, cp_x[3], cp_inv, cp_q)
    wait(cp_wo)

    def seg1(i, carry):
        segment_step(1, i, [(qk_proj(2, i, True, True), 1600), (out_proj(0, i), 800),
                            (fwd_fft(i), 2560)], [], [])
        return carry

    with jax.named_scope("seg1"):
        lax.fori_loop(0, 4, seg1, 0)
    start(cp_ob[0])
    wait(cp_x[3])

    def seg2(i, carry):
        segment_step(2, i, [(qk_proj(3, i, True, False), 1600), (out_proj(1, i), 800)],
                     [(spectra((0, 1, 2), [4 * i + a for a in range(4)]), 12 * SPEC_STEPS)],
                     [spare_t])
        return carry

    with jax.named_scope("seg2"):
        lax.fori_loop(0, 4, seg2, 0)
    wait(cp_ob[0])
    start(cp_ob[1])

    def seg3(i, carry):
        segment_step(3, i, [(out_proj(2, i), 800)],
                     [(spectra((3, 4), [4 * i + a for a in range(4)]), 8 * SPEC_STEPS)],
                     [spare_t])
        return carry

    with jax.named_scope("seg3"):
        lax.fori_loop(0, 4, seg3, 0)
    wait(cp_ob[1])
    start(cp_ob[2])
    wait(cp_inv, cp_q)

    def epilogue(i, carry):
        _Paced([(out_proj(3, i), 800), (inverse(i), 1024)]).finish()
        start([out_a(i)])
        return carry

    with jax.named_scope("epilogue"):
        lax.fori_loop(0, 4, epilogue, 0)
    wait(cp_ob[2])
    start(cp_ob[3])
    _Paced([(inverse(4), 1024)]).finish()
    start(cp_oa[4:])
    wait(cp_ob[3], cp_oa)


@jax.jit
def pallas_concat_heads__ssm_conv_h3__memory_aug_infini_attn__prompt_kernel(
    A_q: jax.Array,
    A_k: jax.Array,
    A_v: jax.Array,
    A_shift_k: jax.Array,
    A_ssm_k: jax.Array,
    A_ssm_D: jax.Array,
    B_x: jax.Array,
    B_wq: jax.Array,
    B_wk: jax.Array,
    B_wv: jax.Array,
    B_wo: jax.Array,
    B_beta: jax.Array,
):
    hbm = pl.BlockSpec(memory_space=pltpu.HBM)
    vmem = pl.BlockSpec(memory_space=pltpu.VMEM)
    seg_tiles = pltpu.VMEM((NT, L, 128), BF16)
    seq_tiles = pltpu.VMEM((NT, S // 2, 128), U32)
    w_tiles = pltpu.VMEM((NT, D // 2, 128), U32)
    scratch = [
        seq_tiles,
        w_tiles, w_tiles, w_tiles, w_tiles, w_tiles,
        pltpu.VMEM((S // 128 + 1, D // 2, 128), U32),
        pltpu.VMEM((NT, 256, 128), U32),
        pltpu.VMEM((NT + 1, S // 2 + 8, 128), U32),
        seq_tiles, seq_tiles,
        pltpu.VMEM((N2, N1, 128), U32),
        pltpu.VMEM((N2, 2, N1 // 2, 128), U32),
        pltpu.VMEM((NT, N2, N1, 128), F32),
        pltpu.VMEM((NT, N2, N1 // 2, 128), U32),
        pltpu.VMEM((NT, N2, N1 // 2, 128), U32),
        pltpu.VMEM((NT, N1 // 8, 4, 4, 2, 8, 128), F32),
        pltpu.VMEM((NT + 1, N1 // 8, 4, 4, 2, 8, 128), F32),
        pltpu.VMEM((12, 4, 4, 2, 8, 128), F32),
        pltpu.VMEM((NT, N2, N1, 128), U32),
        seq_tiles,
        pltpu.VMEM((NT, S, 128), BF16),
        pltpu.VMEM((NT, KS + 1, 8, 128), F32),
        pltpu.VMEM((8, 8, 128), F32),
        pltpu.VMEM((3, 64, 128), F32),
        seg_tiles, seg_tiles, seg_tiles, seg_tiles,
        seg_tiles, seg_tiles, seg_tiles, seg_tiles,
        pltpu.VMEM((4, D, 128), BF16),
        pltpu.VMEM((4, D, 128), BF16),
        pltpu.VMEM((8, 96, 128), F32),
        pltpu.VMEM((2, 4, 8, 128), U32),
        pltpu.VMEM((2, 8, 128), jnp.int32),
        pltpu.VMEM((12, 8, 128), jnp.int32),
        pltpu.VMEM((2, L // 2, 128), U32),
        pltpu.VMEM((2, 4, 96, 128), BF16),
        pltpu.VMEM((2, 4, 8, 32, 128), BF16),
        pltpu.VMEM((2, 4, 80, 128), F32),
        pltpu.VMEM((NT, 64, 128), U32),
        pltpu.SemaphoreType.DMA((23,)),
    ] + [pltpu.VMEM((2, 512, 128), F32)] * NSLOT
    return pl.pallas_call(
        _kernel,
        out_shape=jax.ShapeDtypeStruct((1, S, 2 * D), BF16),
        in_specs=[hbm, hbm, hbm, vmem, hbm, vmem, hbm, hbm, hbm, hbm, hbm, vmem, hbm, hbm],
        out_specs=hbm,
        scratch_shapes=scratch,
        compiler_params=pltpu.CompilerParams(vmem_limit_bytes=110 * 1024 * 1024),
        name="h3_infini",
    )(A_q, A_k, A_v, A_shift_k.T, A_ssm_k, A_ssm_D.reshape(NT, 128), B_x, B_wq, B_wk, B_wv, B_wo,
      B_beta.reshape(1, H), _FWD, _INV)
```

```python
import math

import jax
import jax.numpy as jnp
import numpy as np
from jax import lax
from jax.experimental import pallas as pl
from jax.experimental.pallas import tpu as pltpu

S = 2048
D = 640
NT = D // 128
H = 32
DH = D // H
NSEG = 4
L = S // NSEG
KS = 4
N1, N2 = 128, 16

F32 = jnp.float32
BF16 = jnp.bfloat16
U32 = jnp.uint32
NN_DIMS = (((1,), (0,)), ((), ()))
NT_DIMS = (((1,), (1,)), ((), ()))
NEG = -1e30
LOG2E = 1.4426950408889634


def _pack_rows(a):
    u = a.astype(np.float32).astype(BF16).view(np.uint16).astype(np.uint32)
    return u[..., 0::2, :] | (u[..., 1::2, :] << 16)


def _dft_tables():
    k1 = np.arange(N1)
    fwd = np.zeros((N2, 2 * N1, N1), np.float64)
    inv = np.zeros((N2, N1, 2 * N1), np.float64)
    kappa = np.arange(N1)
    n1_in = 16 * (kappa // 16) + 8 * (kappa % 2) + (kappa % 16) // 2
    row_re = 16 * (k1 // 8) + k1 % 8
    for n2 in range(N2):
        ang = 2.0 * np.pi * np.outer(k1 + 0.25, N2 * n1_in + n2) / S
        fwd[n2, row_re] = np.cos(ang)
        fwd[n2, row_re + 8] = np.sin(ang)
        ang = 2.0 * np.pi * np.outer(N2 * np.arange(N1) + n2, k1 + 0.25) / S
        inv[n2][:, 2 * k1] = np.cos(ang) / S
        inv[n2][:, 2 * k1 + 1] = np.sin(ang) / S
    inv = inv.reshape(N2, N1, 2, N1).transpose(0, 2, 1, 3)
    return _pack_rows(fwd), _pack_rows(inv)


_FWD, _INV = _dft_tables()


def _dot(a, b, dims=NN_DIMS):
    return lax.dot_general(a, b, dims, preferred_element_type=F32)


def _u32(x):
    return pltpu.bitcast(x, U32)


def _bf(x):
    return pltpu.bitcast(x, BF16)


def _u32_word(x):
    return lax.bitcast_convert_type(x, U32)


def _pack2(a, b):
    return pltpu.pack_elementwise([a, b], packed_dtype=BF16).astype(U32)


def _lo(w):
    return pltpu.unpack_elementwise(w, index=0, packed_dtype=BF16, unpacked_dtype=F32)


def _hi(w):
    return pltpu.unpack_elementwise(w, index=1, packed_dtype=BF16, unpacked_dtype=F32)


def _radix4(x0, x1, x2, x3, sign):
    ar, ai = x0[0] + x2[0], x0[1] + x2[1]
    br, bi = x0[0] - x2[0], x0[1] - x2[1]
    cr, ci = x1[0] + x3[0], x1[1] + x3[1]
    dr, di = x1[0] - x3[0], x1[1] - x3[1]
    y0 = (ar + cr, ai + ci)
    y2 = (ar - cr, ai - ci)
    yp = (br - di, bi + dr)
    ym = (br + di, bi - dr)
    return (y0, yp, y2, ym) if sign > 0 else (y0, ym, y2, yp)


def _twiddle(x, e, sign):
    xr, xi = x
    if e == 0:
        return x
    if e == 4:
        return (-xi, xr) if sign > 0 else (xi, -xr)
    r = math.sqrt(0.5)
    if e == 2:
        return ((xr - xi) * r, (xr + xi) * r) if sign > 0 else ((xr + xi) * r, (xi - xr) * r)
    if e == 6:
        return ((xr + xi) * -r, (xr - xi) * r) if sign > 0 else ((xi - xr) * r, (xr + xi) * -r)
    c, s = math.cos(math.pi * e / 8), sign * math.sin(math.pi * e / 8)
    return (xr * c - xi * s, xr * s + xi * c)


def _radix4_tw(x0, x1, x2, x3, sign, b):
    if b != 2:
        return _radix4(x0, _twiddle(x1, b, sign), _twiddle(x2, 2 * b, sign),
                       _twiddle(x3, 3 * b, sign), sign)
    x1, x3 = _twiddle(x1, 2, sign), _twiddle(x3, 6, sign)
    if sign > 0:
        ar, ai = x0[0] - x2[1], x0[1] + x2[0]
        br, bi = x0[0] + x2[1], x0[1] - x2[0]
    else:
        ar, ai = x0[0] + x2[1], x0[1] - x2[0]
        br, bi = x0[0] - x2[1], x0[1] + x2[0]
    cr, ci = x1[0] + x3[0], x1[1] + x3[1]
    dr, di = x1[0] - x3[0], x1[1] - x3[1]
    y0 = (ar + cr, ai + ci)
    y2 = (ar - cr, ai - ci)
    yp = (br - di, bi + dr)
    ym = (br + di, bi - dr)
    return (y0, yp, y2, ym) if sign > 0 else (y0, ym, y2, yp)


class _Paced:
    def __init__(self, streams, sequential=False):
        self.live = [[g, total, 0] for g, total in streams]
        self.total = sum(total for _, total in streams)
        self.done = 0
        self.sequential = sequential

    def step(self):
        cur = self.live[0] if self.sequential else min(self.live, key=lambda e: e[2] / e[1])
        cost = next(cur[0], None)
        if cost is None:
            self.live.remove(cur)
        else:
            cur[2] += cost
            self.done += cost

    def advance(self, fraction):
        while self.live and self.done < fraction * self.total:
            self.step()

    def finish(self):
        self.advance(math.inf)


DEPTH = 3
TAIL = 0.0
EARLY = 1.0
PACE_ON = 3
PACE_ALL = 0
HEAD = 4
SEQ_FILL = True
FCH = 256
VSPLIT = ((0, 1),)
EARLY_TILES = (0, 1, 2)
LATE_TILES = tuple(c for c in range(NT) if c not in EARLY_TILES)
LW = 1.0
AW = 3.0
NSLOT = 4
LAST_ORDER = (0, 1, 2, 3)
QCH = 256


def _kernel(aq_hbm, ak_hbm, av_hbm, shift_hbm, h_hbm, ssmd_hbm, x_hbm, wq_hbm, wk_hbm,
            wv_hbm, wo_hbm, beta_hbm, fwd_hbm, inv_hbm, out_hbm, shift_ref, ssmd_ref, beta_ref,
            xb, wqb, wkb, wvb, wob, wvt, hb, ht, kb, vb, qb, fwd, inv,
            kvf, ub, outa, outb, wtab, gtab, cmask,
            q0, q1, k0, k1, pq0, pq1, pk0, pk1, ots, mst,
            hmask, hsel, bmask, kwin, vall, vhead, opart, onat, sems, *rest):
    sets = (rest[0:5], rest[5:10])
    slots = rest[10:]

    def fft_bufs(c):
        if c in EARLY_TILES:
            return EARLY_TILES.index(c), sets[0]
        return LATE_TILES.index(c), sets[1]

    qs, ks, pqs, pks = (q0, q1), (k0, k1), (pq0, pq1), (pk0, pk1)

    def tile_copy(src, dst, t, sem, r0, n, lead=(0,), dst_off=0):
        return lambda: pltpu.make_async_copy(
            src.bitcast(U32).at[(*lead, pl.ds(r0 // 2, n // 2), pl.ds(128 * t, 128))],
            dst.at[t, pl.ds(dst_off + r0 // 2, n // 2), :], sems.at[sem])

    def h_copy(t, c0, n, sem):
        return lambda: pltpu.make_async_copy(
            h_hbm.bitcast(U32).at[pl.ds(64 * c0, 64 * n), pl.ds(128 * t, 128)],
            hb.at[t, pl.ds(64 * c0, 64 * n), :], sems.at[sem])

    def conv_copies(cs, i, sem):
        out = [h_copy(4 * i + t, cs[0], len(cs), sem) for t in range(4)]
        out += [tile_copy(ak_hbm, kb, c, sem, L * i, L, dst_off=8) for c in cs]
        return out + [tile_copy(av_hbm, vb, c, sem, L * i, L) for c in cs]

    cp_x = [[tile_copy(x_hbm, xb, t, s, L * s, L) for t in range(NT)] for s in range(NSEG)]
    cp_w = [[tile_copy(src, dst, n, 4 + n, 0, D, lead=())
             for src, dst in ((wq_hbm, wqb), (wk_hbm, wkb), (wv_hbm, wvb))] for n in range(NT)]
    cp_wo = [tile_copy(wo_hbm, wob, n, 9, 0, D, lead=()) for n in range(NT)]
    cp_early = [conv_copies(EARLY_TILES, i, 10 + i) for i in range(4)]
    cp_late = [cp for i in range(4) for cp in conv_copies(LATE_TILES, i, 14)]
    cp_q = [tile_copy(aq_hbm, qb, c, 15, 0, S) for c in range(NT)]
    cp_fwd = [lambda: pltpu.make_async_copy(fwd_hbm, fwd, sems.at[16])]
    cp_inv = [lambda: pltpu.make_async_copy(inv_hbm, inv, sems.at[17])]
    cp_small = [lambda: pltpu.make_async_copy(shift_hbm, shift_ref, sems.at[18]),
                lambda: pltpu.make_async_copy(ssmd_hbm, ssmd_ref, sems.at[18]),
                lambda: pltpu.make_async_copy(beta_hbm, beta_ref, sems.at[18])]

    def out_a(c):
        return lambda: pltpu.make_async_copy(
            outa.at[c], out_hbm.bitcast(U32).at[0, :, pl.ds(128 * c, 128)], sems.at[19])

    def out_b(r0, n, rows_):
        return lambda: pltpu.make_async_copy(
            outb.at[n, pl.ds(r0, rows_), :],
            out_hbm.at[0, pl.ds(r0, rows_), pl.ds(D + 128 * n, 128)], sems.at[20])

    cp_oa = [out_a(c) for c in range(NT)]
    cp_ob = [[out_b(L * s, n, L) for n in range(NT)] for s in range(NSEG - 1)]
    cp_ob3 = [[out_b(L * 3 + 128 * i, n, 128) for n in range(NT)] for i in range(4)]

    def start(*groups):
        for g in groups:
            for cp in g:
                cp().start()

    def wait(*groups):
        for g in groups:
            for cp in g:
                cp().wait()

    def rows(i, n):
        return pl.ds(pl.multiple_of(i * n, n), n) if not isinstance(i, int) else pl.ds(i * n, n)

    lane = lax.broadcasted_iota(jnp.int32, (8, 128), 1)
    sub = lax.broadcasted_iota(jnp.int32, (8, 128), 0)

    def lanes(n):
        return lax.broadcasted_iota(jnp.int32, (n, 128), 1)

    recent = [None]

    def dot(a, b, dims=NN_DIMS, kind=0):
        out = _dot(a, b, dims)
        if kind & PACE_ON:
            recent[0] = out
        return out

    def pace(i, targets):
        if recent[0] is not None:
            for target in targets:
                target(jnp.minimum(i, 3), recent[0][-8:])
            recent[0] = None

    def qk_proj(s, i, want_pq, want_pk):
        p = s % 2
        tok = rows(4 * s + i, 64)
        for w_ref, dst, fdst, want, scale in (
                (wqb, qs[p], pqs[p], want_pq, DH ** -0.5 * LOG2E),
                (wkb, ks[p], pks[p], want_pk, None)):
            for n in range(NT):
                t = None
                for c in range(NT):
                    part = dot(_bf(xb[c, tok, :]), _bf(w_ref[n, 64 * c:64 * c + 64, :]))
                    t = part if t is None else t + part
                    if c < NT - 1:
                        yield 32
                dst[n, rows(i, 128), :] = (t if scale is None else t * scale).astype(BF16)
                if want:
                    fdst[n, rows(i, 128), :] = jnp.where(t > 0, t + 1.0, jnp.exp(t)).astype(BF16)
                yield 32

    def first_proj(n):
        for w_ref, dst, scale in ((wqb, qs[0], DH ** -0.5 * LOG2E), (wkb, ks[0], None)):
            for j in range(4):
                t = None
                for c in range(NT):
                    part = dot(_bf(xb[c, rows(j, 64), :]), _bf(w_ref[n, 64 * c:64 * c + 64, :]))
                    t = part if t is None else t + part
                dst[n, rows(j, 128), :] = (t if scale is None else t * scale).astype(BF16)
                if scale is None:
                    pks[0][n, rows(j, 128), :] = jnp.where(t > 0, t + 1.0, jnp.exp(t)).astype(BF16)
                if j < NT - 2:
                    c = j + (scale is None) * 3
                    if c < NT:
                        wvt[c, rows(n, 64), :] = _u32(_bf(wvb[n, 64 * c:64 * c + 64, :]).T)

    def untranspose(s, i, slot=0):
        ot = ots.bitcast(U32)
        for c in range(NT):
            onat[slot, c] = _u32(_bf(ot[s % 2, i, 64 * c:64 * c + 64, :]).T)

    def out_proj(s, i, slot=0):
        for n in range(NT):
            t = None
            for c in range(NT):
                part = dot(_bf(onat[slot, c]), _bf(wob[n, 64 * c:64 * c + 64, :]))
                t = part if t is None else t + part
                if c < NT - 1:
                    yield 32
            outb[n, rows(4 * s + i, 128), :] = t.astype(BF16)
            yield 32

    def tile_rows(r, n):
        return jnp.broadcast_to(r[None], (n // 8, 8, 128)).reshape(n, 128)

    class Group:
        def __init__(self, s, g, gi):
            self.s, self.g, self.gi = s, g, gi
            self.t0 = (80 * g) // 128
            self.off = 80 * g - 128 * self.t0
            self.t1 = jnp.minimum(self.t0 + 1, NT - 1)
            rel = (lane - self.off) & 127
            head = sum((rel >= a * DH).astype(jnp.int32) for a in range(1, 5))
            for a in range(4):
                hmask[gi, a] = jnp.where(head == a, np.uint32(0xFFFFFFFF), np.uint32(0))
            hsel[gi] = jnp.left_shift(1, head)
            self.have_keys, self.have_mem = set(), set()

        def window(self, ref, j, r0=0, n=64):
            ref = ref.bitcast(U32)
            at = pl.ds(64 * j + r0, n)
            return jnp.where(lanes(n) >= self.off, ref[self.t0, at, :], ref[self.t1, at, :])

        def keys(self, r0, r1):
            out = []
            for r in range(r0, r1, 64):
                at = pl.ds(r // 2, 32)
                if r in self.have_keys:
                    out.append(kwin[self.gi, at, :])
                else:
                    self.have_keys.add(r)
                    out.append(self.window(ks[self.s % 2], 0, r // 2, 32))
                    kwin[self.gi, at, :] = out[-1]
            return _bf(jnp.concatenate(out, axis=0))

        def park_values(self, j, v80):
            vall[self.gi, j, 0:80, :] = v80.astype(BF16)
            ones8 = jnp.ones((8, 128), F32)
            for pr in range(2):
                for e in range(2):
                    r0 = 40 * pr + 16 * e
                    vhead[self.gi, j, r0 // 8] = jnp.concatenate(
                        [v80[r0:r0 + 24], ones8], axis=0).astype(BF16)

        def mem_read(self):
            for j in range(4):
                r = dot(mst[self.g].astype(BF16), _bf(self.window(pqs[self.s % 2], j)), NT_DIMS)
                coef = gtab[self.g] / (r[80:88] + 1e-6)
                cb = [jnp.broadcast_to(coef[a:a + 1], (8, 128)) for a in range(4)]
                for pr in range(2):
                    ca, cc = cb[2 * pr], cb[2 * pr + 1]
                    for e, scale in enumerate((ca, ca, jnp.where(sub < 4, ca, cc), cc, cc)):
                        r0 = 40 * pr + 8 * e
                        opart[self.gi, j, r0:r0 + 8, :] = r[r0:r0 + 8] * scale
                self.have_mem.add(j)
                yield 24

        def mem_update(self):
            acc = None
            for j in range(4):
                t = dot(_bf(vall.bitcast(U32)[self.gi, j]), _bf(self.window(pks[self.s % 2], j)))
                acc = t if acc is None else acc + t
                if j < 3:
                    yield 24
            for r in range(12):
                new = jnp.where(bmask[r] & hsel[self.gi] != 0, acc[8 * r:8 * r + 8], 0.0)
                at = pl.ds(8 * r, 8)
                mst[self.g, at, :] = new if self.s == 0 else mst[self.g, at, :] + new
            yield 24

        def logits(self, pr, j, slot):
            qw = self.window(qs[self.s % 2], j)
            qa = qw & tile_rows(hmask[self.gi, 2 * pr], 64)
            qh = qw & tile_rows(hmask[self.gi, 2 * pr + 1], 64)
            w_a = _bf(qa)
            w_b = _bf(jnp.concatenate([qh[32:64], qh[0:32]], axis=0))
            w_t = _bf(jnp.concatenate([qh[32:64], qa[32:64]], axis=0))
            n = 128 * j

            def park(t, e, r0, m):
                for r in range(0, t.shape[0], 8):
                    v = t[r:r + 8]
                    if e == 2:
                        v = v + cmask[2, r:r + 8, :]
                    elif r0 + r >= n:
                        v = v + cmask[e, r0 + r - n:r0 + r - n + 8, :]
                    slot[e % 2, 448 * (e // 2) + r0 + r:448 * (e // 2) + r0 + r + 8, :] = v
                    m = v if m is None else jnp.maximum(m, v)
                return m

            m_t = park(dot(self.keys(n + 64, n + 128), w_t, NT_DIMS, 1), 2, 0, None)
            yield 16 * LW
            cuts = list(range(0, n, QCH)) or [0]
            m = [None, None]
            for r0, r1 in zip(cuts, cuts[1:] + [n + 64]):
                for e, w in enumerate((w_a, w_b)):
                    m[e] = park(dot(self.keys(r0, r1), w, NT_DIMS, 1), e, r0, m[e])
                    if r1 == n + 64 and e == 1:
                        m_a = jnp.maximum(m[0], jnp.where(lane >= 64, m_t, NEG))
                        m_b = jnp.maximum(m[1], jnp.where(lane < 64, m_t, NEG))
                        m_a = jnp.broadcast_to(jnp.max(m_a, axis=0, keepdims=True), (8, 128))
                        m_b = jnp.broadcast_to(jnp.max(m_b, axis=0, keepdims=True), (8, 128))
                        slot[1, 448:456, :] = m_a
                        slot[1, 456:464, :] = m_b
                        slot[1, 464:472, :] = jnp.where(lane < 64, m_b, m_a)
                    yield (r1 - r0) // 4 * LW

    def attend(gi, g, parity, add_mem, pr, j, slot, need_values):
        def prob(e, r0, n, which):
            m2 = tile_rows(slot[1, 448 + 8 * which:456 + 8 * which, :], 16)
            return [jnp.exp2(slot[e, r:r + 16, :] - m2).astype(BF16)
                    for r in range(r0, r0 + n, 16)]

        p_t = _u32(jnp.concatenate(prob(0, 448, 64, 2), axis=0))
        tails = (_bf(jnp.where(lanes(32) >= 64, p_t, np.uint32(0))),
                 _bf(jnp.where(lanes(32) >= 64, np.uint32(0), p_t)))
        res = []
        for e in range(2):
            acc = None
            for kt in range(j + 1):
                need_values(kt)
                if kt < j:
                    p = prob(e, 128 * kt, 128, e)
                else:
                    p = prob(e, 128 * kt, 64, e) + [tails[e]]
                t = dot(_bf(vhead.bitcast(U32)[gi, kt, 5 * pr + 2 * e]),
                         jnp.concatenate(p, axis=0), kind=2)
                acc = t if acc is None else acc + t
                if (e, kt) != (1, j):
                    yield 8 * AW
            res.append(acc)
        r_a = res[0]
        r_b = pltpu.roll(res[1], 64, 1)
        keep = 1.0 - gtab[g]
        keep_a = jnp.broadcast_to(keep[2 * pr:2 * pr + 1], (8, 128))
        keep_b = jnp.broadcast_to(keep[2 * pr + 1:2 * pr + 2], (8, 128))
        o_a = r_a[0:24] * tile_rows(keep_a / r_a[24:32], 24)
        o_b = r_b[0:24] * tile_rows(keep_b / r_b[24:32], 24)
        o = jnp.concatenate(
            [o_a[0:16], jnp.where(sub < 4, o_a[16:24], o_b[0:8]), o_b[8:24]], axis=0)
        if add_mem:
            o = o + opart[gi, j, 40 * pr:40 * pr + 40, :]
        if pr == 0:
            opart[gi, j, 0:40, :] = o
        else:
            o = jnp.concatenate([opart[gi, j, 0:40, :], o], axis=0)
            ots[parity, j, rows(g, 80), :] = o.astype(BF16)
        yield 8 * AW

    def v_proj(s, i, groups, have):
        for j in range(4):
            for gis in VSPLIT:
                acc = None
                for c in range(NT):
                    t = dot(_bf(wvt[c, rows(2 * i // len(gis) + gis[0], 40 * len(gis)), :]),
                            _bf(xb[c, rows(4 * s + j, 64), :]), NT_DIMS)
                    acc = t if acc is None else acc + t
                    if c == NT - 1:
                        for k, gi in enumerate(gis):
                            groups[gi].park_values(j, acc[80 * k:80 * k + 80])
                        if gis[-1] == 1:
                            have.append(j)
                    yield 20 * len(gis)

    def chain(*gens):
        for g in gens:
            yield from g

    units = [(gi, pr, j) for gi in range(2) for pr in range(2)
             for j in (LAST_ORDER if (gi, pr) == (1, 1) else range(4))]

    def cost(j):
        return (48 + 64 * j) * LW, (16 + 16 * j) * AW

    def carried(u, g, parity):
        gi, pr, j = units[u]
        return attend(gi, g, parity, True, pr, j, slots[u % NSLOT], lambda kt: None), cost(j)[1]

    def segment_step(s, i, mxu_fill, vpu_fill, targets):
        vt = []
        fill = _Paced(mxu_fill, sequential=SEQ_FILL)
        for _ in range(HEAD if s < NSEG - 1 else HEAD // 2):
            fill.step()
        if s > 0:
            untranspose(s - 1, i)
        groups = [Group(s, 2 * i + gi, gi) for gi in range(2)]
        reads = [grp.mem_read() for grp in groups if s > 0]
        updates = [grp.mem_update() for grp in groups if s < NSEG - 1]
        first = _Paced([(chain(*reads[:1], v_proj(s, i, groups, vt), *reads[1:], *updates),
                         800 + 96 * (len(reads) + len(updates)))])
        side = _Paced(vpu_fill)
        total = first.total + fill.total
        held = 96 * (s > 0) + 160

        def need_values(kt):
            while len(vt) <= kt:
                first.step()

        def pad(fraction, u):
            target = total * fraction
            early = min(target * EARLY, held if u < DEPTH else first.total)
            first.advance(early / first.total)
            fill.advance((target - early) / fill.total)
            if side.live and side.done < fraction * side.total and recent[0] is not None:
                pace(i, targets)
                side.advance(fraction)

        whole = sum(sum(cost(j)) for _, _, j in units) * (1 + TAIL)
        done = 0
        for u in range(len(units)):
            gi, pr, j = units[u]
            streams = [(groups[gi].logits(pr, j, slots[u % NSLOT]), cost(j)[0])]
            v = u - DEPTH
            if v < 0:
                streams.append(carried(v + len(units), (2 * i + 7) & 7,
                                       jnp.where(i > 0, s % 2, 1 - s % 2)))
            else:
                gi, pr, j = units[v]
                while s > 0 and j not in groups[gi].have_mem:
                    first.step()
                streams.append((attend(gi, 2 * i + gi, s % 2, s > 0, pr, j, slots[v % NSLOT],
                                       need_values), cost(j)[1]))
            att = _Paced(streams[::-1], sequential=u == len(units) - 1)
            while att.live:
                att.step()
                pad((done + att.done) / whole, u)
            done += att.total
        first.finish()
        fill.finish()
        side.finish()

    def split_h(i, cs):
        for c in cs:
            k, (_, hp, _, _, _) = fft_bufs(c)
            for t in range(4):
                ht[c, 64 * t:64 * t + 64, :] = _u32(_bf(hb[4 * i + t, 64 * c:64 * c + 64, :]).T)
                yield 16
            for q in range(2):
                for j in range(8):
                    wa = ht[c, pl.ds(128 * q + j, 8, stride=8), :]
                    wb = ht[c, pl.ds(128 * q + 64 + j, 8, stride=8), :]
                    hp[k, 2 * j, rows(2 * i + q, 8), :] = _pack2(_lo(wa), _lo(wb))
                    hp[k, 2 * j + 1, rows(2 * i + q, 8), :] = _pack2(_hi(wa), _hi(wb))
                    if j % 2:
                        yield 4

    def split_kv(i, cs):
        for c in cs:
            k, (xp, _, _, _, _) = fft_bufs(c)
            taps = [wtab[c, j] for j in range(KS)]
            for q in range(2):
                blk = 2 * i + q
                base = [blk * 128 + 64 * e for e in range(2)]
                hist = []
                for e in range(2):
                    w2 = kb[c, pl.ds(base[e] + 6, 8, stride=8), :]
                    w1 = kb[c, pl.ds(base[e] + 7, 8, stride=8), :]
                    hist.append([_hi(w2), _lo(w1), _hi(w1)])
                for j in range(8):
                    kv = [[None, None], [None, None]]
                    for e in range(2):
                        kw = kb[c, pl.ds(base[e] + 8 + j, 8, stride=8), :]
                        vw = vb[c, pl.ds(base[e] + j, 8, stride=8), :]
                        kp = hist[e] + [_lo(kw), _hi(kw)]
                        for half, part in enumerate((_lo, _hi)):
                            acc = kp[3 + half] * taps[0]
                            for d in range(1, KS):
                                acc = acc + kp[3 + half - d] * taps[d]
                            kv[half][e] = acc * part(vw)
                            kvf[c, 2 * j + half, rows(2 * blk + e, 8), :] = kv[half][e]
                        hist[e] = kp[2:]
                    for half in range(2):
                        xp[k, 2 * j + half, rows(blk, 8), :] = _pack2(*kv[half])
                    yield 11

    def fwd_fft(i, cs):
        for c in cs:
            k, (xp, hp, tx, th, _) = fft_bufs(c)
            for src, dst in ((hp, th), (xp, tx)):
                for r0 in range(0, 2 * N1, FCH):
                    g = [dot(_bf(fwd[4 * a + i, r0 // 2:(r0 + FCH) // 2, :]), _bf(src[k, 4 * a + i]))
                         for a in range(4)]
                    for r in range(0, FCH, 16):
                        z = _radix4(*[(g[a][r:r + 8], g[a][r + 8:r + 16]) for a in range(4)], 1)
                        for cc in range(4):
                            dst[k, (r0 + r) // 16, cc, i, 0] = z[cc][0]
                            dst[k, (r0 + r) // 16, cc, i, 1] = z[cc][1]
                    yield FCH

    def spectrum(c, m, slot):
        k, (_, _, tx, th, yb) = fft_bufs(c)
        for cc in range(4):
            zh = _radix4_tw(*[(th[k, m, cc, b, 0], th[k, m, cc, b, 1]) for b in range(4)], 1, cc)
            yield 1
            zx = _radix4_tw(*[(tx[k, m, cc, b, 0], tx[k, m, cc, b, 1]) for b in range(4)], 1, cc)
            yield 1
            y = [(x[0] * h[0] - x[1] * h[1], x[0] * h[1] + x[1] * h[0]) for x, h in zip(zx, zh)]
            yield 1
            u = _radix4(*y, -1)
            for b in range(4):
                ub[slot, b, cc, 0] = u[b][0]
                ub[slot, b, cc, 1] = u[b][1]
            yield 1
        for b in range(4):
            z = _radix4_tw(*[(ub[slot, b, cc, 0], ub[slot, b, cc, 1]) for cc in range(4)], -1, b)
            for a in range(4):
                yb[k, 4 * a + b, rows(m, 8), :] = _pack2(*z[a])
            yield 1

    SPEC_STEPS = 20

    def spectra(cs, ms):
        for slot, (c, m) in enumerate((c, m) for c in cs for m in ms):
            yield from spectrum(c, m, slot)

    def spare_h(d, v):
        hb[S // 128, rows(d, 8), :] = _u32_word(v)

    def spare_k(d, v):
        kb[NT, rows(d, 8), :] = _u32_word(v)
        if PACE_ALL > 0:
            vb[NT, rows(d, 8), :] = _u32_word(v)

    def spare_t(cs):
        _, (_, _, tx, th, _) = fft_bufs(cs[0])

        def store(d, v):
            th[len(cs), d, 0, 0, 0] = v
            if PACE_ALL > 0:
                tx[len(cs), d, 0, 0, 0] = v
            if PACE_ALL > 1:
                ub[12, d, 0, 0] = v
        return store

    def inverse(cs, jps):
        for c in cs:
            k, (_, _, _, _, yb) = fft_bufs(c)
            for jp in jps:
                w = qb[c, pl.ds(jp, N1, stride=8), :]
                res = []
                for e, part in enumerate((_lo, _hi)):
                    n2 = 2 * jp + e
                    y = dot(_bf(inv[n2, 0]), _bf(yb[k, n2, 0:64, :]))
                    yield 32
                    y = y + dot(_bf(inv[n2, 1]), _bf(yb[k, n2, 64:128, :]))
                    res.append(part(w) * (y + kvf[c, n2] * tile_rows(wtab[c, KS], N1)))
                    if e == 0:
                        yield 32
                outa[c, pl.ds(jp, N1, stride=8), :] = _pack2(*res)
                yield 32

    start(cp_small, cp_x[0], cp_w[0])
    kk = lax.broadcasted_iota(jnp.int32, (64, 128), 0)
    ll = lax.broadcasted_iota(jnp.int32, (64, 128), 1)
    cmask[0] = jnp.where(kk <= ll, 0.0, NEG)
    cmask[1] = jnp.where((ll < 64) | (kk <= ll - 64), 0.0, NEG)
    cmask[2] = jnp.where(kk <= (ll & 63), 0.0, NEG)
    for r in range(12):
        row = sub + 8 * r
        hr = sum((row >= a * DH).astype(jnp.int32) for a in range(1, 4)) if r < 10 else row - 80
        bmask[r] = jnp.left_shift(1, hr)
    for gi in range(2):
        for j in range(4):
            vall[gi, j, 80:96, :] = jnp.ones((16, 128), BF16)
    for c in range(NT):
        kb[c, 0:8, :] = jnp.zeros((8, 128), U32)
    for u in range(16 - DEPTH, 16):
        slots[u % NSLOT][...] = jnp.zeros((2, 512, 128), F32)
    vhead[1] = jnp.ones(vhead.shape[1:], BF16)
    opart[1] = jnp.zeros(opart.shape[1:], F32)
    start(cp_w[1])
    wait(cp_small)
    taps_t = shift_ref[...].astype(F32)
    skip = ssmd_ref[...].astype(F32)
    for c in range(NT):
        for j in range(KS):
            wtab[c, j] = jnp.broadcast_to(taps_t[j:j + 1, 128 * c:128 * c + 128], (8, 128))
        wtab[c, KS] = jnp.broadcast_to(skip[c:c + 1], (8, 128))
    gates = jax.nn.sigmoid(beta_ref[...].astype(F32))
    gcol = jnp.broadcast_to(gates, (8, H)).T
    gcol = jnp.broadcast_to(gcol[:, 0:1], (H, 128))
    for g in range(8):
        gtab[g] = jnp.concatenate([gcol[4 * g:4 * g + 4]] * 2, axis=0)
    wait(cp_x[0])
    start(cp_w[2])

    def prologue(n, carry):
        for j in range(NT):
            @pl.when(n == j)
            def _():
                wait(cp_w[j])
                start(*((cp_w[3],), (cp_w[4],), (cp_x[1],), (cp_early[0],), (cp_early[1],))[j])
        first_proj(n)
        return carry

    with jax.named_scope("prologue"):
        lax.fori_loop(0, NT, prologue, 0)
    wait(cp_x[1])
    start(cp_wo, cp_x[2])

    def seg0(i, carry):
        for j in range(4):
            @pl.when(i == j)
            def _():
                wait(cp_early[j])
                start(*((cp_early[2],), (cp_early[3],), (cp_fwd, cp_late), (cp_x[3],))[j])
        segment_step(0, i, [(qk_proj(1, i, True, True), 1600)],
                     [(split_h(i, EARLY_TILES), 96 * len(EARLY_TILES)),
                      (split_kv(i, EARLY_TILES), 176 * len(EARLY_TILES))], [spare_h, spare_k])
        return carry

    with jax.named_scope("seg0"):
        lax.fori_loop(0, 4, seg0, 0)
    wait(cp_fwd, cp_x[2], cp_wo, cp_late)
    start(cp_inv, cp_q)

    def seg1(i, carry):
        segment_step(1, i, [(qk_proj(2, i, True, True), 1600), (out_proj(0, i), 800),
                            (fwd_fft(i, EARLY_TILES), 512 * len(EARLY_TILES))],
                     [(split_h(i, LATE_TILES), 96 * len(LATE_TILES)),
                      (split_kv(i, LATE_TILES), 176 * len(LATE_TILES))], [spare_h, spare_k])
        return carry

    with jax.named_scope("seg1"):
        lax.fori_loop(0, 4, seg1, 0)
    start(cp_ob[0])
    wait(cp_x[3])

    def seg2(i, carry):
        segment_step(2, i, [(qk_proj(3, i, True, False), 1600), (out_proj(1, i), 800),
                            (fwd_fft(i, LATE_TILES), 512 * len(LATE_TILES))],
                     [(spectra(EARLY_TILES, [4 * i + a for a in range(4)]),
                       4 * SPEC_STEPS * len(EARLY_TILES))], [spare_t(EARLY_TILES)])
        return carry

    with jax.named_scope("seg2"):
        lax.fori_loop(0, 4, seg2, 0)
    wait(cp_ob[0], cp_inv, cp_q)
    start(cp_ob[1])

    def seg3(i, carry):
        segment_step(3, i, [(inverse(EARLY_TILES, (2 * i, 2 * i + 1)), 256 * len(EARLY_TILES)),
                            (out_proj(2, i), 800)],
                     [(spectra(LATE_TILES, [4 * i + a for a in range(4)]),
                       4 * SPEC_STEPS * len(LATE_TILES))], [spare_t(LATE_TILES)])
        return carry

    with jax.named_scope("seg3"):
        lax.fori_loop(0, 4, seg3, 0)
    wait(cp_ob[1])
    start(cp_ob[2], [cp_oa[c] for c in EARLY_TILES])
    with jax.named_scope("epilogue"):
        for c in LATE_TILES:
            streams = [(inverse((c,), range(8)), 1024)]
            if c == LATE_TILES[0]:
                streams.append((chain(*[carried(u, 7, 1)[0] for u in range(16 - DEPTH, 16)]),
                                sum(cost(units[u][2])[1] for u in range(16 - DEPTH, 16))))
            _Paced(streams).finish()
            if c == LATE_TILES[0]:
                for i in range(4):
                    untranspose(3, i, i)
            start([cp_oa[c]])
        for i in range(4):
            _Paced([(out_proj(3, i, i), 800)]).finish()
            start(cp_ob3[i])
    wait(cp_ob[2], *cp_ob3, cp_oa)


@jax.jit
def pallas_concat_heads__ssm_conv_h3__memory_aug_infini_attn__prompt_kernel(
    A_q: jax.Array,
    A_k: jax.Array,
    A_v: jax.Array,
    A_shift_k: jax.Array,
    A_ssm_k: jax.Array,
    A_ssm_D: jax.Array,
    B_x: jax.Array,
    B_wq: jax.Array,
    B_wk: jax.Array,
    B_wv: jax.Array,
    B_wo: jax.Array,
    B_beta: jax.Array,
):
    hbm = pl.BlockSpec(memory_space=pltpu.HBM)
    seg_tiles = pltpu.VMEM((NT, L, 128), BF16)
    seq_tiles = pltpu.VMEM((NT, S // 2, 128), U32)
    w_tiles = pltpu.VMEM((NT, D // 2, 128), U32)
    scratch = [
        pltpu.VMEM((KS, D), BF16),
        pltpu.VMEM((NT, 128), BF16),
        pltpu.VMEM((1, H), BF16),
        seq_tiles,
        w_tiles, w_tiles, w_tiles, w_tiles, w_tiles,
        pltpu.VMEM((S // 128 + 1, D // 2, 128), U32),
        pltpu.VMEM((NT, 256, 128), U32),
        pltpu.VMEM((NT + 1, S // 2 + 8, 128), U32),
        pltpu.VMEM((NT + 1, S // 2, 128), U32),
        seq_tiles,
        pltpu.VMEM((N2, N1, 128), U32),
        pltpu.VMEM((N2, 2, N1 // 2, 128), U32),
        pltpu.VMEM((NT, N2, N1, 128), F32),
        pltpu.VMEM((13, 4, 4, 2, 8, 128), F32),
        seq_tiles,
        pltpu.VMEM((NT, S, 128), BF16),
        pltpu.VMEM((NT, KS + 1, 8, 128), F32),
        pltpu.VMEM((8, 8, 128), F32),
        pltpu.VMEM((3, 64, 128), F32),
        seg_tiles, seg_tiles, seg_tiles, seg_tiles,
        seg_tiles, seg_tiles, seg_tiles, seg_tiles,
        pltpu.VMEM((2, 4, D, 128), BF16),
        pltpu.VMEM((8, 96, 128), F32),
        pltpu.VMEM((2, 4, 8, 128), U32),
        pltpu.VMEM((2, 8, 128), jnp.int32),
        pltpu.VMEM((12, 8, 128), jnp.int32),
        pltpu.VMEM((2, L // 2, 128), U32),
        pltpu.VMEM((2, 4, 96, 128), BF16),
        pltpu.VMEM((2, 4, 8, 32, 128), BF16),
        pltpu.VMEM((2, 4, 80, 128), F32),
        pltpu.VMEM((4, NT, 64, 128), U32),
        pltpu.SemaphoreType.DMA((21,)),
    ]
    for n in (len(EARLY_TILES), len(LATE_TILES)):
        scratch += [
            pltpu.VMEM((n, N2, N1 // 2, 128), U32),
            pltpu.VMEM((n, N2, N1 // 2, 128), U32),
            pltpu.VMEM((n + 1, N1 // 8, 4, 4, 2, 8, 128), F32),
            pltpu.VMEM((n + 1, N1 // 8, 4, 4, 2, 8, 128), F32),
            pltpu.VMEM((n, N2, N1, 128), U32),
        ]
    scratch += [pltpu.VMEM((2, 512, 128), F32)] * NSLOT
    return pl.pallas_call(
        _kernel,
        out_shape=jax.ShapeDtypeStruct((1, S, 2 * D), BF16),
        in_specs=[hbm] * 14,
        out_specs=hbm,
        scratch_shapes=scratch,
        compiler_params=pltpu.CompilerParams(vmem_limit_bytes=110 * 1024 * 1024),
        name="h3_infini",
    )(A_q, A_k, A_v, A_shift_k.T, A_ssm_k, A_ssm_D.reshape(NT, 128), B_x, B_wq, B_wk, B_wv, B_wo,
      B_beta.reshape(1, H), _FWD, _INV)
```

```python
import math

import jax
import jax.numpy as jnp
import numpy as np
from jax import lax
from jax.experimental import pallas as pl
from jax.experimental.pallas import tpu as pltpu

S = 2048
D = 640
NT = D // 128
H = 32
DH = D // H
NSEG = 4
L = S // NSEG
KS = 4
N1, N2 = 128, 16

F32 = jnp.float32
BF16 = jnp.bfloat16
U32 = jnp.uint32
NN_DIMS = (((1,), (0,)), ((), ()))
NT_DIMS = (((1,), (1,)), ((), ()))
NEG = -1e30
LOG2E = 1.4426950408889634


def _pack_rows(a):
    u = a.astype(np.float32).astype(BF16).view(np.uint16).astype(np.uint32)
    return u[..., 0::2, :] | (u[..., 1::2, :] << 16)


def _dft_tables():
    k1 = np.arange(N1)
    fwd = np.zeros((N2, 2 * N1, N1), np.float64)
    inv = np.zeros((N2, N1, 2 * N1), np.float64)
    kappa = np.arange(N1)
    n1_in = 16 * (kappa // 16) + 8 * (kappa % 2) + (kappa % 16) // 2
    row_re = 16 * (k1 // 8) + k1 % 8
    for n2 in range(N2):
        ang = 2.0 * np.pi * np.outer(k1 + 0.25, N2 * n1_in + n2) / S
        fwd[n2, row_re] = np.cos(ang)
        fwd[n2, row_re + 8] = np.sin(ang)
        ang = 2.0 * np.pi * np.outer(N2 * np.arange(N1) + n2, k1 + 0.25) / S
        inv[n2][:, 2 * k1] = np.cos(ang) / S
        inv[n2][:, 2 * k1 + 1] = np.sin(ang) / S
    inv = inv.reshape(N2, N1, 2, N1).transpose(0, 2, 1, 3)
    return _pack_rows(fwd), _pack_rows(inv)


_FWD, _INV = _dft_tables()


def _dot(a, b, dims=NN_DIMS):
    return lax.dot_general(a, b, dims, preferred_element_type=F32)


def _u32(x):
    return pltpu.bitcast(x, U32)


def _bf(x):
    return pltpu.bitcast(x, BF16)


def _u32_word(x):
    return lax.bitcast_convert_type(x, U32)


def _pack2(a, b):
    return pltpu.pack_elementwise([a, b], packed_dtype=BF16).astype(U32)


def _lo(w):
    return pltpu.unpack_elementwise(w, index=0, packed_dtype=BF16, unpacked_dtype=F32)


def _hi(w):
    return pltpu.unpack_elementwise(w, index=1, packed_dtype=BF16, unpacked_dtype=F32)


def _radix4(x0, x1, x2, x3, sign):
    ar, ai = x0[0] + x2[0], x0[1] + x2[1]
    br, bi = x0[0] - x2[0], x0[1] - x2[1]
    cr, ci = x1[0] + x3[0], x1[1] + x3[1]
    dr, di = x1[0] - x3[0], x1[1] - x3[1]
    y0 = (ar + cr, ai + ci)
    y2 = (ar - cr, ai - ci)
    yp = (br - di, bi + dr)
    ym = (br + di, bi - dr)
    return (y0, yp, y2, ym) if sign > 0 else (y0, ym, y2, yp)


def _twiddle(x, e, sign):
    xr, xi = x
    if e == 0:
        return x
    if e == 4:
        return (-xi, xr) if sign > 0 else (xi, -xr)
    r = math.sqrt(0.5)
    if e == 2:
        return ((xr - xi) * r, (xr + xi) * r) if sign > 0 else ((xr + xi) * r, (xi - xr) * r)
    if e == 6:
        return ((xr + xi) * -r, (xr - xi) * r) if sign > 0 else ((xi - xr) * r, (xr + xi) * -r)
    c, s = math.cos(math.pi * e / 8), sign * math.sin(math.pi * e / 8)
    return (xr * c - xi * s, xr * s + xi * c)


def _radix4_tw(x0, x1, x2, x3, sign, b):
    if b != 2:
        return _radix4(x0, _twiddle(x1, b, sign), _twiddle(x2, 2 * b, sign),
                       _twiddle(x3, 3 * b, sign), sign)
    x1, x3 = _twiddle(x1, 2, sign), _twiddle(x3, 6, sign)
    if sign > 0:
        ar, ai = x0[0] - x2[1], x0[1] + x2[0]
        br, bi = x0[0] + x2[1], x0[1] - x2[0]
    else:
        ar, ai = x0[0] + x2[1], x0[1] - x2[0]
        br, bi = x0[0] - x2[1], x0[1] + x2[0]
    cr, ci = x1[0] + x3[0], x1[1] + x3[1]
    dr, di = x1[0] - x3[0], x1[1] - x3[1]
    y0 = (ar + cr, ai + ci)
    y2 = (ar - cr, ai - ci)
    yp = (br - di, bi + dr)
    ym = (br + di, bi - dr)
    return (y0, yp, y2, ym) if sign > 0 else (y0, ym, y2, yp)


class _Paced:
    def __init__(self, streams, sequential=False):
        self.live = [[g, total, 0] for g, total in streams]
        self.total = sum(total for _, total in streams)
        self.done = 0
        self.sequential = sequential

    def step(self):
        cur = self.live[0] if self.sequential else min(self.live, key=lambda e: e[2] / e[1])
        cost = next(cur[0], None)
        if cost is None:
            self.live.remove(cur)
        else:
            cur[2] += cost
            self.done += cost

    def advance(self, fraction):
        while self.live and self.done < fraction * self.total:
            self.step()

    def finish(self):
        self.advance(math.inf)


DEPTH = 3
TAIL = 0.0
EARLY = 1.0
PACE_ON = [3]
MID = 3
SHIFT = 0
UNROLL = (0, 0, 0, 0)
FLAGS = None
HEAD = 4
SEQ_FILL = True
FCH = 256
VSPLIT = ((0, 1),)
EARLY_TILES = (0, 1)
LATE_TILES = tuple(c for c in range(NT) if c not in EARLY_TILES)
LW = 1.0
AW = 3.0
NSLOT = 4
LAST_ORDER = (0, 1, 2, 3)
QCH = 256


def _kernel(aq_hbm, ak_hbm, av_hbm, shift_hbm, h_hbm, ssmd_hbm, x_hbm, wq_hbm, wk_hbm,
            wv_hbm, wo_hbm, beta_hbm, fwd_hbm, inv_hbm, out_hbm, shift_ref, ssmd_ref, beta_ref,
            xb, wqb, wkb, wvb, wob, wvt, hb, ht, kb, vb, qb, fwd, inv,
            kvf, ub, outa, outb, wtab, gtab, cmask,
            q0, q1, k0, k1, pq0, pq1, pk0, pk1, ots, mst,
            hmask, hsel, bmask, kwin, vall, vhead, opart, onat, sem_zero, sems, *rest):
    xp, hp, tx, th, yb = (rest[NT * k:NT * k + NT] for k in range(5))
    slots = rest[5 * NT:]
    PACE_ON[0] = 3
    qs, ks, pqs, pks = (q0, q1), (k0, k1), (pq0, pq1), (pk0, pk1)

    def tile_copy(src, dst, t, sem, r0, n, lead=(0,), dst_off=0):
        return lambda: pltpu.make_async_copy(
            src.bitcast(U32).at[(*lead, pl.ds(r0 // 2, n // 2), pl.ds(128 * t, 128))],
            dst.at[t, pl.ds(dst_off + r0 // 2, n // 2), :], sems.at[sem])

    def h_copy(t, c0, n, sem):
        return lambda: pltpu.make_async_copy(
            h_hbm.bitcast(U32).at[pl.ds(64 * c0, 64 * n), pl.ds(128 * t, 128)],
            hb.at[t, pl.ds(64 * c0, 64 * n), :], sems.at[sem])

    def conv_copies(cs, i, sem):
        out = [h_copy(4 * i + t, cs[0], len(cs), sem) for t in range(4)]
        out += [tile_copy(ak_hbm, kb, c, sem, L * i, L, dst_off=8) for c in cs]
        return out + [tile_copy(av_hbm, vb, c, sem, L * i, L) for c in cs]

    cp_x = [[tile_copy(x_hbm, xb, t, s, L * s, L) for t in range(NT)] for s in range(NSEG)]
    cp_x1 = [[tile_copy(x_hbm, xb, t, 10 + i, L + 128 * i, 128) for t in range(NT)]
             for i in range(4)]
    cp_w = [[tile_copy(src, dst, n, 4 + n, 0, D, lead=())
             for src, dst in ((wq_hbm, wqb), (wk_hbm, wkb))] for n in range(NT)]
    cp_wv = [tile_copy(wv_hbm, wvb, n, 1, 0, D, lead=()) for n in range(NT)]
    cp_wo = [tile_copy(wo_hbm, wob, n, 9, 0, D, lead=()) for n in range(NT)]
    cp_early = [conv_copies(EARLY_TILES, i, 10 + i) + cp_x1[i] for i in range(4)]
    cp_late = [cp for i in range(4) for cp in conv_copies(LATE_TILES, i, 14)]
    cp_q = [tile_copy(aq_hbm, qb, c, 15, 0, S) for c in range(NT)]
    cp_fwd = [lambda: pltpu.make_async_copy(fwd_hbm, fwd, sems.at[16])]
    cp_inv = [lambda: pltpu.make_async_copy(inv_hbm, inv, sems.at[17])]
    cp_small = [lambda: pltpu.make_async_copy(shift_hbm, shift_ref, sems.at[18]),
                lambda: pltpu.make_async_copy(ssmd_hbm, ssmd_ref, sems.at[18]),
                lambda: pltpu.make_async_copy(beta_hbm, beta_ref, sems.at[18])]

    def out_a(c):
        return lambda: pltpu.make_async_copy(
            outa.at[c], out_hbm.bitcast(U32).at[0, :, pl.ds(128 * c, 128)], sems.at[19])

    def out_b(r0, n, rows_):
        return lambda: pltpu.make_async_copy(
            outb.at[n, pl.ds(r0, rows_), :],
            out_hbm.at[0, pl.ds(r0, rows_), pl.ds(D + 128 * n, 128)], sems.at[20])

    cp_oa = [out_a(c) for c in range(NT)]
    cp_ob = [[out_b(L * s, n, L) for n in range(NT)] for s in range(NSEG - 1)]
    cp_ob3 = [[out_b(L * 3 + 128 * i, n, 128) for n in range(NT)] for i in range(4)]

    def start(*groups):
        for g in groups:
            for cp in g:
                cp().start()

    def wait(*groups):
        for g in groups:
            for cp in g:
                cp().wait()

    def rows(i, n):
        return pl.ds(pl.multiple_of(i * n, n), n) if not isinstance(i, int) else pl.ds(i * n, n)

    lane = lax.broadcasted_iota(jnp.int32, (8, 128), 1)
    sub = lax.broadcasted_iota(jnp.int32, (8, 128), 0)

    def lanes(n):
        return lax.broadcasted_iota(jnp.int32, (n, 128), 1)

    recent = [None]

    def dot(a, b, dims=NN_DIMS, kind=4):
        out = _dot(a, b, dims)
        if kind & PACE_ON[0]:
            recent[0] = out
        return out

    def pace(i, targets):
        if recent[0] is not None:
            for target in targets:
                target(sem_zero[0] if isinstance(i, int) else jnp.minimum(i, 3), recent[0][-8:])
            recent[0] = None

    def qk_proj(s, i, want_pq, want_pk):
        p = s % 2
        tok = rows(4 * s + i, 64)
        for w_ref, dst, fdst, want, scale in (
                (wqb, qs[p], pqs[p], want_pq, DH ** -0.5 * LOG2E),
                (wkb, ks[p], pks[p], want_pk, None)):
            for n in range(NT):
                t = None
                for c in range(NT):
                    part = dot(_bf(xb[c, tok, :]), _bf(w_ref[n, 64 * c:64 * c + 64, :]))
                    t = part if t is None else t + part
                    if c < NT - 1:
                        yield 32
                dst[n, rows(i, 128), :] = (t if scale is None else t * scale).astype(BF16)
                if want:
                    fdst[n, rows(i, 128), :] = jnp.where(t > 0, t + 1.0, jnp.exp(t)).astype(BF16)
                yield 32

    def first_proj(n):
        for w_ref, dst, scale in ((wqb, qs[0], DH ** -0.5 * LOG2E), (wkb, ks[0], None)):
            for j in range(4):
                t = None
                for c in range(NT):
                    part = dot(_bf(xb[c, rows(j, 64), :]), _bf(w_ref[n, 64 * c:64 * c + 64, :]))
                    t = part if t is None else t + part
                dst[n, rows(j, 128), :] = (t if scale is None else t * scale).astype(BF16)
                if scale is None:
                    pks[0][n, rows(j, 128), :] = jnp.where(t > 0, t + 1.0, jnp.exp(t)).astype(BF16)

    def untranspose(s, i, slot=0):
        ot = ots.bitcast(U32)
        for c in range(NT):
            onat[slot, c] = _u32(_bf(ot[s % 2, i, 64 * c:64 * c + 64, :]).T)

    def out_proj(s, i, slot=0, copies=None):
        for n in range(NT):
            t = None
            for c in range(NT):
                part = dot(_bf(onat[slot, c]), _bf(wob[n, 64 * c:64 * c + 64, :]))
                t = part if t is None else t + part
                if c < NT - 1:
                    yield 32
            outb[n, rows(4 * s + i, 128), :] = t.astype(BF16)
            if copies is not None:
                start([copies[n]])
            yield 32

    def tile_rows(r, n):
        return jnp.broadcast_to(r[None], (n // 8, 8, 128)).reshape(n, 128)

    class Group:
        def __init__(self, s, g, gi):
            self.s, self.g, self.gi = s, g, gi
            self.t0 = (80 * g) // 128
            self.off = 80 * g - 128 * self.t0
            self.static = isinstance(g, int)
            self.t1 = min(self.t0 + 1, NT - 1) if self.static else jnp.minimum(self.t0 + 1, NT - 1)
            rel = (lane - self.off) & 127
            head = sum((rel >= a * DH).astype(jnp.int32) for a in range(1, 5))
            for a in range(4):
                hmask[gi, a] = jnp.where(head == a, np.uint32(0xFFFFFFFF), np.uint32(0))
            hsel[gi] = jnp.left_shift(1, head)
            self.have_keys, self.have_mem = set(), set()

        def window(self, ref, j, r0=0, n=64):
            ref = ref.bitcast(U32)
            at = pl.ds(64 * j + r0, n)
            if self.static and self.off + 80 <= 128:
                return ref[self.t0, at, :]
            return jnp.where(lanes(n) >= self.off, ref[self.t0, at, :], ref[self.t1, at, :])

        def keys(self, r0, r1):
            out = []
            for r in range(r0, r1, 64):
                at = pl.ds(r // 2, 32)
                if r in self.have_keys:
                    out.append(kwin[self.gi, at, :])
                else:
                    self.have_keys.add(r)
                    out.append(self.window(ks[self.s % 2], 0, r // 2, 32))
                    kwin[self.gi, at, :] = out[-1]
            return _bf(jnp.concatenate(out, axis=0))

        def park_values(self, j, v80):
            vall[self.gi, j, 0:80, :] = v80.astype(BF16)
            ones8 = jnp.ones((8, 128), F32)
            for pr in range(2):
                for e in range(2):
                    r0 = 40 * pr + 16 * e
                    vhead[self.gi, j, r0 // 8] = jnp.concatenate(
                        [v80[r0:r0 + 24], ones8], axis=0).astype(BF16)

        def mem_read(self):
            for j in range(4):
                r = dot(mst[self.g].astype(BF16), _bf(self.window(pqs[self.s % 2], j)), NT_DIMS)
                coef = gtab[self.g] / (r[80:88] + 1e-6)
                cb = [jnp.broadcast_to(coef[a:a + 1], (8, 128)) for a in range(4)]
                for pr in range(2):
                    ca, cc = cb[2 * pr], cb[2 * pr + 1]
                    for e, scale in enumerate((ca, ca, jnp.where(sub < 4, ca, cc), cc, cc)):
                        r0 = 40 * pr + 8 * e
                        opart[self.gi, j, r0:r0 + 8, :] = r[r0:r0 + 8] * scale
                self.have_mem.add(j)
                yield 24

        def mem_update(self):
            acc = None
            for j in range(4):
                t = dot(_bf(vall.bitcast(U32)[self.gi, j]), _bf(self.window(pks[self.s % 2], j)))
                acc = t if acc is None else acc + t
                if j < 3:
                    yield 24
            for r in range(12):
                new = jnp.where(bmask[r] & hsel[self.gi] != 0, acc[8 * r:8 * r + 8], 0.0)
                at = pl.ds(8 * r, 8)
                mst[self.g, at, :] = new if self.s == 0 else mst[self.g, at, :] + new
            yield 24

        def logits(self, pr, j, slot):
            qw = self.window(qs[self.s % 2], j)
            qa = qw & tile_rows(hmask[self.gi, 2 * pr], 64)
            qh = qw & tile_rows(hmask[self.gi, 2 * pr + 1], 64)
            w_a = _bf(qa)
            w_b = _bf(jnp.concatenate([qh[32:64], qh[0:32]], axis=0))
            w_t = _bf(jnp.concatenate([qh[32:64], qa[32:64]], axis=0))
            n = 128 * j

            def park(t, e, r0, m):
                for r in range(0, t.shape[0], 8):
                    v = t[r:r + 8]
                    if e == 2:
                        v = v + cmask[2, r:r + 8, :]
                    elif r0 + r >= n:
                        v = v + cmask[e, r0 + r - n:r0 + r - n + 8, :]
                    slot[e % 2, 448 * (e // 2) + r0 + r:448 * (e // 2) + r0 + r + 8, :] = v
                    m = v if m is None else jnp.maximum(m, v)
                return m

            m_t = park(dot(self.keys(n + 64, n + 128), w_t, NT_DIMS, 1), 2, 0, None)
            yield 16 * LW
            cuts = list(range(0, n, QCH)) or [0]
            m = [None, None]
            for r0, r1 in zip(cuts, cuts[1:] + [n + 64]):
                for e, w in enumerate((w_a, w_b)):
                    m[e] = park(dot(self.keys(r0, r1), w, NT_DIMS, 1), e, r0, m[e])
                    if r1 == n + 64 and e == 1:
                        m_a = jnp.maximum(m[0], jnp.where(lane >= 64, m_t, NEG))
                        m_b = jnp.maximum(m[1], jnp.where(lane < 64, m_t, NEG))
                        m_a = jnp.broadcast_to(jnp.max(m_a, axis=0, keepdims=True), (8, 128))
                        m_b = jnp.broadcast_to(jnp.max(m_b, axis=0, keepdims=True), (8, 128))
                        slot[1, 448:456, :] = m_a
                        slot[1, 456:464, :] = m_b
                        slot[1, 464:472, :] = jnp.where(lane < 64, m_b, m_a)
                    yield (r1 - r0) // 4 * LW

    def attend(gi, g, parity, add_mem, pr, j, slot, need_values):
        def prob(e, r0, n, which):
            m2 = tile_rows(slot[1, 448 + 8 * which:456 + 8 * which, :], 16)
            return [jnp.exp2(slot[e, r:r + 16, :] - m2).astype(BF16)
                    for r in range(r0, r0 + n, 16)]

        p_t = _u32(jnp.concatenate(prob(0, 448, 64, 2), axis=0))
        tails = (_bf(jnp.where(lanes(32) >= 64, p_t, np.uint32(0))),
                 _bf(jnp.where(lanes(32) >= 64, np.uint32(0), p_t)))
        res = []
        for e in range(2):
            acc = None
            for kt in range(j + 1):
                need_values(kt)
                if kt < j:
                    p = prob(e, 128 * kt, 128, e)
                else:
                    p = prob(e, 128 * kt, 64, e) + [tails[e]]
                t = dot(_bf(vhead.bitcast(U32)[gi, kt, 5 * pr + 2 * e]),
                         jnp.concatenate(p, axis=0), kind=2)
                acc = t if acc is None else acc + t
                if (e, kt) != (1, j):
                    yield 8 * AW
            res.append(acc)
        r_a = res[0]
        r_b = pltpu.roll(res[1], 64, 1)
        keep = 1.0 - gtab[g]
        keep_a = jnp.broadcast_to(keep[2 * pr:2 * pr + 1], (8, 128))
        keep_b = jnp.broadcast_to(keep[2 * pr + 1:2 * pr + 2], (8, 128))
        o_a = r_a[0:24] * tile_rows(keep_a / r_a[24:32], 24)
        o_b = r_b[0:24] * tile_rows(keep_b / r_b[24:32], 24)
        o = jnp.concatenate(
            [o_a[0:16], jnp.where(sub < 4, o_a[16:24], o_b[0:8]), o_b[8:24]], axis=0)
        if add_mem:
            o = o + opart[gi, j, 40 * pr:40 * pr + 40, :]
        if pr == 0:
            opart[gi, j, 0:40, :] = o
        else:
            o = jnp.concatenate([opart[gi, j, 0:40, :], o], axis=0)
            ots[parity, j, rows(g, 80), :] = o.astype(BF16)
        yield 8 * AW

    def v_proj(s, i, groups, have):
        for j in range(4):
            for gis in VSPLIT:
                acc = None
                for c in range(NT):
                    t = dot(_bf(wvt[c, rows(2 * i // len(gis) + gis[0], 40 * len(gis)), :]),
                            _bf(xb[c, rows(4 * s + j, 64), :]), NT_DIMS)
                    acc = t if acc is None else acc + t
                    if c == NT - 1:
                        for k, gi in enumerate(gis):
                            groups[gi].park_values(j, acc[80 * k:80 * k + 80])
                        if gis[-1] == 1:
                            have.append(j)
                    yield 20 * len(gis)

    def chain(*gens):
        for g in gens:
            yield from g

    units = [(gi, pr, j) for gi in range(2) for pr in range(2)
             for j in (LAST_ORDER if (gi, pr) == (1, 1) else range(4))]

    def cost(j):
        return (48 + 64 * j) * LW, (16 + 16 * j) * AW

    def carried(u, g, parity, weight=None):
        gi, pr, j = units[u]
        return attend(gi, g, parity, True, pr, j, slots[u % NSLOT], lambda kt: None), cost(j)[1]

    def segment_step(s, i, mxu_fill, vpu_fill, targets):
        vt = []
        fill = _Paced(mxu_fill, sequential=SEQ_FILL)
        for _ in range(HEAD if s < NSEG - 1 else HEAD // 2):
            fill.step()
        if s > 0:
            untranspose(s - 1, i)
        groups = [Group(s, 2 * i + gi, gi) for gi in range(2)]
        reads = [grp.mem_read() for grp in groups if s > 0]
        updates = [grp.mem_update() for grp in groups if s < NSEG - 1]
        first = _Paced([(chain(*reads[:1], v_proj(s, i, groups, vt), *reads[1:], *updates),
                         800 + 96 * (len(reads) + len(updates)))])
        side = _Paced(vpu_fill)
        total = first.total + fill.total
        held = 96 * (s > 0) + 160

        def need_values(kt):
            while len(vt) <= kt:
                first.step()

        def pad(fraction, u):
            target = total * fraction
            early = min(target * EARLY, held if u < DEPTH else first.total)
            first.advance(early / first.total)
            fill.advance((target - early) / fill.total)
            if side.live and side.done < fraction * side.total and recent[0] is not None:
                pace(i, targets)
                side.advance(fraction)

        whole = sum(sum(cost(j)) for _, _, j in units) * (1 + TAIL)
        done = 0
        for u in range(len(units)):
            gi, pr, j = units[u]
            streams = [(groups[gi].logits(pr, j, slots[u % NSLOT]), cost(j)[0])]
            v = u - DEPTH
            if v < 0:
                parity = (s - (i == 0)) % 2 if isinstance(i, int) else jnp.where(
                    i > 0, s % 2, 1 - s % 2)
                streams.append(carried(v + len(units), (2 * i + 7) & 7, parity))
            else:
                gi, pr, j = units[v]
                while s > 0 and j not in groups[gi].have_mem:
                    first.step()
                streams.append((attend(gi, 2 * i + gi, s % 2, s > 0, pr, j, slots[v % NSLOT],
                                       need_values), cost(j)[1]))
            att = _Paced(streams[::-1], sequential=u == len(units) - 1)
            while att.live:
                att.step()
                pad((done + att.done) / whole, u)
            done += att.total
        first.finish()
        fill.finish()
        side.finish()

    def split_h(i, cs):
        for c in cs:
            for t in range(4):
                ht[c, 64 * t:64 * t + 64, :] = _u32(_bf(hb[4 * i + t, 64 * c:64 * c + 64, :]).T)
                yield 16
            for q in range(2):
                for j in range(8):
                    wa = ht[c, pl.ds(128 * q + j, 8, stride=8), :]
                    wb = ht[c, pl.ds(128 * q + 64 + j, 8, stride=8), :]
                    hp[c][2 * j, rows(2 * i + q, 8), :] = _pack2(_lo(wa), _lo(wb))
                    hp[c][2 * j + 1, rows(2 * i + q, 8), :] = _pack2(_hi(wa), _hi(wb))
                    if j % 2:
                        yield 4

    def split_kv(i, cs):
        for c in cs:
            taps = [wtab[c, j] for j in range(KS)]
            for q in range(2):
                blk = 2 * i + q
                base = [blk * 128 + 64 * e for e in range(2)]
                hist = []
                for e in range(2):
                    w2 = kb[c, pl.ds(base[e] + 6, 8, stride=8), :]
                    w1 = kb[c, pl.ds(base[e] + 7, 8, stride=8), :]
                    hist.append([_hi(w2), _lo(w1), _hi(w1)])
                for j in range(8):
                    kv = [[None, None], [None, None]]
                    for e in range(2):
                        kw = kb[c, pl.ds(base[e] + 8 + j, 8, stride=8), :]
                        vw = vb[c, pl.ds(base[e] + j, 8, stride=8), :]
                        kp = hist[e] + [_lo(kw), _hi(kw)]
                        for half, part in enumerate((_lo, _hi)):
                            acc = kp[3 + half] * taps[0]
                            for d in range(1, KS):
                                acc = acc + kp[3 + half - d] * taps[d]
                            kv[half][e] = acc * part(vw)
                            kvf[c, 2 * j + half, rows(2 * blk + e, 8), :] = kv[half][e]
                        hist[e] = kp[2:]
                    for half in range(2):
                        xp[c][2 * j + half, rows(blk, 8), :] = _pack2(*kv[half])
                    yield 11

    def fwd_fft(i, cs):
        for c in cs:
            for src, dst in ((hp[c], th[c]), (xp[c], tx[c])):
                for r0 in range(0, 2 * N1, FCH):
                    g = [dot(_bf(fwd[4 * a + i, r0 // 2:(r0 + FCH) // 2, :]), _bf(src[4 * a + i]))
                         for a in range(4)]
                    for r in range(0, FCH, 16):
                        z = _radix4(*[(g[a][r:r + 8], g[a][r + 8:r + 16]) for a in range(4)], 1)
                        for cc in range(4):
                            dst[(r0 + r) // 16, cc, i, 0] = z[cc][0]
                            dst[(r0 + r) // 16, cc, i, 1] = z[cc][1]
                    yield FCH

    current = [None]

    def spectrum(c, m, slot):
        current[0] = c
        for cc in range(4):
            zh = _radix4_tw(*[(th[c][m, cc, b, 0], th[c][m, cc, b, 1]) for b in range(4)], 1, cc)
            yield 1
            zx = _radix4_tw(*[(tx[c][m, cc, b, 0], tx[c][m, cc, b, 1]) for b in range(4)], 1, cc)
            yield 1
            y = [(x[0] * h[0] - x[1] * h[1], x[0] * h[1] + x[1] * h[0]) for x, h in zip(zx, zh)]
            yield 1
            u = _radix4(*y, -1)
            for b in range(4):
                ub[slot, b, cc, 0] = u[b][0]
                ub[slot, b, cc, 1] = u[b][1]
            yield 1
        for b in range(4):
            z = _radix4_tw(*[(ub[slot, b, cc, 0], ub[slot, b, cc, 1]) for cc in range(4)], -1, b)
            for a in range(4):
                yb[c][4 * a + b, rows(m, 8), :] = _pack2(*z[a])
            yield 1

    SPEC_STEPS = 20

    def spectra(cs, ms, slot0=0):
        for slot, (c, m) in enumerate(((c, m) for c in cs for m in ms), slot0):
            yield from spectrum(c, m, slot)

    def spare_h(d, v):
        hb[S // 128, rows(d, 8), :] = _u32_word(v)

    def spare_k(d, v):
        kb[NT, rows(d, 8), :] = _u32_word(v)

    def spare_t(d, v):
        if current[0] is not None:
            th[current[0]][N1 // 8, d, 0, 0] = v

    def inverse(cs, jps):
        for c in cs:
            for jp in jps:
                w = qb[c, pl.ds(jp, N1, stride=8), :]
                res = []
                for e, part in enumerate((_lo, _hi)):
                    n2 = 2 * jp + e
                    y = dot(_bf(inv[n2, 0]), _bf(yb[c][n2, 0:64, :]))
                    yield 32
                    y = y + dot(_bf(inv[n2, 1]), _bf(yb[c][n2, 64:128, :]))
                    res.append(part(w) * (y + kvf[c, n2] * tile_rows(wtab[c, KS], N1)))
                    if e == 0:
                        yield 32
                outa[c, pl.ds(jp, N1, stride=8), :] = _pack2(*res)
                yield 32

    def loop(s, body):
        if UNROLL[s]:
            for i in range(4):
                body(i, 0)
        else:
            lax.fori_loop(0, 4, body, 0)

    def when(cond):
        if isinstance(cond, bool):
            return lambda f: f() if cond else None
        return pl.when(cond)

    start(cp_small, cp_x[0], cp_w[0])
    sem_zero[0] = 0
    kk = lax.broadcasted_iota(jnp.int32, (64, 128), 0)
    ll = lax.broadcasted_iota(jnp.int32, (64, 128), 1)
    cmask[0] = jnp.where(kk <= ll, 0.0, NEG)
    cmask[1] = jnp.where((ll < 64) | (kk <= ll - 64), 0.0, NEG)
    cmask[2] = jnp.where(kk <= (ll & 63), 0.0, NEG)
    for r in range(12):
        row = sub + 8 * r
        hr = sum((row >= a * DH).astype(jnp.int32) for a in range(1, 4)) if r < 10 else row - 80
        bmask[r] = jnp.left_shift(1, hr)
    for gi in range(2):
        for j in range(4):
            vall[gi, j, 80:96, :] = jnp.ones((16, 128), BF16)
    for c in range(NT):
        kb[c, 0:8, :] = jnp.zeros((8, 128), U32)
    for u in range(16 - DEPTH, 16):
        slots[u % NSLOT][...] = jnp.zeros((2, 512, 128), F32)
    vhead[1] = jnp.ones(vhead.shape[1:], BF16)
    opart[1] = jnp.zeros(opart.shape[1:], F32)
    start(cp_w[1])
    wait(cp_small)
    taps_t = shift_ref[...].astype(F32)
    skip = ssmd_ref[...].astype(F32)
    for c in range(NT):
        for j in range(KS):
            wtab[c, j] = jnp.broadcast_to(taps_t[j:j + 1, 128 * c:128 * c + 128], (8, 128))
        wtab[c, KS] = jnp.broadcast_to(skip[c:c + 1], (8, 128))
    gates = jax.nn.sigmoid(beta_ref[...].astype(F32))
    gcol = jnp.broadcast_to(gates, (8, H)).T
    gcol = jnp.broadcast_to(gcol[:, 0:1], (H, 128))
    for g in range(8):
        gtab[g] = jnp.concatenate([gcol[4 * g:4 * g + 4]] * 2, axis=0)
    start(cp_w[2])
    with jax.named_scope("prologue"):
        wait(cp_x[0], cp_w[0])
        start(cp_w[3], cp_w[4], cp_wv)
        first_proj(0)
        wait(cp_w[1], cp_w[2])
        start(cp_early[0])
        first_proj(1)
        first_proj(2)
        wait(cp_w[3], cp_w[4], cp_wv)
        start(cp_early[1])
        for n in range(NT):
            for c in range(NT):
                wvt[c, rows(n, 64), :] = _u32(_bf(wvb[n, 64 * c:64 * c + 64, :]).T)
        first_proj(3)
        first_proj(4)
    start(cp_wo, cp_x[2])

    def seg0(i, carry):
        for j in range(4):
            @when(i == j)
            def _():
                wait(cp_early[j])
                start(*((cp_early[2],), (cp_early[3],), (cp_fwd, cp_late), (cp_x[3],))[j])
        segment_step(0, i, [(qk_proj(1, i, True, True), 1600)],
                     [(split_h(i, EARLY_TILES), 96 * len(EARLY_TILES)),
                      (split_kv(i, EARLY_TILES), 176 * len(EARLY_TILES))], [spare_h, spare_k])
        return carry

    with jax.named_scope("seg0"):
        loop(0, seg0)
    wait(cp_fwd, cp_x[2], cp_wo, cp_late)
    start(cp_inv, cp_q)

    def seg1(i, carry):
        segment_step(1, i, [(qk_proj(2, i, True, True), 1600), (out_proj(0, i), 800),
                            (fwd_fft(i, EARLY_TILES), 512 * len(EARLY_TILES))],
                     [(split_h(i, LATE_TILES), 96 * len(LATE_TILES)),
                      (split_kv(i, LATE_TILES), 176 * len(LATE_TILES))], [spare_h, spare_k])
        return carry

    with jax.named_scope("seg1"):
        loop(1, seg1)
    start(cp_ob[0])
    wait(cp_x[3])

    def seg2(i, carry):
        segment_step(2, i, [(qk_proj(3, i, True, False), 1600), (out_proj(1, i), 800),
                            (fwd_fft(i, LATE_TILES), 512 * len(LATE_TILES))],
                     [(spectra(EARLY_TILES, [4 * i + a for a in range(4)]),
                       4 * SPEC_STEPS * len(EARLY_TILES))], [spare_t])
        return carry

    with jax.named_scope("seg2"):
        loop(2, seg2)
    wait(cp_ob[0], cp_inv, cp_q)
    start(cp_ob[1])

    def seg3(i, carry):
        segment_step(3, i, [(inverse(EARLY_TILES, (2 * i, 2 * i + 1)), 256 * len(EARLY_TILES)),
                            (out_proj(2, i), 800)],
                     [(chain(spectra(LATE_TILES[:-1], [4 * i + a for a in range(4)]),
                             spectra(LATE_TILES[-1:], [SHIFT * i + a for a in range(SHIFT)], 12)),
                       SPEC_STEPS * (4 * len(LATE_TILES[:-1]) + SHIFT))], [spare_t])
        return carry

    with jax.named_scope("seg3"):
        loop(3, seg3)
    wait(cp_ob[1])
    start(cp_ob[2], [cp_oa[c] for c in EARLY_TILES])
    with jax.named_scope("epilogue"):
        last = LATE_TILES[-1]
        PACE_ON[0] = 7
        side = _Paced([(spectra((last,), range(4 * SHIFT, 16)), (16 - 4 * SHIFT) * SPEC_STEPS)])
        span = 1024 * len(LATE_TILES[:-1]) + 800 * MID
        done = 0

        def run(streams):
            nonlocal done
            work = _Paced(streams)
            while work.live:
                before = work.done
                work.step()
                done += work.done - before
                if side.live and side.done < done / span * side.total and recent[0] is not None:
                    pace(0, [spare_t])
                    side.advance(done / span)

        for c in LATE_TILES[:-1]:
            streams = [(inverse((c,), range(8)), 1024)]
            if c == LATE_TILES[0]:
                streams.append((chain(*[carried(u, 7, 1, 0)[0] for u in range(16 - DEPTH, 16)]),
                                sum(cost(units[u][2])[1] for u in range(16 - DEPTH, 16))))
            run(streams)
            if c == LATE_TILES[0]:
                for i in range(4):
                    untranspose(3, i, i)
            start([cp_oa[c]])
        for i in range(4):
            if i == MID:
                side.finish()
                run([(inverse((last,), range(8)), 1024)])
                start([cp_oa[last]])
            run([(out_proj(3, i, i, cp_ob3[i]), 800)])
    wait(cp_ob[2], *cp_ob3, cp_oa)


@jax.jit
def pallas_concat_heads__ssm_conv_h3__memory_aug_infini_attn__prompt_kernel(
    A_q: jax.Array,
    A_k: jax.Array,
    A_v: jax.Array,
    A_shift_k: jax.Array,
    A_ssm_k: jax.Array,
    A_ssm_D: jax.Array,
    B_x: jax.Array,
    B_wq: jax.Array,
    B_wk: jax.Array,
    B_wv: jax.Array,
    B_wo: jax.Array,
    B_beta: jax.Array,
):
    hbm = pl.BlockSpec(memory_space=pltpu.HBM)
    seg_tiles = pltpu.VMEM((NT, L, 128), BF16)
    seq_tiles = pltpu.VMEM((NT, S // 2, 128), U32)
    w_tiles = pltpu.VMEM((NT, D // 2, 128), U32)
    scratch = [
        pltpu.VMEM((KS, D), BF16),
        pltpu.VMEM((NT, 128), BF16),
        pltpu.VMEM((1, H), BF16),
        seq_tiles,
        w_tiles, w_tiles, w_tiles, w_tiles, w_tiles,
        pltpu.VMEM((S // 128 + 1, D // 2, 128), U32),
        pltpu.VMEM((NT, 256, 128), U32),
        pltpu.VMEM((NT + 1, S // 2 + 8, 128), U32),
        seq_tiles, seq_tiles,
        pltpu.VMEM((N2, N1, 128), U32),
        pltpu.VMEM((N2, 2, N1 // 2, 128), U32),
        pltpu.VMEM((NT, N2, N1, 128), F32),
        pltpu.VMEM((16, 4, 4, 2, 8, 128), F32),
        seq_tiles,
        pltpu.VMEM((NT, S, 128), BF16),
        pltpu.VMEM((NT, KS + 1, 8, 128), F32),
        pltpu.VMEM((8, 8, 128), F32),
        pltpu.VMEM((3, 64, 128), F32),
        seg_tiles, seg_tiles, seg_tiles, seg_tiles,
        seg_tiles, seg_tiles, seg_tiles, seg_tiles,
        pltpu.VMEM((2, 4, D, 128), BF16),
        pltpu.VMEM((8, 96, 128), F32),
        pltpu.VMEM((2, 4, 8, 128), U32),
        pltpu.VMEM((2, 8, 128), jnp.int32),
        pltpu.VMEM((12, 8, 128), jnp.int32),
        pltpu.VMEM((2, L // 2, 128), U32),
        pltpu.VMEM((2, 4, 96, 128), BF16),
        pltpu.VMEM((2, 4, 8, 32, 128), BF16),
        pltpu.VMEM((2, 4, 80, 128), F32),
        pltpu.VMEM((4, NT, 64, 128), U32),
        pltpu.SMEM((1,), jnp.int32),
        pltpu.SemaphoreType.DMA((21,)),
    ]
    scratch += [pltpu.VMEM((N2, N1 // 2, 128), U32)] * (2 * NT)
    scratch += [pltpu.VMEM((N1 // 8 + 1, 4, 4, 2, 8, 128), F32)] * (2 * NT)
    scratch += [pltpu.VMEM((N2, N1, 128), U32)] * NT
    scratch += [pltpu.VMEM((2, 512, 128), F32)] * NSLOT
    return pl.pallas_call(
        _kernel,
        out_shape=jax.ShapeDtypeStruct((1, S, 2 * D), BF16),
        in_specs=[hbm] * 14,
        out_specs=hbm,
        scratch_shapes=scratch,
        compiler_params=pltpu.CompilerParams(vmem_limit_bytes=110 * 1024 * 1024, flags=FLAGS),
        name="h3_infini",
    )(A_q, A_k, A_v, A_shift_k.T, A_ssm_k, A_ssm_D.reshape(NT, 128), B_x, B_wq, B_wk, B_wv, B_wo,
      B_beta.reshape(1, H), _FWD, _INV)
```

```python
import math

import jax
import jax.numpy as jnp
import numpy as np
from jax import lax
from jax.experimental import pallas as pl
from jax.experimental.pallas import tpu as pltpu

S = 2048
D = 640
NT = D // 128
H = 32
DH = D // H
NSEG = 4
L = S // NSEG
KS = 4
N1, N2 = 128, 16

F32 = jnp.float32
BF16 = jnp.bfloat16
U32 = jnp.uint32
NN_DIMS = (((1,), (0,)), ((), ()))
NT_DIMS = (((1,), (1,)), ((), ()))
NEG = -1e30
LOG2E = 1.4426950408889634


def _pack_rows(a):
    u = a.astype(np.float32).astype(BF16).view(np.uint16).astype(np.uint32)
    return u[..., 0::2, :] | (u[..., 1::2, :] << 16)


def _dft_tables():
    k1 = np.arange(N1)
    fwd = np.zeros((N2, 2 * N1, N1), np.float64)
    inv = np.zeros((N2, N1, 2 * N1), np.float64)
    kappa = np.arange(N1)
    n1_in = 16 * (kappa // 16) + 8 * (kappa % 2) + (kappa % 16) // 2
    row_re = 16 * (k1 // 8) + k1 % 8
    for n2 in range(N2):
        ang = 2.0 * np.pi * np.outer(k1 + 0.25, N2 * n1_in + n2) / S
        fwd[n2, row_re] = np.cos(ang)
        fwd[n2, row_re + 8] = np.sin(ang)
        ang = 2.0 * np.pi * np.outer(N2 * np.arange(N1) + n2, k1 + 0.25) / S
        inv[n2][:, 2 * k1] = np.cos(ang) / S
        inv[n2][:, 2 * k1 + 1] = np.sin(ang) / S
    inv = inv.reshape(N2, N1, 2, N1).transpose(2, 0, 1, 3).reshape(2 * N2, N1, N1)
    return _pack_rows(fwd), _pack_rows(inv)


_FWD, _INV = _dft_tables()


def _dot(a, b, dims=NN_DIMS):
    return lax.dot_general(a, b, dims, preferred_element_type=F32)


def _u32(x):
    return pltpu.bitcast(x, U32)


def _bf(x):
    return pltpu.bitcast(x, BF16)


def _u32_word(x):
    return lax.bitcast_convert_type(x, U32)


def _pack2(a, b):
    return pltpu.pack_elementwise([a, b], packed_dtype=BF16).astype(U32)


def _lo(w):
    return pltpu.unpack_elementwise(w, index=0, packed_dtype=BF16, unpacked_dtype=F32)


def _hi(w):
    return pltpu.unpack_elementwise(w, index=1, packed_dtype=BF16, unpacked_dtype=F32)


def _radix4(x0, x1, x2, x3, sign):
    ar, ai = x0[0] + x2[0], x0[1] + x2[1]
    br, bi = x0[0] - x2[0], x0[1] - x2[1]
    cr, ci = x1[0] + x3[0], x1[1] + x3[1]
    dr, di = x1[0] - x3[0], x1[1] - x3[1]
    y0 = (ar + cr, ai + ci)
    y2 = (ar - cr, ai - ci)
    yp = (br - di, bi + dr)
    ym = (br + di, bi - dr)
    return (y0, yp, y2, ym) if sign > 0 else (y0, ym, y2, yp)


def _twiddle(x, e, sign):
    xr, xi = x
    if e == 0:
        return x
    if e == 4:
        return (-xi, xr) if sign > 0 else (xi, -xr)
    r = math.sqrt(0.5)
    if e == 2:
        return ((xr - xi) * r, (xr + xi) * r) if sign > 0 else ((xr + xi) * r, (xi - xr) * r)
    if e == 6:
        return ((xr + xi) * -r, (xr - xi) * r) if sign > 0 else ((xi - xr) * r, (xr + xi) * -r)
    c, s = math.cos(math.pi * e / 8), sign * math.sin(math.pi * e / 8)
    return (xr * c - xi * s, xr * s + xi * c)


def _radix4_tw(x0, x1, x2, x3, sign, b):
    if b != 2:
        return _radix4(x0, _twiddle(x1, b, sign), _twiddle(x2, 2 * b, sign),
                       _twiddle(x3, 3 * b, sign), sign)
    x1, x3 = _twiddle(x1, 2, sign), _twiddle(x3, 6, sign)
    if sign > 0:
        ar, ai = x0[0] - x2[1], x0[1] + x2[0]
        br, bi = x0[0] + x2[1], x0[1] - x2[0]
    else:
        ar, ai = x0[0] + x2[1], x0[1] - x2[0]
        br, bi = x0[0] - x2[1], x0[1] + x2[0]
    cr, ci = x1[0] + x3[0], x1[1] + x3[1]
    dr, di = x1[0] - x3[0], x1[1] - x3[1]
    y0 = (ar + cr, ai + ci)
    y2 = (ar - cr, ai - ci)
    yp = (br - di, bi + dr)
    ym = (br + di, bi - dr)
    return (y0, yp, y2, ym) if sign > 0 else (y0, ym, y2, yp)


class _Paced:
    def __init__(self, streams, sequential=False):
        self.live = [[g, total, 0] for g, total in streams if total]
        self.total = sum(total for _, total in streams)
        self.done = 0
        self.sequential = sequential

    def step(self):
        cur = self.live[0] if self.sequential else min(self.live, key=lambda e: e[2] / e[1])
        cost = next(cur[0], None)
        if cost is None:
            self.live.remove(cur)
        else:
            cur[2] += cost
            self.done += cost

    def advance(self, fraction):
        while self.live and self.done < fraction * self.total:
            self.step()

    def finish(self):
        self.advance(math.inf)


PLAN_SPLIT = (2, 3, 4, 3, 2, 2, 2, 2, 0, 0, 0, 0, 0, 0, 0, 0)
PLAN_FORWARD = (0, 0, 2, 2, 2, 2, 2, 2, 2, 2, 2, 2, 0, 0, 0, 0)
PLAN_SPECTRUM = (0, 0, 0, 0, 4, 4, 4, 4, 8, 8, 8, 8, 6, 6, 6, 6)
PLAN_INVERSE = (0, 0, 0, 0, 0, 0, 0, 0, 2, 2, 2, 2, 4, 4, 4, 4)
BLOCKS = (4, 4, 4, 4)
ONLY = None
DEPTH = 3
NSLOT = 4
LAST_ORDER = (0, 1, 2, 3)
TAIL = [0.0] * 16
LW = [1.0] * 16
AW = [3.0] * 16
QCH = [128] * 16
HEAD = [4] * 16
SEQ_FILL = [True] * 16
PACE_ON = [3] * 15 + [7, 7]
MID = 3


def _deal(items, counts, ready):
    runs, pos = [], 0
    for t, n in enumerate(counts):
        runs.append(items[pos:pos + n])
        assert all(ready(item, t) for item in runs[-1])
        pos += n
    return runs + [items[pos:]]


def _done_before(runs, c, t):
    return all(item[0] != c for run in runs[t:] for item in run)


_SPLIT = _deal([(c, q) for c in range(NT) for q in range(4)], PLAN_SPLIT, lambda it, t: True)
_FORWARD = _deal([(c, b) for c in range(NT) for b in range(4)], PLAN_FORWARD,
                 lambda it, t: _done_before(_SPLIT, it[0], t))
_SPECTRUM = _deal([(c, m) for c in range(NT) for m in range(16)], PLAN_SPECTRUM,
                  lambda it, t: _done_before(_FORWARD, it[0], t))
_INVERSE = _deal([(c, jp) for c in range(NT) for jp in range(8)], PLAN_INVERSE,
                 lambda it, t: _done_before(_SPECTRUM, it[0], t))
assert not _SPLIT[-1] and not _FORWARD[-1]


def _kernel(aq_hbm, ak_hbm, av_hbm, shift_hbm, h_hbm, ssmd_hbm, x_hbm, wq_hbm, wk_hbm,
            wv_hbm, wo_hbm, beta_hbm, fwd_hbm, inv_hbm, out_hbm, shift_ref, ssmd_ref, beta_ref,
            xb, wqb, wkb, wvb, wob, wvt, hb, ht, kb, vb, qb, fwd, inv,
            ub, outb, wtab, gtab, cmask,
            q0, q1, k0, k1, pq0, pq1, pk0, pk1, ots, mst,
            hmask, hsel, bmask, kwin, vall, vhead, opart, onat, sem_zero, sems, *rest):
    xp, hp, tx, th, yb, kvf, outa = (rest[NT * k:NT * k + NT] for k in range(7))
    slots = rest[7 * NT:]
    qs, ks, pqs, pks = (q0, q1), (k0, k1), (pq0, pq1), (pk0, pk1)

    def tile_copy(src, dst, t, sem, r0, n, lead=(0,), dst_off=0):
        return lambda: pltpu.make_async_copy(
            src.bitcast(U32).at[(*lead, pl.ds(r0 // 2, n // 2), pl.ds(128 * t, 128))],
            dst.at[t, pl.ds(dst_off + r0 // 2, n // 2), :], sems.at[sem])

    def h_copy(t, c0, n, sem):
        return lambda: pltpu.make_async_copy(
            h_hbm.bitcast(U32).at[pl.ds(64 * c0, 64 * n), pl.ds(128 * t, 128)],
            hb.at[t, pl.ds(64 * c0, 64 * n), :], sems.at[sem])

    def step_copies(t):
        sem, out = 21 + t, []
        for c, q in _SPLIT[t]:
            out += [h_copy(4 * q + k, c, 1, sem) for k in range(4)]
            out += [tile_copy(ak_hbm, kb, c, sem, L * q, L, dst_off=8),
                    tile_copy(av_hbm, vb, c, sem, L * q, L)]
        if t < 12:
            out += [tile_copy(x_hbm, xb, c, sem, L + 128 * t, 128) for c in range(NT)]
        return out

    cp_x0 = [tile_copy(x_hbm, xb, c, 0, 0, L) for c in range(NT)]
    cp_w = [[tile_copy(src, dst, n, 4 + n, 0, D, lead=())
             for src, dst in ((wq_hbm, wqb), (wk_hbm, wkb))] for n in range(NT)]
    cp_wv = [tile_copy(wv_hbm, wvb, n, 1, 0, D, lead=()) for n in range(NT)]
    cp_wo = [tile_copy(wo_hbm, wob, n, 9, 0, D, lead=()) for n in range(NT)]
    cp_step = [step_copies(t) for t in range(12)]
    cp_q = [tile_copy(aq_hbm, qb, c, 15, 0, S) for c in range(NT)]
    cp_fwd = [lambda: pltpu.make_async_copy(fwd_hbm, fwd, sems.at[16])]
    cp_inv = [lambda: pltpu.make_async_copy(inv_hbm, inv, sems.at[17])]
    cp_small = [lambda: pltpu.make_async_copy(shift_hbm, shift_ref, sems.at[18]),
                lambda: pltpu.make_async_copy(ssmd_hbm, ssmd_ref, sems.at[18]),
                lambda: pltpu.make_async_copy(beta_hbm, beta_ref, sems.at[18])]

    def out_a(c):
        return lambda: pltpu.make_async_copy(
            outa[c], out_hbm.bitcast(U32).at[0, :, pl.ds(128 * c, 128)], sems.at[19])

    def out_b(r0, n, rows_):
        return lambda: pltpu.make_async_copy(
            outb.at[n, pl.ds(r0, rows_), :],
            out_hbm.at[0, pl.ds(r0, rows_), pl.ds(D + 128 * n, 128)], sems.at[20])

    cp_oa = [out_a(c) for c in range(NT)]
    cp_ob = [[out_b(L * s, n, L) for n in range(NT)] for s in range(NSEG - 1)]
    cp_ob3 = [[out_b(L * 3 + 128 * i, n, 128) for n in range(NT)] for i in range(4)]

    def start(*groups):
        for g in groups:
            for cp in g:
                cp().start()

    def wait(*groups):
        for g in groups:
            for cp in g:
                cp().wait()

    def rows(i, n):
        return pl.ds(i * n, n)

    lane = lax.broadcasted_iota(jnp.int32, (8, 128), 1)
    sub = lax.broadcasted_iota(jnp.int32, (8, 128), 0)

    def lanes(n):
        return lax.broadcasted_iota(jnp.int32, (n, 128), 1)

    recent = [None]
    step = [0]

    def dot(a, b, dims=NN_DIMS, kind=4):
        out = _dot(a, b, dims)
        if kind & PACE_ON[step[0]]:
            recent[0] = out
        return out

    def pace(targets):
        if recent[0] is not None:
            for target in targets:
                target(sem_zero[0], recent[0][-8:])
            recent[0] = None

    def qk_proj(s, i, want_pq, want_pk):
        p = s % 2
        tok = rows(4 * s + i, 64)
        for w_ref, dst, fdst, want, scale in (
                (wqb, qs[p], pqs[p], want_pq, DH ** -0.5 * LOG2E),
                (wkb, ks[p], pks[p], want_pk, None)):
            for n in range(NT):
                t = None
                for c in range(NT):
                    part = dot(_bf(xb[c, tok, :]), _bf(w_ref[n, 64 * c:64 * c + 64, :]))
                    t = part if t is None else t + part
                    if c < NT - 1:
                        yield 32
                dst[n, rows(i, 128), :] = (t if scale is None else t * scale).astype(BF16)
                if want:
                    fdst[n, rows(i, 128), :] = jnp.where(t > 0, t + 1.0, jnp.exp(t)).astype(BF16)
                yield 32

    def first_proj(n):
        for w_ref, dst, scale in ((wqb, qs[0], DH ** -0.5 * LOG2E), (wkb, ks[0], None)):
            for j in range(4):
                t = None
                for c in range(NT):
                    part = dot(_bf(xb[c, rows(j, 64), :]), _bf(w_ref[n, 64 * c:64 * c + 64, :]))
                    t = part if t is None else t + part
                dst[n, rows(j, 128), :] = (t if scale is None else t * scale).astype(BF16)
                if scale is None:
                    pks[0][n, rows(j, 128), :] = jnp.where(t > 0, t + 1.0, jnp.exp(t)).astype(BF16)

    def untranspose(s, i, slot=0):
        ot = ots.bitcast(U32)
        for c in range(NT):
            onat[slot, c] = _u32(_bf(ot[s % 2, i, 64 * c:64 * c + 64, :]).T)

    def out_proj(s, i, slot=0, copies=None):
        for n in range(NT):
            t = None
            for c in range(NT):
                part = dot(_bf(onat[slot, c]), _bf(wob[n, 64 * c:64 * c + 64, :]))
                t = part if t is None else t + part
                if c < NT - 1:
                    yield 32
            outb[n, rows(4 * s + i, 128), :] = t.astype(BF16)
            if copies is not None:
                start([copies[n]])
            yield 32

    def tile_rows(r, n):
        return jnp.broadcast_to(r[None], (n // 8, 8, 128)).reshape(n, 128)

    class Group:
        def __init__(self, s, g, gi):
            self.s, self.g, self.gi = s, g, gi
            self.t0 = (80 * g) // 128
            self.off = 80 * g - 128 * self.t0
            rel = (lane - self.off) & 127
            head = sum((rel >= a * DH).astype(jnp.int32) for a in range(1, 5))
            for a in range(4):
                hmask[gi, a] = jnp.where(head == a, np.uint32(0xFFFFFFFF), np.uint32(0))
            hsel[gi] = jnp.left_shift(1, head)
            self.have_keys, self.have_mem = set(), set()

        def window(self, ref, j, r0=0, n=64):
            ref = ref.bitcast(U32)
            at = pl.ds(64 * j + r0, n)
            if self.off + 80 <= 128:
                return ref[self.t0, at, :]
            return jnp.where(lanes(n) >= self.off, ref[self.t0, at, :], ref[self.t0 + 1, at, :])

        def keys(self, r0, r1):
            out = []
            for r in range(r0, r1, 64):
                at = pl.ds(r // 2, 32)
                if r in self.have_keys:
                    out.append(kwin[self.gi, at, :])
                else:
                    self.have_keys.add(r)
                    out.append(self.window(ks[self.s % 2], 0, r // 2, 32))
                    kwin[self.gi, at, :] = out[-1]
            return _bf(jnp.concatenate(out, axis=0))

        def park_values(self, j, v80):
            vall[self.gi, j, 0:80, :] = v80.astype(BF16)
            ones8 = jnp.ones((8, 128), F32)
            for pr in range(2):
                for e in range(2):
                    r0 = 40 * pr + 16 * e
                    vhead[self.gi, j, r0 // 8] = jnp.concatenate(
                        [v80[r0:r0 + 24], ones8], axis=0).astype(BF16)

        def mem_read(self):
            for j in range(4):
                r = dot(mst[self.g].astype(BF16), _bf(self.window(pqs[self.s % 2], j)), NT_DIMS)
                coef = gtab[self.g] / (r[80:88] + 1e-6)
                cb = [jnp.broadcast_to(coef[a:a + 1], (8, 128)) for a in range(4)]
                for pr in range(2):
                    ca, cc = cb[2 * pr], cb[2 * pr + 1]
                    for e, scale in enumerate((ca, ca, jnp.where(sub < 4, ca, cc), cc, cc)):
                        r0 = 40 * pr + 8 * e
                        opart[self.gi, j, r0:r0 + 8, :] = r[r0:r0 + 8] * scale
                self.have_mem.add(j)
                yield 24

        def mem_update(self):
            acc = None
            for j in range(4):
                t = dot(_bf(vall.bitcast(U32)[self.gi, j]), _bf(self.window(pks[self.s % 2], j)))
                acc = t if acc is None else acc + t
                if j < 3:
                    yield 24
            for r in range(12):
                new = jnp.where(bmask[r] & hsel[self.gi] != 0, acc[8 * r:8 * r + 8], 0.0)
                at = pl.ds(8 * r, 8)
                mst[self.g, at, :] = new if self.s == 0 else mst[self.g, at, :] + new
            yield 24

        def logits(self, pr, j, slot):
            qw = self.window(qs[self.s % 2], j)
            qa = qw & tile_rows(hmask[self.gi, 2 * pr], 64)
            qh = qw & tile_rows(hmask[self.gi, 2 * pr + 1], 64)
            w_a = _bf(qa)
            w_b = _bf(jnp.concatenate([qh[32:64], qh[0:32]], axis=0))
            w_t = _bf(jnp.concatenate([qh[32:64], qa[32:64]], axis=0))
            n = 128 * j

            def park(t, e, r0, m):
                for r in range(0, t.shape[0], 8):
                    v = t[r:r + 8]
                    if e == 2:
                        v = v + cmask[2, r:r + 8, :]
                    elif r0 + r >= n:
                        v = v + cmask[e, r0 + r - n:r0 + r - n + 8, :]
                    slot[e % 2, 448 * (e // 2) + r0 + r:448 * (e // 2) + r0 + r + 8, :] = v
                    m = v if m is None else jnp.maximum(m, v)
                return m

            m_t = park(dot(self.keys(n + 64, n + 128), w_t, NT_DIMS, 1), 2, 0, None)
            yield 16 * LW[step[0]]
            cuts = list(range(0, n, QCH[step[0]])) or [0]
            m = [None, None]
            for r0, r1 in zip(cuts, cuts[1:] + [n + 64]):
                for e, w in enumerate((w_a, w_b)):
                    m[e] = park(dot(self.keys(r0, r1), w, NT_DIMS, 1), e, r0, m[e])
                    if r1 == n + 64 and e == 1:
                        m_a = jnp.maximum(m[0], jnp.where(lane >= 64, m_t, NEG))
                        m_b = jnp.maximum(m[1], jnp.where(lane < 64, m_t, NEG))
                        m_a = jnp.broadcast_to(jnp.max(m_a, axis=0, keepdims=True), (8, 128))
                        m_b = jnp.broadcast_to(jnp.max(m_b, axis=0, keepdims=True), (8, 128))
                        slot[1, 448:456, :] = m_a
                        slot[1, 456:464, :] = m_b
                        slot[1, 464:472, :] = jnp.where(lane < 64, m_b, m_a)
                    yield (r1 - r0) // 4 * LW[step[0]]

    def attend(gi, g, parity, add_mem, pr, j, slot, need_values):
        def prob(e, r0, n, which):
            m2 = tile_rows(slot[1, 448 + 8 * which:456 + 8 * which, :], 16)
            return [jnp.exp2(slot[e, r:r + 16, :] - m2) for r in range(r0, r0 + n, 16)]

        res = [None, None]
        order = [(0, j), (1, j)] + [(e, kt) for e in range(2) for kt in range(j)]
        for n, (e, kt) in enumerate(order):
            need_values(kt)
            if n == 0:
                p_t = prob(0, 448, 64, 2)
            if kt < j:
                p = prob(e, 128 * kt, 128, e)
            else:
                mine = lanes(16) >= 64 if e == 0 else lanes(16) < 64
                p = prob(e, 128 * kt, 64, e) + [jnp.where(mine, t, 0.0) for t in p_t]
            t = dot(_bf(vhead.bitcast(U32)[gi, kt, 5 * pr + 2 * e]),
                    jnp.concatenate(p, axis=0).astype(BF16), kind=2)
            res[e] = t if res[e] is None else res[e] + t
            if n < len(order) - 1:
                yield 8 * AW[step[0]]
        r_a = res[0]
        r_b = pltpu.roll(res[1], 64, 1)
        keep = 1.0 - gtab[g]
        keep_a = jnp.broadcast_to(keep[2 * pr:2 * pr + 1], (8, 128))
        keep_b = jnp.broadcast_to(keep[2 * pr + 1:2 * pr + 2], (8, 128))
        o_a = r_a[0:24] * tile_rows(keep_a / r_a[24:32], 24)
        o_b = r_b[0:24] * tile_rows(keep_b / r_b[24:32], 24)
        o = jnp.concatenate(
            [o_a[0:16], jnp.where(sub < 4, o_a[16:24], o_b[0:8]), o_b[8:24]], axis=0)
        if add_mem:
            o = o + opart[gi, j, 40 * pr:40 * pr + 40, :]
        if pr == 0:
            opart[gi, j, 0:40, :] = o
        else:
            o = jnp.concatenate([opart[gi, j, 0:40, :], o], axis=0)
            ots[parity, j, rows(g, 80), :] = o.astype(BF16)
        yield 8 * AW[step[0]]

    def v_proj(s, i, groups, have):
        for j in range(4):
            acc = None
            for c in range(NT):
                t = dot(_bf(wvt[c, rows(i, 80), :]), _bf(xb[c, rows(4 * s + j, 64), :]), NT_DIMS)
                acc = t if acc is None else acc + t
                if c == NT - 1:
                    for gi in range(2):
                        groups[gi].park_values(j, acc[80 * gi:80 * gi + 80])
                    have.append(j)
                yield 40

    def chain(*gens):
        for g in gens:
            yield from g

    units = [(gi, pr, j) for gi in range(2) for pr in range(2)
             for j in (LAST_ORDER if (gi, pr) == (1, 1) else range(4))]

    def cost(j):
        return (48 + 64 * j) * LW[step[0]], (16 + 16 * j) * AW[step[0]]

    def carried(u, g, parity):
        gi, pr, j = units[u]
        return attend(gi, g, parity, step[0] - (step[0] % 4 == 0) > 3, pr, j, slots[u % NSLOT], lambda kt: None), cost(j)[1]

    def segment_step(s, i, mxu_fill, vpu_fill):
        vt = []
        fill = _Paced(mxu_fill, sequential=SEQ_FILL[step[0]])
        for _ in range(HEAD[step[0]]):
            fill.step()
        if s > 0:
            untranspose(s - 1, i)
        groups = [Group(s, 2 * i + gi, gi) for gi in range(2)]
        reads = [grp.mem_read() for grp in groups if s > 0]
        updates = [grp.mem_update() for grp in groups if s < NSEG - 1]
        first = _Paced([(chain(*reads[:1], v_proj(s, i, groups, vt), *reads[1:], *updates),
                         800 + 96 * (len(reads) + len(updates)))])
        side = _Paced(vpu_fill, sequential=True)
        total = first.total + fill.total
        held = 96 * (s > 0) + 160

        def need_values(kt):
            while len(vt) <= kt:
                first.step()

        def pad(fraction, u):
            target = total * fraction
            early = min(target, held if u < DEPTH else first.total)
            first.advance(early / first.total)
            fill.advance((target - early) / fill.total)
            if side.live and side.done < fraction * side.total and recent[0] is not None:
                pace([spare_h, spare_k, spare_t])
                side.advance(fraction)

        whole = sum(sum(cost(j)) for _, _, j in units) * (1 + TAIL[step[0]])
        done = 0
        for u in range(len(units)):
            gi, pr, j = units[u]
            streams = [(groups[gi].logits(pr, j, slots[u % NSLOT]), cost(j)[0])]
            v = u - DEPTH
            if v < 0:
                if s or i:
                    streams.append(carried(v + len(units), (2 * i + 7) & 7, (s - (i == 0)) % 2))
            else:
                gi, pr, j = units[v]
                while s > 0 and j not in groups[gi].have_mem:
                    first.step()
                streams.append((attend(gi, 2 * i + gi, s % 2, s > 0, pr, j, slots[v % NSLOT],
                                       need_values), cost(j)[1]))
            att = _Paced(streams[::-1], sequential=u == len(units) - 1)
            while att.live:
                att.step()
                pad((done + att.done) / whole, u)
            done += att.total
        first.finish()
        fill.finish()
        side.finish()

    current = {}

    def split_h(c, i):
        current.clear()
        current["h"] = True
        for t in range(4):
            ht[4 * c + i, 64 * t:64 * t + 64, :] = _u32(
                _bf(hb[4 * i + t, 64 * c:64 * c + 64, :]).T)
            yield 4
        for q in range(2):
            for j in range(8):
                wa = ht[4 * c + i, pl.ds(128 * q + j, 8, stride=8), :]
                wb = ht[4 * c + i, pl.ds(128 * q + 64 + j, 8, stride=8), :]
                hp[c][2 * j, rows(2 * i + q, 8), :] = _pack2(_lo(wa), _lo(wb))
                hp[c][2 * j + 1, rows(2 * i + q, 8), :] = _pack2(_hi(wa), _hi(wb))
                if j % 2:
                    yield 16

    def split_kv(c, i):
        current.clear()
        current["k"] = True
        taps = [wtab[c, j] for j in range(KS)]
        for q in range(2):
            blk = 2 * i + q
            base = [blk * 128 + 64 * e for e in range(2)]
            hist = []
            for e in range(2):
                w2 = kb[c, pl.ds(base[e] + 6, 8, stride=8), :]
                w1 = kb[c, pl.ds(base[e] + 7, 8, stride=8), :]
                hist.append([_hi(w2), _lo(w1), _hi(w1)])
            for j in range(8):
                kv = [[None, None], [None, None]]
                for e in range(2):
                    kw = kb[c, pl.ds(base[e] + 8 + j, 8, stride=8), :]
                    vw = vb[c, pl.ds(base[e] + j, 8, stride=8), :]
                    kp = hist[e] + [_lo(kw), _hi(kw)]
                    for half, part in enumerate((_lo, _hi)):
                        acc = kp[3 + half] * taps[0]
                        for d in range(1, KS):
                            acc = acc + kp[3 + half - d] * taps[d]
                        kv[half][e] = acc * part(vw)
                        kvf[c][2 * j + half, rows(2 * blk + e, 8), :] = kv[half][e]
                    hist[e] = kp[2:]
                    if e == 0:
                        yield 22
                for half in range(2):
                    xp[c][2 * j + half, rows(blk, 8), :] = _pack2(*kv[half])
                yield 22

    def fwd_fft(items):
        for c, i in items:
            for src, dst in ((hp[c], th[c]), (xp[c], tx[c])):
                g = [dot(_bf(fwd[4 * a + i]), _bf(src[4 * a + i])) for a in range(4)]
                for r in range(0, 2 * N1, 16):
                    z = _radix4(*[(g[a][r:r + 8], g[a][r + 8:r + 16]) for a in range(4)], 1)
                    for cc in range(4):
                        dst[r // 16, cc, i, 0] = z[cc][0]
                        dst[r // 16, cc, i, 1] = z[cc][1]
                yield 256

    def spectrum(c, m, slot):
        current.clear()
        current["t"] = c
        for cc in range(4):
            zh = _radix4_tw(*[(th[c][m, cc, b, 0], th[c][m, cc, b, 1]) for b in range(4)], 1, cc)
            yield 17
            zx = _radix4_tw(*[(tx[c][m, cc, b, 0], tx[c][m, cc, b, 1]) for b in range(4)], 1, cc)
            yield 17
            y = [(x[0] * h[0] - x[1] * h[1], x[0] * h[1] + x[1] * h[0]) for x, h in zip(zx, zh)]
            yield 17
            u = _radix4(*y, -1)
            for b in range(4):
                ub[slot, b, cc, 0] = u[b][0]
                ub[slot, b, cc, 1] = u[b][1]
            yield 17
        for b in range(4):
            z = _radix4_tw(*[(ub[slot, b, cc, 0], ub[slot, b, cc, 1]) for cc in range(4)], -1, b)
            for a in range(4):
                yb[c][4 * a + b, rows(m, 8), :] = _pack2(*z[a])
            yield 17

    SPEC_COST = 17 * 20

    def spectra(items):
        for slot, (c, m) in enumerate(items):
            yield from spectrum(c, m, slot)

    def spare_h(d, v):
        if "h" in current:
            hb[S // 128, rows(d, 8), :] = _u32_word(v)

    def spare_k(d, v):
        if "k" in current:
            kb[NT, rows(d, 8), :] = _u32_word(v)

    def spare_t(d, v):
        if "t" in current:
            th[current["t"]][N1 // 8, d, 0, 0] = v

    def inverse(items):
        for c, jp in items:
            w = qb[c, pl.ds(jp, N1, stride=8), :]
            res = []
            for e, part in enumerate((_lo, _hi)):
                n2 = 2 * jp + e
                y = dot(_bf(inv[n2]), _bf(yb[c][n2, 0:64, :]))
                yield 32
                y = y + dot(_bf(inv[N2 + n2]), _bf(yb[c][n2, 64:128, :]))
                res.append(part(w) * (y + kvf[c][n2] * tile_rows(wtab[c, KS], N1)))
                if e == 0:
                    yield 32
            outa[c][pl.ds(jp, N1, stride=8), :] = _pack2(*res)
            if jp == 7:
                start([cp_oa[c]])
            yield 32

    start(cp_small, cp_x0, cp_w[0])
    sem_zero[0] = 0
    kk = lax.broadcasted_iota(jnp.int32, (64, 128), 0)
    ll = lax.broadcasted_iota(jnp.int32, (64, 128), 1)
    cmask[0] = jnp.where(kk <= ll, 0.0, NEG)
    cmask[1] = jnp.where((ll < 64) | (kk <= ll - 64), 0.0, NEG)
    cmask[2] = jnp.where(kk <= (ll & 63), 0.0, NEG)
    for r in range(12):
        row = sub + 8 * r
        hr = sum((row >= a * DH).astype(jnp.int32) for a in range(1, 4)) if r < 10 else row - 80
        bmask[r] = jnp.left_shift(1, hr)
    for gi in range(2):
        for j in range(4):
            vall[gi, j, 80:96, :] = jnp.ones((16, 128), BF16)
    for c in range(NT):
        kb[c, 0:8, :] = jnp.zeros((8, 128), U32)
    start(cp_w[1])
    wait(cp_small)
    taps_t = shift_ref[...].astype(F32)
    skip = ssmd_ref[...].astype(F32)
    for c in range(NT):
        for j in range(KS):
            wtab[c, j] = jnp.broadcast_to(taps_t[j:j + 1, 128 * c:128 * c + 128], (8, 128))
        wtab[c, KS] = jnp.broadcast_to(skip[c:c + 1], (8, 128))
    gates = jax.nn.sigmoid(beta_ref[...].astype(F32))
    gcol = jnp.broadcast_to(gates, (8, H)).T
    gcol = jnp.broadcast_to(gcol[:, 0:1], (H, 128))
    for g in range(8):
        gtab[g] = jnp.concatenate([gcol[4 * g:4 * g + 4]] * 2, axis=0)
    start(cp_w[2])
    with jax.named_scope("prologue"):
        wait(cp_x0, cp_w[0])
        start(cp_w[3], cp_w[4], cp_wv)
        first_proj(0)
        wait(cp_w[1], cp_w[2])
        start(cp_step[0])
        first_proj(1)
        first_proj(2)
        wait(cp_w[3], cp_w[4], cp_wv)
        start(cp_step[1])
        for n in range(NT):
            for c in range(NT):
                wvt[c, rows(n, 64), :] = _u32(_bf(wvb[n, 64 * c:64 * c + 64, :]).T)
        first_proj(3)
        first_proj(4)

    extra_start = {0: (cp_fwd,), 1: (cp_wo,), 4: (cp_inv, cp_q), 9: (cp_ob[0],), 13: (cp_ob[1],)}
    extra_wait = {2: (cp_fwd,), 4: (cp_wo,), 8: (cp_inv, cp_q), 13: (cp_ob[0],)}

    def run_step(t):
        s, i = divmod(t, 4)
        step[0] = t
        if t < 12:
            wait(cp_step[t])
        wait(*extra_wait.get(t, ()))
        if t + 2 < 12:
            start(cp_step[t + 2])
        start(*extra_start.get(t, ()))
        fill = []
        if s < NSEG - 1:
            fill.append((qk_proj(s + 1, i, True, s + 1 < NSEG - 1), 1600))
        if _FORWARD[t]:
            fill.append((fwd_fft(_FORWARD[t][:1]), 512))
        if _INVERSE[t]:
            fill.append((inverse(_INVERSE[t]), 128 * len(_INVERSE[t])))
        if s > 0:
            fill.append((out_proj(s - 1, i), 800))
        if _FORWARD[t][1:]:
            fill.append((fwd_fft(_FORWARD[t][1:]), 512 * len(_FORWARD[t][1:])))
        side = [(spectra(_SPECTRUM[t]), SPEC_COST * len(_SPECTRUM[t]))]
        for c, q in _SPLIT[t]:
            side += [(split_h(c, q), 144), (split_kv(c, q), 704)]
        segment_step(s, i, fill, side)

    t0 = 0
    for s in range(NSEG):
        for _ in range(4 // BLOCKS[s]):
            steps = range(t0, t0 + BLOCKS[s])
            t0 += BLOCKS[s]
            if ONLY is not None and s != ONLY:
                continue

            @pl.when(sem_zero[0] == 0)
            def _():
                for t in steps:
                    run_step(t)

    wait(cp_ob[1])
    start(cp_ob[2])
    with jax.named_scope("epilogue"):
        step[0] = 16
        side = _Paced([(spectra(_SPECTRUM[16]), SPEC_COST * len(_SPECTRUM[16]))])
        early = [it for it in _INVERSE[16] if it[0] != NT - 1]
        span = 128 * len(early) + 800 * MID
        done = 0

        def run(streams):
            nonlocal done
            work = _Paced(streams)
            while work.live:
                before = work.done
                work.step()
                done += work.done - before
                if side.live and side.done < done / span * side.total and recent[0] is not None:
                    pace([spare_t])
                    side.advance(done / span)

        step[0] = 15
        tail = [carried(u, 7, 1) for u in range(16 - DEPTH, 16)]
        run([(inverse(early), 128 * len(early)),
             (chain(*[g for g, _ in tail]), sum(w for _, w in tail))])
        for i in range(4):
            untranspose(3, i, i)
        for i in range(4):
            if i == MID:
                side.finish()
                run([(inverse([it for it in _INVERSE[16] if it[0] == NT - 1]), 1024)])
            run([(out_proj(3, i, i, cp_ob3[i]), 800)])
    wait(cp_ob[2], *cp_ob3, cp_oa)


@jax.jit
def pallas_concat_heads__ssm_conv_h3__memory_aug_infini_attn__prompt_kernel(
    A_q: jax.Array,
    A_k: jax.Array,
    A_v: jax.Array,
    A_shift_k: jax.Array,
    A_ssm_k: jax.Array,
    A_ssm_D: jax.Array,
    B_x: jax.Array,
    B_wq: jax.Array,
    B_wk: jax.Array,
    B_wv: jax.Array,
    B_wo: jax.Array,
    B_beta: jax.Array,
):
    hbm = pl.BlockSpec(memory_space=pltpu.HBM)
    seg_tiles = pltpu.VMEM((NT, L, 128), BF16)
    seq_tiles = pltpu.VMEM((NT, S // 2, 128), U32)
    w_tiles = pltpu.VMEM((NT, D // 2, 128), U32)
    scratch = [
        pltpu.VMEM((KS, D), BF16),
        pltpu.VMEM((NT, 128), BF16),
        pltpu.VMEM((1, H), BF16),
        seq_tiles,
        w_tiles, w_tiles, w_tiles, w_tiles, w_tiles,
        pltpu.VMEM((S // 128 + 1, D // 2, 128), U32),
        pltpu.VMEM((4 * NT, 256, 128), U32),
        pltpu.VMEM((NT + 1, S // 2 + 8, 128), U32),
        seq_tiles, seq_tiles,
        pltpu.VMEM((N2, N1, 128), U32),
        pltpu.VMEM((2 * N2, N1 // 2, 128), U32),
        pltpu.VMEM((16, 4, 4, 2, 8, 128), F32),
        pltpu.VMEM((NT, S, 128), BF16),
        pltpu.VMEM((NT, KS + 1, 8, 128), F32),
        pltpu.VMEM((8, 8, 128), F32),
        pltpu.VMEM((3, 64, 128), F32),
        seg_tiles, seg_tiles, seg_tiles, seg_tiles,
        seg_tiles, seg_tiles, seg_tiles, seg_tiles,
        pltpu.VMEM((2, 4, D, 128), BF16),
        pltpu.VMEM((8, 96, 128), F32),
        pltpu.VMEM((2, 4, 8, 128), U32),
        pltpu.VMEM((2, 8, 128), jnp.int32),
        pltpu.VMEM((12, 8, 128), jnp.int32),
        pltpu.VMEM((2, L // 2, 128), U32),
        pltpu.VMEM((2, 4, 96, 128), BF16),
        pltpu.VMEM((2, 4, 8, 32, 128), BF16),
        pltpu.VMEM((2, 4, 80, 128), F32),
        pltpu.VMEM((4, NT, 64, 128), U32),
        pltpu.SMEM((1,), jnp.int32),
        pltpu.SemaphoreType.DMA((33,)),
    ]
    scratch += [pltpu.VMEM((N2, N1 // 2, 128), U32)] * (2 * NT)
    scratch += [pltpu.VMEM((N1 // 8 + 1, 4, 4, 2, 8, 128), F32)] * (2 * NT)
    scratch += [pltpu.VMEM((N2, N1, 128), U32)] * NT
    scratch += [pltpu.VMEM((N2, N1, 128), F32)] * NT
    scratch += [pltpu.VMEM((S // 2, 128), U32)] * NT
    scratch += [pltpu.VMEM((2, 512, 128), F32)] * NSLOT
    return pl.pallas_call(
        _kernel,
        out_shape=jax.ShapeDtypeStruct((1, S, 2 * D), BF16),
        in_specs=[hbm] * 14,
        out_specs=hbm,
        scratch_shapes=scratch,
        compiler_params=pltpu.CompilerParams(vmem_limit_bytes=110 * 1024 * 1024),
        name="h3_infini",
    )(A_q, A_k, A_v, A_shift_k.T, A_ssm_k, A_ssm_D.reshape(NT, 128), B_x, B_wq, B_wk, B_wv, B_wo,
      B_beta.reshape(1, H), _FWD, _INV)
```

```python
import math

import jax
import jax.numpy as jnp
import numpy as np
from jax import lax
from jax.experimental import pallas as pl
from jax.experimental.pallas import tpu as pltpu

S = 2048
D = 640
NT = D // 128
H = 32
DH = D // H
NSEG = 4
L = S // NSEG
KS = 4
N1, N2 = 128, 16

F32 = jnp.float32
BF16 = jnp.bfloat16
U32 = jnp.uint32
NN_DIMS = (((1,), (0,)), ((), ()))
NT_DIMS = (((1,), (1,)), ((), ()))
NEG = -1e30
LOG2E = 1.4426950408889634


def _pack_rows(a):
    u = a.astype(np.float32).astype(BF16).view(np.uint16).astype(np.uint32)
    return u[..., 0::2, :] | (u[..., 1::2, :] << 16)


def _dft_tables():
    k1 = np.arange(N1)
    fwd = np.zeros((N2, 2 * N1, N1), np.float64)
    inv = np.zeros((N2, N1, 2 * N1), np.float64)
    kappa = np.arange(N1)
    n1_in = 16 * (kappa // 16) + 8 * (kappa % 2) + (kappa % 16) // 2
    row_re = 16 * (k1 // 8) + k1 % 8
    for n2 in range(N2):
        ang = 2.0 * np.pi * np.outer(k1 + 0.25, N2 * n1_in + n2) / S
        fwd[n2, row_re] = np.cos(ang)
        fwd[n2, row_re + 8] = np.sin(ang)
        ang = 2.0 * np.pi * np.outer(N2 * np.arange(N1) + n2, k1 + 0.25) / S
        inv[n2][:, 2 * k1] = np.cos(ang) / S
        inv[n2][:, 2 * k1 + 1] = np.sin(ang) / S
    inv = inv.reshape(N2, N1, 2, N1).transpose(0, 2, 1, 3)
    return _pack_rows(fwd), _pack_rows(inv)


_FWD, _INV = _dft_tables()


def _dot(a, b, dims=NN_DIMS):
    return lax.dot_general(a, b, dims, preferred_element_type=F32)


def _u32(x):
    return pltpu.bitcast(x, U32)


def _bf(x):
    return pltpu.bitcast(x, BF16)


def _u32_word(x):
    return lax.bitcast_convert_type(x, U32)


def _pack2(a, b):
    return pltpu.pack_elementwise([a, b], packed_dtype=BF16).astype(U32)


def _lo(w):
    return pltpu.unpack_elementwise(w, index=0, packed_dtype=BF16, unpacked_dtype=F32)


def _hi(w):
    return pltpu.unpack_elementwise(w, index=1, packed_dtype=BF16, unpacked_dtype=F32)


def _radix4(x0, x1, x2, x3, sign):
    ar, ai = x0[0] + x2[0], x0[1] + x2[1]
    br, bi = x0[0] - x2[0], x0[1] - x2[1]
    cr, ci = x1[0] + x3[0], x1[1] + x3[1]
    dr, di = x1[0] - x3[0], x1[1] - x3[1]
    y0 = (ar + cr, ai + ci)
    y2 = (ar - cr, ai - ci)
    yp = (br - di, bi + dr)
    ym = (br + di, bi - dr)
    return (y0, yp, y2, ym) if sign > 0 else (y0, ym, y2, yp)


def _twiddle(x, e, sign):
    xr, xi = x
    if e == 0:
        return x
    if e == 4:
        return (-xi, xr) if sign > 0 else (xi, -xr)
    r = math.sqrt(0.5)
    if e == 2:
        return ((xr - xi) * r, (xr + xi) * r) if sign > 0 else ((xr + xi) * r, (xi - xr) * r)
    if e == 6:
        return ((xr + xi) * -r, (xr - xi) * r) if sign > 0 else ((xi - xr) * r, (xr + xi) * -r)
    c, s = math.cos(math.pi * e / 8), sign * math.sin(math.pi * e / 8)
    return (xr * c - xi * s, xr * s + xi * c)


def _radix4_tw(x0, x1, x2, x3, sign, b):
    if b != 2:
        return _radix4(x0, _twiddle(x1, b, sign), _twiddle(x2, 2 * b, sign),
                       _twiddle(x3, 3 * b, sign), sign)
    x1, x3 = _twiddle(x1, 2, sign), _twiddle(x3, 6, sign)
    if sign > 0:
        ar, ai = x0[0] - x2[1], x0[1] + x2[0]
        br, bi = x0[0] + x2[1], x0[1] - x2[0]
    else:
        ar, ai = x0[0] + x2[1], x0[1] - x2[0]
        br, bi = x0[0] - x2[1], x0[1] + x2[0]
    cr, ci = x1[0] + x3[0], x1[1] + x3[1]
    dr, di = x1[0] - x3[0], x1[1] - x3[1]
    y0 = (ar + cr, ai + ci)
    y2 = (ar - cr, ai - ci)
    yp = (br - di, bi + dr)
    ym = (br + di, bi - dr)
    return (y0, yp, y2, ym) if sign > 0 else (y0, ym, y2, yp)


class _Paced:
    def __init__(self, streams, sequential=False):
        self.live = [[g, total, 0] for g, total in streams if total]
        self.total = sum(total for _, total in streams)
        self.done = 0
        self.sequential = sequential

    def step(self):
        cur = self.live[0] if self.sequential else min(self.live, key=lambda e: e[2] / e[1])
        cost = next(cur[0], None)
        if cost is None:
            self.live.remove(cur)
        else:
            cur[2] += cost
            self.done += cost

    def advance(self, fraction):
        while self.live and self.done < fraction * self.total:
            self.step()

    def finish(self):
        self.advance(math.inf)


SPLIT = ((0, 1, 2), (3, 4), (), ())
FORWARD = ((), (0, 1), (2, 3, 4), ())
SPECTRUM = ((), (), (0, 1), (2, 3))
INVERSE = ((), (), (), (0, 1))
DEPTH = 3
NSLOT = 4
ORDER = ((0, 1, 2, 3), (0, 1, 2, 3), (0, 1, 2, 3), (0, 1, 2, 3))
TAIL = (0.0, 0.0, 0.0, 0.0)
LW = (1.0, 1.0, 1.0, 1.0)
AW = (3.0, 3.0, 3.0, 3.0, 3.0)
QCH = (128, 128, 128, 128)
HEAD = (4, 4, 4, 2)
FILL_ORDER = (0, 0, 0, 0)
PACE_ON = (3, 3, 3, 3, 7)
SIDE_SPEED = (1.0, 1.0, 1.0, 1.0)
MID = 3


def _kernel(aq_hbm, ak_hbm, av_hbm, shift_hbm, h_hbm, ssmd_hbm, x_hbm, wq_hbm, wk_hbm,
            wv_hbm, wo_hbm, beta_hbm, fwd_hbm, inv_hbm, out_hbm, shift_ref, ssmd_ref, beta_ref,
            xb, wqb, wkb, wvb, wob, wvt, hb, ht, kb, vb, qb, fwd, inv,
            ub, outb, wtab, gtab, cmask,
            q0, q1, k0, k1, pq0, pq1, pk0, pk1, ots, mst,
            hmask, hsel, bmask, kwin, vall, vhead, opart, onat, sem_zero, sems, *rest):
    xp, hp, tx, th, yb, kvf, outa = (rest[NT * k:NT * k + NT] for k in range(7))
    slots = rest[7 * NT:]
    qs, ks, pqs, pks = (q0, q1), (k0, k1), (pq0, pq1), (pk0, pk1)

    def tile_copy(src, dst, t, sem, r0, n, lead=(0,), dst_off=0):
        return lambda: pltpu.make_async_copy(
            src.bitcast(U32).at[(*lead, pl.ds(r0 // 2, n // 2), pl.ds(128 * t, 128))],
            dst.at[t, pl.ds(dst_off + r0 // 2, n // 2), :], sems.at[sem])

    def h_copy(t, c0, n, sem):
        return lambda: pltpu.make_async_copy(
            h_hbm.bitcast(U32).at[pl.ds(64 * c0, 64 * n), pl.ds(128 * t, 128)],
            hb.at[t, pl.ds(64 * c0, 64 * n), :], sems.at[sem])

    def conv_copies(cs, i, sem):
        out = [h_copy(4 * i + t, cs[0], len(cs), sem) for t in range(4)]
        out += [tile_copy(ak_hbm, kb, c, sem, L * i, L, dst_off=8) for c in cs]
        return out + [tile_copy(av_hbm, vb, c, sem, L * i, L) for c in cs]

    cp_x = [[tile_copy(x_hbm, xb, t, s, L * s, L) for t in range(NT)] for s in range(NSEG)]
    cp_x1 = [[tile_copy(x_hbm, xb, t, 10 + i, L + 128 * i, 128) for t in range(NT)]
             for i in range(4)]
    cp_w = [[tile_copy(src, dst, n, 4 + n, 0, D, lead=())
             for src, dst in ((wq_hbm, wqb), (wk_hbm, wkb))] for n in range(NT)]
    cp_wv = [tile_copy(wv_hbm, wvb, n, 1, 0, D, lead=()) for n in range(NT)]
    cp_wo = [tile_copy(wo_hbm, wob, n, 9, 0, D, lead=()) for n in range(NT)]
    cp_early = [conv_copies(SPLIT[0], i, 10 + i) + cp_x1[i] for i in range(4)]
    cp_late = [cp for i in range(4) for cp in conv_copies(SPLIT[1], i, 14)]
    cp_q = [tile_copy(aq_hbm, qb, c, 15, 0, S) for c in range(NT)]
    cp_fwd = [lambda: pltpu.make_async_copy(fwd_hbm, fwd, sems.at[16])]
    cp_inv = [lambda: pltpu.make_async_copy(inv_hbm, inv, sems.at[17])]
    cp_small = [lambda: pltpu.make_async_copy(shift_hbm, shift_ref, sems.at[18]),
                lambda: pltpu.make_async_copy(ssmd_hbm, ssmd_ref, sems.at[18]),
                lambda: pltpu.make_async_copy(beta_hbm, beta_ref, sems.at[18])]

    def out_a(c):
        return lambda: pltpu.make_async_copy(
            outa[c], out_hbm.bitcast(U32).at[0, :, pl.ds(128 * c, 128)], sems.at[19])

    def out_b(r0, n, rows_):
        return lambda: pltpu.make_async_copy(
            outb.at[n, pl.ds(r0, rows_), :],
            out_hbm.at[0, pl.ds(r0, rows_), pl.ds(D + 128 * n, 128)], sems.at[20])

    cp_oa = [out_a(c) for c in range(NT)]
    cp_ob = [[out_b(L * s, n, L) for n in range(NT)] for s in range(NSEG - 1)]
    cp_ob3 = [[out_b(L * 3 + 128 * i, n, 128) for n in range(NT)] for i in range(4)]

    def start(*groups):
        for g in groups:
            for cp in g:
                cp().start()

    def wait(*groups):
        for g in groups:
            for cp in g:
                cp().wait()

    def rows(i, n):
        return pl.ds(pl.multiple_of(i * n, n), n) if not isinstance(i, int) else pl.ds(i * n, n)

    lane = lax.broadcasted_iota(jnp.int32, (8, 128), 1)
    sub = lax.broadcasted_iota(jnp.int32, (8, 128), 0)

    def lanes(n):
        return lax.broadcasted_iota(jnp.int32, (n, 128), 1)

    recent = [None]
    seg = [0]

    def dot(a, b, dims=NN_DIMS, kind=4):
        out = _dot(a, b, dims)
        if kind & PACE_ON[seg[0]]:
            recent[0] = out
        return out

    current = {}

    def pace(zero):
        v = recent[0][-8:]
        recent[0] = None
        if "h" in current:
            hb[S // 128, rows(zero, 8), :] = _u32_word(v)
        if "k" in current:
            kb[NT, rows(zero, 8), :] = _u32_word(v)
        if "t" in current:
            th[current["t"]][N1 // 8, zero, 0, 0] = v

    def qk_proj(s, i, want_pq, want_pk):
        p = s % 2
        tok = rows(4 * s + i, 64)
        for w_ref, dst, fdst, want, scale in (
                (wqb, qs[p], pqs[p], want_pq, DH ** -0.5 * LOG2E),
                (wkb, ks[p], pks[p], want_pk, None)):
            for n in range(NT):
                t = None
                for c in range(NT):
                    part = dot(_bf(xb[c, tok, :]), _bf(w_ref[n, 64 * c:64 * c + 64, :]))
                    t = part if t is None else t + part
                    if c < NT - 1:
                        yield 32
                dst[n, rows(i, 128), :] = (t if scale is None else t * scale).astype(BF16)
                if want:
                    fdst[n, rows(i, 128), :] = jnp.where(t > 0, t + 1.0, jnp.exp(t)).astype(BF16)
                yield 32

    def first_proj(n):
        for w_ref, dst, scale in ((wqb, qs[0], DH ** -0.5 * LOG2E), (wkb, ks[0], None)):
            for j in range(4):
                t = None
                for c in range(NT):
                    part = dot(_bf(xb[c, rows(j, 64), :]), _bf(w_ref[n, 64 * c:64 * c + 64, :]))
                    t = part if t is None else t + part
                dst[n, rows(j, 128), :] = (t if scale is None else t * scale).astype(BF16)
                if scale is None:
                    pks[0][n, rows(j, 128), :] = jnp.where(t > 0, t + 1.0, jnp.exp(t)).astype(BF16)

    def untranspose(s, i, slot=0):
        ot = ots.bitcast(U32)
        for c in range(NT):
            onat[slot, c] = _u32(_bf(ot[s % 2, i, 64 * c:64 * c + 64, :]).T)

    def out_proj(s, i, slot=0, copies=None):
        for n in range(NT):
            t = None
            for c in range(NT):
                part = dot(_bf(onat[slot, c]), _bf(wob[n, 64 * c:64 * c + 64, :]))
                t = part if t is None else t + part
                if c < NT - 1:
                    yield 32
            outb[n, rows(4 * s + i, 128), :] = t.astype(BF16)
            if copies is not None:
                start([copies[n]])
            yield 32

    def tile_rows(r, n):
        return jnp.broadcast_to(r[None], (n // 8, 8, 128)).reshape(n, 128)

    class Group:
        def __init__(self, s, g, gi):
            self.s, self.g, self.gi = s, g, gi
            self.t0 = (80 * g) // 128
            self.off = 80 * g - 128 * self.t0
            self.t1 = jnp.minimum(self.t0 + 1, NT - 1)
            rel = (lane - self.off) & 127
            head = sum((rel >= a * DH).astype(jnp.int32) for a in range(1, 5))
            for a in range(4):
                hmask[gi, a] = jnp.where(head == a, np.uint32(0xFFFFFFFF), np.uint32(0))
            hsel[gi] = jnp.left_shift(1, head)
            self.have_keys, self.have_mem = set(), set()

        def window(self, ref, j, r0=0, n=64):
            ref = ref.bitcast(U32)
            at = pl.ds(64 * j + r0, n)
            return jnp.where(lanes(n) >= self.off, ref[self.t0, at, :], ref[self.t1, at, :])

        def keys(self, r0, r1):
            out = []
            for r in range(r0, r1, 64):
                at = pl.ds(r // 2, 32)
                if r in self.have_keys:
                    out.append(kwin[self.gi, at, :])
                else:
                    self.have_keys.add(r)
                    out.append(self.window(ks[self.s % 2], 0, r // 2, 32))
                    kwin[self.gi, at, :] = out[-1]
            return _bf(jnp.concatenate(out, axis=0))

        def park_values(self, j, v80):
            vall[self.gi, j, 0:80, :] = v80.astype(BF16)
            ones8 = jnp.ones((8, 128), F32)
            for pr in range(2):
                for e in range(2):
                    r0 = 40 * pr + 16 * e
                    vhead[self.gi, j, r0 // 8] = jnp.concatenate(
                        [v80[r0:r0 + 24], ones8], axis=0).astype(BF16)

        def mem_read(self):
            for j in range(4):
                r = dot(mst[self.g].astype(BF16), _bf(self.window(pqs[self.s % 2], j)), NT_DIMS)
                coef = gtab[self.g] / (r[80:88] + 1e-6)
                cb = [jnp.broadcast_to(coef[a:a + 1], (8, 128)) for a in range(4)]
                for pr in range(2):
                    ca, cc = cb[2 * pr], cb[2 * pr + 1]
                    for e, scale in enumerate((ca, ca, jnp.where(sub < 4, ca, cc), cc, cc)):
                        r0 = 40 * pr + 8 * e
                        opart[self.gi, j, r0:r0 + 8, :] = r[r0:r0 + 8] * scale
                self.have_mem.add(j)
                yield 24

        def mem_update(self):
            acc = None
            for j in range(4):
                t = dot(_bf(vall.bitcast(U32)[self.gi, j]), _bf(self.window(pks[self.s % 2], j)))
                acc = t if acc is None else acc + t
                if j < 3:
                    yield 24
            for r in range(12):
                new = jnp.where(bmask[r] & hsel[self.gi] != 0, acc[8 * r:8 * r + 8], 0.0)
                at = pl.ds(8 * r, 8)
                mst[self.g, at, :] = new if self.s == 0 else mst[self.g, at, :] + new
            yield 24

        def logits(self, pr, j, slot):
            qw = self.window(qs[self.s % 2], j)
            qa = qw & tile_rows(hmask[self.gi, 2 * pr], 64)
            qh = qw & tile_rows(hmask[self.gi, 2 * pr + 1], 64)
            w_a = _bf(qa)
            w_b = _bf(jnp.concatenate([qh[32:64], qh[0:32]], axis=0))
            w_t = _bf(jnp.concatenate([qh[32:64], qa[32:64]], axis=0))
            n = 128 * j

            def park(t, e, r0, m):
                for r in range(0, t.shape[0], 8):
                    v = t[r:r + 8]
                    if e == 2:
                        v = v + cmask[2, r:r + 8, :]
                    elif r0 + r >= n:
                        v = v + cmask[e, r0 + r - n:r0 + r - n + 8, :]
                    slot[e % 2, 448 * (e // 2) + r0 + r:448 * (e // 2) + r0 + r + 8, :] = v
                    m = v if m is None else jnp.maximum(m, v)
                return m

            m_t = park(dot(self.keys(n + 64, n + 128), w_t, NT_DIMS, 1), 2, 0, None)
            yield 16 * LW[seg[0] % 4]
            cuts = list(range(0, n, QCH[seg[0]])) or [0]
            m = [None, None]
            for r0, r1 in zip(cuts, cuts[1:] + [n + 64]):
                for e, w in enumerate((w_a, w_b)):
                    m[e] = park(dot(self.keys(r0, r1), w, NT_DIMS, 1), e, r0, m[e])
                    if r1 == n + 64 and e == 1:
                        m_a = jnp.maximum(m[0], jnp.where(lane >= 64, m_t, NEG))
                        m_b = jnp.maximum(m[1], jnp.where(lane < 64, m_t, NEG))
                        m_a = jnp.broadcast_to(jnp.max(m_a, axis=0, keepdims=True), (8, 128))
                        m_b = jnp.broadcast_to(jnp.max(m_b, axis=0, keepdims=True), (8, 128))
                        slot[1, 448:456, :] = m_a
                        slot[1, 456:464, :] = m_b
                        slot[1, 464:472, :] = jnp.where(lane < 64, m_b, m_a)
                    yield (r1 - r0) // 4 * LW[seg[0] % 4]

    def attend(gi, g, parity, add_mem, pr, j, slot, need_values):
        def prob(e, r0, n, which):
            m2 = tile_rows(slot[1, 448 + 8 * which:456 + 8 * which, :], 16)
            return [jnp.exp2(slot[e, r:r + 16, :] - m2) for r in range(r0, r0 + n, 16)]

        res = [None, None]
        order = [(0, j), (1, j)] + [(e, kt) for e in range(2) for kt in range(j)]
        for n, (e, kt) in enumerate(order):
            need_values(kt)
            if n == 0:
                p_t = prob(0, 448, 64, 2)
            if kt < j:
                p = prob(e, 128 * kt, 128, e)
            else:
                mine = lanes(16) >= 64 if e == 0 else lanes(16) < 64
                p = prob(e, 128 * kt, 64, e) + [jnp.where(mine, t, 0.0) for t in p_t]
            t = dot(_bf(vhead.bitcast(U32)[gi, kt, 5 * pr + 2 * e]),
                    jnp.concatenate(p, axis=0).astype(BF16), kind=2)
            res[e] = t if res[e] is None else res[e] + t
            if n < len(order) - 1:
                yield 8 * AW[seg[0]]
        r_a = res[0]
        r_b = pltpu.roll(res[1], 64, 1)
        keep = 1.0 - gtab[g]
        keep_a = jnp.broadcast_to(keep[2 * pr:2 * pr + 1], (8, 128))
        keep_b = jnp.broadcast_to(keep[2 * pr + 1:2 * pr + 2], (8, 128))
        o_a = r_a[0:24] * tile_rows(keep_a / r_a[24:32], 24)
        o_b = r_b[0:24] * tile_rows(keep_b / r_b[24:32], 24)
        o = jnp.concatenate(
            [o_a[0:16], jnp.where(sub < 4, o_a[16:24], o_b[0:8]), o_b[8:24]], axis=0)
        if add_mem:
            o = o + opart[gi, j, 40 * pr:40 * pr + 40, :]
        if pr == 0:
            opart[gi, j, 0:40, :] = o
        else:
            o = jnp.concatenate([opart[gi, j, 0:40, :], o], axis=0)
            ots[parity, j, rows(g, 80), :] = o.astype(BF16)
        yield 8 * AW[seg[0]]

    def v_proj(s, i, groups, have):
        for j in range(4):
            acc = None
            for c in range(NT):
                t = dot(_bf(wvt[c, rows(i, 80), :]), _bf(xb[c, rows(4 * s + j, 64), :]), NT_DIMS)
                acc = t if acc is None else acc + t
                if c == NT - 1:
                    for gi in range(2):
                        groups[gi].park_values(j, acc[80 * gi:80 * gi + 80])
                    have.append(j)
                yield 40

    def chain(*gens):
        for g in gens:
            yield from g

    def units(s):
        return [(gi, pr, j) for gi in range(2) for pr in range(2)
                for j in (range(4) if (gi, pr) == (1, 1) else ORDER[s] if gi + pr else range(4))]

    def cost(j):
        return (48 + 64 * j) * LW[seg[0] % 4], (16 + 16 * j) * AW[seg[0]]

    def carried(u, g, parity):
        gi, pr, j = units(0)[u]
        return attend(gi, g, parity, True, pr, j, slots[u % NSLOT], lambda kt: None), cost(j)[1]

    def segment_step(s, i):
        seg[0] = s
        parts = {}
        if s < NSEG - 1:
            parts["qk"] = (qk_proj(s + 1, i, True, s + 1 < NSEG - 1), 1600)
        if s > 0:
            parts["out"] = (out_proj(s - 1, i), 800)
        if FORWARD[s]:
            parts["fwd"] = (fwd_fft(i, FORWARD[s]), 512 * len(FORWARD[s]))
        if INVERSE[s]:
            parts["inv"] = (inverse(INVERSE[s], (2 * i, 2 * i + 1)), 256 * len(INVERSE[s]))
        names = (("qk", "inv", "out", "fwd"), ("qk", "inv", "fwd", "out"),
                 ("inv", "fwd", "qk", "out"), ("qk", "inv", "out", "fwd"))[FILL_ORDER[s]]
        fill = _Paced([parts[n] for n in names if n in parts], sequential=FILL_ORDER[s] < 3)
        side = []
        if SPECTRUM[s]:
            side.append((spectra(SPECTRUM[s], [4 * i + a for a in range(4)]),
                         4 * SPEC_COST * len(SPECTRUM[s])))
        for c in SPLIT[s]:
            side += [(split_h(i, c), 144), (split_kv(i, c), 704)]
        side = _Paced(side, sequential=True)
        current.clear()
        recent[0] = None
        for _ in range(HEAD[s]):
            fill.step()
        if s > 0:
            untranspose(s - 1, i)
        vt = []
        groups = [Group(s, 2 * i + gi, gi) for gi in range(2)]
        reads = [grp.mem_read() for grp in groups if s > 0]
        updates = [grp.mem_update() for grp in groups if s < NSEG - 1]
        first = _Paced([(chain(*reads[:1], v_proj(s, i, groups, vt), *reads[1:], *updates),
                         800 + 96 * (len(reads) + len(updates)))])
        total = first.total + fill.total
        held = 96 * (s > 0) + 160

        def need_values(kt):
            while len(vt) <= kt:
                first.step()

        def pad(fraction, u):
            target = total * fraction / (1 + TAIL[s])
            early = min(target, held if u < DEPTH else first.total)
            first.advance(early / first.total)
            fill.advance((target - early) / fill.total)
            goal = fraction * SIDE_SPEED[s]
            if side.live and side.done < goal * side.total and recent[0] is not None:
                pace(jnp.minimum(i, 3))
                side.advance(goal)

        todo = units(s)
        whole = sum(sum(cost(j)) for _, _, j in todo)
        done = 0
        for u, (gi, pr, j) in enumerate(todo):
            streams = [(groups[gi].logits(pr, j, slots[u % NSLOT]), cost(j)[0])]
            v = u - DEPTH
            if v < 0:
                streams.append(carried(v + len(todo), (2 * i + 7) & 7,
                                       jnp.where(i > 0, s % 2, 1 - s % 2)))
            else:
                gi, pr, j = todo[v]
                while s > 0 and j not in groups[gi].have_mem:
                    first.step()
                streams.append((attend(gi, 2 * i + gi, s % 2, s > 0, pr, j, slots[v % NSLOT],
                                       need_values), cost(j)[1]))
            att = _Paced(streams[::-1], sequential=u == len(todo) - 1)
            while att.live:
                att.step()
                pad((done + att.done) / whole, u)
            done += att.total
        first.finish()
        fill.finish()
        side.finish()

    def split_h(i, c):
        current.clear()
        current["h"] = True
        for t in range(4):
            ht[c, 64 * t:64 * t + 64, :] = _u32(
                _bf(hb[4 * i + t, 64 * c:64 * c + 64, :]).T)
            yield 4
        for q in range(2):
            for j in range(8):
                wa = ht[c, pl.ds(128 * q + j, 8, stride=8), :]
                wb = ht[c, pl.ds(128 * q + 64 + j, 8, stride=8), :]
                hp[c][2 * j, rows(2 * i + q, 8), :] = _pack2(_lo(wa), _lo(wb))
                hp[c][2 * j + 1, rows(2 * i + q, 8), :] = _pack2(_hi(wa), _hi(wb))
                if j % 2:
                    yield 16

    def split_kv(i, c):
        current.clear()
        current["k"] = True
        taps = [wtab[c, j] for j in range(KS)]
        for q in range(2):
            blk = 2 * i + q
            base = [blk * 128 + 64 * e for e in range(2)]
            hist = []
            for e in range(2):
                w2 = kb[c, pl.ds(base[e] + 6, 8, stride=8), :]
                w1 = kb[c, pl.ds(base[e] + 7, 8, stride=8), :]
                hist.append([_hi(w2), _lo(w1), _hi(w1)])
            for j in range(8):
                kv = [[None, None], [None, None]]
                for e in range(2):
                    kw = kb[c, pl.ds(base[e] + 8 + j, 8, stride=8), :]
                    vw = vb[c, pl.ds(base[e] + j, 8, stride=8), :]
                    kp = hist[e] + [_lo(kw), _hi(kw)]
                    for half, part in enumerate((_lo, _hi)):
                        acc = kp[3 + half] * taps[0]
                        for d in range(1, KS):
                            acc = acc + kp[3 + half - d] * taps[d]
                        kv[half][e] = acc * part(vw)
                        kvf[c][2 * j + half, rows(2 * blk + e, 8), :] = kv[half][e]
                    hist[e] = kp[2:]
                    if e == 0:
                        yield 22
                for half in range(2):
                    xp[c][2 * j + half, rows(blk, 8), :] = _pack2(*kv[half])
                yield 22

    def fwd_fft(i, cs):
        for c in cs:
            for src, dst in ((hp[c], th[c]), (xp[c], tx[c])):
                g = [dot(_bf(fwd[4 * a + i]), _bf(src[4 * a + i])) for a in range(4)]
                for r in range(0, 2 * N1, 16):
                    z = _radix4(*[(g[a][r:r + 8], g[a][r + 8:r + 16]) for a in range(4)], 1)
                    for cc in range(4):
                        dst[r // 16, cc, i, 0] = z[cc][0]
                        dst[r // 16, cc, i, 1] = z[cc][1]
                yield 256

    def spectrum(c, m, slot):
        current.clear()
        current["t"] = c
        for cc in range(4):
            zh = _radix4_tw(*[(th[c][m, cc, b, 0], th[c][m, cc, b, 1]) for b in range(4)], 1, cc)
            yield 17
            zx = _radix4_tw(*[(tx[c][m, cc, b, 0], tx[c][m, cc, b, 1]) for b in range(4)], 1, cc)
            yield 17
            y = [(x[0] * h[0] - x[1] * h[1], x[0] * h[1] + x[1] * h[0]) for x, h in zip(zx, zh)]
            yield 17
            u = _radix4(*y, -1)
            for b in range(4):
                ub[slot, b, cc, 0] = u[b][0]
                ub[slot, b, cc, 1] = u[b][1]
            yield 17
        for b in range(4):
            z = _radix4_tw(*[(ub[slot, b, cc, 0], ub[slot, b, cc, 1]) for cc in range(4)], -1, b)
            for a in range(4):
                yb[c][4 * a + b, rows(m, 8), :] = _pack2(*z[a])
            yield 17

    SPEC_COST = 17 * 20

    def spectra(cs, ms, slot0=0):
        for slot, (c, m) in enumerate(((c, m) for c in cs for m in ms), slot0):
            yield from spectrum(c, m, slot)

    def inverse(cs, jps):
        for c in cs:
            for jp in jps:
                w = qb[c, pl.ds(jp, N1, stride=8), :]
                res = []
                for e, part in enumerate((_lo, _hi)):
                    n2 = 2 * jp + e
                    y = dot(_bf(inv[n2, 0]), _bf(yb[c][n2, 0:64, :]))
                    yield 32
                    y = y + dot(_bf(inv[n2, 1]), _bf(yb[c][n2, 64:128, :]))
                    res.append(part(w) * (y + kvf[c][n2] * tile_rows(wtab[c, KS], N1)))
                    if e == 0:
                        yield 32
                outa[c][pl.ds(jp, N1, stride=8), :] = _pack2(*res)
                yield 32

    start(cp_small, cp_x[0], cp_w[0])
    sem_zero[0] = 0
    kk = lax.broadcasted_iota(jnp.int32, (64, 128), 0)
    ll = lax.broadcasted_iota(jnp.int32, (64, 128), 1)
    cmask[0] = jnp.where(kk <= ll, 0.0, NEG)
    cmask[1] = jnp.where((ll < 64) | (kk <= ll - 64), 0.0, NEG)
    cmask[2] = jnp.where(kk <= (ll & 63), 0.0, NEG)
    for r in range(12):
        row = sub + 8 * r
        hr = sum((row >= a * DH).astype(jnp.int32) for a in range(1, 4)) if r < 10 else row - 80
        bmask[r] = jnp.left_shift(1, hr)
    for gi in range(2):
        for j in range(4):
            vall[gi, j, 80:96, :] = jnp.ones((16, 128), BF16)
    for c in range(NT):
        kb[c, 0:8, :] = jnp.zeros((8, 128), U32)
    for u in range(16 - DEPTH, 16):
        slots[u % NSLOT][...] = jnp.zeros((2, 512, 128), F32)
    vhead[1] = jnp.ones(vhead.shape[1:], BF16)
    opart[1] = jnp.zeros(opart.shape[1:], F32)
    start(cp_w[1])
    wait(cp_small)
    taps_t = shift_ref[...].astype(F32)
    skip = ssmd_ref[...].astype(F32)
    for c in range(NT):
        for j in range(KS):
            wtab[c, j] = jnp.broadcast_to(taps_t[j:j + 1, 128 * c:128 * c + 128], (8, 128))
        wtab[c, KS] = jnp.broadcast_to(skip[c:c + 1], (8, 128))
    gates = jax.nn.sigmoid(beta_ref[...].astype(F32))
    gcol = jnp.broadcast_to(gates, (8, H)).T
    gcol = jnp.broadcast_to(gcol[:, 0:1], (H, 128))
    for g in range(8):
        gtab[g] = jnp.concatenate([gcol[4 * g:4 * g + 4]] * 2, axis=0)
    start(cp_w[2])
    with jax.named_scope("prologue"):
        wait(cp_x[0], cp_w[0])
        start(cp_w[3], cp_w[4], cp_wv)
        first_proj(0)
        wait(cp_w[1], cp_w[2])
        start(cp_early[0])
        first_proj(1)
        first_proj(2)
        wait(cp_w[3], cp_w[4], cp_wv)
        start(cp_early[1])
        for n in range(NT):
            for c in range(NT):
                wvt[c, rows(n, 64), :] = _u32(_bf(wvb[n, 64 * c:64 * c + 64, :]).T)
        first_proj(3)
        first_proj(4)
    start(cp_wo, cp_x[2])

    def segment(s):
        def body(i, carry):
            if s == 0:
                for j in range(4):
                    @pl.when(i == j)
                    def _():
                        wait(cp_early[j])
                        start(*((cp_early[2],), (cp_early[3],), (cp_fwd, cp_late), (cp_x[3],))[j])
            segment_step(s, i)
            return carry

        with jax.named_scope(f"seg{s}"):
            lax.fori_loop(0, 4, body, 0)

    segment(0)
    wait(cp_fwd, cp_x[2], cp_wo, cp_late)
    start(cp_inv, cp_q)
    segment(1)
    start(cp_ob[0])
    wait(cp_x[3])
    segment(2)
    wait(cp_ob[0], cp_inv, cp_q)
    start(cp_ob[1])
    segment(3)
    wait(cp_ob[1])
    start(cp_ob[2], [cp_oa[c] for c in INVERSE[3]])
    with jax.named_scope("epilogue"):
        seg[0] = 4
        current.clear()
        recent[0] = None
        last = NT - 1
        rest_tiles = [c for c in range(last) if c not in INVERSE[3]]
        side = _Paced([(spectra((last,), range(16)), 16 * SPEC_COST)])
        span = 1024 * len(rest_tiles) + 800 * MID
        done = 0

        def run(streams):
            nonlocal done
            work = _Paced(streams)
            while work.live:
                before = work.done
                work.step()
                done += work.done - before
                if side.live and side.done < done / span * side.total and recent[0] is not None:
                    pace(sem_zero[0])
                    side.advance(done / span)

        for c in rest_tiles:
            streams = [(inverse((c,), range(8)), 1024)]
            if c == rest_tiles[0]:
                tail = [carried(u, 7, 1) for u in range(16 - DEPTH, 16)]
                streams.append((chain(*[g for g, _ in tail]), sum(w for _, w in tail)))
            run(streams)
            if c == rest_tiles[0]:
                for i in range(4):
                    untranspose(3, i, i)
            start([cp_oa[c]])
        for i in range(4):
            if i == MID:
                side.finish()
                run([(inverse((last,), range(8)), 1024)])
                start([cp_oa[last]])
            run([(out_proj(3, i, i, cp_ob3[i]), 800)])
    wait(cp_ob[2], *cp_ob3, cp_oa)


@jax.jit
def pallas_concat_heads__ssm_conv_h3__memory_aug_infini_attn__prompt_kernel(
    A_q: jax.Array,
    A_k: jax.Array,
    A_v: jax.Array,
    A_shift_k: jax.Array,
    A_ssm_k: jax.Array,
    A_ssm_D: jax.Array,
    B_x: jax.Array,
    B_wq: jax.Array,
    B_wk: jax.Array,
    B_wv: jax.Array,
    B_wo: jax.Array,
    B_beta: jax.Array,
):
    hbm = pl.BlockSpec(memory_space=pltpu.HBM)
    seg_tiles = pltpu.VMEM((NT, L, 128), BF16)
    seq_tiles = pltpu.VMEM((NT, S // 2, 128), U32)
    w_tiles = pltpu.VMEM((NT, D // 2, 128), U32)
    scratch = [
        pltpu.VMEM((KS, D), BF16),
        pltpu.VMEM((NT, 128), BF16),
        pltpu.VMEM((1, H), BF16),
        seq_tiles,
        w_tiles, w_tiles, w_tiles, w_tiles, w_tiles,
        pltpu.VMEM((S // 128 + 1, D // 2, 128), U32),
        pltpu.VMEM((NT, 256, 128), U32),
        pltpu.VMEM((NT + 1, S // 2 + 8, 128), U32),
        seq_tiles, seq_tiles,
        pltpu.VMEM((N2, N1, 128), U32),
        pltpu.VMEM((N2, 2, N1 // 2, 128), U32),
        pltpu.VMEM((16, 4, 4, 2, 8, 128), F32),
        pltpu.VMEM((NT, S, 128), BF16),
        pltpu.VMEM((NT, KS + 1, 8, 128), F32),
        pltpu.VMEM((8, 8, 128), F32),
        pltpu.VMEM((3, 64, 128), F32),
        seg_tiles, seg_tiles, seg_tiles, seg_tiles,
        seg_tiles, seg_tiles, seg_tiles, seg_tiles,
        pltpu.VMEM((2, 4, D, 128), BF16),
        pltpu.VMEM((8, 96, 128), F32),
        pltpu.VMEM((2, 4, 8, 128), U32),
        pltpu.VMEM((2, 8, 128), jnp.int32),
        pltpu.VMEM((12, 8, 128), jnp.int32),
        pltpu.VMEM((2, L // 2, 128), U32),
        pltpu.VMEM((2, 4, 96, 128), BF16),
        pltpu.VMEM((2, 4, 8, 32, 128), BF16),
        pltpu.VMEM((2, 4, 80, 128), F32),
        pltpu.VMEM((4, NT, 64, 128), U32),
        pltpu.SMEM((1,), jnp.int32),
        pltpu.SemaphoreType.DMA((21,)),
    ]
    scratch += [pltpu.VMEM((N2, N1 // 2, 128), U32)] * (2 * NT)
    scratch += [pltpu.VMEM((N1 // 8 + 1, 4, 4, 2, 8, 128), F32)] * (2 * NT)
    scratch += [pltpu.VMEM((N2, N1, 128), U32)] * NT
    scratch += [pltpu.VMEM((N2, N1, 128), F32)] * NT
    scratch += [pltpu.VMEM((S // 2, 128), U32)] * NT
    scratch += [pltpu.VMEM((2, 512, 128), F32)] * NSLOT
    return pl.pallas_call(
        _kernel,
        out_shape=jax.ShapeDtypeStruct((1, S, 2 * D), BF16),
        in_specs=[hbm] * 14,
        out_specs=hbm,
        scratch_shapes=scratch,
        compiler_params=pltpu.CompilerParams(vmem_limit_bytes=110 * 1024 * 1024),
        name="h3_infini",
    )(A_q, A_k, A_v, A_shift_k.T, A_ssm_k, A_ssm_D.reshape(NT, 128), B_x, B_wq, B_wk, B_wv, B_wo,
      B_beta.reshape(1, H), _FWD, _INV)
```

```python
import math

import jax
import jax.numpy as jnp
import numpy as np
from jax import lax
from jax.experimental import pallas as pl
from jax.experimental.pallas import tpu as pltpu

S = 2048
D = 640
NT = D // 128
H = 32
DH = D // H
NSEG = 4
L = S // NSEG
KS = 4
N1, N2 = 128, 16

F32 = jnp.float32
BF16 = jnp.bfloat16
U32 = jnp.uint32
NN_DIMS = (((1,), (0,)), ((), ()))
NT_DIMS = (((1,), (1,)), ((), ()))
NEG = -1e30
LOG2E = 1.4426950408889634


def _pack_rows(a):
    u = a.astype(np.float32).astype(BF16).view(np.uint16).astype(np.uint32)
    return u[..., 0::2, :] | (u[..., 1::2, :] << 16)


def _dft_tables():
    k1 = np.arange(N1)
    fwd = np.zeros((N2, 2 * N1, N1), np.float64)
    inv = np.zeros((N2, N1, 2 * N1), np.float64)
    kappa = np.arange(N1)
    n1_in = 16 * (kappa // 16) + 8 * (kappa % 2) + (kappa % 16) // 2
    row_re = 16 * (k1 // 8) + k1 % 8
    for n2 in range(N2):
        ang = 2.0 * np.pi * np.outer(k1 + 0.25, N2 * n1_in + n2) / S
        fwd[n2, row_re] = np.cos(ang)
        fwd[n2, row_re + 8] = np.sin(ang)
        ang = 2.0 * np.pi * np.outer(N2 * np.arange(N1) + n2, k1 + 0.25) / S
        inv[n2][:, 2 * k1] = np.cos(ang) / S
        inv[n2][:, 2 * k1 + 1] = np.sin(ang) / S
    inv = inv.reshape(N2, N1, 2, N1).transpose(0, 2, 1, 3)
    return _pack_rows(fwd), _pack_rows(inv)


_FWD, _INV = _dft_tables()


def _dot(a, b, dims=NN_DIMS):
    return lax.dot_general(a, b, dims, preferred_element_type=F32)


def _u32(x):
    return pltpu.bitcast(x, U32)


def _bf(x):
    return pltpu.bitcast(x, BF16)


def _u32_word(x):
    return lax.bitcast_convert_type(x, U32)


def _pack2(a, b):
    return pltpu.pack_elementwise([a, b], packed_dtype=BF16).astype(U32)


def _lo(w):
    return pltpu.unpack_elementwise(w, index=0, packed_dtype=BF16, unpacked_dtype=F32)


def _hi(w):
    return pltpu.unpack_elementwise(w, index=1, packed_dtype=BF16, unpacked_dtype=F32)


def _radix4(x0, x1, x2, x3, sign):
    ar, ai = x0[0] + x2[0], x0[1] + x2[1]
    br, bi = x0[0] - x2[0], x0[1] - x2[1]
    cr, ci = x1[0] + x3[0], x1[1] + x3[1]
    dr, di = x1[0] - x3[0], x1[1] - x3[1]
    y0 = (ar + cr, ai + ci)
    y2 = (ar - cr, ai - ci)
    yp = (br - di, bi + dr)
    ym = (br + di, bi - dr)
    return (y0, yp, y2, ym) if sign > 0 else (y0, ym, y2, yp)


def _twiddle(x, e, sign):
    xr, xi = x
    if e == 0:
        return x
    if e == 4:
        return (-xi, xr) if sign > 0 else (xi, -xr)
    r = math.sqrt(0.5)
    if e == 2:
        return ((xr - xi) * r, (xr + xi) * r) if sign > 0 else ((xr + xi) * r, (xi - xr) * r)
    if e == 6:
        return ((xr + xi) * -r, (xr - xi) * r) if sign > 0 else ((xi - xr) * r, (xr + xi) * -r)
    c, s = math.cos(math.pi * e / 8), sign * math.sin(math.pi * e / 8)
    return (xr * c - xi * s, xr * s + xi * c)


def _radix4_tw(x0, x1, x2, x3, sign, b):
    if b != 2:
        return _radix4(x0, _twiddle(x1, b, sign), _twiddle(x2, 2 * b, sign),
                       _twiddle(x3, 3 * b, sign), sign)
    x1, x3 = _twiddle(x1, 2, sign), _twiddle(x3, 6, sign)
    if sign > 0:
        ar, ai = x0[0] - x2[1], x0[1] + x2[0]
        br, bi = x0[0] + x2[1], x0[1] - x2[0]
    else:
        ar, ai = x0[0] + x2[1], x0[1] - x2[0]
        br, bi = x0[0] - x2[1], x0[1] + x2[0]
    cr, ci = x1[0] + x3[0], x1[1] + x3[1]
    dr, di = x1[0] - x3[0], x1[1] - x3[1]
    y0 = (ar + cr, ai + ci)
    y2 = (ar - cr, ai - ci)
    yp = (br - di, bi + dr)
    ym = (br + di, bi - dr)
    return (y0, yp, y2, ym) if sign > 0 else (y0, ym, y2, yp)


class _Paced:
    def __init__(self, streams, sequential=False):
        self.live = [[g, total, 0] for g, total in streams if total]
        self.total = sum(total for _, total in streams)
        self.done = 0
        self.sequential = sequential

    def step(self):
        cur = self.live[0] if self.sequential else min(self.live, key=lambda e: e[2] / e[1])
        cost = next(cur[0], None)
        if cost is None:
            self.live.remove(cur)
        else:
            cur[2] += cost
            self.done += cost

    def advance(self, fraction):
        while self.live and self.done < fraction * self.total:
            self.step()

    def finish(self):
        self.advance(math.inf)


SPLIT = ((0, 1, 2), (3, 4), (), ())
FORWARD = ((), (0, 1), (2, 3, 4), ())
SPECTRUM = ((), (), (0, 1), (2, 3))
INVERSE = ((), (), (), (0, 1))
DEPTH = 3
NSLOT = 4
ORDER = ((0, 1, 2, 3), (0, 1, 2, 3), (0, 1, 2, 3), (0, 1, 2, 3))
TAIL = (0.0, 0.0, 0.0, 0.0)
LW = (1.0, 1.0, 1.0, 1.0)
AW = (3.0, 3.0, 3.0, 3.0, 3.0)
QCH = (128, 128, 128, 128)
HEAD = (4, 4, 4, 2)
FILL_ORDER = (0, 0, 0, 0)
PACE_ON = (3, 3, 3, 3, 7)
SIDE_SPEED = (1.0, 1.0, 1.0, 1.0)
MID = 3
W_STAGES = ((0, 1), (1, 3), (3, 5))


def _kernel(aq_hbm, ak_hbm, av_hbm, shift_hbm, h_hbm, ssmd_hbm, x_hbm, wq_hbm, wk_hbm,
            wv_hbm, wo_hbm, beta_hbm, fwd_hbm, inv_hbm, out_hbm, shift_ref, ssmd_ref, beta_ref,
            xb, wqb, wkb, wvb, wob, wvt, hb, ht, kb, vb, qb, fwd, inv,
            ub, outb, wtab, gtab, cmask,
            q0, q1, k0, k1, pq0, pq1, pk0, pk1, ots, mst,
            hmask, hsel, bmask, kwin, vall, vhead, opart, onat, sem_zero, sems, *rest):
    xp, hp, tx, th, yb, kvf, outa = (rest[NT * k:NT * k + NT] for k in range(7))
    slots = rest[7 * NT:]
    qs, ks, pqs, pks = (q0, q1), (k0, k1), (pq0, pq1), (pk0, pk1)

    def tile_copy(src, dst, t, sem, r0, n, lead=(0,), dst_off=0):
        return lambda: pltpu.make_async_copy(
            src.bitcast(U32).at[(*lead, pl.ds(r0 // 2, n // 2), pl.ds(128 * t, 128))],
            dst.at[t, pl.ds(dst_off + r0 // 2, n // 2), :], sems.at[sem])

    def h_copy(t, c0, n, sem):
        return lambda: pltpu.make_async_copy(
            h_hbm.bitcast(U32).at[pl.ds(64 * c0, 64 * n), pl.ds(128 * t, 128)],
            hb.at[t, pl.ds(64 * c0, 64 * n), :], sems.at[sem])

    def conv_copies(cs, i, sem):
        out = [h_copy(4 * i + t, cs[0], len(cs), sem) for t in range(4)]
        out += [tile_copy(ak_hbm, kb, c, sem, L * i, L, dst_off=8) for c in cs]
        return out + [tile_copy(av_hbm, vb, c, sem, L * i, L) for c in cs]

    def whole(ref, sem):
        return [lambda: pltpu.make_async_copy(ref, ref, sems.at[sem])]

    def x_copies(r0, n, sem):
        return ([tile_copy(x_hbm, xb, c, sem, r0, n) for c in range(NT)],
                whole(xb.at[:, pl.ds(r0 // 2, n // 2), :], sem))

    def w_copies(src, dst, n0, n1, sem):
        return ([tile_copy(src, dst, n, sem, 0, D, lead=()) for n in range(n0, n1)],
                whole(dst.at[pl.ds(n0, n1 - n0)], sem))

    cp_x0 = [x_copies(256 * k, 256, k) for k in range(2)]
    cp_x1 = [x_copies(L + 128 * i, 128, 2 + i) for i in range(4)]
    cp_x = {s: x_copies(L * s, L, 4 + s) for s in (2, 3)}
    cp_wq = [w_copies(wq_hbm, wqb, n0, n1, 8 + k) for k, (n0, n1) in enumerate(W_STAGES)]
    cp_wk = [w_copies(wk_hbm, wkb, n0, n1, 11 + k) for k, (n0, n1) in enumerate(W_STAGES)]
    cp_wv = w_copies(wv_hbm, wvb, 0, NT, 14)
    cp_wo = w_copies(wo_hbm, wob, 0, NT, 15)
    cp_early = [conv_copies(SPLIT[0], i, 16 + i) for i in range(4)]
    cp_late = [cp for i in range(4) for cp in conv_copies(SPLIT[1], i, 20)]
    cp_q = ([tile_copy(aq_hbm, qb, c, 21, 0, S) for c in range(NT)], whole(qb, 21))
    cp_fwd = [lambda: pltpu.make_async_copy(fwd_hbm, fwd, sems.at[22])]
    cp_inv = [lambda: pltpu.make_async_copy(inv_hbm, inv, sems.at[23])]
    cp_small = [lambda: pltpu.make_async_copy(shift_hbm, shift_ref, sems.at[24]),
                lambda: pltpu.make_async_copy(ssmd_hbm, ssmd_ref, sems.at[24]),
                lambda: pltpu.make_async_copy(beta_hbm, beta_ref, sems.at[24])]

    def out_a(c):
        return [lambda: pltpu.make_async_copy(
            outa[c], out_hbm.bitcast(U32).at[0, :, pl.ds(128 * c, 128)], sems.at[25 + c])]

    def out_b(r0, n, rows_, sem):
        return lambda: pltpu.make_async_copy(
            outb.at[n, pl.ds(r0, rows_), :],
            out_hbm.at[0, pl.ds(r0, rows_), pl.ds(D + 128 * n, 128)], sems.at[sem])

    cp_oa = [out_a(c) for c in range(NT)]
    cp_ob3 = [[out_b(L * 3 + 128 * i, n, 128, 30) for n in range(NT)] for i in range(4)]
    ob_done = whole(outb, 30)

    def start(*groups):
        for g in groups:
            for cp in (g[0] if isinstance(g, tuple) else g):
                cp().start()

    def wait(*groups):
        for g in groups:
            for cp in (g[1] if isinstance(g, tuple) else g):
                cp().wait()

    def rows(i, n):
        return pl.ds(pl.multiple_of(i * n, n), n) if not isinstance(i, int) else pl.ds(i * n, n)

    lane = lax.broadcasted_iota(jnp.int32, (8, 128), 1)
    sub = lax.broadcasted_iota(jnp.int32, (8, 128), 0)

    def lanes(n):
        return lax.broadcasted_iota(jnp.int32, (n, 128), 1)

    recent = [None]
    seg = [0]

    def dot(a, b, dims=NN_DIMS, kind=4):
        out = _dot(a, b, dims)
        if kind & PACE_ON[seg[0]]:
            recent[0] = out
        return out

    current = {}

    def pace(zero):
        v = recent[0][-8:]
        recent[0] = None
        if "h" in current:
            hb[S // 128, rows(zero, 8), :] = _u32_word(v)
        if "k" in current:
            kb[NT, rows(zero, 8), :] = _u32_word(v)
        if "t" in current:
            th[current["t"]][N1 // 8, zero, 0, 0] = v

    def qk_proj(s, i, want_pq, want_pk):
        p = s % 2
        tok = rows(4 * s + i, 64)
        for w_ref, dst, fdst, want, scale in (
                (wqb, qs[p], pqs[p], want_pq, DH ** -0.5 * LOG2E),
                (wkb, ks[p], pks[p], want_pk, None)):
            for n in range(NT):
                t = None
                for c in range(NT):
                    part = dot(_bf(xb[c, tok, :]), _bf(w_ref[n, 64 * c:64 * c + 64, :]))
                    t = part if t is None else t + part
                    if c < NT - 1:
                        yield 32
                dst[n, rows(i, 128), :] = (t if scale is None else t * scale).astype(BF16)
                if want:
                    fdst[n, rows(i, 128), :] = jnp.where(t > 0, t + 1.0, jnp.exp(t)).astype(BF16)
                yield 32

    def first_proj(n, js=range(4)):
        for w_ref, dst, scale in ((wqb, qs[0], DH ** -0.5 * LOG2E), (wkb, ks[0], None)):
            for j in js:
                t = None
                for c in range(NT):
                    part = dot(_bf(xb[c, rows(j, 64), :]), _bf(w_ref[n, 64 * c:64 * c + 64, :]))
                    t = part if t is None else t + part
                dst[n, rows(j, 128), :] = (t if scale is None else t * scale).astype(BF16)
                if scale is None:
                    pks[0][n, rows(j, 128), :] = jnp.where(t > 0, t + 1.0, jnp.exp(t)).astype(BF16)

    def untranspose(s, i, slot=0):
        ot = ots.bitcast(U32)
        for c in range(NT):
            onat[slot, c] = _u32(_bf(ot[s % 2, i, 64 * c:64 * c + 64, :]).T)

    def out_proj(s, i, slot=0, copies=None):
        for n in range(NT):
            t = None
            for c in range(NT):
                part = dot(_bf(onat[slot, c]), _bf(wob[n, 64 * c:64 * c + 64, :]))
                t = part if t is None else t + part
                if c < NT - 1:
                    yield 32
            outb[n, rows(4 * s + i, 128), :] = t.astype(BF16)
            if copies is not None:
                start([copies[n]])
            yield 32

    def tile_rows(r, n):
        return jnp.broadcast_to(r[None], (n // 8, 8, 128)).reshape(n, 128)

    class Group:
        def __init__(self, s, g, gi):
            self.s, self.g, self.gi = s, g, gi
            self.t0 = (80 * g) // 128
            self.off = 80 * g - 128 * self.t0
            self.t1 = jnp.minimum(self.t0 + 1, NT - 1)
            rel = (lane - self.off) & 127
            head = sum((rel >= a * DH).astype(jnp.int32) for a in range(1, 5))
            for a in range(4):
                hmask[gi, a] = jnp.where(head == a, np.uint32(0xFFFFFFFF), np.uint32(0))
            hsel[gi] = jnp.left_shift(1, head)
            self.have_keys, self.have_mem = set(), set()

        def window(self, ref, j, r0=0, n=64):
            ref = ref.bitcast(U32)
            at = pl.ds(64 * j + r0, n)
            return jnp.where(lanes(n) >= self.off, ref[self.t0, at, :], ref[self.t1, at, :])

        def keys(self, r0, r1):
            out = []
            for r in range(r0, r1, 64):
                at = pl.ds(r // 2, 32)
                if r in self.have_keys:
                    out.append(kwin[self.gi, at, :])
                else:
                    self.have_keys.add(r)
                    out.append(self.window(ks[self.s % 2], 0, r // 2, 32))
                    kwin[self.gi, at, :] = out[-1]
            return _bf(jnp.concatenate(out, axis=0))

        def park_values(self, j, v80):
            vall[self.gi, j, 0:80, :] = v80.astype(BF16)
            ones8 = jnp.ones((8, 128), F32)
            for pr in range(2):
                for e in range(2):
                    r0 = 40 * pr + 16 * e
                    vhead[self.gi, j, r0 // 8] = jnp.concatenate(
                        [v80[r0:r0 + 24], ones8], axis=0).astype(BF16)

        def mem_read(self):
            for j in range(4):
                r = dot(mst[self.g].astype(BF16), _bf(self.window(pqs[self.s % 2], j)), NT_DIMS)
                coef = gtab[self.g] / (r[80:88] + 1e-6)
                cb = [jnp.broadcast_to(coef[a:a + 1], (8, 128)) for a in range(4)]
                for pr in range(2):
                    ca, cc = cb[2 * pr], cb[2 * pr + 1]
                    for e, scale in enumerate((ca, ca, jnp.where(sub < 4, ca, cc), cc, cc)):
                        r0 = 40 * pr + 8 * e
                        opart[self.gi, j, r0:r0 + 8, :] = r[r0:r0 + 8] * scale
                self.have_mem.add(j)
                yield 24

        def mem_update(self):
            acc = None
            for j in range(4):
                t = dot(_bf(vall.bitcast(U32)[self.gi, j]), _bf(self.window(pks[self.s % 2], j)))
                acc = t if acc is None else acc + t
                if j < 3:
                    yield 24
            for r in range(12):
                new = jnp.where(bmask[r] & hsel[self.gi] != 0, acc[8 * r:8 * r + 8], 0.0)
                at = pl.ds(8 * r, 8)
                mst[self.g, at, :] = new if self.s == 0 else mst[self.g, at, :] + new
            yield 24

        def logits(self, pr, j, slot):
            qw = self.window(qs[self.s % 2], j)
            qa = qw & tile_rows(hmask[self.gi, 2 * pr], 64)
            qh = qw & tile_rows(hmask[self.gi, 2 * pr + 1], 64)
            w_a = _bf(qa)
            w_b = _bf(jnp.concatenate([qh[32:64], qh[0:32]], axis=0))
            w_t = _bf(jnp.concatenate([qh[32:64], qa[32:64]], axis=0))
            n = 128 * j

            def park(t, e, r0, m):
                for r in range(0, t.shape[0], 8):
                    v = t[r:r + 8]
                    if e == 2:
                        v = v + cmask[2, r:r + 8, :]
                    elif r0 + r >= n:
                        v = v + cmask[e, r0 + r - n:r0 + r - n + 8, :]
                    slot[e % 2, 448 * (e // 2) + r0 + r:448 * (e // 2) + r0 + r + 8, :] = v
                    m = v if m is None else jnp.maximum(m, v)
                return m

            m_t = park(dot(self.keys(n + 64, n + 128), w_t, NT_DIMS, 1), 2, 0, None)
            yield 16 * LW[seg[0] % 4]
            cuts = list(range(0, n, QCH[seg[0]])) or [0]
            m = [None, None]
            for r0, r1 in zip(cuts, cuts[1:] + [n + 64]):
                for e, w in enumerate((w_a, w_b)):
                    m[e] = park(dot(self.keys(r0, r1), w, NT_DIMS, 1), e, r0, m[e])
                    if r1 == n + 64 and e == 1:
                        m_a = jnp.maximum(m[0], jnp.where(lane >= 64, m_t, NEG))
                        m_b = jnp.maximum(m[1], jnp.where(lane < 64, m_t, NEG))
                        m_a = jnp.broadcast_to(jnp.max(m_a, axis=0, keepdims=True), (8, 128))
                        m_b = jnp.broadcast_to(jnp.max(m_b, axis=0, keepdims=True), (8, 128))
                        slot[1, 448:456, :] = m_a
                        slot[1, 456:464, :] = m_b
                        slot[1, 464:472, :] = jnp.where(lane < 64, m_b, m_a)
                    yield (r1 - r0) // 4 * LW[seg[0] % 4]

    def attend(gi, g, parity, add_mem, pr, j, slot, need_values):
        def prob(e, r0, n, which):
            m2 = tile_rows(slot[1, 448 + 8 * which:456 + 8 * which, :], 16)
            return [jnp.exp2(slot[e, r:r + 16, :] - m2) for r in range(r0, r0 + n, 16)]

        res = [None, None]
        order = [(0, j), (1, j)] + [(e, kt) for e in range(2) for kt in range(j)]
        for n, (e, kt) in enumerate(order):
            need_values(kt)
            if n == 0:
                p_t = prob(0, 448, 64, 2)
            if kt < j:
                p = prob(e, 128 * kt, 128, e)
            else:
                mine = lanes(16) >= 64 if e == 0 else lanes(16) < 64
                p = prob(e, 128 * kt, 64, e) + [jnp.where(mine, t, 0.0) for t in p_t]
            t = dot(_bf(vhead.bitcast(U32)[gi, kt, 5 * pr + 2 * e]),
                    jnp.concatenate(p, axis=0).astype(BF16), kind=2)
            res[e] = t if res[e] is None else res[e] + t
            if n < len(order) - 1:
                yield 8 * AW[seg[0]]
        r_a = res[0]
        r_b = pltpu.roll(res[1], 64, 1)
        keep = 1.0 - gtab[g]
        keep_a = jnp.broadcast_to(keep[2 * pr:2 * pr + 1], (8, 128))
        keep_b = jnp.broadcast_to(keep[2 * pr + 1:2 * pr + 2], (8, 128))
        o_a = r_a[0:24] * tile_rows(keep_a / r_a[24:32], 24)
        o_b = r_b[0:24] * tile_rows(keep_b / r_b[24:32], 24)
        o = jnp.concatenate(
            [o_a[0:16], jnp.where(sub < 4, o_a[16:24], o_b[0:8]), o_b[8:24]], axis=0)
        if add_mem:
            o = o + opart[gi, j, 40 * pr:40 * pr + 40, :]
        if pr == 0:
            opart[gi, j, 0:40, :] = o
        else:
            o = jnp.concatenate([opart[gi, j, 0:40, :], o], axis=0)
            ots[parity, j, rows(g, 80), :] = o.astype(BF16)
        yield 8 * AW[seg[0]]

    def v_proj(s, i, groups, have):
        for j in range(4):
            acc = None
            for c in range(NT):
                t = dot(_bf(wvt[c, rows(i, 80), :]), _bf(xb[c, rows(4 * s + j, 64), :]), NT_DIMS)
                acc = t if acc is None else acc + t
                if c == NT - 1:
                    for gi in range(2):
                        groups[gi].park_values(j, acc[80 * gi:80 * gi + 80])
                    have.append(j)
                yield 40

    def chain(*gens):
        for g in gens:
            yield from g

    def units(s):
        return [(gi, pr, j) for gi in range(2) for pr in range(2)
                for j in (range(4) if (gi, pr) == (1, 1) else ORDER[s] if gi + pr else range(4))]

    def cost(j):
        return (48 + 64 * j) * LW[seg[0] % 4], (16 + 16 * j) * AW[seg[0]]

    def carried(u, g, parity):
        gi, pr, j = units(0)[u]
        return attend(gi, g, parity, True, pr, j, slots[u % NSLOT], lambda kt: None), cost(j)[1]

    def segment_step(s, i):
        seg[0] = s
        parts = {}
        if s < NSEG - 1:
            parts["qk"] = (qk_proj(s + 1, i, True, s + 1 < NSEG - 1), 1600)
        if s > 0:
            parts["out"] = (out_proj(s - 1, i), 800)
        if FORWARD[s]:
            parts["fwd"] = (fwd_fft(i, FORWARD[s]), 512 * len(FORWARD[s]))
        if INVERSE[s]:
            parts["inv"] = (inverse(INVERSE[s], (2 * i, 2 * i + 1)), 256 * len(INVERSE[s]))
        names = (("qk", "inv", "out", "fwd"), ("qk", "inv", "fwd", "out"),
                 ("inv", "fwd", "qk", "out"), ("qk", "inv", "out", "fwd"))[FILL_ORDER[s]]
        fill = _Paced([parts[n] for n in names if n in parts], sequential=FILL_ORDER[s] < 3)
        side = []
        if SPECTRUM[s]:
            side.append((spectra(SPECTRUM[s], [4 * i + a for a in range(4)]),
                         4 * SPEC_COST * len(SPECTRUM[s])))
        for c in SPLIT[s]:
            side += [(split_h(i, c), 144), (split_kv(i, c), 704)]
        side = _Paced(side, sequential=True)
        current.clear()
        recent[0] = None
        for _ in range(HEAD[s]):
            fill.step()
        if s > 0:
            untranspose(s - 1, i)
        vt = []
        groups = [Group(s, 2 * i + gi, gi) for gi in range(2)]
        reads = [grp.mem_read() for grp in groups if s > 0]
        updates = [grp.mem_update() for grp in groups if s < NSEG - 1]
        first = _Paced([(chain(*reads[:1], v_proj(s, i, groups, vt), *reads[1:], *updates),
                         800 + 96 * (len(reads) + len(updates)))])
        total = first.total + fill.total
        held = 96 * (s > 0) + 160

        def need_values(kt):
            while len(vt) <= kt:
                first.step()

        def pad(fraction, u):
            target = total * fraction / (1 + TAIL[s])
            early = min(target, held if u < DEPTH else first.total)
            first.advance(early / first.total)
            fill.advance((target - early) / fill.total)
            goal = fraction * SIDE_SPEED[s]
            if side.live and side.done < goal * side.total and recent[0] is not None:
                pace(jnp.minimum(i, 3))
                side.advance(goal)

        todo = units(s)
        whole = sum(sum(cost(j)) for _, _, j in todo)
        done = 0
        for u, (gi, pr, j) in enumerate(todo):
            streams = [(groups[gi].logits(pr, j, slots[u % NSLOT]), cost(j)[0])]
            v = u - DEPTH
            if v < 0:
                streams.append(carried(v + len(todo), (2 * i + 7) & 7,
                                       jnp.where(i > 0, s % 2, 1 - s % 2)))
            else:
                gi, pr, j = todo[v]
                while s > 0 and j not in groups[gi].have_mem:
                    first.step()
                streams.append((attend(gi, 2 * i + gi, s % 2, s > 0, pr, j, slots[v % NSLOT],
                                       need_values), cost(j)[1]))
            att = _Paced(streams[::-1], sequential=u == len(todo) - 1)
            while att.live:
                att.step()
                pad((done + att.done) / whole, u)
            done += att.total
        first.finish()
        fill.finish()
        side.finish()

    def split_h(i, c):
        current.clear()
        current["h"] = True
        for t in range(4):
            ht[c, 64 * t:64 * t + 64, :] = _u32(
                _bf(hb[4 * i + t, 64 * c:64 * c + 64, :]).T)
            yield 4
        for q in range(2):
            for j in range(8):
                wa = ht[c, pl.ds(128 * q + j, 8, stride=8), :]
                wb = ht[c, pl.ds(128 * q + 64 + j, 8, stride=8), :]
                hp[c][2 * j, rows(2 * i + q, 8), :] = _pack2(_lo(wa), _lo(wb))
                hp[c][2 * j + 1, rows(2 * i + q, 8), :] = _pack2(_hi(wa), _hi(wb))
                if j % 2:
                    yield 16

    def split_kv(i, c):
        current.clear()
        current["k"] = True
        taps = [wtab[c, j] for j in range(KS)]
        for q in range(2):
            blk = 2 * i + q
            base = [blk * 128 + 64 * e for e in range(2)]
            hist = []
            for e in range(2):
                w2 = kb[c, pl.ds(base[e] + 6, 8, stride=8), :]
                w1 = kb[c, pl.ds(base[e] + 7, 8, stride=8), :]
                hist.append([_hi(w2), _lo(w1), _hi(w1)])
            for j in range(8):
                kv = [[None, None], [None, None]]
                for e in range(2):
                    kw = kb[c, pl.ds(base[e] + 8 + j, 8, stride=8), :]
                    vw = vb[c, pl.ds(base[e] + j, 8, stride=8), :]
                    kp = hist[e] + [_lo(kw), _hi(kw)]
                    for half, part in enumerate((_lo, _hi)):
                        acc = kp[3 + half] * taps[0]
                        for d in range(1, KS):
                            acc = acc + kp[3 + half - d] * taps[d]
                        kv[half][e] = acc * part(vw)
                        kvf[c][2 * j + half, rows(2 * blk + e, 8), :] = kv[half][e]
                    hist[e] = kp[2:]
                    if e == 0:
                        yield 22
                for half in range(2):
                    xp[c][2 * j + half, rows(blk, 8), :] = _pack2(*kv[half])
                yield 22

    def fwd_fft(i, cs):
        for c in cs:
            for src, dst in ((hp[c], th[c]), (xp[c], tx[c])):
                g = [dot(_bf(fwd[4 * a + i]), _bf(src[4 * a + i])) for a in range(4)]
                for r in range(0, 2 * N1, 16):
                    z = _radix4(*[(g[a][r:r + 8], g[a][r + 8:r + 16]) for a in range(4)], 1)
                    for cc in range(4):
                        dst[r // 16, cc, i, 0] = z[cc][0]
                        dst[r // 16, cc, i, 1] = z[cc][1]
                yield 256

    def spectrum(c, m, slot):
        current.clear()
        current["t"] = c
        for cc in range(4):
            zh = _radix4_tw(*[(th[c][m, cc, b, 0], th[c][m, cc, b, 1]) for b in range(4)], 1, cc)
            yield 17
            zx = _radix4_tw(*[(tx[c][m, cc, b, 0], tx[c][m, cc, b, 1]) for b in range(4)], 1, cc)
            yield 17
            y = [(x[0] * h[0] - x[1] * h[1], x[0] * h[1] + x[1] * h[0]) for x, h in zip(zx, zh)]
            yield 17
            u = _radix4(*y, -1)
            for b in range(4):
                ub[slot, b, cc, 0] = u[b][0]
                ub[slot, b, cc, 1] = u[b][1]
            yield 17
        for b in range(4):
            z = _radix4_tw(*[(ub[slot, b, cc, 0], ub[slot, b, cc, 1]) for cc in range(4)], -1, b)
            for a in range(4):
                yb[c][4 * a + b, rows(m, 8), :] = _pack2(*z[a])
            yield 17

    SPEC_COST = 17 * 20

    def spectra(cs, ms, slot0=0):
        for slot, (c, m) in enumerate(((c, m) for c in cs for m in ms), slot0):
            yield from spectrum(c, m, slot)

    def inverse(cs, jps):
        for c in cs:
            for jp in jps:
                w = qb[c, pl.ds(jp, N1, stride=8), :]
                res = []
                for e, part in enumerate((_lo, _hi)):
                    n2 = 2 * jp + e
                    y = dot(_bf(inv[n2, 0]), _bf(yb[c][n2, 0:64, :]))
                    yield 32
                    y = y + dot(_bf(inv[n2, 1]), _bf(yb[c][n2, 64:128, :]))
                    res.append(part(w) * (y + kvf[c][n2] * tile_rows(wtab[c, KS], N1)))
                    if e == 0:
                        yield 32
                outa[c][pl.ds(jp, N1, stride=8), :] = _pack2(*res)
                yield 32

    start(cp_wq[0], cp_wk[0], cp_x0[0], cp_x0[1], cp_wq[1], cp_wk[1])
    sem_zero[0] = 0
    kk = lax.broadcasted_iota(jnp.int32, (64, 128), 0)
    ll = lax.broadcasted_iota(jnp.int32, (64, 128), 1)
    cmask[0] = jnp.where(kk <= ll, 0.0, NEG)
    cmask[1] = jnp.where((ll < 64) | (kk <= ll - 64), 0.0, NEG)
    cmask[2] = jnp.where(kk <= (ll & 63), 0.0, NEG)
    for r in range(12):
        row = sub + 8 * r
        hr = sum((row >= a * DH).astype(jnp.int32) for a in range(1, 4)) if r < 10 else row - 80
        bmask[r] = jnp.left_shift(1, hr)
    for gi in range(2):
        for j in range(4):
            vall[gi, j, 80:96, :] = jnp.ones((16, 128), BF16)
    for c in range(NT):
        kb[c, 0:8, :] = jnp.zeros((8, 128), U32)
    for u in range(16 - DEPTH, 16):
        slots[u % NSLOT][...] = jnp.zeros((2, 512, 128), F32)
    vhead[1] = jnp.ones(vhead.shape[1:], BF16)
    opart[1] = jnp.zeros(opart.shape[1:], F32)
    with jax.named_scope("prologue"):
        wait(cp_wq[0], cp_wk[0], cp_x0[0])
        start(cp_wq[2], cp_wk[2], cp_wv, cp_small, cp_x1[0], cp_early[0])
        first_proj(0, (0, 1))
        wait(cp_x0[1])
        first_proj(0, (2, 3))
        wait(cp_wq[1], cp_wk[1])
        for n in range(*W_STAGES[1]):
            first_proj(n)
        wait(cp_wq[2], cp_wk[2])
        first_proj(W_STAGES[2][0])
        wait(cp_wv, cp_small)
        start(cp_x1[1], cp_early[1])
        taps_t = shift_ref[...].astype(F32)
        skip = ssmd_ref[...].astype(F32)
        for c in range(NT):
            for j in range(KS):
                wtab[c, j] = jnp.broadcast_to(taps_t[j:j + 1, 128 * c:128 * c + 128], (8, 128))
            wtab[c, KS] = jnp.broadcast_to(skip[c:c + 1], (8, 128))
        gates = jax.nn.sigmoid(beta_ref[...].astype(F32))
        gcol = jnp.broadcast_to(gates, (8, H)).T
        gcol = jnp.broadcast_to(gcol[:, 0:1], (H, 128))
        for g in range(8):
            gtab[g] = jnp.concatenate([gcol[4 * g:4 * g + 4]] * 2, axis=0)
        for n in range(NT):
            for c in range(NT):
                wvt[c, rows(n, 64), :] = _u32(_bf(wvb[n, 64 * c:64 * c + 64, :]).T)
        for n in range(W_STAGES[2][0] + 1, NT):
            first_proj(n)
    start(cp_wo, cp_x[2])

    def segment(s):
        def body(i, carry):
            if s == 0:
                for j in range(4):
                    @pl.when(i == j)
                    def _():
                        wait(cp_x1[j], cp_early[j])
                        start(*((cp_x1[2], cp_early[2]), (cp_x1[3], cp_early[3]),
                                (cp_fwd, cp_late), (cp_x[3],))[j])
            segment_step(s, i)
            if s > 0:
                r0 = pl.multiple_of(L * (s - 1) + 128 * i, 128)
                start([out_b(r0, n, 128, 30) for n in range(NT)])
            return carry

        with jax.named_scope(f"seg{s}"):
            lax.fori_loop(0, 4, body, 0)

    segment(0)
    wait(cp_fwd, cp_x[2], cp_wo, cp_late)
    start(cp_inv, cp_q)
    segment(1)
    wait(cp_x[3])
    segment(2)
    wait(cp_inv, cp_q)
    segment(3)
    start(*[cp_oa[c] for c in INVERSE[3]])
    with jax.named_scope("epilogue"):
        seg[0] = 4
        current.clear()
        recent[0] = None
        last = NT - 1
        rest_tiles = [c for c in range(last) if c not in INVERSE[3]]
        side = _Paced([(spectra((last,), range(16)), 16 * SPEC_COST)])
        span = 1024 * len(rest_tiles) + 800 * MID
        done = 0

        def run(streams):
            nonlocal done
            work = _Paced(streams)
            while work.live:
                before = work.done
                work.step()
                done += work.done - before
                if side.live and side.done < done / span * side.total and recent[0] is not None:
                    pace(sem_zero[0])
                    side.advance(done / span)

        for c in rest_tiles:
            streams = [(inverse((c,), range(8)), 1024)]
            if c == rest_tiles[0]:
                tail = [carried(u, 7, 1) for u in range(16 - DEPTH, 16)]
                streams.append((chain(*[g for g, _ in tail]), sum(w for _, w in tail)))
            run(streams)
            if c == rest_tiles[0]:
                for i in range(4):
                    untranspose(3, i, i)
            start(cp_oa[c])
        for i in range(4):
            if i == MID:
                side.finish()
                run([(inverse((last,), range(8)), 1024)])
                start(cp_oa[last])
            run([(out_proj(3, i, i, cp_ob3[i]), 800)])
    wait(*cp_oa, ob_done)


@jax.jit
def pallas_concat_heads__ssm_conv_h3__memory_aug_infini_attn__prompt_kernel(
    A_q: jax.Array,
    A_k: jax.Array,
    A_v: jax.Array,
    A_shift_k: jax.Array,
    A_ssm_k: jax.Array,
    A_ssm_D: jax.Array,
    B_x: jax.Array,
    B_wq: jax.Array,
    B_wk: jax.Array,
    B_wv: jax.Array,
    B_wo: jax.Array,
    B_beta: jax.Array,
):
    hbm = pl.BlockSpec(memory_space=pltpu.HBM)
    seg_tiles = pltpu.VMEM((NT, L, 128), BF16)
    seq_tiles = pltpu.VMEM((NT, S // 2, 128), U32)
    w_tiles = pltpu.VMEM((NT, D // 2, 128), U32)
    scratch = [
        pltpu.VMEM((KS, D), BF16),
        pltpu.VMEM((NT, 128), BF16),
        pltpu.VMEM((1, H), BF16),
        seq_tiles,
        w_tiles, w_tiles, w_tiles, w_tiles, w_tiles,
        pltpu.VMEM((S // 128 + 1, D // 2, 128), U32),
        pltpu.VMEM((NT, 256, 128), U32),
        pltpu.VMEM((NT + 1, S // 2 + 8, 128), U32),
        seq_tiles, seq_tiles,
        pltpu.VMEM((N2, N1, 128), U32),
        pltpu.VMEM((N2, 2, N1 // 2, 128), U32),
        pltpu.VMEM((16, 4, 4, 2, 8, 128), F32),
        pltpu.VMEM((NT, S, 128), BF16),
        pltpu.VMEM((NT, KS + 1, 8, 128), F32),
        pltpu.VMEM((8, 8, 128), F32),
        pltpu.VMEM((3, 64, 128), F32),
        seg_tiles, seg_tiles, seg_tiles, seg_tiles,
        seg_tiles, seg_tiles, seg_tiles, seg_tiles,
        pltpu.VMEM((2, 4, D, 128), BF16),
        pltpu.VMEM((8, 96, 128), F32),
        pltpu.VMEM((2, 4, 8, 128), U32),
        pltpu.VMEM((2, 8, 128), jnp.int32),
        pltpu.VMEM((12, 8, 128), jnp.int32),
        pltpu.VMEM((2, L // 2, 128), U32),
        pltpu.VMEM((2, 4, 96, 128), BF16),
        pltpu.VMEM((2, 4, 8, 32, 128), BF16),
        pltpu.VMEM((2, 4, 80, 128), F32),
        pltpu.VMEM((4, NT, 64, 128), U32),
        pltpu.SMEM((1,), jnp.int32),
        pltpu.SemaphoreType.DMA((31,)),
    ]
    scratch += [pltpu.VMEM((N2, N1 // 2, 128), U32)] * (2 * NT)
    scratch += [pltpu.VMEM((N1 // 8 + 1, 4, 4, 2, 8, 128), F32)] * (2 * NT)
    scratch += [pltpu.VMEM((N2, N1, 128), U32)] * NT
    scratch += [pltpu.VMEM((N2, N1, 128), F32)] * NT
    scratch += [pltpu.VMEM((S // 2, 128), U32)] * NT
    scratch += [pltpu.VMEM((2, 512, 128), F32)] * NSLOT
    return pl.pallas_call(
        _kernel,
        out_shape=jax.ShapeDtypeStruct((1, S, 2 * D), BF16),
        in_specs=[hbm] * 14,
        out_specs=hbm,
        scratch_shapes=scratch,
        compiler_params=pltpu.CompilerParams(vmem_limit_bytes=110 * 1024 * 1024),
        name="h3_infini",
    )(A_q, A_k, A_v, A_shift_k.T, A_ssm_k, A_ssm_D.reshape(NT, 128), B_x, B_wq, B_wk, B_wv, B_wo,
      B_beta.reshape(1, H), _FWD, _INV)
```

```python
import math

import jax
import jax.numpy as jnp
import numpy as np
from jax import lax
from jax.experimental import pallas as pl
from jax.experimental.pallas import tpu as pltpu

S = 2048
D = 640
NT = D // 128
H = 32
DH = D // H
NSEG = 4
L = S // NSEG
KS = 4
N1, N2 = 128, 16

F32 = jnp.float32
BF16 = jnp.bfloat16
U32 = jnp.uint32
NN_DIMS = (((1,), (0,)), ((), ()))
NT_DIMS = (((1,), (1,)), ((), ()))
NEG = -1e30
LOG2E = 1.4426950408889634


def _pack_rows(a):
    u = a.astype(np.float32).astype(BF16).view(np.uint16).astype(np.uint32)
    return u[..., 0::2, :] | (u[..., 1::2, :] << 16)


def _dft_tables():
    k1 = np.arange(N1)
    fwd = np.zeros((N2, 2 * N1, N1), np.float64)
    inv = np.zeros((N2, N1, 2 * N1), np.float64)
    kappa = np.arange(N1)
    n1_in = 16 * (kappa // 16) + 8 * (kappa % 2) + (kappa % 16) // 2
    row_re = 16 * (k1 // 8) + k1 % 8
    for n2 in range(N2):
        ang = 2.0 * np.pi * np.outer(k1 + 0.25, N2 * n1_in + n2) / S
        fwd[n2, row_re] = np.cos(ang)
        fwd[n2, row_re + 8] = np.sin(ang)
        ang = 2.0 * np.pi * np.outer(N2 * np.arange(N1) + n2, k1 + 0.25) / S
        inv[n2][:, 2 * k1] = np.cos(ang) / S
        inv[n2][:, 2 * k1 + 1] = np.sin(ang) / S
    inv = inv.reshape(N2, N1, 2, N1).transpose(0, 2, 1, 3)
    return _pack_rows(fwd), _pack_rows(inv)


_FWD, _INV = _dft_tables()


def _dot(a, b, dims=NN_DIMS):
    return lax.dot_general(a, b, dims, preferred_element_type=F32)


def _u32(x):
    return pltpu.bitcast(x, U32)


def _bf(x):
    return pltpu.bitcast(x, BF16)


def _u32_word(x):
    return lax.bitcast_convert_type(x, U32)


def _pack2(a, b):
    return pltpu.pack_elementwise([a, b], packed_dtype=BF16).astype(U32)


def _lo(w):
    return pltpu.unpack_elementwise(w, index=0, packed_dtype=BF16, unpacked_dtype=F32)


def _hi(w):
    return pltpu.unpack_elementwise(w, index=1, packed_dtype=BF16, unpacked_dtype=F32)


def _radix4(x0, x1, x2, x3, sign):
    ar, ai = x0[0] + x2[0], x0[1] + x2[1]
    br, bi = x0[0] - x2[0], x0[1] - x2[1]
    cr, ci = x1[0] + x3[0], x1[1] + x3[1]
    dr, di = x1[0] - x3[0], x1[1] - x3[1]
    y0 = (ar + cr, ai + ci)
    y2 = (ar - cr, ai - ci)
    yp = (br - di, bi + dr)
    ym = (br + di, bi - dr)
    return (y0, yp, y2, ym) if sign > 0 else (y0, ym, y2, yp)


def _twiddle(x, e, sign):
    xr, xi = x
    if e == 0:
        return x
    if e == 4:
        return (-xi, xr) if sign > 0 else (xi, -xr)
    r = math.sqrt(0.5)
    if e == 2:
        return ((xr - xi) * r, (xr + xi) * r) if sign > 0 else ((xr + xi) * r, (xi - xr) * r)
    if e == 6:
        return ((xr + xi) * -r, (xr - xi) * r) if sign > 0 else ((xi - xr) * r, (xr + xi) * -r)
    c, s = math.cos(math.pi * e / 8), sign * math.sin(math.pi * e / 8)
    return (xr * c - xi * s, xr * s + xi * c)


def _radix4_tw(x0, x1, x2, x3, sign, b):
    if b != 2:
        return _radix4(x0, _twiddle(x1, b, sign), _twiddle(x2, 2 * b, sign),
                       _twiddle(x3, 3 * b, sign), sign)
    x1, x3 = _twiddle(x1, 2, sign), _twiddle(x3, 6, sign)
    if sign > 0:
        ar, ai = x0[0] - x2[1], x0[1] + x2[0]
        br, bi = x0[0] + x2[1], x0[1] - x2[0]
    else:
        ar, ai = x0[0] + x2[1], x0[1] - x2[0]
        br, bi = x0[0] - x2[1], x0[1] + x2[0]
    cr, ci = x1[0] + x3[0], x1[1] + x3[1]
    dr, di = x1[0] - x3[0], x1[1] - x3[1]
    y0 = (ar + cr, ai + ci)
    y2 = (ar - cr, ai - ci)
    yp = (br - di, bi + dr)
    ym = (br + di, bi - dr)
    return (y0, yp, y2, ym) if sign > 0 else (y0, ym, y2, yp)


class _Paced:
    def __init__(self, streams, sequential=False):
        self.live = [[g, total, 0] for g, total in streams if total]
        self.total = sum(total for _, total in streams)
        self.done = 0
        self.sequential = sequential

    def step(self):
        cur = self.live[0] if self.sequential else min(self.live, key=lambda e: e[2] / e[1])
        cost = next(cur[0], None)
        if cost is None:
            self.live.remove(cur)
        else:
            cur[2] += cost
            self.done += cost

    def advance(self, fraction):
        while self.live and self.done < fraction * self.total:
            self.step()

    def finish(self):
        self.advance(math.inf)


SPLIT = ((0, 1, 2), (3, 4), (), ())
FORWARD = ((), (0, 1), (2, 3, 4), ())
SPECTRUM = ((), (), (0, 1), (2, 3))
INVERSE = ((), (), (), (0, 1))
DEPTH = 3
NSLOT = 4
ORDER = ((0, 1, 2, 3), (0, 1, 2, 3), (0, 1, 2, 3), (0, 1, 2, 3))
TAIL = (0.0, 0.0, 0.0, 0.0)
LW = (1.0, 1.0, 1.0, 1.0)
AW = (3.0, 3.0, 3.0, 3.0, 3.0)
QCH = (128, 128, 128, 128)
HEAD = (4, 4, 4, 2)
FILL_ORDER = (0, 0, 0, 0)
PACE_ON = (3, 3, 3, 3, 7)
SIDE_SPEED = (1.0, 1.0, 1.0, 1.0)
MID = 3
PACE_ALL = (0, 0, 3, 3, 0)
SPEC_V = (0, 0, 0, 0, 1)
W_STAGES = ((0, 1), (1, 3), (3, 5))


def _kernel(aq_hbm, ak_hbm, av_hbm, shift_hbm, h_hbm, ssmd_hbm, x_hbm, wq_hbm, wk_hbm,
            wv_hbm, wo_hbm, beta_hbm, fwd_hbm, inv_hbm, out_hbm, shift_ref, ssmd_ref, beta_ref,
            xb, wqb, wkb, wvb, wob, wvt, hb, ht, kb, vb, qb, fwd, inv,
            ub, outb, wtab, gtab, cmask,
            q0, q1, k0, k1, pq0, pq1, pk0, pk1, ots, mst,
            hmask, hsel, bmask, kwin, vall, vhead, opart, onat, sem_zero, sems, *rest):
    xp, hp, tx, th, yb, kvf, outa = (rest[NT * k:NT * k + NT] for k in range(7))
    slots = rest[7 * NT:]
    qs, ks, pqs, pks = (q0, q1), (k0, k1), (pq0, pq1), (pk0, pk1)

    def tile_copy(src, dst, t, sem, r0, n, lead=(0,), dst_off=0):
        return lambda: pltpu.make_async_copy(
            src.bitcast(U32).at[(*lead, pl.ds(r0 // 2, n // 2), pl.ds(128 * t, 128))],
            dst.at[t, pl.ds(dst_off + r0 // 2, n // 2), :], sems.at[sem])

    def h_copy(t, c0, n, sem):
        return lambda: pltpu.make_async_copy(
            h_hbm.bitcast(U32).at[pl.ds(64 * c0, 64 * n), pl.ds(128 * t, 128)],
            hb.at[t, pl.ds(64 * c0, 64 * n), :], sems.at[sem])

    def conv_copies(cs, i, sem):
        out = [h_copy(4 * i + t, cs[0], len(cs), sem) for t in range(4)]
        out += [tile_copy(ak_hbm, kb, c, sem, L * i, L, dst_off=8) for c in cs]
        return out + [tile_copy(av_hbm, vb, c, sem, L * i, L) for c in cs]

    def whole(ref, sem):
        return [lambda: pltpu.make_async_copy(ref, ref, sems.at[sem])]

    def x_copies(r0, n, sem):
        return ([tile_copy(x_hbm, xb, c, sem, r0, n) for c in range(NT)],
                whole(xb.at[:, pl.ds(r0 // 2, n // 2), :], sem))

    def w_copies(src, dst, n0, n1, sem):
        return ([tile_copy(src, dst, n, sem, 0, D, lead=()) for n in range(n0, n1)],
                whole(dst.at[pl.ds(n0, n1 - n0)], sem))

    cp_x0 = [x_copies(256 * k, 256, k) for k in range(2)]
    cp_x1 = [x_copies(L + 128 * i, 128, 2 + i) for i in range(4)]
    cp_x = {s: x_copies(L * s, L, 4 + s) for s in (2, 3)}
    cp_wq = [w_copies(wq_hbm, wqb, n0, n1, 8 + k) for k, (n0, n1) in enumerate(W_STAGES)]
    cp_wk = [w_copies(wk_hbm, wkb, n0, n1, 11 + k) for k, (n0, n1) in enumerate(W_STAGES)]
    cp_wv = w_copies(wv_hbm, wvb, 0, NT, 14)
    cp_wo = w_copies(wo_hbm, wob, 0, NT, 15)
    cp_early = [conv_copies(SPLIT[0], i, 16 + i) for i in range(4)]
    cp_late = [cp for i in range(4) for cp in conv_copies(SPLIT[1], i, 20)]
    cp_q = ([tile_copy(aq_hbm, qb, c, 21, 0, S) for c in range(NT)], whole(qb, 21))
    cp_fwd = [lambda: pltpu.make_async_copy(fwd_hbm, fwd, sems.at[22])]
    cp_inv = [lambda: pltpu.make_async_copy(inv_hbm, inv, sems.at[23])]
    cp_small = [lambda: pltpu.make_async_copy(shift_hbm, shift_ref, sems.at[24]),
                lambda: pltpu.make_async_copy(ssmd_hbm, ssmd_ref, sems.at[24]),
                lambda: pltpu.make_async_copy(beta_hbm, beta_ref, sems.at[24])]

    def out_a(c):
        return [lambda: pltpu.make_async_copy(
            outa[c], out_hbm.bitcast(U32).at[0, :, pl.ds(128 * c, 128)], sems.at[25 + c])]

    def out_b(r0, n, rows_, sem):
        return lambda: pltpu.make_async_copy(
            outb.at[n, pl.ds(r0, rows_), :],
            out_hbm.at[0, pl.ds(r0, rows_), pl.ds(D + 128 * n, 128)], sems.at[sem])

    cp_oa = [out_a(c) for c in range(NT)]
    cp_ob3 = [[out_b(L * 3 + 128 * i, n, 128, 30) for n in range(NT)] for i in range(4)]
    ob_done = whole(outb, 30)

    def start(*groups):
        for g in groups:
            for cp in (g[0] if isinstance(g, tuple) else g):
                cp().start()

    def wait(*groups):
        for g in groups:
            for cp in (g[1] if isinstance(g, tuple) else g):
                cp().wait()

    def rows(i, n):
        return pl.ds(pl.multiple_of(i * n, n), n) if not isinstance(i, int) else pl.ds(i * n, n)

    lane = lax.broadcasted_iota(jnp.int32, (8, 128), 1)
    sub = lax.broadcasted_iota(jnp.int32, (8, 128), 0)

    def lanes(n):
        return lax.broadcasted_iota(jnp.int32, (n, 128), 1)

    recent = [None]
    seg = [0]

    def dot(a, b, dims=NN_DIMS, kind=4):
        out = _dot(a, b, dims)
        if kind & PACE_ON[seg[0]]:
            recent[0] = out
        return out

    current = {}

    def pace(zero):
        v = recent[0][-8:]
        recent[0] = None
        if "h" in current:
            hb[S // 128, rows(zero, 8), :] = _u32_word(v)
        if "k" in current:
            kb[NT, rows(zero, 8), :] = _u32_word(v)
        if "t" in current:
            th[current["t"]][N1 // 8, zero, 0, 0] = v
            if PACE_ALL[seg[0]] & 1:
                tx[current["t"]][N1 // 8, zero, 0, 0] = v
            if PACE_ALL[seg[0]] & 2:
                ub[16, zero, 0, 0] = v

    def qk_proj(s, i, want_pq, want_pk):
        p = s % 2
        tok = rows(4 * s + i, 64)
        for w_ref, dst, fdst, want, scale in (
                (wqb, qs[p], pqs[p], want_pq, DH ** -0.5 * LOG2E),
                (wkb, ks[p], pks[p], want_pk, None)):
            for n in range(NT):
                t = None
                for c in range(NT):
                    part = dot(_bf(xb[c, tok, :]), _bf(w_ref[n, 64 * c:64 * c + 64, :]))
                    t = part if t is None else t + part
                    if c < NT - 1:
                        yield 32
                dst[n, rows(i, 128), :] = (t if scale is None else t * scale).astype(BF16)
                if want:
                    fdst[n, rows(i, 128), :] = jnp.where(t > 0, t + 1.0, jnp.exp(t)).astype(BF16)
                yield 32

    def first_proj(n, js=range(4)):
        for w_ref, dst, scale in ((wqb, qs[0], DH ** -0.5 * LOG2E), (wkb, ks[0], None)):
            for j in js:
                t = None
                for c in range(NT):
                    part = dot(_bf(xb[c, rows(j, 64), :]), _bf(w_ref[n, 64 * c:64 * c + 64, :]))
                    t = part if t is None else t + part
                dst[n, rows(j, 128), :] = (t if scale is None else t * scale).astype(BF16)
                if scale is None:
                    pks[0][n, rows(j, 128), :] = jnp.where(t > 0, t + 1.0, jnp.exp(t)).astype(BF16)

    def untranspose(s, i, slot=0):
        ot = ots.bitcast(U32)
        for c in range(NT):
            onat[slot, c] = _u32(_bf(ot[s % 2, i, 64 * c:64 * c + 64, :]).T)

    def out_proj(s, i, slot=0, copies=None):
        for n in range(NT):
            t = None
            for c in range(NT):
                part = dot(_bf(onat[slot, c]), _bf(wob[n, 64 * c:64 * c + 64, :]))
                t = part if t is None else t + part
                if c < NT - 1:
                    yield 32
            outb[n, rows(4 * s + i, 128), :] = t.astype(BF16)
            if copies is not None:
                start([copies[n]])
            yield 32

    def tile_rows(r, n):
        return jnp.broadcast_to(r[None], (n // 8, 8, 128)).reshape(n, 128)

    class Group:
        def __init__(self, s, g, gi):
            self.s, self.g, self.gi = s, g, gi
            self.t0 = (80 * g) // 128
            self.off = 80 * g - 128 * self.t0
            self.t1 = jnp.minimum(self.t0 + 1, NT - 1)
            rel = (lane - self.off) & 127
            head = sum((rel >= a * DH).astype(jnp.int32) for a in range(1, 5))
            for a in range(4):
                hmask[gi, a] = jnp.where(head == a, np.uint32(0xFFFFFFFF), np.uint32(0))
            hsel[gi] = jnp.left_shift(1, head)
            self.have_keys, self.have_mem = set(), set()

        def window(self, ref, j, r0=0, n=64):
            ref = ref.bitcast(U32)
            at = pl.ds(64 * j + r0, n)
            return jnp.where(lanes(n) >= self.off, ref[self.t0, at, :], ref[self.t1, at, :])

        def keys(self, r0, r1):
            out = []
            for r in range(r0, r1, 64):
                at = pl.ds(r // 2, 32)
                if r in self.have_keys:
                    out.append(kwin[self.gi, at, :])
                else:
                    self.have_keys.add(r)
                    out.append(self.window(ks[self.s % 2], 0, r // 2, 32))
                    kwin[self.gi, at, :] = out[-1]
            return _bf(jnp.concatenate(out, axis=0))

        def park_values(self, j, v80):
            if self.s < NSEG - 1:
                vall[self.gi, j, 0:80, :] = v80
            ones8 = jnp.ones((8, 128), F32)
            for pr in range(2):
                for e in range(2):
                    r0 = 40 * pr + 16 * e
                    vhead[self.gi, j, r0 // 8] = jnp.concatenate(
                        [v80[r0:r0 + 24], ones8], axis=0).astype(BF16)

        def mem_read(self):
            for j in range(4):
                r = dot(mst[self.g, 0:88, :], _bf(self.window(pqs[self.s % 2], j)), NT_DIMS)
                coef = gtab[self.g] / (r[80:88] + 1e-6)
                cb = [jnp.broadcast_to(coef[a:a + 1], (8, 128)) for a in range(4)]
                for pr in range(2):
                    ca, cc = cb[2 * pr], cb[2 * pr + 1]
                    for e, scale in enumerate((ca, ca, jnp.where(sub < 4, ca, cc), cc, cc)):
                        r0 = 40 * pr + 8 * e
                        opart[self.gi, j, r0:r0 + 8, :] = r[r0:r0 + 8] * scale
                self.have_mem.add(j)
                yield 24

        def mem_update(self):
            acc = None
            for j in range(4):
                t = dot(vall[self.gi, j], _bf(self.window(pks[self.s % 2], j)))
                acc = t if acc is None else acc + t
                if j < 3:
                    yield 24
            for r in range(11):
                new = jnp.where(bmask[r] & hsel[self.gi] != 0, acc[8 * r:8 * r + 8], 0.0)
                at = pl.ds(8 * r, 8)
                mst[self.g, at, :] = new if self.s == 0 else mst[self.g, at, :] + new
            yield 24

        def logits(self, pr, j, slot):
            qw = self.window(qs[self.s % 2], j)
            qa = qw & tile_rows(hmask[self.gi, 2 * pr], 64)
            qh = qw & tile_rows(hmask[self.gi, 2 * pr + 1], 64)
            w_a = _bf(qa)
            w_b = _bf(jnp.concatenate([qh[32:64], qh[0:32]], axis=0))
            w_t = _bf(jnp.concatenate([qh[32:64], qa[32:64]], axis=0))
            n = 128 * j

            def park(t, e, r0, m):
                for r in range(0, t.shape[0], 8):
                    v = t[r:r + 8]
                    if e == 2:
                        v = v + cmask[2, r:r + 8, :]
                    elif r0 + r >= n:
                        v = v + cmask[e, r0 + r - n:r0 + r - n + 8, :]
                    slot[e % 2, 448 * (e // 2) + r0 + r:448 * (e // 2) + r0 + r + 8, :] = v
                    m = v if m is None else jnp.maximum(m, v)
                return m

            m_t = park(dot(self.keys(n + 64, n + 128), w_t, NT_DIMS, 1), 2, 0, None)
            yield 16 * LW[seg[0] % 4]
            cuts = list(range(0, n, QCH[seg[0]])) or [0]
            m = [None, None]
            for r0, r1 in zip(cuts, cuts[1:] + [n + 64]):
                for e, w in enumerate((w_a, w_b)):
                    m[e] = park(dot(self.keys(r0, r1), w, NT_DIMS, 1), e, r0, m[e])
                    if r1 == n + 64 and e == 1:
                        m_a = jnp.maximum(m[0], jnp.where(lane >= 64, m_t, NEG))
                        m_b = jnp.maximum(m[1], jnp.where(lane < 64, m_t, NEG))
                        m_a = jnp.broadcast_to(jnp.max(m_a, axis=0, keepdims=True), (8, 128))
                        m_b = jnp.broadcast_to(jnp.max(m_b, axis=0, keepdims=True), (8, 128))
                        slot[1, 448:456, :] = m_a
                        slot[1, 456:464, :] = m_b
                        slot[1, 464:472, :] = jnp.where(lane < 64, m_b, m_a)
                    yield (r1 - r0) // 4 * LW[seg[0] % 4]

    def attend(gi, g, parity, add_mem, pr, j, slot, need_values):
        def prob(e, r0, n, which):
            m2 = tile_rows(slot[1, 448 + 8 * which:456 + 8 * which, :], 16)
            return [jnp.exp2(slot[e, r:r + 16, :] - m2) for r in range(r0, r0 + n, 16)]

        res = [None, None]
        order = [(0, j), (1, j)] + [(e, kt) for e in range(2) for kt in range(j)]
        for n, (e, kt) in enumerate(order):
            need_values(kt)
            if n == 0:
                p_t = prob(0, 448, 64, 2)
            if kt < j:
                p = prob(e, 128 * kt, 128, e)
            else:
                mine = lanes(16) >= 64 if e == 0 else lanes(16) < 64
                p = prob(e, 128 * kt, 64, e) + [jnp.where(mine, t, 0.0) for t in p_t]
            t = dot(_bf(vhead.bitcast(U32)[gi, kt, 5 * pr + 2 * e]),
                    jnp.concatenate(p, axis=0).astype(BF16), kind=2)
            res[e] = t if res[e] is None else res[e] + t
            if n < len(order) - 1:
                yield 8 * AW[seg[0]]
        r_a = res[0]
        r_b = pltpu.roll(res[1], 64, 1)
        keep = 1.0 - gtab[g]
        keep_a = jnp.broadcast_to(keep[2 * pr:2 * pr + 1], (8, 128))
        keep_b = jnp.broadcast_to(keep[2 * pr + 1:2 * pr + 2], (8, 128))
        o_a = r_a[0:24] * tile_rows(keep_a / r_a[24:32], 24)
        o_b = r_b[0:24] * tile_rows(keep_b / r_b[24:32], 24)
        o = jnp.concatenate(
            [o_a[0:16], jnp.where(sub < 4, o_a[16:24], o_b[0:8]), o_b[8:24]], axis=0)
        if add_mem:
            o = o + opart[gi, j, 40 * pr:40 * pr + 40, :]
        if pr == 0:
            opart[gi, j, 0:40, :] = o
        else:
            o = jnp.concatenate([opart[gi, j, 0:40, :], o], axis=0)
            ots[parity, j, rows(g, 80), :] = o.astype(BF16)
        yield 8 * AW[seg[0]]

    def v_proj(s, i, groups, have):
        for j in range(4):
            acc = None
            for c in range(NT):
                t = dot(_bf(wvt[c, rows(i, 80), :]), _bf(xb[c, rows(4 * s + j, 64), :]), NT_DIMS)
                acc = t if acc is None else acc + t
                if c == NT - 1:
                    for gi in range(2):
                        groups[gi].park_values(j, acc[80 * gi:80 * gi + 80])
                    have.append(j)
                yield 40

    def chain(*gens):
        for g in gens:
            yield from g

    def units(s):
        return [(gi, pr, j) for gi in range(2) for pr in range(2)
                for j in (range(4) if (gi, pr) == (1, 1) else ORDER[s] if gi + pr else range(4))]

    def cost(j):
        return (48 + 64 * j) * LW[seg[0] % 4], (16 + 16 * j) * AW[seg[0]]

    def carried(u, g, parity):
        gi, pr, j = units(0)[u]
        return attend(gi, g, parity, True, pr, j, slots[u % NSLOT], lambda kt: None), cost(j)[1]

    def segment_step(s, i):
        seg[0] = s
        parts = {}
        if s < NSEG - 1:
            parts["qk"] = (qk_proj(s + 1, i, True, s + 1 < NSEG - 1), 1600)
        if s > 0:
            parts["out"] = (out_proj(s - 1, i), 800)
        if FORWARD[s]:
            parts["fwd"] = (fwd_fft(i, FORWARD[s]), 512 * len(FORWARD[s]))
        if INVERSE[s]:
            parts["inv"] = (inverse(INVERSE[s], (2 * i, 2 * i + 1)), 256 * len(INVERSE[s]))
        names = (("qk", "inv", "out", "fwd"), ("qk", "inv", "fwd", "out"),
                 ("inv", "fwd", "qk", "out"), ("qk", "inv", "out", "fwd"))[FILL_ORDER[s]]
        fill = _Paced([parts[n] for n in names if n in parts], sequential=FILL_ORDER[s] < 3)
        side = []
        if SPECTRUM[s]:
            side.append((spectra(SPECTRUM[s], [4 * i + a for a in range(4)]),
                         4 * SPEC_COST * len(SPECTRUM[s])))
        for c in SPLIT[s]:
            side += [(split_h(i, c), 144), (split_kv(i, c), 704)]
        side = _Paced(side, sequential=True)
        current.clear()
        recent[0] = None
        for _ in range(HEAD[s]):
            fill.step()
        if s > 0:
            untranspose(s - 1, i)
        vt = []
        groups = [Group(s, 2 * i + gi, gi) for gi in range(2)]
        reads = [grp.mem_read() for grp in groups if s > 0]
        updates = [grp.mem_update() for grp in groups if s < NSEG - 1]
        first = _Paced([(chain(*reads[:1], v_proj(s, i, groups, vt), *reads[1:], *updates),
                         800 + 96 * (len(reads) + len(updates)))])
        total = first.total + fill.total
        held = 96 * (s > 0) + 160

        def need_values(kt):
            while len(vt) <= kt:
                first.step()

        def pad(fraction, u):
            target = total * fraction / (1 + TAIL[s])
            early = min(target, held if u < DEPTH else first.total)
            first.advance(early / first.total)
            fill.advance((target - early) / fill.total)
            goal = fraction * SIDE_SPEED[s]
            if side.live and side.done < goal * side.total and recent[0] is not None:
                pace(jnp.minimum(i, 3))
                side.advance(goal)

        todo = units(s)
        whole = sum(sum(cost(j)) for _, _, j in todo)
        done = 0
        for u, (gi, pr, j) in enumerate(todo):
            streams = [(groups[gi].logits(pr, j, slots[u % NSLOT]), cost(j)[0])]
            v = u - DEPTH
            if v < 0:
                streams.append(carried(v + len(todo), (2 * i + 7) & 7,
                                       jnp.where(i > 0, s % 2, 1 - s % 2)))
            else:
                gi, pr, j = todo[v]
                while s > 0 and j not in groups[gi].have_mem:
                    first.step()
                streams.append((attend(gi, 2 * i + gi, s % 2, s > 0, pr, j, slots[v % NSLOT],
                                       need_values), cost(j)[1]))
            att = _Paced(streams[::-1], sequential=u == len(todo) - 1)
            while att.live:
                att.step()
                pad((done + att.done) / whole, u)
            done += att.total
        first.finish()
        fill.finish()
        side.finish()

    def split_h(i, c):
        current.clear()
        current["h"] = True
        for t in range(4):
            ht[c, 64 * t:64 * t + 64, :] = _u32(
                _bf(hb[4 * i + t, 64 * c:64 * c + 64, :]).T)
            yield 4
        for q in range(2):
            for j in range(8):
                wa = ht[c, pl.ds(128 * q + j, 8, stride=8), :]
                wb = ht[c, pl.ds(128 * q + 64 + j, 8, stride=8), :]
                hp[c][2 * j, rows(2 * i + q, 8), :] = _pack2(_lo(wa), _lo(wb))
                hp[c][2 * j + 1, rows(2 * i + q, 8), :] = _pack2(_hi(wa), _hi(wb))
                if j % 2:
                    yield 16

    def split_kv(i, c):
        current.clear()
        current["k"] = True
        taps = [wtab[c, j] for j in range(KS)]
        for q in range(2):
            blk = 2 * i + q
            base = [blk * 128 + 64 * e for e in range(2)]
            hist = []
            for e in range(2):
                w2 = kb[c, pl.ds(base[e] + 6, 8, stride=8), :]
                w1 = kb[c, pl.ds(base[e] + 7, 8, stride=8), :]
                hist.append([_hi(w2), _lo(w1), _hi(w1)])
            for j in range(8):
                kv = [[None, None], [None, None]]
                for e in range(2):
                    kw = kb[c, pl.ds(base[e] + 8 + j, 8, stride=8), :]
                    vw = vb[c, pl.ds(base[e] + j, 8, stride=8), :]
                    kp = hist[e] + [_lo(kw), _hi(kw)]
                    for half, part in enumerate((_lo, _hi)):
                        acc = kp[3 + half] * taps[0]
                        for d in range(1, KS):
                            acc = acc + kp[3 + half - d] * taps[d]
                        kv[half][e] = acc * part(vw)
                        kvf[c][2 * j + half, rows(2 * blk + e, 8), :] = kv[half][e]
                    hist[e] = kp[2:]
                    if e == 0:
                        yield 22
                for half in range(2):
                    xp[c][2 * j + half, rows(blk, 8), :] = _pack2(*kv[half])
                yield 22

    def fwd_fft(i, cs):
        for c in cs:
            for src, dst in ((hp[c], th[c]), (xp[c], tx[c])):
                g = [dot(_bf(fwd[4 * a + i]), _bf(src[4 * a + i])) for a in range(4)]
                for r in range(0, 2 * N1, 16):
                    z = _radix4(*[(g[a][r:r + 8], g[a][r + 8:r + 16]) for a in range(4)], 1)
                    for cc in range(4):
                        dst[r // 16, cc, i, 0] = z[cc][0]
                        dst[r // 16, cc, i, 1] = z[cc][1]
                yield 256

    def spectrum(c, m, slot):
        current.clear()
        current["t"] = c
        for cc in range(4):
            zh = _radix4_tw(*[(th[c][m, cc, b, 0], th[c][m, cc, b, 1]) for b in range(4)], 1, cc)
            yield 17
            zx = _radix4_tw(*[(tx[c][m, cc, b, 0], tx[c][m, cc, b, 1]) for b in range(4)], 1, cc)
            yield 17
            y = [(x[0] * h[0] - x[1] * h[1], x[0] * h[1] + x[1] * h[0]) for x, h in zip(zx, zh)]
            yield 17
            u = _radix4(*y, -1)
            for b in range(4):
                ub[slot, b, cc, 0] = u[b][0]
                ub[slot, b, cc, 1] = u[b][1]
            yield 17
        if SPEC_V[seg[0]]:
            return

        yield from spectrum_end(c, m, slot)

    def spectrum_end(c, m, slot):
        for b in range(4):
            z = _radix4_tw(*[(ub[slot, b, cc, 0], ub[slot, b, cc, 1]) for cc in range(4)], -1, b)
            for a in range(4):
                yb[c][4 * a + b, rows(m, 8), :] = _pack2(*z[a])
            yield 17

    SPEC_COST = 17 * 20

    def spectra(cs, ms, slot0=0):
        prev = None
        for slot, (c, m) in enumerate(((c, m) for c in cs for m in ms), slot0):
            yield from spectrum(c, m, slot)
            if SPEC_V[seg[0]] and prev is not None:
                yield from spectrum_end(*prev)
            prev = (c, m, slot)
        if SPEC_V[seg[0]]:
            yield from spectrum_end(*prev)

    def inverse(cs, jps):
        for c in cs:
            for jp in jps:
                w = qb[c, pl.ds(jp, N1, stride=8), :]
                res = []
                for e, part in enumerate((_lo, _hi)):
                    n2 = 2 * jp + e
                    y = dot(_bf(inv[n2, 0]), _bf(yb[c][n2, 0:64, :]))
                    yield 32
                    y = y + dot(_bf(inv[n2, 1]), _bf(yb[c][n2, 64:128, :]))
                    res.append(part(w) * (y + kvf[c][n2] * tile_rows(wtab[c, KS], N1)))
                    if e == 0:
                        yield 32
                outa[c][pl.ds(jp, N1, stride=8), :] = _pack2(*res)
                yield 32

    start(cp_wq[0], cp_wk[0], cp_x0[0], cp_x0[1], cp_wq[1], cp_wk[1])
    sem_zero[0] = 0
    kk = lax.broadcasted_iota(jnp.int32, (64, 128), 0)
    ll = lax.broadcasted_iota(jnp.int32, (64, 128), 1)
    cmask[0] = jnp.where(kk <= ll, 0.0, NEG)
    cmask[1] = jnp.where((ll < 64) | (kk <= ll - 64), 0.0, NEG)
    cmask[2] = jnp.where(kk <= (ll & 63), 0.0, NEG)
    for r in range(11):
        row = sub + 8 * r
        hr = sum((row >= a * DH).astype(jnp.int32) for a in range(1, 4)) if r < 10 else row - 80
        bmask[r] = jnp.left_shift(1, hr)
    for gi in range(2):
        for j in range(4):
            vall[gi, j, 80:88, :] = jnp.ones((8, 128), F32)
    for c in range(NT):
        kb[c, 0:8, :] = jnp.zeros((8, 128), U32)
    for u in range(16 - DEPTH, 16):
        slots[u % NSLOT][...] = jnp.zeros((2, 512, 128), F32)
    vhead[1] = jnp.ones(vhead.shape[1:], BF16)
    opart[1] = jnp.zeros(opart.shape[1:], F32)
    with jax.named_scope("prologue"):
        wait(cp_wq[0], cp_wk[0], cp_x0[0])
        start(cp_wq[2], cp_wk[2], cp_wv, cp_small, cp_x1[0], cp_early[0])
        first_proj(0, (0, 1))
        wait(cp_x0[1])
        first_proj(0, (2, 3))
        wait(cp_wq[1], cp_wk[1])
        for n in range(*W_STAGES[1]):
            first_proj(n)
        wait(cp_wq[2], cp_wk[2])
        first_proj(W_STAGES[2][0])
        wait(cp_wv, cp_small)
        start(cp_x1[1], cp_early[1])
        taps_t = shift_ref[...].astype(F32)
        skip = ssmd_ref[...].astype(F32)
        for c in range(NT):
            for j in range(KS):
                wtab[c, j] = jnp.broadcast_to(taps_t[j:j + 1, 128 * c:128 * c + 128], (8, 128))
            wtab[c, KS] = jnp.broadcast_to(skip[c:c + 1], (8, 128))
        gates = jax.nn.sigmoid(beta_ref[...].astype(F32))
        gcol = jnp.broadcast_to(gates, (8, H)).T
        gcol = jnp.broadcast_to(gcol[:, 0:1], (H, 128))
        for g in range(8):
            gtab[g] = jnp.concatenate([gcol[4 * g:4 * g + 4]] * 2, axis=0)
        for n in range(NT):
            for c in range(NT):
                wvt[c, rows(n, 64), :] = _u32(_bf(wvb[n, 64 * c:64 * c + 64, :]).T)
        for n in range(W_STAGES[2][0] + 1, NT):
            first_proj(n)
    start(cp_wo, cp_x[2])

    def segment(s):
        def body(i, carry):
            if s == 0:
                for j in range(4):
                    @pl.when(i == j)
                    def _():
                        wait(cp_x1[j], cp_early[j])
                        start(*((cp_x1[2], cp_early[2]), (cp_x1[3], cp_early[3]),
                                (cp_fwd, cp_late), (cp_x[3],))[j])
            segment_step(s, i)
            if s > 0:
                r0 = pl.multiple_of(L * (s - 1) + 128 * i, 128)
                start([out_b(r0, n, 128, 30) for n in range(NT)])
            return carry

        with jax.named_scope(f"seg{s}"):
            lax.fori_loop(0, 4, body, 0)

    segment(0)
    wait(cp_fwd, cp_x[2], cp_wo, cp_late)
    start(cp_inv, cp_q)
    segment(1)
    wait(cp_x[3])
    segment(2)
    wait(cp_inv, cp_q)
    segment(3)
    start(*[cp_oa[c] for c in INVERSE[3]])
    with jax.named_scope("epilogue"):
        seg[0] = 4
        current.clear()
        recent[0] = None
        last = NT - 1
        rest_tiles = [c for c in range(last) if c not in INVERSE[3]]
        side = _Paced([(spectra((last,), range(16)), 16 * SPEC_COST)])
        span = 1024 * len(rest_tiles) + 800 * MID
        done = 0

        def run(streams):
            nonlocal done
            work = _Paced(streams)
            while work.live:
                before = work.done
                work.step()
                done += work.done - before
                if side.live and side.done < done / span * side.total and recent[0] is not None:
                    pace(sem_zero[0])
                    side.advance(done / span)

        for c in rest_tiles:
            streams = [(inverse((c,), range(8)), 1024)]
            if c == rest_tiles[0]:
                tail = [carried(u, 7, 1) for u in range(16 - DEPTH, 16)]
                streams.append((chain(*[g for g, _ in tail]), sum(w for _, w in tail)))
            run(streams)
            if c == rest_tiles[0]:
                for i in range(4):
                    untranspose(3, i, i)
            start(cp_oa[c])
        for i in range(4):
            if i == MID:
                side.finish()
                run([(inverse((last,), range(8)), 1024)])
                start(cp_oa[last])
            run([(out_proj(3, i, i, cp_ob3[i]), 800)])
    wait(*cp_oa, ob_done)


@jax.jit
def pallas_concat_heads__ssm_conv_h3__memory_aug_infini_attn__prompt_kernel(
    A_q: jax.Array,
    A_k: jax.Array,
    A_v: jax.Array,
    A_shift_k: jax.Array,
    A_ssm_k: jax.Array,
    A_ssm_D: jax.Array,
    B_x: jax.Array,
    B_wq: jax.Array,
    B_wk: jax.Array,
    B_wv: jax.Array,
    B_wo: jax.Array,
    B_beta: jax.Array,
):
    hbm = pl.BlockSpec(memory_space=pltpu.HBM)
    seg_tiles = pltpu.VMEM((NT, L, 128), BF16)
    seq_tiles = pltpu.VMEM((NT, S // 2, 128), U32)
    w_tiles = pltpu.VMEM((NT, D // 2, 128), U32)
    scratch = [
        pltpu.VMEM((KS, D), BF16),
        pltpu.VMEM((NT, 128), BF16),
        pltpu.VMEM((1, H), BF16),
        seq_tiles,
        w_tiles, w_tiles, w_tiles, w_tiles, w_tiles,
        pltpu.VMEM((S // 128 + 1, D // 2, 128), U32),
        pltpu.VMEM((NT, 256, 128), U32),
        pltpu.VMEM((NT + 1, S // 2 + 8, 128), U32),
        seq_tiles, seq_tiles,
        pltpu.VMEM((N2, N1, 128), U32),
        pltpu.VMEM((N2, 2, N1 // 2, 128), U32),
        pltpu.VMEM((17, 4, 4, 2, 8, 128), F32),
        pltpu.VMEM((NT, S, 128), BF16),
        pltpu.VMEM((NT, KS + 1, 8, 128), F32),
        pltpu.VMEM((8, 8, 128), F32),
        pltpu.VMEM((3, 64, 128), F32),
        seg_tiles, seg_tiles, seg_tiles, seg_tiles,
        seg_tiles, seg_tiles, seg_tiles, seg_tiles,
        pltpu.VMEM((2, 4, D, 128), BF16),
        pltpu.VMEM((8, 88, 128), F32),
        pltpu.VMEM((2, 4, 8, 128), U32),
        pltpu.VMEM((2, 8, 128), jnp.int32),
        pltpu.VMEM((11, 8, 128), jnp.int32),
        pltpu.VMEM((2, L // 2, 128), U32),
        pltpu.VMEM((2, 4, 88, 128), F32),
        pltpu.VMEM((2, 4, 8, 32, 128), BF16),
        pltpu.VMEM((2, 4, 80, 128), F32),
        pltpu.VMEM((4, NT, 64, 128), U32),
        pltpu.SMEM((1,), jnp.int32),
        pltpu.SemaphoreType.DMA((31,)),
    ]
    scratch += [pltpu.VMEM((N2, N1 // 2, 128), U32)] * (2 * NT)
    scratch += [pltpu.VMEM((N1 // 8 + 1, 4, 4, 2, 8, 128), F32)] * (2 * NT)
    scratch += [pltpu.VMEM((N2, N1, 128), U32)] * NT
    scratch += [pltpu.VMEM((N2, N1, 128), F32)] * NT
    scratch += [pltpu.VMEM((S // 2, 128), U32)] * NT
    scratch += [pltpu.VMEM((2, 512, 128), F32)] * NSLOT
    return pl.pallas_call(
        _kernel,
        out_shape=jax.ShapeDtypeStruct((1, S, 2 * D), BF16),
        in_specs=[hbm] * 14,
        out_specs=hbm,
        scratch_shapes=scratch,
        compiler_params=pltpu.CompilerParams(vmem_limit_bytes=110 * 1024 * 1024),
        name="h3_infini",
    )(A_q, A_k, A_v, A_shift_k.T, A_ssm_k, A_ssm_D.reshape(NT, 128), B_x, B_wq, B_wk, B_wv, B_wo,
      B_beta.reshape(1, H), _FWD, _INV)
```

```python
import math

import jax
import jax.numpy as jnp
import numpy as np
from jax import lax
from jax.experimental import pallas as pl
from jax.experimental.pallas import tpu as pltpu

S = 2048
D = 640
NT = D // 128
H = 32
DH = D // H
NSEG = 4
L = S // NSEG
KS = 4
N1, N2 = 128, 16

F32 = jnp.float32
BF16 = jnp.bfloat16
U32 = jnp.uint32
NN_DIMS = (((1,), (0,)), ((), ()))
NT_DIMS = (((1,), (1,)), ((), ()))
NEG = -1e30
LOG2E = 1.4426950408889634


def _pack_rows(a):
    u = a.astype(np.float32).astype(BF16).view(np.uint16).astype(np.uint32)
    return u[..., 0::2, :] | (u[..., 1::2, :] << 16)


def _dft_tables():
    k1 = np.arange(N1)
    fwd = np.zeros((N2, 2 * N1, N1), np.float64)
    inv = np.zeros((N2, N1, 2 * N1), np.float64)
    kappa = np.arange(N1)
    n1_in = 16 * (kappa // 16) + 8 * (kappa % 2) + (kappa % 16) // 2
    row_re = 16 * (k1 // 8) + k1 % 8
    for n2 in range(N2):
        ang = 2.0 * np.pi * np.outer(k1 + 0.25, N2 * n1_in + n2) / S
        fwd[n2, row_re] = np.cos(ang)
        fwd[n2, row_re + 8] = np.sin(ang)
        ang = 2.0 * np.pi * np.outer(N2 * np.arange(N1) + n2, k1 + 0.25) / S
        inv[n2][:, 2 * k1] = np.cos(ang) / S
        inv[n2][:, 2 * k1 + 1] = np.sin(ang) / S
    inv = inv.reshape(N2, N1, 2, N1).transpose(0, 2, 1, 3)
    return _pack_rows(fwd), _pack_rows(inv)


_FWD, _INV = _dft_tables()


def _dot(a, b, dims=NN_DIMS):
    return lax.dot_general(a, b, dims, preferred_element_type=F32)


def _u32(x):
    return pltpu.bitcast(x, U32)


def _bf(x):
    return pltpu.bitcast(x, BF16)


def _u32_word(x):
    return lax.bitcast_convert_type(x, U32)


def _pack2(a, b):
    return pltpu.pack_elementwise([a, b], packed_dtype=BF16).astype(U32)


def _lo(w):
    return pltpu.unpack_elementwise(w, index=0, packed_dtype=BF16, unpacked_dtype=F32)


def _hi(w):
    return pltpu.unpack_elementwise(w, index=1, packed_dtype=BF16, unpacked_dtype=F32)


def _radix4(x0, x1, x2, x3, sign):
    ar, ai = x0[0] + x2[0], x0[1] + x2[1]
    br, bi = x0[0] - x2[0], x0[1] - x2[1]
    cr, ci = x1[0] + x3[0], x1[1] + x3[1]
    dr, di = x1[0] - x3[0], x1[1] - x3[1]
    y0 = (ar + cr, ai + ci)
    y2 = (ar - cr, ai - ci)
    yp = (br - di, bi + dr)
    ym = (br + di, bi - dr)
    return (y0, yp, y2, ym) if sign > 0 else (y0, ym, y2, yp)


def _twiddle(x, e, sign):
    xr, xi = x
    if e == 0:
        return x
    if e == 4:
        return (-xi, xr) if sign > 0 else (xi, -xr)
    r = math.sqrt(0.5)
    if e == 2:
        return ((xr - xi) * r, (xr + xi) * r) if sign > 0 else ((xr + xi) * r, (xi - xr) * r)
    if e == 6:
        return ((xr + xi) * -r, (xr - xi) * r) if sign > 0 else ((xi - xr) * r, (xr + xi) * -r)
    c, s = math.cos(math.pi * e / 8), sign * math.sin(math.pi * e / 8)
    return (xr * c - xi * s, xr * s + xi * c)


def _radix4_tw(x0, x1, x2, x3, sign, b):
    if b != 2:
        return _radix4(x0, _twiddle(x1, b, sign), _twiddle(x2, 2 * b, sign),
                       _twiddle(x3, 3 * b, sign), sign)
    x1, x3 = _twiddle(x1, 2, sign), _twiddle(x3, 6, sign)
    if sign > 0:
        ar, ai = x0[0] - x2[1], x0[1] + x2[0]
        br, bi = x0[0] + x2[1], x0[1] - x2[0]
    else:
        ar, ai = x0[0] + x2[1], x0[1] - x2[0]
        br, bi = x0[0] - x2[1], x0[1] + x2[0]
    cr, ci = x1[0] + x3[0], x1[1] + x3[1]
    dr, di = x1[0] - x3[0], x1[1] - x3[1]
    y0 = (ar + cr, ai + ci)
    y2 = (ar - cr, ai - ci)
    yp = (br - di, bi + dr)
    ym = (br + di, bi - dr)
    return (y0, yp, y2, ym) if sign > 0 else (y0, ym, y2, yp)


class _Paced:
    def __init__(self, streams, sequential=False):
        self.live = [[g, total, 0] for g, total in streams if total]
        self.total = sum(total for _, total in streams)
        self.done = 0
        self.sequential = sequential

    def step(self):
        cur = self.live[0] if self.sequential else min(self.live, key=lambda e: e[2] / e[1])
        cost = next(cur[0], None)
        if cost is None:
            self.live.remove(cur)
        else:
            cur[2] += cost
            self.done += cost

    def advance(self, fraction):
        while self.live and self.done < fraction * self.total:
            self.step()

    def finish(self):
        self.advance(math.inf)


SPLIT = ((0, 1, 2), (3, 4), (), ())
FORWARD = ((), (0, 1), (2, 3, 4), ())
SPECTRUM = ((), (), (0, 1), (2, 3))
INVERSE = ((), (), (), (0, 1))
DEPTH = 3
NSLOT = 4
ORDER = ((1, 3, 0, 2), (3, 2, 1, 0), (0, 2, 1, 3), (0, 1, 2, 3))
TAIL = (-0.03, -0.03, 0.02, -0.03)
LW = (1.0, 1.0, 1.0, 1.0)
AW = (4.0, 2.0, 4.0, 2.0, 3.0)
QCH = (128, 256, 128, 128)
HEAD = (4, 6, 6, 6)
FILL_ORDER = (0, 1, 1, 2)
PACE_ON = (3, 3, 7, 7, 7)
SIDE_SPEED = (1.03, 1.0, 1.03, 1.0)
MID = 3
PACE_ALL = (3, 2, 2, 3, 0)
SPEC_V = (0, 0, 0, 0, 1)
W_STAGES = ((0, 1), (1, 3), (3, 5))


def _kernel(aq_hbm, ak_hbm, av_hbm, shift_hbm, h_hbm, ssmd_hbm, x_hbm, wq_hbm, wk_hbm,
            wv_hbm, wo_hbm, beta_hbm, fwd_hbm, inv_hbm, out_hbm, shift_ref, ssmd_ref, beta_ref,
            xb, wqb, wkb, wvb, wob, wvt, hb, ht, kb, vb, qb, fwd, inv,
            ub, outb, wtab, gtab, cmask,
            q0, q1, k0, k1, pq0, pq1, pk0, pk1, ots, mst,
            hmask, hsel, bmask, kwin, vall, vhead, opart, onat, sem_zero, sems, *rest):
    xp, hp, tx, th, yb, kvf, outa = (rest[NT * k:NT * k + NT] for k in range(7))
    slots = rest[7 * NT:]
    qs, ks, pqs, pks = (q0, q1), (k0, k1), (pq0, pq1), (pk0, pk1)

    def tile_copy(src, dst, t, sem, r0, n, lead=(0,), dst_off=0):
        return lambda: pltpu.make_async_copy(
            src.bitcast(U32).at[(*lead, pl.ds(r0 // 2, n // 2), pl.ds(128 * t, 128))],
            dst.at[t, pl.ds(dst_off + r0 // 2, n // 2), :], sems.at[sem])

    def h_copy(t, c0, n, sem):
        return lambda: pltpu.make_async_copy(
            h_hbm.bitcast(U32).at[pl.ds(64 * c0, 64 * n), pl.ds(128 * t, 128)],
            hb.at[t, pl.ds(64 * c0, 64 * n), :], sems.at[sem])

    def conv_copies(cs, i, sem):
        out = [h_copy(4 * i + t, cs[0], len(cs), sem) for t in range(4)]
        out += [tile_copy(ak_hbm, kb, c, sem, L * i, L, dst_off=8) for c in cs]
        return out + [tile_copy(av_hbm, vb, c, sem, L * i, L) for c in cs]

    def whole(ref, sem):
        return [lambda: pltpu.make_async_copy(ref, ref, sems.at[sem])]

    def x_copies(r0, n, sem):
        return ([tile_copy(x_hbm, xb, c, sem, r0, n) for c in range(NT)],
                whole(xb.at[:, pl.ds(r0 // 2, n // 2), :], sem))

    def w_copies(src, dst, n0, n1, sem):
        return ([tile_copy(src, dst, n, sem, 0, D, lead=()) for n in range(n0, n1)],
                whole(dst.at[pl.ds(n0, n1 - n0)], sem))

    cp_x0 = [x_copies(256 * k, 256, k) for k in range(2)]
    cp_x1 = [x_copies(L + 128 * i, 128, 2 + i) for i in range(4)]
    cp_x = {s: x_copies(L * s, L, 4 + s) for s in (2, 3)}
    cp_wq = [w_copies(wq_hbm, wqb, n0, n1, 8 + k) for k, (n0, n1) in enumerate(W_STAGES)]
    cp_wk = [w_copies(wk_hbm, wkb, n0, n1, 11 + k) for k, (n0, n1) in enumerate(W_STAGES)]
    cp_wv = w_copies(wv_hbm, wvb, 0, NT, 14)
    cp_wo = w_copies(wo_hbm, wob, 0, NT, 15)
    cp_early = [conv_copies(SPLIT[0], i, 16 + i) for i in range(4)]
    cp_late = [cp for i in range(4) for cp in conv_copies(SPLIT[1], i, 20)]
    cp_q = ([tile_copy(aq_hbm, qb, c, 21, 0, S) for c in range(NT)], whole(qb, 21))
    cp_fwd = [lambda: pltpu.make_async_copy(fwd_hbm, fwd, sems.at[22])]
    cp_inv = [lambda: pltpu.make_async_copy(inv_hbm, inv, sems.at[23])]
    cp_small = [lambda: pltpu.make_async_copy(shift_hbm, shift_ref, sems.at[24]),
                lambda: pltpu.make_async_copy(ssmd_hbm, ssmd_ref, sems.at[24]),
                lambda: pltpu.make_async_copy(beta_hbm, beta_ref, sems.at[24])]

    def out_a(c):
        return [lambda: pltpu.make_async_copy(
            outa[c], out_hbm.bitcast(U32).at[0, :, pl.ds(128 * c, 128)], sems.at[25 + c])]

    def out_b(r0, n, rows_, sem):
        return lambda: pltpu.make_async_copy(
            outb.at[n, pl.ds(r0, rows_), :],
            out_hbm.at[0, pl.ds(r0, rows_), pl.ds(D + 128 * n, 128)], sems.at[sem])

    cp_oa = [out_a(c) for c in range(NT)]
    cp_ob3 = [[out_b(L * 3 + 128 * i, n, 128, 30) for n in range(NT)] for i in range(4)]
    ob_done = whole(outb, 30)

    def start(*groups):
        for g in groups:
            for cp in (g[0] if isinstance(g, tuple) else g):
                cp().start()

    def wait(*groups):
        for g in groups:
            for cp in (g[1] if isinstance(g, tuple) else g):
                cp().wait()

    def rows(i, n):
        return pl.ds(pl.multiple_of(i * n, n), n) if not isinstance(i, int) else pl.ds(i * n, n)

    lane = lax.broadcasted_iota(jnp.int32, (8, 128), 1)
    sub = lax.broadcasted_iota(jnp.int32, (8, 128), 0)

    def lanes(n):
        return lax.broadcasted_iota(jnp.int32, (n, 128), 1)

    recent = [None]
    seg = [0]

    def dot(a, b, dims=NN_DIMS, kind=4):
        out = _dot(a, b, dims)
        if kind & PACE_ON[seg[0]]:
            recent[0] = out
        return out

    current = {}

    def pace(zero):
        v = recent[0][-8:]
        recent[0] = None
        if "h" in current:
            hb[S // 128, rows(zero, 8), :] = _u32_word(v)
        if "k" in current:
            kb[NT, rows(zero, 8), :] = _u32_word(v)
        if "t" in current:
            th[current["t"]][N1 // 8, zero, 0, 0] = v
            if PACE_ALL[seg[0]] & 1:
                tx[current["t"]][N1 // 8, zero, 0, 0] = v
            if PACE_ALL[seg[0]] & 2:
                ub[16, zero, 0, 0] = v

    def qk_proj(s, i, want_pq, want_pk):
        p = s % 2
        tok = rows(4 * s + i, 64)
        for w_ref, dst, fdst, want, scale in (
                (wqb, qs[p], pqs[p], want_pq, DH ** -0.5 * LOG2E),
                (wkb, ks[p], pks[p], want_pk, None)):
            for n in range(NT):
                t = None
                for c in range(NT):
                    part = dot(_bf(xb[c, tok, :]), _bf(w_ref[n, 64 * c:64 * c + 64, :]))
                    t = part if t is None else t + part
                    if c < NT - 1:
                        yield 32
                dst[n, rows(i, 128), :] = (t if scale is None else t * scale).astype(BF16)
                if want:
                    fdst[n, rows(i, 128), :] = jnp.where(t > 0, t + 1.0, jnp.exp(t)).astype(BF16)
                yield 32

    def first_proj(n, js=range(4)):
        for w_ref, dst, scale in ((wqb, qs[0], DH ** -0.5 * LOG2E), (wkb, ks[0], None)):
            for j in js:
                t = None
                for c in range(NT):
                    part = dot(_bf(xb[c, rows(j, 64), :]), _bf(w_ref[n, 64 * c:64 * c + 64, :]))
                    t = part if t is None else t + part
                dst[n, rows(j, 128), :] = (t if scale is None else t * scale).astype(BF16)
                if scale is None:
                    pks[0][n, rows(j, 128), :] = jnp.where(t > 0, t + 1.0, jnp.exp(t)).astype(BF16)

    def untranspose(s, i, slot=0):
        ot = ots.bitcast(U32)
        for c in range(NT):
            onat[slot, c] = _u32(_bf(ot[s % 2, i, 64 * c:64 * c + 64, :]).T)

    def out_proj(s, i, slot=0, copies=None):
        for n in range(NT):
            t = None
            for c in range(NT):
                part = dot(_bf(onat[slot, c]), _bf(wob[n, 64 * c:64 * c + 64, :]))
                t = part if t is None else t + part
                if c < NT - 1:
                    yield 32
            outb[n, rows(4 * s + i, 128), :] = t.astype(BF16)
            if copies is not None:
                start([copies[n]])
            yield 32

    def tile_rows(r, n):
        return jnp.broadcast_to(r[None], (n // 8, 8, 128)).reshape(n, 128)

    class Group:
        def __init__(self, s, g, gi):
            self.s, self.g, self.gi = s, g, gi
            self.t0 = (80 * g) // 128
            self.off = 80 * g - 128 * self.t0
            self.t1 = jnp.minimum(self.t0 + 1, NT - 1)
            rel = (lane - self.off) & 127
            head = sum((rel >= a * DH).astype(jnp.int32) for a in range(1, 5))
            for a in range(4):
                hmask[gi, a] = jnp.where(head == a, np.uint32(0xFFFFFFFF), np.uint32(0))
            hsel[gi] = jnp.left_shift(1, head)
            self.have_keys, self.have_mem = set(), set()

        def window(self, ref, j, r0=0, n=64):
            ref = ref.bitcast(U32)
            at = pl.ds(64 * j + r0, n)
            return jnp.where(lanes(n) >= self.off, ref[self.t0, at, :], ref[self.t1, at, :])

        def keys(self, r0, r1):
            out = []
            for r in range(r0, r1, 64):
                at = pl.ds(r // 2, 32)
                if r in self.have_keys:
                    out.append(kwin[self.gi, at, :])
                else:
                    self.have_keys.add(r)
                    out.append(self.window(ks[self.s % 2], 0, r // 2, 32))
                    kwin[self.gi, at, :] = out[-1]
            return _bf(jnp.concatenate(out, axis=0))

        def park_values(self, j, v80):
            if self.s < NSEG - 1:
                vall[self.gi, j, 0:80, :] = v80
            ones8 = jnp.ones((8, 128), F32)
            for pr in range(2):
                for e in range(2):
                    r0 = 40 * pr + 16 * e
                    vhead[self.gi, j, r0 // 8] = jnp.concatenate(
                        [v80[r0:r0 + 24], ones8], axis=0).astype(BF16)

        def mem_read(self):
            for j in range(4):
                r = dot(mst[self.g, 0:88, :], _bf(self.window(pqs[self.s % 2], j)), NT_DIMS)
                coef = gtab[self.g] / (r[80:88] + 1e-6)
                cb = [jnp.broadcast_to(coef[a:a + 1], (8, 128)) for a in range(4)]
                for pr in range(2):
                    ca, cc = cb[2 * pr], cb[2 * pr + 1]
                    for e, scale in enumerate((ca, ca, jnp.where(sub < 4, ca, cc), cc, cc)):
                        r0 = 40 * pr + 8 * e
                        opart[self.gi, j, r0:r0 + 8, :] = r[r0:r0 + 8] * scale
                self.have_mem.add(j)
                yield 24

        def mem_update(self):
            acc = None
            for j in range(4):
                t = dot(vall[self.gi, j], _bf(self.window(pks[self.s % 2], j)))
                acc = t if acc is None else acc + t
                if j < 3:
                    yield 24
            for r in range(11):
                new = jnp.where(bmask[r] & hsel[self.gi] != 0, acc[8 * r:8 * r + 8], 0.0)
                at = pl.ds(8 * r, 8)
                mst[self.g, at, :] = new if self.s == 0 else mst[self.g, at, :] + new
            yield 24

        def logits(self, pr, j, slot):
            qw = self.window(qs[self.s % 2], j)
            qa = qw & tile_rows(hmask[self.gi, 2 * pr], 64)
            qh = qw & tile_rows(hmask[self.gi, 2 * pr + 1], 64)
            w_a = _bf(qa)
            w_b = _bf(jnp.concatenate([qh[32:64], qh[0:32]], axis=0))
            w_t = _bf(jnp.concatenate([qh[32:64], qa[32:64]], axis=0))
            n = 128 * j

            def park(t, e, r0, m):
                for r in range(0, t.shape[0], 8):
                    v = t[r:r + 8]
                    if e == 2:
                        v = v + cmask[2, r:r + 8, :]
                    elif r0 + r >= n:
                        v = v + cmask[e, r0 + r - n:r0 + r - n + 8, :]
                    slot[e % 2, 448 * (e // 2) + r0 + r:448 * (e // 2) + r0 + r + 8, :] = v
                    m = v if m is None else jnp.maximum(m, v)
                return m

            m_t = park(dot(self.keys(n + 64, n + 128), w_t, NT_DIMS, 1), 2, 0, None)
            yield 16 * LW[seg[0] % 4]
            cuts = list(range(0, n, QCH[seg[0]])) or [0]
            m = [None, None]
            for r0, r1 in zip(cuts, cuts[1:] + [n + 64]):
                for e, w in enumerate((w_a, w_b)):
                    m[e] = park(dot(self.keys(r0, r1), w, NT_DIMS, 1), e, r0, m[e])
                    if r1 == n + 64 and e == 1:
                        m_a = jnp.maximum(m[0], jnp.where(lane >= 64, m_t, NEG))
                        m_b = jnp.maximum(m[1], jnp.where(lane < 64, m_t, NEG))
                        m_a = jnp.broadcast_to(jnp.max(m_a, axis=0, keepdims=True), (8, 128))
                        m_b = jnp.broadcast_to(jnp.max(m_b, axis=0, keepdims=True), (8, 128))
                        slot[1, 448:456, :] = m_a
                        slot[1, 456:464, :] = m_b
                        slot[1, 464:472, :] = jnp.where(lane < 64, m_b, m_a)
                    yield (r1 - r0) // 4 * LW[seg[0] % 4]

    def attend(gi, g, parity, add_mem, pr, j, slot, need_values):
        def prob(e, r0, n, which):
            m2 = tile_rows(slot[1, 448 + 8 * which:456 + 8 * which, :], 16)
            return [jnp.exp2(slot[e, r:r + 16, :] - m2) for r in range(r0, r0 + n, 16)]

        res = [None, None]
        order = [(0, j), (1, j)] + [(e, kt) for e in range(2) for kt in range(j)]
        for n, (e, kt) in enumerate(order):
            need_values(kt)
            if n == 0:
                p_t = prob(0, 448, 64, 2)
            if kt < j:
                p = prob(e, 128 * kt, 128, e)
            else:
                mine = lanes(16) >= 64 if e == 0 else lanes(16) < 64
                p = prob(e, 128 * kt, 64, e) + [jnp.where(mine, t, 0.0) for t in p_t]
            t = dot(_bf(vhead.bitcast(U32)[gi, kt, 5 * pr + 2 * e]),
                    jnp.concatenate(p, axis=0).astype(BF16), kind=2)
            res[e] = t if res[e] is None else res[e] + t
            if n < len(order) - 1:
                yield 8 * AW[seg[0]]
        r_a = res[0]
        r_b = pltpu.roll(res[1], 64, 1)
        keep = 1.0 - gtab[g]
        keep_a = jnp.broadcast_to(keep[2 * pr:2 * pr + 1], (8, 128))
        keep_b = jnp.broadcast_to(keep[2 * pr + 1:2 * pr + 2], (8, 128))
        o_a = r_a[0:24] * tile_rows(keep_a / r_a[24:32], 24)
        o_b = r_b[0:24] * tile_rows(keep_b / r_b[24:32], 24)
        o = jnp.concatenate(
            [o_a[0:16], jnp.where(sub < 4, o_a[16:24], o_b[0:8]), o_b[8:24]], axis=0)
        if add_mem:
            o = o + opart[gi, j, 40 * pr:40 * pr + 40, :]
        if pr == 0:
            opart[gi, j, 0:40, :] = o
        else:
            o = jnp.concatenate([opart[gi, j, 0:40, :], o], axis=0)
            ots[parity, j, rows(g, 80), :] = o.astype(BF16)
        yield 8 * AW[seg[0]]

    def v_proj(s, i, groups, have):
        for j in range(4):
            acc = None
            for c in range(NT):
                t = dot(_bf(wvt[c, rows(i, 80), :]), _bf(xb[c, rows(4 * s + j, 64), :]), NT_DIMS)
                acc = t if acc is None else acc + t
                if c == NT - 1:
                    for gi in range(2):
                        groups[gi].park_values(j, acc[80 * gi:80 * gi + 80])
                    have.append(j)
                yield 40

    def chain(*gens):
        for g in gens:
            yield from g

    def units(s):
        return [(gi, pr, j) for gi in range(2) for pr in range(2)
                for j in (range(4) if (gi, pr) == (1, 1) else ORDER[s] if gi + pr else range(4))]

    def cost(j):
        return (48 + 64 * j) * LW[seg[0] % 4], (16 + 16 * j) * AW[seg[0]]

    def carried(u, g, parity):
        gi, pr, j = units(0)[u]
        return attend(gi, g, parity, True, pr, j, slots[u % NSLOT], lambda kt: None), cost(j)[1]

    def segment_step(s, i):
        seg[0] = s
        parts = {}
        if s < NSEG - 1:
            parts["qk"] = (qk_proj(s + 1, i, True, s + 1 < NSEG - 1), 1600)
        if s > 0:
            parts["out"] = (out_proj(s - 1, i), 800)
        if FORWARD[s]:
            parts["fwd"] = (fwd_fft(i, FORWARD[s]), 512 * len(FORWARD[s]))
        if INVERSE[s]:
            parts["inv"] = (inverse(INVERSE[s], (2 * i, 2 * i + 1)), 256 * len(INVERSE[s]))
        names = (("qk", "inv", "out", "fwd"), ("qk", "inv", "fwd", "out"),
                 ("inv", "fwd", "qk", "out"), ("qk", "inv", "out", "fwd"))[FILL_ORDER[s]]
        fill = _Paced([parts[n] for n in names if n in parts], sequential=FILL_ORDER[s] < 3)
        side = []
        if SPECTRUM[s]:
            side.append((spectra(SPECTRUM[s], [4 * i + a for a in range(4)]),
                         4 * SPEC_COST * len(SPECTRUM[s])))
        for c in SPLIT[s]:
            side += [(split_h(i, c), 144), (split_kv(i, c), 704)]
        side = _Paced(side, sequential=True)
        current.clear()
        recent[0] = None
        for _ in range(HEAD[s]):
            fill.step()
        if s > 0:
            untranspose(s - 1, i)
        vt = []
        groups = [Group(s, 2 * i + gi, gi) for gi in range(2)]
        reads = [grp.mem_read() for grp in groups if s > 0]
        updates = [grp.mem_update() for grp in groups if s < NSEG - 1]
        first = _Paced([(chain(*reads[:1], v_proj(s, i, groups, vt), *reads[1:], *updates),
                         800 + 96 * (len(reads) + len(updates)))])
        total = first.total + fill.total
        held = 96 * (s > 0) + 160

        def need_values(kt):
            while len(vt) <= kt:
                first.step()

        def pad(fraction, u):
            target = total * fraction / (1 + TAIL[s])
            early = min(target, held if u < DEPTH else first.total)
            first.advance(early / first.total)
            fill.advance((target - early) / fill.total)
            goal = fraction * SIDE_SPEED[s]
            if side.live and side.done < goal * side.total and recent[0] is not None:
                pace(jnp.minimum(i, 3))
                side.advance(goal)

        todo = units(s)
        whole = sum(sum(cost(j)) for _, _, j in todo)
        done = 0
        for u, (gi, pr, j) in enumerate(todo):
            streams = [(groups[gi].logits(pr, j, slots[u % NSLOT]), cost(j)[0])]
            v = u - DEPTH
            if v < 0:
                streams.append(carried(v + len(todo), (2 * i + 7) & 7,
                                       jnp.where(i > 0, s % 2, 1 - s % 2)))
            else:
                gi, pr, j = todo[v]
                while s > 0 and j not in groups[gi].have_mem:
                    first.step()
                streams.append((attend(gi, 2 * i + gi, s % 2, s > 0, pr, j, slots[v % NSLOT],
                                       need_values), cost(j)[1]))
            att = _Paced(streams[::-1], sequential=u == len(todo) - 1)
            while att.live:
                att.step()
                pad((done + att.done) / whole, u)
            done += att.total
        first.finish()
        fill.finish()
        side.finish()

    def split_h(i, c):
        current.clear()
        current["h"] = True
        for t in range(4):
            ht[c, 64 * t:64 * t + 64, :] = _u32(
                _bf(hb[4 * i + t, 64 * c:64 * c + 64, :]).T)
            yield 4
        for q in range(2):
            for j in range(8):
                wa = ht[c, pl.ds(128 * q + j, 8, stride=8), :]
                wb = ht[c, pl.ds(128 * q + 64 + j, 8, stride=8), :]
                hp[c][2 * j, rows(2 * i + q, 8), :] = _pack2(_lo(wa), _lo(wb))
                hp[c][2 * j + 1, rows(2 * i + q, 8), :] = _pack2(_hi(wa), _hi(wb))
                if j % 2:
                    yield 16

    def split_kv(i, c):
        current.clear()
        current["k"] = True
        taps = [wtab[c, j] for j in range(KS)]
        for q in range(2):
            blk = 2 * i + q
            base = [blk * 128 + 64 * e for e in range(2)]
            hist = []
            for e in range(2):
                w2 = kb[c, pl.ds(base[e] + 6, 8, stride=8), :]
                w1 = kb[c, pl.ds(base[e] + 7, 8, stride=8), :]
                hist.append([_hi(w2), _lo(w1), _hi(w1)])
            for j in range(8):
                kv = [[None, None], [None, None]]
                for e in range(2):
                    kw = kb[c, pl.ds(base[e] + 8 + j, 8, stride=8), :]
                    vw = vb[c, pl.ds(base[e] + j, 8, stride=8), :]
                    kp = hist[e] + [_lo(kw), _hi(kw)]
                    for half, part in enumerate((_lo, _hi)):
                        acc = kp[3 + half] * taps[0]
                        for d in range(1, KS):
                            acc = acc + kp[3 + half - d] * taps[d]
                        kv[half][e] = acc * part(vw)
                        kvf[c][2 * j + half, rows(2 * blk + e, 8), :] = kv[half][e]
                    hist[e] = kp[2:]
                    if e == 0:
                        yield 22
                for half in range(2):
                    xp[c][2 * j + half, rows(blk, 8), :] = _pack2(*kv[half])
                yield 22

    def fwd_fft(i, cs):
        for c in cs:
            for src, dst in ((hp[c], th[c]), (xp[c], tx[c])):
                g = [dot(_bf(fwd[4 * a + i]), _bf(src[4 * a + i])) for a in range(4)]
                for r in range(0, 2 * N1, 16):
                    z = _radix4(*[(g[a][r:r + 8], g[a][r + 8:r + 16]) for a in range(4)], 1)
                    for cc in range(4):
                        dst[r // 16, cc, i, 0] = z[cc][0]
                        dst[r // 16, cc, i, 1] = z[cc][1]
                yield 256

    def spectrum(c, m, slot):
        current.clear()
        current["t"] = c
        for cc in range(4):
            zh = _radix4_tw(*[(th[c][m, cc, b, 0], th[c][m, cc, b, 1]) for b in range(4)], 1, cc)
            yield 17
            zx = _radix4_tw(*[(tx[c][m, cc, b, 0], tx[c][m, cc, b, 1]) for b in range(4)], 1, cc)
            yield 17
            y = [(x[0] * h[0] - x[1] * h[1], x[0] * h[1] + x[1] * h[0]) for x, h in zip(zx, zh)]
            yield 17
            u = _radix4(*y, -1)
            for b in range(4):
                ub[slot, b, cc, 0] = u[b][0]
                ub[slot, b, cc, 1] = u[b][1]
            yield 17
        if SPEC_V[seg[0]]:
            return

        yield from spectrum_end(c, m, slot)

    def spectrum_end(c, m, slot):
        for b in range(4):
            z = _radix4_tw(*[(ub[slot, b, cc, 0], ub[slot, b, cc, 1]) for cc in range(4)], -1, b)
            for a in range(4):
                yb[c][4 * a + b, rows(m, 8), :] = _pack2(*z[a])
            yield 17

    SPEC_COST = 17 * 20

    def spectra(cs, ms, slot0=0):
        prev = None
        for slot, (c, m) in enumerate(((c, m) for c in cs for m in ms), slot0):
            yield from spectrum(c, m, slot)
            if SPEC_V[seg[0]] and prev is not None:
                yield from spectrum_end(*prev)
            prev = (c, m, slot)
        if SPEC_V[seg[0]]:
            yield from spectrum_end(*prev)

    def inverse(cs, jps):
        for c in cs:
            for jp in jps:
                w = qb[c, pl.ds(jp, N1, stride=8), :]
                res = []
                for e, part in enumerate((_lo, _hi)):
                    n2 = 2 * jp + e
                    y = dot(_bf(inv[n2, 0]), _bf(yb[c][n2, 0:64, :]))
                    yield 32
                    y = y + dot(_bf(inv[n2, 1]), _bf(yb[c][n2, 64:128, :]))
                    res.append(part(w) * (y + kvf[c][n2] * tile_rows(wtab[c, KS], N1)))
                    if e == 0:
                        yield 32
                outa[c][pl.ds(jp, N1, stride=8), :] = _pack2(*res)
                yield 32

    start(cp_wq[0], cp_wk[0], cp_x0[0], cp_x0[1], cp_wq[1], cp_wk[1])
    sem_zero[0] = 0
    kk = lax.broadcasted_iota(jnp.int32, (64, 128), 0)
    ll = lax.broadcasted_iota(jnp.int32, (64, 128), 1)
    cmask[0] = jnp.where(kk <= ll, 0.0, NEG)
    cmask[1] = jnp.where((ll < 64) | (kk <= ll - 64), 0.0, NEG)
    cmask[2] = jnp.where(kk <= (ll & 63), 0.0, NEG)
    for r in range(11):
        row = sub + 8 * r
        hr = sum((row >= a * DH).astype(jnp.int32) for a in range(1, 4)) if r < 10 else row - 80
        bmask[r] = jnp.left_shift(1, hr)
    for gi in range(2):
        for j in range(4):
            vall[gi, j, 80:88, :] = jnp.ones((8, 128), F32)
    for c in range(NT):
        kb[c, 0:8, :] = jnp.zeros((8, 128), U32)
    for u in range(16 - DEPTH, 16):
        slots[u % NSLOT][...] = jnp.zeros((2, 512, 128), F32)
    vhead[1] = jnp.ones(vhead.shape[1:], BF16)
    opart[1] = jnp.zeros(opart.shape[1:], F32)
    with jax.named_scope("prologue"):
        wait(cp_wq[0], cp_wk[0], cp_x0[0])
        start(cp_wq[2], cp_wk[2], cp_wv, cp_small, cp_x1[0], cp_early[0])
        first_proj(0, (0, 1))
        wait(cp_x0[1])
        first_proj(0, (2, 3))
        wait(cp_wq[1], cp_wk[1])
        for n in range(*W_STAGES[1]):
            first_proj(n)
        wait(cp_wq[2], cp_wk[2])
        first_proj(W_STAGES[2][0])
        wait(cp_wv, cp_small)
        start(cp_x1[1], cp_early[1])
        taps_t = shift_ref[...].astype(F32)
        skip = ssmd_ref[...].astype(F32)
        for c in range(NT):
            for j in range(KS):
                wtab[c, j] = jnp.broadcast_to(taps_t[j:j + 1, 128 * c:128 * c + 128], (8, 128))
            wtab[c, KS] = jnp.broadcast_to(skip[c:c + 1], (8, 128))
        gates = jax.nn.sigmoid(beta_ref[...].astype(F32))
        gcol = jnp.broadcast_to(gates, (8, H)).T
        gcol = jnp.broadcast_to(gcol[:, 0:1], (H, 128))
        for g in range(8):
            gtab[g] = jnp.concatenate([gcol[4 * g:4 * g + 4]] * 2, axis=0)
        for n in range(NT):
            for c in range(NT):
                wvt[c, rows(n, 64), :] = _u32(_bf(wvb[n, 64 * c:64 * c + 64, :]).T)
        for n in range(W_STAGES[2][0] + 1, NT):
            first_proj(n)
    start(cp_wo, cp_x[2])

    def segment(s):
        def body(i, carry):
            if s == 0:
                for j in range(4):
                    @pl.when(i == j)
                    def _():
                        wait(cp_x1[j], cp_early[j])
                        start(*((cp_x1[2], cp_early[2]), (cp_x1[3], cp_early[3]),
                                (cp_fwd, cp_late), (cp_x[3],))[j])
            segment_step(s, i)
            if s > 0:
                r0 = pl.multiple_of(L * (s - 1) + 128 * i, 128)
                start([out_b(r0, n, 128, 30) for n in range(NT)])
            return carry

        with jax.named_scope(f"seg{s}"):
            lax.fori_loop(0, 4, body, 0)

    segment(0)
    wait(cp_fwd, cp_x[2], cp_wo, cp_late)
    start(cp_inv, cp_q)
    segment(1)
    wait(cp_x[3])
    segment(2)
    wait(cp_inv, cp_q)
    segment(3)
    start(*[cp_oa[c] for c in INVERSE[3]])
    with jax.named_scope("epilogue"):
        seg[0] = 4
        current.clear()
        recent[0] = None
        last = NT - 1
        rest_tiles = [c for c in range(last) if c not in INVERSE[3]]
        side = _Paced([(spectra((last,), range(16)), 16 * SPEC_COST)])
        span = 1024 * len(rest_tiles) + 800 * MID
        done = 0

        def run(streams):
            nonlocal done
            work = _Paced(streams)
            while work.live:
                before = work.done
                work.step()
                done += work.done - before
                if side.live and side.done < done / span * side.total and recent[0] is not None:
                    pace(sem_zero[0])
                    side.advance(done / span)

        for c in rest_tiles:
            streams = [(inverse((c,), range(8)), 1024)]
            if c == rest_tiles[0]:
                tail = [carried(u, 7, 1) for u in range(16 - DEPTH, 16)]
                streams.append((chain(*[g for g, _ in tail]), sum(w for _, w in tail)))
            run(streams)
            if c == rest_tiles[0]:
                for i in range(4):
                    untranspose(3, i, i)
            start(cp_oa[c])
        for i in range(4):
            if i == MID:
                side.finish()
                run([(inverse((last,), range(8)), 1024)])
                start(cp_oa[last])
            run([(out_proj(3, i, i, cp_ob3[i]), 800)])
    wait(*cp_oa, ob_done)


@jax.jit
def pallas_concat_heads__ssm_conv_h3__memory_aug_infini_attn__prompt_kernel(
    A_q: jax.Array,
    A_k: jax.Array,
    A_v: jax.Array,
    A_shift_k: jax.Array,
    A_ssm_k: jax.Array,
    A_ssm_D: jax.Array,
    B_x: jax.Array,
    B_wq: jax.Array,
    B_wk: jax.Array,
    B_wv: jax.Array,
    B_wo: jax.Array,
    B_beta: jax.Array,
):
    hbm = pl.BlockSpec(memory_space=pltpu.HBM)
    seg_tiles = pltpu.VMEM((NT, L, 128), BF16)
    seq_tiles = pltpu.VMEM((NT, S // 2, 128), U32)
    w_tiles = pltpu.VMEM((NT, D // 2, 128), U32)
    scratch = [
        pltpu.VMEM((KS, D), BF16),
        pltpu.VMEM((NT, 128), BF16),
        pltpu.VMEM((1, H), BF16),
        seq_tiles,
        w_tiles, w_tiles, w_tiles, w_tiles, w_tiles,
        pltpu.VMEM((S // 128 + 1, D // 2, 128), U32),
        pltpu.VMEM((NT, 256, 128), U32),
        pltpu.VMEM((NT + 1, S // 2 + 8, 128), U32),
        seq_tiles, seq_tiles,
        pltpu.VMEM((N2, N1, 128), U32),
        pltpu.VMEM((N2, 2, N1 // 2, 128), U32),
        pltpu.VMEM((17, 4, 4, 2, 8, 128), F32),
        pltpu.VMEM((NT, S, 128), BF16),
        pltpu.VMEM((NT, KS + 1, 8, 128), F32),
        pltpu.VMEM((8, 8, 128), F32),
        pltpu.VMEM((3, 64, 128), F32),
        seg_tiles, seg_tiles, seg_tiles, seg_tiles,
        seg_tiles, seg_tiles, seg_tiles, seg_tiles,
        pltpu.VMEM((2, 4, D, 128), BF16),
        pltpu.VMEM((8, 88, 128), F32),
        pltpu.VMEM((2, 4, 8, 128), U32),
        pltpu.VMEM((2, 8, 128), jnp.int32),
        pltpu.VMEM((11, 8, 128), jnp.int32),
        pltpu.VMEM((2, L // 2, 128), U32),
        pltpu.VMEM((2, 4, 88, 128), F32),
        pltpu.VMEM((2, 4, 8, 32, 128), BF16),
        pltpu.VMEM((2, 4, 80, 128), F32),
        pltpu.VMEM((4, NT, 64, 128), U32),
        pltpu.SMEM((1,), jnp.int32),
        pltpu.SemaphoreType.DMA((31,)),
    ]
    scratch += [pltpu.VMEM((N2, N1 // 2, 128), U32)] * (2 * NT)
    scratch += [pltpu.VMEM((N1 // 8 + 1, 4, 4, 2, 8, 128), F32)] * (2 * NT)
    scratch += [pltpu.VMEM((N2, N1, 128), U32)] * NT
    scratch += [pltpu.VMEM((N2, N1, 128), F32)] * NT
    scratch += [pltpu.VMEM((S // 2, 128), U32)] * NT
    scratch += [pltpu.VMEM((2, 512, 128), F32)] * NSLOT
    return pl.pallas_call(
        _kernel,
        out_shape=jax.ShapeDtypeStruct((1, S, 2 * D), BF16),
        in_specs=[hbm] * 14,
        out_specs=hbm,
        scratch_shapes=scratch,
        compiler_params=pltpu.CompilerParams(vmem_limit_bytes=110 * 1024 * 1024),
        name="h3_infini",
    )(A_q, A_k, A_v, A_shift_k.T, A_ssm_k, A_ssm_D.reshape(NT, 128), B_x, B_wq, B_wk, B_wv, B_wo,
      B_beta.reshape(1, H), _FWD, _INV)
```

```python
import math

import jax
import jax.numpy as jnp
import numpy as np
from jax import lax
from jax.experimental import pallas as pl
from jax.experimental.pallas import tpu as pltpu

S = 2048
D = 640
NT = D // 128
H = 32
DH = D // H
NSEG = 4
L = S // NSEG
KS = 4
N1, N2 = 128, 16

F32 = jnp.float32
BF16 = jnp.bfloat16
U32 = jnp.uint32
NN_DIMS = (((1,), (0,)), ((), ()))
NT_DIMS = (((1,), (1,)), ((), ()))
NEG = -1e30
LOG2E = 1.4426950408889634


def _pack_rows(a):
    u = a.astype(np.float32).astype(BF16).view(np.uint16).astype(np.uint32)
    return u[..., 0::2, :] | (u[..., 1::2, :] << 16)


def _dft_tables():
    k1 = np.arange(N1)
    fwd = np.zeros((N2, 2 * N1, N1), np.float64)
    inv = np.zeros((N2, N1, 2 * N1), np.float64)
    kappa = np.arange(N1)
    n1_in = 16 * (kappa // 16) + 8 * (kappa % 2) + (kappa % 16) // 2
    row_re = 16 * (k1 // 8) + k1 % 8
    for n2 in range(N2):
        ang = 2.0 * np.pi * np.outer(k1 + 0.25, N2 * n1_in + n2) / S
        fwd[n2, row_re] = np.cos(ang)
        fwd[n2, row_re + 8] = np.sin(ang)
        ang = 2.0 * np.pi * np.outer(N2 * np.arange(N1) + n2, k1 + 0.25) / S
        inv[n2][:, 2 * k1] = np.cos(ang) / S
        inv[n2][:, 2 * k1 + 1] = np.sin(ang) / S
    inv = inv.reshape(N2, N1, 2, N1).transpose(0, 2, 1, 3)
    return _pack_rows(fwd), _pack_rows(inv)


_FWD, _INV = _dft_tables()


def _dot(a, b, dims=NN_DIMS):
    return lax.dot_general(a, b, dims, preferred_element_type=F32)


def _u32(x):
    return pltpu.bitcast(x, U32)


def _bf(x):
    return pltpu.bitcast(x, BF16)


def _u32_word(x):
    return lax.bitcast_convert_type(x, U32)


def _pack2(a, b):
    return pltpu.pack_elementwise([a, b], packed_dtype=BF16).astype(U32)


def _lo(w):
    return pltpu.unpack_elementwise(w, index=0, packed_dtype=BF16, unpacked_dtype=F32)


def _hi(w):
    return pltpu.unpack_elementwise(w, index=1, packed_dtype=BF16, unpacked_dtype=F32)


def _radix4(x0, x1, x2, x3, sign):
    ar, ai = x0[0] + x2[0], x0[1] + x2[1]
    br, bi = x0[0] - x2[0], x0[1] - x2[1]
    cr, ci = x1[0] + x3[0], x1[1] + x3[1]
    dr, di = x1[0] - x3[0], x1[1] - x3[1]
    y0 = (ar + cr, ai + ci)
    y2 = (ar - cr, ai - ci)
    yp = (br - di, bi + dr)
    ym = (br + di, bi - dr)
    return (y0, yp, y2, ym) if sign > 0 else (y0, ym, y2, yp)


def _twiddle(x, e, sign):
    xr, xi = x
    if e == 0:
        return x
    if e == 4:
        return (-xi, xr) if sign > 0 else (xi, -xr)
    r = math.sqrt(0.5)
    if e == 2:
        return ((xr - xi) * r, (xr + xi) * r) if sign > 0 else ((xr + xi) * r, (xi - xr) * r)
    if e == 6:
        return ((xr + xi) * -r, (xr - xi) * r) if sign > 0 else ((xi - xr) * r, (xr + xi) * -r)
    c, s = math.cos(math.pi * e / 8), sign * math.sin(math.pi * e / 8)
    return (xr * c - xi * s, xr * s + xi * c)


def _radix4_tw(x0, x1, x2, x3, sign, b):
    if b != 2:
        return _radix4(x0, _twiddle(x1, b, sign), _twiddle(x2, 2 * b, sign),
                       _twiddle(x3, 3 * b, sign), sign)
    x1, x3 = _twiddle(x1, 2, sign), _twiddle(x3, 6, sign)
    if sign > 0:
        ar, ai = x0[0] - x2[1], x0[1] + x2[0]
        br, bi = x0[0] + x2[1], x0[1] - x2[0]
    else:
        ar, ai = x0[0] + x2[1], x0[1] - x2[0]
        br, bi = x0[0] - x2[1], x0[1] + x2[0]
    cr, ci = x1[0] + x3[0], x1[1] + x3[1]
    dr, di = x1[0] - x3[0], x1[1] - x3[1]
    y0 = (ar + cr, ai + ci)
    y2 = (ar - cr, ai - ci)
    yp = (br - di, bi + dr)
    ym = (br + di, bi - dr)
    return (y0, yp, y2, ym) if sign > 0 else (y0, ym, y2, yp)


class _Paced:
    def __init__(self, streams, sequential=False):
        self.live = [[g, total, 0] for g, total in streams if total]
        self.total = sum(total for _, total in streams)
        self.done = 0
        self.sequential = sequential

    def step(self):
        cur = self.live[0] if self.sequential else min(self.live, key=lambda e: e[2] / e[1])
        cost = next(cur[0], None)
        if cost is None:
            self.live.remove(cur)
        else:
            cur[2] += cost
            self.done += cost

    def advance(self, fraction):
        while self.live and self.done < fraction * self.total:
            self.step()

    def finish(self):
        self.advance(math.inf)


SPLIT = ((0, 1, 2), (3, 4), (), ())
FORWARD = ((), (0, 1), (2, 3, 4), ())
SPECTRUM = ((), (), (0, 1), (2, 3))
INVERSE = ((), (), (), (0, 1))
DEPTH = 3
NSLOT = 4
ORDER = ((1, 3, 0, 2), (3, 2, 1, 0), (0, 2, 1, 3), (0, 1, 2, 3))
TAIL = (-0.03, -0.03, 0.02, -0.03)
LW = (1.0, 1.0, 1.0, 1.0)
AW = (4.0, 2.0, 4.0, 2.0, 3.0)
QCH = (128, 256, 128, 128)
HEAD = (4, 6, 6, 6)
FILL_ORDER = (0, 1, 1, 2)
PACE_ON = (3, 3, 7, 7, 7)
SIDE_SPEED = (1.03, 1.0, 1.03, 1.0)
MID = 3
PACE_ALL = (3, 2, 2, 3, 0)
SPEC_V = (0, 0, 0, 0, 1)
W_STAGES = ((0, 1), (1, 3), (3, 5))


def _kernel(aq_hbm, ak_hbm, av_hbm, shift_hbm, h_hbm, ssmd_hbm, x_hbm, wq_hbm, wk_hbm,
            wv_hbm, wo_hbm, beta_hbm, fwd_hbm, inv_hbm, out_hbm, shift_ref, ssmd_ref, beta_ref,
            xb, wqb, wkb, wvb, wob, wvt, hb, ht, kb, vb, qb, fwd, inv,
            ub, outb, wtab, gtab, cmask,
            q0, q1, k0, k1, pq0, pq1, pk0, pk1, ots, mst,
            hmask, hsel, bmask, kwin, vall, vhead, opart, onat, sem_zero, sems, *rest):
    xp, hp, tx, th, yb, kvf, outa = (rest[NT * k:NT * k + NT] for k in range(7))
    slots = rest[7 * NT:]
    qs, ks, pqs, pks = (q0, q1), (k0, k1), (pq0, pq1), (pk0, pk1)

    def copy(src, dst, sem):
        return [lambda: pltpu.make_async_copy(src, dst, sems.at[sem])]

    def tiles(src, dst, sem, r0, n, ts=range(NT), off=0):
        src = src.bitcast(U32)
        lead = (0,) * (len(src.shape) - 2)
        return [cp for t in ts for cp in copy(
            src.at[lead + (pl.ds(r0 // 2, n // 2), pl.ds(128 * t, 128))],
            dst.at[t, pl.ds(off + r0 // 2, n // 2), :], sem)]

    def conv_inputs(cs, r0, n, sem):
        return (tiles(h_hbm, hb, sem, 128 * cs[0], 128 * len(cs), range(r0 // 128, (r0 + n) // 128))
                + tiles(ak_hbm, kb, sem, r0, n, cs, off=8) + tiles(av_hbm, vb, sem, r0, n, cs))

    def w_stage(k, sem):
        return (tiles(wq_hbm, wqb, sem, 0, D, range(*W_STAGES[k]))
                + tiles(wk_hbm, wkb, sem, 0, D, range(*W_STAGES[k])))

    cp_first = w_stage(0, 0) + tiles(x_hbm, xb, 0, 0, 256)
    cp_x0 = tiles(x_hbm, xb, 1, 256, 256)
    cp_w1, cp_w2 = w_stage(1, 2), w_stage(2, 3)
    cp_wv = (tiles(wv_hbm, wvb, 0, 0, D) + copy(shift_hbm, shift_ref, 0)
             + copy(ssmd_hbm, ssmd_ref, 0) + copy(beta_hbm, beta_ref, 0))
    cp_step = [tiles(x_hbm, xb, sem, L + 128 * i, 128) + conv_inputs(SPLIT[0], L * i, L, sem)
               for i, sem in enumerate((4, 0, 1, 2))]
    cp_seg1 = (tiles(wo_hbm, wob, 3, 0, D) + tiles(x_hbm, xb, 3, 2 * L, L)
               + copy(fwd_hbm, fwd, 3) + conv_inputs(SPLIT[1], 0, S, 3))
    cp_seg2 = (tiles(x_hbm, xb, 4, 3 * L, L) + copy(inv_hbm, inv, 4)
               + tiles(aq_hbm, qb, 4, 0, S))
    cp_oa = [copy(outa[c].at[pl.ds(0, S // 2), :],
                  out_hbm.bitcast(U32).at[0, :, pl.ds(128 * c, 128)], 0) for c in range(NT)]

    def out_b(tile, ns=range(NT)):
        at = pl.ds(128 * tile if isinstance(tile, int) else pl.multiple_of(128 * tile, 128), 128)
        return [cp for n in ns for cp in copy(
            outb.at[n, at, :], out_hbm.at[0, at, pl.ds(D + 128 * n, 128)], 1)]

    all_of_b = copy(outb, outb, 1)

    def start(*groups):
        for g in groups:
            for cp in g:
                cp().start()

    def wait(*groups):
        for g in groups:
            for cp in g:
                cp().wait()

    def rows(i, n):
        return pl.ds(pl.multiple_of(i * n, n), n) if not isinstance(i, int) else pl.ds(i * n, n)

    lane = lax.broadcasted_iota(jnp.int32, (8, 128), 1)
    sub = lax.broadcasted_iota(jnp.int32, (8, 128), 0)

    def lanes(n):
        return lax.broadcasted_iota(jnp.int32, (n, 128), 1)

    recent = [None]
    seg = [0]

    def dot(a, b, dims=NN_DIMS, kind=4):
        out = _dot(a, b, dims)
        if kind & PACE_ON[seg[0]]:
            recent[0] = out
        return out

    current = {}

    def pace(zero):
        v = recent[0][-8:]
        recent[0] = None
        if "h" in current:
            hb[S // 128, rows(zero, 8), :] = _u32_word(v)
        if "k" in current:
            kb[NT, rows(zero, 8), :] = _u32_word(v)
        if "t" in current:
            th[current["t"]][N1 // 8, zero, 0, 0] = v
            if PACE_ALL[seg[0]] & 1:
                tx[current["t"]][N1 // 8, zero, 0, 0] = v
            if PACE_ALL[seg[0]] & 2:
                ub[16, zero, 0, 0] = v

    def qk_proj(s, i, want_pq, want_pk):
        p = s % 2
        tok = rows(4 * s + i, 64)
        for w_ref, dst, fdst, want, scale in (
                (wqb, qs[p], pqs[p], want_pq, DH ** -0.5 * LOG2E),
                (wkb, ks[p], pks[p], want_pk, None)):
            for n in range(NT):
                t = None
                for c in range(NT):
                    part = dot(_bf(xb[c, tok, :]), _bf(w_ref[n, 64 * c:64 * c + 64, :]))
                    t = part if t is None else t + part
                    if c < NT - 1:
                        yield 32
                dst[n, rows(i, 128), :] = (t if scale is None else t * scale).astype(BF16)
                if want:
                    fdst[n, rows(i, 128), :] = jnp.where(t > 0, t + 1.0, jnp.exp(t)).astype(BF16)
                yield 32

    def first_proj(n, js=range(4)):
        for w_ref, dst, scale in ((wqb, qs[0], DH ** -0.5 * LOG2E), (wkb, ks[0], None)):
            for j in js:
                t = None
                for c in range(NT):
                    part = dot(_bf(xb[c, rows(j, 64), :]), _bf(w_ref[n, 64 * c:64 * c + 64, :]))
                    t = part if t is None else t + part
                dst[n, rows(j, 128), :] = (t if scale is None else t * scale).astype(BF16)
                if scale is None:
                    pks[0][n, rows(j, 128), :] = jnp.where(t > 0, t + 1.0, jnp.exp(t)).astype(BF16)

    def untranspose(s, i, slot=0):
        ot = ots.bitcast(U32)
        for c in range(NT):
            onat[slot, c] = _u32(_bf(ot[s % 2, i, 64 * c:64 * c + 64, :]).T)

    def out_proj(s, i, slot=0):
        for n in range(NT):
            t = None
            for c in range(NT):
                part = dot(_bf(onat[slot, c]), _bf(wob[n, 64 * c:64 * c + 64, :]))
                t = part if t is None else t + part
                if c < NT - 1:
                    yield 32
            outb[n, rows(4 * s + i, 128), :] = t.astype(BF16)
            if s == NSEG - 1:
                start(out_b(4 * s + i, (n,)))
            yield 32

    def tile_rows(r, n):
        return jnp.broadcast_to(r[None], (n // 8, 8, 128)).reshape(n, 128)

    class Group:
        def __init__(self, s, g, gi):
            self.s, self.g, self.gi = s, g, gi
            self.t0 = (80 * g) // 128
            self.off = 80 * g - 128 * self.t0
            self.t1 = jnp.minimum(self.t0 + 1, NT - 1)
            rel = (lane - self.off) & 127
            head = sum((rel >= a * DH).astype(jnp.int32) for a in range(1, 5))
            for a in range(4):
                hmask[gi, a] = jnp.where(head == a, np.uint32(0xFFFFFFFF), np.uint32(0))
            hsel[gi] = jnp.left_shift(1, head)
            self.have_keys, self.have_mem = set(), set()

        def window(self, ref, j, r0=0, n=64):
            ref = ref.bitcast(U32)
            at = pl.ds(64 * j + r0, n)
            return jnp.where(lanes(n) >= self.off, ref[self.t0, at, :], ref[self.t1, at, :])

        def keys(self, r0, r1):
            out = []
            for r in range(r0, r1, 64):
                at = pl.ds(r // 2, 32)
                if r in self.have_keys:
                    out.append(kwin[self.gi, at, :])
                else:
                    self.have_keys.add(r)
                    out.append(self.window(ks[self.s % 2], 0, r // 2, 32))
                    kwin[self.gi, at, :] = out[-1]
            return _bf(jnp.concatenate(out, axis=0))

        def park_values(self, j, v80):
            if self.s < NSEG - 1:
                vall[self.gi, j, 0:80, :] = v80
            ones8 = jnp.ones((8, 128), F32)
            for pr in range(2):
                for e in range(2):
                    r0 = 40 * pr + 16 * e
                    vhead[self.gi, j, r0 // 8] = jnp.concatenate(
                        [v80[r0:r0 + 24], ones8], axis=0).astype(BF16)

        def mem_read(self):
            for j in range(4):
                r = dot(mst[self.g, 0:88, :], _bf(self.window(pqs[self.s % 2], j)), NT_DIMS)
                coef = gtab[self.g] / (r[80:88] + 1e-6)
                cb = [jnp.broadcast_to(coef[a:a + 1], (8, 128)) for a in range(4)]
                for pr in range(2):
                    ca, cc = cb[2 * pr], cb[2 * pr + 1]
                    for e, scale in enumerate((ca, ca, jnp.where(sub < 4, ca, cc), cc, cc)):
                        r0 = 40 * pr + 8 * e
                        opart[self.gi, j, r0:r0 + 8, :] = r[r0:r0 + 8] * scale
                self.have_mem.add(j)
                yield 24

        def mem_update(self):
            acc = None
            for j in range(4):
                t = dot(vall[self.gi, j], _bf(self.window(pks[self.s % 2], j)))
                acc = t if acc is None else acc + t
                if j < 3:
                    yield 24
            for r in range(11):
                new = jnp.where(bmask[r] & hsel[self.gi] != 0, acc[8 * r:8 * r + 8], 0.0)
                at = pl.ds(8 * r, 8)
                mst[self.g, at, :] = new if self.s == 0 else mst[self.g, at, :] + new
            yield 24

        def logits(self, pr, j, slot):
            qw = self.window(qs[self.s % 2], j)
            qa = qw & tile_rows(hmask[self.gi, 2 * pr], 64)
            qh = qw & tile_rows(hmask[self.gi, 2 * pr + 1], 64)
            w_a = _bf(qa)
            w_b = _bf(jnp.concatenate([qh[32:64], qh[0:32]], axis=0))
            w_t = _bf(jnp.concatenate([qh[32:64], qa[32:64]], axis=0))
            n = 128 * j

            def park(t, e, r0, m):
                for r in range(0, t.shape[0], 8):
                    v = t[r:r + 8]
                    if e == 2:
                        v = v + cmask[2, r:r + 8, :]
                    elif r0 + r >= n:
                        v = v + cmask[e, r0 + r - n:r0 + r - n + 8, :]
                    slot[e % 2, 448 * (e // 2) + r0 + r:448 * (e // 2) + r0 + r + 8, :] = v
                    m = v if m is None else jnp.maximum(m, v)
                return m

            m_t = park(dot(self.keys(n + 64, n + 128), w_t, NT_DIMS, 1), 2, 0, None)
            yield 16 * LW[seg[0] % 4]
            cuts = list(range(0, n, QCH[seg[0]])) or [0]
            m = [None, None]
            for r0, r1 in zip(cuts, cuts[1:] + [n + 64]):
                for e, w in enumerate((w_a, w_b)):
                    m[e] = park(dot(self.keys(r0, r1), w, NT_DIMS, 1), e, r0, m[e])
                    if r1 == n + 64 and e == 1:
                        m_a = jnp.maximum(m[0], jnp.where(lane >= 64, m_t, NEG))
                        m_b = jnp.maximum(m[1], jnp.where(lane < 64, m_t, NEG))
                        m_a = jnp.broadcast_to(jnp.max(m_a, axis=0, keepdims=True), (8, 128))
                        m_b = jnp.broadcast_to(jnp.max(m_b, axis=0, keepdims=True), (8, 128))
                        slot[1, 448:456, :] = m_a
                        slot[1, 456:464, :] = m_b
                        slot[1, 464:472, :] = jnp.where(lane < 64, m_b, m_a)
                    yield (r1 - r0) // 4 * LW[seg[0] % 4]

    def attend(gi, g, parity, add_mem, pr, j, slot, need_values):
        def prob(e, r0, n, which):
            m2 = tile_rows(slot[1, 448 + 8 * which:456 + 8 * which, :], 16)
            return [jnp.exp2(slot[e, r:r + 16, :] - m2) for r in range(r0, r0 + n, 16)]

        res = [None, None]
        order = [(0, j), (1, j)] + [(e, kt) for e in range(2) for kt in range(j)]
        for n, (e, kt) in enumerate(order):
            need_values(kt)
            if n == 0:
                p_t = prob(0, 448, 64, 2)
            if kt < j:
                p = prob(e, 128 * kt, 128, e)
            else:
                mine = lanes(16) >= 64 if e == 0 else lanes(16) < 64
                p = prob(e, 128 * kt, 64, e) + [jnp.where(mine, t, 0.0) for t in p_t]
            t = dot(_bf(vhead.bitcast(U32)[gi, kt, 5 * pr + 2 * e]),
                    jnp.concatenate(p, axis=0).astype(BF16), kind=2)
            res[e] = t if res[e] is None else res[e] + t
            if n < len(order) - 1:
                yield 8 * AW[seg[0]]
        r_a = res[0]
        r_b = pltpu.roll(res[1], 64, 1)
        keep = 1.0 - gtab[g]
        keep_a = jnp.broadcast_to(keep[2 * pr:2 * pr + 1], (8, 128))
        keep_b = jnp.broadcast_to(keep[2 * pr + 1:2 * pr + 2], (8, 128))
        o_a = r_a[0:24] * tile_rows(keep_a / r_a[24:32], 24)
        o_b = r_b[0:24] * tile_rows(keep_b / r_b[24:32], 24)
        o = jnp.concatenate(
            [o_a[0:16], jnp.where(sub < 4, o_a[16:24], o_b[0:8]), o_b[8:24]], axis=0)
        if add_mem:
            o = o + opart[gi, j, 40 * pr:40 * pr + 40, :]
        if pr == 0:
            opart[gi, j, 0:40, :] = o
        else:
            o = jnp.concatenate([opart[gi, j, 0:40, :], o], axis=0)
            ots[parity, j, rows(g, 80), :] = o.astype(BF16)
        yield 8 * AW[seg[0]]

    def v_proj(s, i, groups, have):
        for j in range(4):
            acc = None
            for c in range(NT):
                t = dot(_bf(wvt[c, rows(i, 80), :]), _bf(xb[c, rows(4 * s + j, 64), :]), NT_DIMS)
                acc = t if acc is None else acc + t
                if c == NT - 1:
                    for gi in range(2):
                        groups[gi].park_values(j, acc[80 * gi:80 * gi + 80])
                    have.append(j)
                yield 40

    def chain(*gens):
        for g in gens:
            yield from g

    def units(s):
        return [(gi, pr, j) for gi in range(2) for pr in range(2)
                for j in (range(4) if (gi, pr) == (1, 1) else ORDER[s] if gi + pr else range(4))]

    def cost(j):
        return (48 + 64 * j) * LW[seg[0] % 4], (16 + 16 * j) * AW[seg[0]]

    def carried(u, g, parity):
        gi, pr, j = units(0)[u]
        return attend(gi, g, parity, True, pr, j, slots[u % NSLOT], lambda kt: None), cost(j)[1]

    def segment_step(s, i):
        seg[0] = s
        parts = {}
        if s < NSEG - 1:
            parts["qk"] = (qk_proj(s + 1, i, True, s + 1 < NSEG - 1), 1600)
        if s > 0:
            parts["out"] = (out_proj(s - 1, i), 800)
        if FORWARD[s]:
            parts["fwd"] = (fwd_fft(i, FORWARD[s]), 512 * len(FORWARD[s]))
        if INVERSE[s]:
            parts["inv"] = (inverse(INVERSE[s], (2 * i, 2 * i + 1)), 256 * len(INVERSE[s]))
        names = (("qk", "inv", "out", "fwd"), ("qk", "inv", "fwd", "out"),
                 ("inv", "fwd", "qk", "out"), ("qk", "inv", "out", "fwd"))[FILL_ORDER[s]]
        fill = _Paced([parts[n] for n in names if n in parts], sequential=FILL_ORDER[s] < 3)
        side = []
        if SPECTRUM[s]:
            side.append((spectra(SPECTRUM[s], [4 * i + a for a in range(4)]),
                         4 * SPEC_COST * len(SPECTRUM[s])))
        for c in SPLIT[s]:
            side += [(split_h(i, c), 144), (split_kv(i, c), 704)]
        side = _Paced(side, sequential=True)
        current.clear()
        recent[0] = None
        for _ in range(HEAD[s]):
            fill.step()
        if s > 0:
            untranspose(s - 1, i)
        vt = []
        groups = [Group(s, 2 * i + gi, gi) for gi in range(2)]
        reads = [grp.mem_read() for grp in groups if s > 0]
        updates = [grp.mem_update() for grp in groups if s < NSEG - 1]
        first = _Paced([(chain(*reads[:1], v_proj(s, i, groups, vt), *reads[1:], *updates),
                         800 + 96 * (len(reads) + len(updates)))])
        total = first.total + fill.total
        held = 96 * (s > 0) + 159

        def need_values(kt):
            while len(vt) <= kt:
                first.step()

        def pad(fraction, u):
            target = total * fraction / (1 + TAIL[s])
            early = min(target, held if u < DEPTH else first.total)
            first.advance(early / first.total)
            fill.advance((target - early) / fill.total)
            goal = fraction * SIDE_SPEED[s]
            if side.live and side.done < goal * side.total and recent[0] is not None:
                pace(jnp.minimum(i, 3))
                side.advance(goal)

        todo = units(s)
        whole = sum(sum(cost(j)) for _, _, j in todo)
        done = 0
        for u, (gi, pr, j) in enumerate(todo):
            streams = [(groups[gi].logits(pr, j, slots[u % NSLOT]), cost(j)[0])]
            v = u - DEPTH
            if v < 0:
                streams.append(carried(v + len(todo), (2 * i + 7) & 7,
                                       jnp.where(i > 0, s % 2, 1 - s % 2)))
            else:
                gi, pr, j = todo[v]
                while s > 0 and j not in groups[gi].have_mem:
                    first.step()
                streams.append((attend(gi, 2 * i + gi, s % 2, s > 0, pr, j, slots[v % NSLOT],
                                       need_values), cost(j)[1]))
            att = _Paced(streams[::-1], sequential=u == len(todo) - 1)
            while att.live:
                att.step()
                pad((done + att.done) / whole, u)
            done += att.total
        first.finish()
        fill.finish()
        side.finish()

    def split_h(i, c):
        current.clear()
        current["h"] = True
        for t in range(4):
            ht[c, 64 * t:64 * t + 64, :] = _u32(
                _bf(hb[4 * i + t, 64 * c:64 * c + 64, :]).T)
            yield 4
        for q in range(2):
            for j in range(8):
                wa = ht[c, pl.ds(128 * q + j, 8, stride=8), :]
                wb = ht[c, pl.ds(128 * q + 64 + j, 8, stride=8), :]
                hp[c][2 * j, rows(2 * i + q, 8), :] = _pack2(_lo(wa), _lo(wb))
                hp[c][2 * j + 1, rows(2 * i + q, 8), :] = _pack2(_hi(wa), _hi(wb))
                if j % 2:
                    yield 16

    def split_kv(i, c):
        current.clear()
        current["k"] = True
        taps = [wtab[c, j] for j in range(KS)]
        for q in range(2):
            blk = 2 * i + q
            base = [blk * 128 + 64 * e for e in range(2)]
            hist = []
            for e in range(2):
                w2 = kb[c, pl.ds(base[e] + 6, 8, stride=8), :]
                w1 = kb[c, pl.ds(base[e] + 7, 8, stride=8), :]
                hist.append([_hi(w2), _lo(w1), _hi(w1)])
            for j in range(8):
                kv = [[None, None], [None, None]]
                for e in range(2):
                    kw = kb[c, pl.ds(base[e] + 8 + j, 8, stride=8), :]
                    vw = vb[c, pl.ds(base[e] + j, 8, stride=8), :]
                    kp = hist[e] + [_lo(kw), _hi(kw)]
                    for half, part in enumerate((_lo, _hi)):
                        acc = kp[3 + half] * taps[0]
                        for d in range(1, KS):
                            acc = acc + kp[3 + half - d] * taps[d]
                        kv[half][e] = acc * part(vw)
                        kvf[c][2 * j + half, rows(2 * blk + e, 8), :] = kv[half][e]
                    hist[e] = kp[2:]
                    if e == 0:
                        yield 22
                for half in range(2):
                    xp[c][2 * j + half, rows(blk, 8), :] = _pack2(*kv[half])
                yield 22

    def fwd_fft(i, cs):
        for c in cs:
            for src, dst in ((hp[c], th[c]), (xp[c], tx[c])):
                g = [dot(_bf(fwd[4 * a + i]), _bf(src[4 * a + i])) for a in range(4)]
                for r in range(0, 2 * N1, 16):
                    z = _radix4(*[(g[a][r:r + 8], g[a][r + 8:r + 16]) for a in range(4)], 1)
                    for cc in range(4):
                        dst[r // 16, cc, i, 0] = z[cc][0]
                        dst[r // 16, cc, i, 1] = z[cc][1]
                yield 256

    def spectrum(c, m, slot):
        current.clear()
        current["t"] = c
        for cc in range(4):
            zh = _radix4_tw(*[(th[c][m, cc, b, 0], th[c][m, cc, b, 1]) for b in range(4)], 1, cc)
            yield 17
            zx = _radix4_tw(*[(tx[c][m, cc, b, 0], tx[c][m, cc, b, 1]) for b in range(4)], 1, cc)
            yield 17
            y = [(x[0] * h[0] - x[1] * h[1], x[0] * h[1] + x[1] * h[0]) for x, h in zip(zx, zh)]
            yield 17
            u = _radix4(*y, -1)
            for b in range(4):
                ub[slot, b, cc, 0] = u[b][0]
                ub[slot, b, cc, 1] = u[b][1]
            yield 17
        if SPEC_V[seg[0]]:
            return

        yield from spectrum_end(c, m, slot)

    def spectrum_end(c, m, slot):
        for b in range(4):
            z = _radix4_tw(*[(ub[slot, b, cc, 0], ub[slot, b, cc, 1]) for cc in range(4)], -1, b)
            for a in range(4):
                yb[c][4 * a + b, rows(m, 8), :] = _pack2(*z[a])
            yield 17

    SPEC_COST = 17 * 20

    def spectra(cs, ms, slot0=0):
        prev = None
        for slot, (c, m) in enumerate(((c, m) for c in cs for m in ms), slot0):
            yield from spectrum(c, m, slot)
            if SPEC_V[seg[0]] and prev is not None:
                yield from spectrum_end(*prev)
            prev = (c, m, slot)
        if SPEC_V[seg[0]]:
            yield from spectrum_end(*prev)

    def inverse(cs, jps):
        for c in cs:
            for jp in jps:
                w = qb[c, pl.ds(jp, N1, stride=8), :]
                res = []
                for e, part in enumerate((_lo, _hi)):
                    n2 = 2 * jp + e
                    y = dot(_bf(inv[n2, 0]), _bf(yb[c][n2, 0:64, :]))
                    yield 32
                    y = y + dot(_bf(inv[n2, 1]), _bf(yb[c][n2, 64:128, :]))
                    res.append(part(w) * (y + kvf[c][n2] * tile_rows(wtab[c, KS], N1)))
                    if e == 0:
                        yield 32
                outa[c][pl.ds(jp, N1, stride=8), :] = _pack2(*res)
                yield 32

    start(cp_first, cp_x0, cp_w1)
    sem_zero[0] = 0
    kk = lax.broadcasted_iota(jnp.int32, (64, 128), 0)
    ll = lax.broadcasted_iota(jnp.int32, (64, 128), 1)
    cmask[0] = jnp.where(kk <= ll, 0.0, NEG)
    cmask[1] = jnp.where((ll < 64) | (kk <= ll - 64), 0.0, NEG)
    cmask[2] = jnp.where(kk <= (ll & 63), 0.0, NEG)
    for r in range(11):
        row = sub + 8 * r
        hr = sum((row >= a * DH).astype(jnp.int32) for a in range(1, 4)) if r < 10 else row - 80
        bmask[r] = jnp.left_shift(1, hr)
    for gi in range(2):
        for j in range(4):
            vall[gi, j, 80:88, :] = jnp.ones((8, 128), F32)
    for c in range(NT):
        kb[c, 0:8, :] = jnp.zeros((8, 128), U32)
    for u in range(16 - DEPTH, 16):
        slots[u % NSLOT][...] = jnp.zeros((2, 512, 128), F32)
    vhead[1] = jnp.ones(vhead.shape[1:], BF16)
    opart[1] = jnp.zeros(opart.shape[1:], F32)
    with jax.named_scope("prologue"):
        wait(cp_first)
        start(cp_w2, cp_wv, cp_step[0])
        first_proj(0, (0, 1))
        wait(cp_x0)
        first_proj(0, (2, 3))
        wait(cp_w1)
        for n in range(*W_STAGES[1]):
            first_proj(n)
        wait(cp_w2)
        first_proj(W_STAGES[2][0])
        wait(cp_wv)
        start(cp_step[1])
        taps_t = shift_ref[...].astype(F32)
        skip = ssmd_ref[...].astype(F32)
        for c in range(NT):
            for j in range(KS):
                wtab[c, j] = jnp.broadcast_to(taps_t[j:j + 1, 128 * c:128 * c + 128], (8, 128))
            wtab[c, KS] = jnp.broadcast_to(skip[c:c + 1], (8, 128))
        gates = jax.nn.sigmoid(beta_ref[...].astype(F32))
        gcol = jnp.broadcast_to(gates, (8, H)).T
        gcol = jnp.broadcast_to(gcol[:, 0:1], (H, 128))
        for g in range(8):
            gtab[g] = jnp.concatenate([gcol[4 * g:4 * g + 4]] * 2, axis=0)
        for n in range(NT):
            for c in range(NT):
                wvt[c, rows(n, 64), :] = _u32(_bf(wvb[n, 64 * c:64 * c + 64, :]).T)
        for n in range(W_STAGES[2][0] + 1, NT):
            first_proj(n)

    def segment(s):
        def body(i, carry):
            if s == 0:
                for j in range(4):
                    @pl.when(i == j)
                    def _():
                        wait(cp_step[j])
                        start(*((cp_step[2],), (cp_step[3],), (cp_seg1,), (cp_seg2,))[j])
            segment_step(s, i)
            if s > 0:
                start(out_b(4 * (s - 1) + i))
            return carry

        with jax.named_scope(f"seg{s}"):
            lax.fori_loop(0, 4, body, 0)

    segment(0)
    wait(cp_seg1)
    segment(1)
    wait(cp_seg2)
    segment(2)
    segment(3)
    start(*[cp_oa[c] for c in INVERSE[3]])
    with jax.named_scope("epilogue"):
        seg[0] = 4
        current.clear()
        recent[0] = None
        last = NT - 1
        rest_tiles = [c for c in range(last) if c not in INVERSE[3]]
        side = _Paced([(spectra((last,), range(16)), 16 * SPEC_COST)])
        span = 1024 * len(rest_tiles) + 800 * MID
        done = 0

        def run(streams):
            nonlocal done
            work = _Paced(streams)
            while work.live:
                before = work.done
                work.step()
                done += work.done - before
                if side.live and side.done < done / span * side.total and recent[0] is not None:
                    pace(sem_zero[0])
                    side.advance(done / span)

        for c in rest_tiles:
            streams = [(inverse((c,), range(8)), 1024)]
            if c == rest_tiles[0]:
                tail = [carried(u, 7, 1) for u in range(16 - DEPTH, 16)]
                streams.append((chain(*[g for g, _ in tail]), sum(w for _, w in tail)))
            run(streams)
            if c == rest_tiles[0]:
                for i in range(4):
                    untranspose(3, i, i)
            start(cp_oa[c])
        for i in range(4):
            if i == MID:
                side.finish()
                run([(inverse((last,), range(8)), 1024)])
                start(cp_oa[last])
            run([(out_proj(3, i, i), 800)])
    wait(*cp_oa, all_of_b)


@jax.jit
def pallas_concat_heads__ssm_conv_h3__memory_aug_infini_attn__prompt_kernel(
    A_q: jax.Array,
    A_k: jax.Array,
    A_v: jax.Array,
    A_shift_k: jax.Array,
    A_ssm_k: jax.Array,
    A_ssm_D: jax.Array,
    B_x: jax.Array,
    B_wq: jax.Array,
    B_wk: jax.Array,
    B_wv: jax.Array,
    B_wo: jax.Array,
    B_beta: jax.Array,
):
    hbm = pl.BlockSpec(memory_space=pltpu.HBM)
    seg_tiles = pltpu.VMEM((NT, L, 128), BF16)
    weight = pltpu.VMEM((NT, D // 2, 128), U32)
    scratch = [
        pltpu.VMEM((KS, D), BF16),
        pltpu.VMEM((NT, 128), BF16),
        pltpu.VMEM((1, H), BF16),
        pltpu.VMEM((NT, S // 2, 128), U32),
        weight, weight, weight, weight,
        pltpu.VMEM((NT, D // 2, 128), U32),
        pltpu.VMEM((S // 128 + 1, D // 2, 128), U32),
        pltpu.VMEM((NT, 256 + 32, 128), U32),
        pltpu.VMEM((NT + 1, S // 2 + 40, 128), U32),
        pltpu.VMEM((NT, S // 2 + 32, 128), U32),
        pltpu.VMEM((NT, S // 2 + 32, 128), U32),
        pltpu.VMEM((N2, N1, 128), U32),
        pltpu.VMEM((N2, 2, N1 // 2, 128), U32),
        pltpu.VMEM((17, 4, 4, 2, 8, 128), F32),
        pltpu.VMEM((NT, S, 128), BF16),
        pltpu.VMEM((NT, KS + 1, 8, 128), F32),
        pltpu.VMEM((8, 8, 128), F32),
        pltpu.VMEM((3, 64, 128), F32),
        seg_tiles, seg_tiles, seg_tiles, seg_tiles,
        seg_tiles, seg_tiles, seg_tiles, seg_tiles,
        pltpu.VMEM((2, 4, D, 128), BF16),
        pltpu.VMEM((8, 88, 128), F32),
        pltpu.VMEM((2, 4, 8, 128), U32),
        pltpu.VMEM((2, 8, 128), jnp.int32),
        pltpu.VMEM((11, 8, 128), jnp.int32),
        pltpu.VMEM((2, L // 2, 128), U32),
        pltpu.VMEM((2, 4, 88, 128), F32),
        pltpu.VMEM((2, 4, 8, 32, 128), BF16),
        pltpu.VMEM((2, 4, 80, 128), F32),
        pltpu.VMEM((4, NT, 64, 128), U32),
        pltpu.SMEM((1,), jnp.int32),
        pltpu.SemaphoreType.DMA((5,)),
    ]
    scratch += [pltpu.VMEM((N2, N1 // 2, 128), U32)] * (2 * NT)
    scratch += [pltpu.VMEM((N1 // 8 + 1, 4, 4, 2, 8, 128), F32)] * (2 * NT)
    scratch += [pltpu.VMEM((N2, N1, 128), U32)] * NT
    scratch += [pltpu.VMEM((N2, N1, 128), F32)] * NT
    scratch += [pltpu.VMEM((S // 2 + 32, 128), U32)] * NT
    scratch += [pltpu.VMEM((2, 512, 128), F32)] * NSLOT
    return pl.pallas_call(
        _kernel,
        out_shape=jax.ShapeDtypeStruct((1, S, 2 * D), BF16),
        in_specs=[hbm] * 14,
        out_specs=hbm,
        scratch_shapes=scratch,
        compiler_params=pltpu.CompilerParams(vmem_limit_bytes=110 * 1024 * 1024),
        name="h3_infini",
    )(A_q, A_k, A_v, A_shift_k.T, A_ssm_k, A_ssm_D.reshape(NT, 128), B_x, B_wq, B_wk, B_wv, B_wo,
      B_beta.reshape(1, H), _FWD, _INV)
```

```python
import math

import jax
import jax.numpy as jnp
import numpy as np
from jax import lax
from jax.experimental import pallas as pl
from jax.experimental.pallas import tpu as pltpu

S = 2048
D = 640
NT = D // 128
H = 32
DH = D // H
NSEG = 4
L = S // NSEG
KS = 4
N1, N2 = 128, 16

F32 = jnp.float32
BF16 = jnp.bfloat16
U32 = jnp.uint32
NN_DIMS = (((1,), (0,)), ((), ()))
NT_DIMS = (((1,), (1,)), ((), ()))
NEG = -1e30
LOG2E = 1.4426950408889634


def _pack_rows(a):
    u = a.astype(np.float32).astype(BF16).view(np.uint16).astype(np.uint32)
    return u[..., 0::2, :] | (u[..., 1::2, :] << 16)


def _dft_tables():
    k1 = np.arange(N1)
    fwd = np.zeros((N2, 2 * N1, N1), np.float64)
    inv = np.zeros((N2, N1, 2 * N1), np.float64)
    kappa = np.arange(N1)
    n1_in = 16 * (kappa // 16) + 8 * (kappa % 2) + (kappa % 16) // 2
    row_re = 16 * (k1 // 8) + k1 % 8
    for n2 in range(N2):
        ang = 2.0 * np.pi * np.outer(k1 + 0.25, N2 * n1_in + n2) / S
        fwd[n2, row_re] = np.cos(ang)
        fwd[n2, row_re + 8] = np.sin(ang)
        ang = 2.0 * np.pi * np.outer(N2 * np.arange(N1) + n2, k1 + 0.25) / S
        inv[n2][:, 2 * k1] = np.cos(ang) / S
        inv[n2][:, 2 * k1 + 1] = np.sin(ang) / S
    inv = inv.reshape(N2, N1, 2, N1).transpose(0, 2, 1, 3)
    return _pack_rows(fwd), _pack_rows(inv)


_FWD, _INV = _dft_tables()


def _dot(a, b, dims=NN_DIMS):
    return lax.dot_general(a, b, dims, preferred_element_type=F32)


def _u32(x):
    return pltpu.bitcast(x, U32)


def _bf(x):
    return pltpu.bitcast(x, BF16)


def _u32_word(x):
    return lax.bitcast_convert_type(x, U32)


def _pack2(a, b):
    return pltpu.pack_elementwise([a, b], packed_dtype=BF16).astype(U32)


def _lo(w):
    return pltpu.unpack_elementwise(w, index=0, packed_dtype=BF16, unpacked_dtype=F32)


def _hi(w):
    return pltpu.unpack_elementwise(w, index=1, packed_dtype=BF16, unpacked_dtype=F32)


def _radix4(x0, x1, x2, x3, sign):
    ar, ai = x0[0] + x2[0], x0[1] + x2[1]
    br, bi = x0[0] - x2[0], x0[1] - x2[1]
    cr, ci = x1[0] + x3[0], x1[1] + x3[1]
    dr, di = x1[0] - x3[0], x1[1] - x3[1]
    y0 = (ar + cr, ai + ci)
    y2 = (ar - cr, ai - ci)
    yp = (br - di, bi + dr)
    ym = (br + di, bi - dr)
    return (y0, yp, y2, ym) if sign > 0 else (y0, ym, y2, yp)


def _twiddle(x, e, sign):
    xr, xi = x
    if e == 0:
        return x
    if e == 4:
        return (-xi, xr) if sign > 0 else (xi, -xr)
    r = math.sqrt(0.5)
    if e == 2:
        return ((xr - xi) * r, (xr + xi) * r) if sign > 0 else ((xr + xi) * r, (xi - xr) * r)
    if e == 6:
        return ((xr + xi) * -r, (xr - xi) * r) if sign > 0 else ((xi - xr) * r, (xr + xi) * -r)
    c, s = math.cos(math.pi * e / 8), sign * math.sin(math.pi * e / 8)
    return (xr * c - xi * s, xr * s + xi * c)


def _radix4_tw(x0, x1, x2, x3, sign, b):
    if b != 2:
        return _radix4(x0, _twiddle(x1, b, sign), _twiddle(x2, 2 * b, sign),
                       _twiddle(x3, 3 * b, sign), sign)
    x1, x3 = _twiddle(x1, 2, sign), _twiddle(x3, 6, sign)
    if sign > 0:
        ar, ai = x0[0] - x2[1], x0[1] + x2[0]
        br, bi = x0[0] + x2[1], x0[1] - x2[0]
    else:
        ar, ai = x0[0] + x2[1], x0[1] - x2[0]
        br, bi = x0[0] - x2[1], x0[1] + x2[0]
    cr, ci = x1[0] + x3[0], x1[1] + x3[1]
    dr, di = x1[0] - x3[0], x1[1] - x3[1]
    y0 = (ar + cr, ai + ci)
    y2 = (ar - cr, ai - ci)
    yp = (br - di, bi + dr)
    ym = (br + di, bi - dr)
    return (y0, yp, y2, ym) if sign > 0 else (y0, ym, y2, yp)


class _Paced:
    def __init__(self, streams, sequential=False):
        self.live = [[g, total, 0] for g, total in streams if total]
        self.total = sum(total for _, total in streams)
        self.done = 0
        self.sequential = sequential

    def step(self):
        cur = self.live[0] if self.sequential else min(self.live, key=lambda e: e[2] / e[1])
        cost = next(cur[0], None)
        if cost is None:
            self.live.remove(cur)
        else:
            cur[2] += cost
            self.done += cost

    def advance(self, fraction):
        while self.live and self.done < fraction * self.total:
            self.step()

    def finish(self):
        self.advance(math.inf)


SPLIT = ((0, 1, 2), (3, 4), (), ())
FORWARD = ((), (0, 1), (2, 3, 4), ())
SPECTRUM = ((), (), (0, 1), (2, 3))
INVERSE = ((), (), (), (0, 1))
DEPTH = 3
NSLOT = 4
ORDER = ((1, 3, 0, 2), (3, 2, 1, 0), (0, 2, 1, 3), (0, 1, 2, 3))
TAIL = (-0.03, -0.03, 0.02, -0.03)
LW = (1.0, 1.0, 1.0, 1.0)
AW = (4.0, 2.0, 4.0, 2.0, 3.0)
QCH = (128, 256, 128, 128)
HEAD = (4, 6, 6, 6)
FILL_ORDER = (0, 1, 1, 2)
PACE_ON = (3, 3, 7, 7, 7)
SIDE_SPEED = (1.03, 1.0, 1.03, 1.0)
MID = 3
PACE_ALL = (3, 2, 2, 3, 0)
SPEC_V = (0, 0, 0, 0, 1)
W_STAGES = ((0, 1), (1, 3), (3, 5))


def _kernel(aq_hbm, ak_hbm, av_hbm, shift_hbm, h_hbm, ssmd_hbm, x_hbm, wq_hbm, wk_hbm,
            wv_hbm, wo_hbm, beta_hbm, fwd_hbm, inv_hbm, out_hbm,
            xb, wqb, wkb, wvb, wob, wvt, hb, ht, kb, vb, qb, fwd, inv,
            ub, outb, wtab, gtab, cmask,
            q0, q1, k0, k1, pq0, pq1, pk0, pk1, ots, mst,
            hmask, hsel, bmask, kwin, vall, vhead, opart, onat, sem_zero, sems, *rest):
    xp, hp, tx, th, yb, kvf, outa = (rest[NT * k:NT * k + NT] for k in range(7))
    slots = rest[7 * NT:7 * NT + NSLOT]
    shift_ref, ssmd_ref, beta_ref = rest[7 * NT + NSLOT:]
    qs, ks, pqs, pks = (q0, q1), (k0, k1), (pq0, pq1), (pk0, pk1)

    def copy(src, dst, sem):
        return [lambda: pltpu.make_async_copy(src, dst, sems.at[sem])]

    def tiles(src, dst, sem, r0, n, ts=range(NT), off=0):
        src = src.bitcast(U32)
        lead = (0,) * (len(src.shape) - 2)
        return [cp for t in ts for cp in copy(
            src.at[lead + (pl.ds(r0 // 2, n // 2), pl.ds(128 * t, 128))],
            dst.at[t, pl.ds(off + r0 // 2, n // 2), :], sem)]

    def conv_inputs(cs, r0, n, sem):
        return (tiles(h_hbm, hb, sem, 128 * cs[0], 128 * len(cs), range(r0 // 128, (r0 + n) // 128))
                + tiles(ak_hbm, kb, sem, r0, n, cs, off=32) + tiles(av_hbm, vb, sem, r0, n, cs))

    def w_stage(k, sem):
        return (tiles(wq_hbm, wqb, sem, 0, D, range(*W_STAGES[k]))
                + tiles(wk_hbm, wkb, sem, 0, D, range(*W_STAGES[k])))

    cp_first = w_stage(0, 0) + tiles(x_hbm, xb, 0, 0, 256)
    cp_x0 = tiles(x_hbm, xb, 1, 256, 256)
    cp_w1, cp_w2 = w_stage(1, 2), w_stage(2, 3)
    cp_wv = (tiles(wv_hbm, wvb, 0, 0, D) + copy(shift_hbm, shift_ref, 0)
             + copy(ssmd_hbm, ssmd_ref, 0) + copy(beta_hbm, beta_ref, 0))
    cp_step = [tiles(x_hbm, xb, sem, L + 128 * i, 128) + conv_inputs(SPLIT[0], L * i, L, sem)
               for i, sem in enumerate((4, 0, 1, 2))]
    cp_seg1 = (tiles(wo_hbm, wob, 3, 0, D) + tiles(x_hbm, xb, 3, 2 * L, L)
               + copy(fwd_hbm, fwd, 3) + conv_inputs(SPLIT[1], 0, S, 3))
    cp_seg2 = (tiles(x_hbm, xb, 4, 3 * L, L) + copy(inv_hbm, inv, 4)
               + tiles(aq_hbm, qb, 4, 0, S))
    cp_oa = [copy(outa[c].at[pl.ds(0, S // 2), :],
                  out_hbm.bitcast(U32).at[0, :, pl.ds(128 * c, 128)], 0) for c in range(NT)]

    def out_b(tile, ns=range(NT)):
        at = pl.ds(128 * tile if isinstance(tile, int) else pl.multiple_of(128 * tile, 128), 128)
        return [cp for n in ns for cp in copy(
            outb.at[n, at, :], out_hbm.at[0, at, pl.ds(D + 128 * n, 128)], 1)]

    all_of_b = copy(outb, outb, 1)

    def start(*groups):
        for g in groups:
            for cp in g:
                cp().start()

    def wait(*groups):
        for g in groups:
            for cp in g:
                cp().wait()

    def rows(i, n):
        return pl.ds(pl.multiple_of(i * n, n), n) if not isinstance(i, int) else pl.ds(i * n, n)

    lane = lax.broadcasted_iota(jnp.int32, (8, 128), 1)
    sub = lax.broadcasted_iota(jnp.int32, (8, 128), 0)

    def lanes(n):
        return lax.broadcasted_iota(jnp.int32, (n, 128), 1)

    recent = [None]
    seg = [0]

    def dot(a, b, dims=NN_DIMS, kind=4):
        out = _dot(a, b, dims)
        if kind & PACE_ON[seg[0]]:
            recent[0] = out
        return out

    current = {}

    def pace(zero):
        v = recent[0][-8:]
        recent[0] = None
        if "h" in current:
            hb[S // 128, rows(zero, 8), :] = _u32_word(v)
        if "k" in current:
            kb[NT, rows(zero, 8), :] = _u32_word(v)
        if "t" in current:
            th[current["t"]][N1 // 8, zero, 0, 0] = v
            if PACE_ALL[seg[0]] & 1:
                tx[current["t"]][N1 // 8, zero, 0, 0] = v
            if PACE_ALL[seg[0]] & 2:
                ub[16, zero, 0, 0] = v

    def qk_proj(s, i, want_pq, want_pk):
        p = s % 2
        tok = rows(4 * s + i, 64)
        for w_ref, dst, fdst, want, scale in (
                (wqb, qs[p], pqs[p], want_pq, DH ** -0.5 * LOG2E),
                (wkb, ks[p], pks[p], want_pk, None)):
            for n in range(NT):
                t = None
                for c in range(NT):
                    part = dot(_bf(xb[c, tok, :]), _bf(w_ref[n, 64 * c:64 * c + 64, :]))
                    t = part if t is None else t + part
                    if c < NT - 1:
                        yield 32
                dst[n, rows(i, 128), :] = (t if scale is None else t * scale).astype(BF16)
                if want:
                    fdst[n, rows(i, 128), :] = jnp.where(t > 0, t + 1.0, jnp.exp(t)).astype(BF16)
                yield 32

    def first_proj(n, js=range(4)):
        for w_ref, dst, scale in ((wqb, qs[0], DH ** -0.5 * LOG2E), (wkb, ks[0], None)):
            for j in js:
                t = None
                for c in range(NT):
                    part = dot(_bf(xb[c, rows(j, 64), :]), _bf(w_ref[n, 64 * c:64 * c + 64, :]))
                    t = part if t is None else t + part
                dst[n, rows(j, 128), :] = (t if scale is None else t * scale).astype(BF16)
                if scale is None:
                    pks[0][n, rows(j, 128), :] = jnp.where(t > 0, t + 1.0, jnp.exp(t)).astype(BF16)

    def untranspose(s, i, slot=0):
        ot = ots.bitcast(U32)
        for c in range(NT):
            onat[slot, c] = _u32(_bf(ot[s % 2, i, 64 * c:64 * c + 64, :]).T)

    def out_proj(s, i, slot=0):
        for n in range(NT):
            t = None
            for c in range(NT):
                part = dot(_bf(onat[slot, c]), _bf(wob[n, 64 * c:64 * c + 64, :]))
                t = part if t is None else t + part
                if c < NT - 1:
                    yield 32
            outb[n, rows(4 * s + i, 128), :] = t.astype(BF16)
            if s == NSEG - 1:
                start(out_b(4 * s + i, (n,)))
            yield 32

    def tile_rows(r, n):
        return jnp.broadcast_to(r[None], (n // 8, 8, 128)).reshape(n, 128)

    class Group:
        def __init__(self, s, g, gi):
            self.s, self.g, self.gi = s, g, gi
            self.t0 = (80 * g) // 128
            self.off = 80 * g - 128 * self.t0
            self.t1 = jnp.minimum(self.t0 + 1, NT - 1)
            rel = (lane - self.off) & 127
            head = sum((rel >= a * DH).astype(jnp.int32) for a in range(1, 5))
            for a in range(4):
                hmask[gi, a] = jnp.where(head == a, np.uint32(0xFFFFFFFF), np.uint32(0))
            hsel[gi] = jnp.left_shift(1, head)
            self.have_keys, self.have_mem = set(), set()

        def window(self, ref, j, r0=0, n=64):
            ref = ref.bitcast(U32)
            at = pl.ds(64 * j + r0, n)
            return jnp.where(lanes(n) >= self.off, ref[self.t0, at, :], ref[self.t1, at, :])

        def keys(self, r0, r1):
            out = []
            for r in range(r0, r1, 64):
                at = pl.ds(r // 2, 32)
                if r in self.have_keys:
                    out.append(kwin[self.gi, at, :])
                else:
                    self.have_keys.add(r)
                    out.append(self.window(ks[self.s % 2], 0, r // 2, 32))
                    kwin[self.gi, at, :] = out[-1]
            return _bf(jnp.concatenate(out, axis=0))

        def park_values(self, j, v80):
            if self.s < NSEG - 1:
                vall[self.gi, j, 0:80, :] = v80
            ones8 = jnp.ones((8, 128), F32)
            for pr in range(2):
                for e in range(2):
                    r0 = 40 * pr + 16 * e
                    vhead[self.gi, j, r0 // 8] = jnp.concatenate(
                        [v80[r0:r0 + 24], ones8], axis=0).astype(BF16)

        def mem_read(self):
            for j in range(4):
                r = dot(mst[self.g, 0:88, :], _bf(self.window(pqs[self.s % 2], j)), NT_DIMS)
                coef = gtab[self.g] / (r[80:88] + 1e-6)
                cb = [jnp.broadcast_to(coef[a:a + 1], (8, 128)) for a in range(4)]
                for pr in range(2):
                    ca, cc = cb[2 * pr], cb[2 * pr + 1]
                    for e, scale in enumerate((ca, ca, jnp.where(sub < 4, ca, cc), cc, cc)):
                        r0 = 40 * pr + 8 * e
                        opart[self.gi, j, r0:r0 + 8, :] = r[r0:r0 + 8] * scale
                self.have_mem.add(j)
                yield 24

        def mem_update(self):
            acc = None
            for j in range(4):
                t = dot(vall[self.gi, j], _bf(self.window(pks[self.s % 2], j)))
                acc = t if acc is None else acc + t
                if j < 3:
                    yield 24
            for r in range(11):
                new = jnp.where(bmask[r] & hsel[self.gi] != 0, acc[8 * r:8 * r + 8], 0.0)
                at = pl.ds(8 * r, 8)
                mst[self.g, at, :] = new if self.s == 0 else mst[self.g, at, :] + new
            yield 24

        def logits(self, pr, j, slot):
            qw = self.window(qs[self.s % 2], j)
            qa = qw & tile_rows(hmask[self.gi, 2 * pr], 64)
            qh = qw & tile_rows(hmask[self.gi, 2 * pr + 1], 64)
            w_a = _bf(qa)
            w_b = _bf(jnp.concatenate([qh[32:64], qh[0:32]], axis=0))
            w_t = _bf(jnp.concatenate([qh[32:64], qa[32:64]], axis=0))
            n = 128 * j

            def park(t, e, r0, m):
                for r in range(0, t.shape[0], 8):
                    v = t[r:r + 8]
                    if e == 2:
                        v = v + cmask[2, r:r + 8, :]
                    elif r0 + r >= n:
                        v = v + cmask[e, r0 + r - n:r0 + r - n + 8, :]
                    slot[e % 2, 448 * (e // 2) + r0 + r:448 * (e // 2) + r0 + r + 8, :] = v
                    m = v if m is None else jnp.maximum(m, v)
                return m

            m_t = park(dot(self.keys(n + 64, n + 128), w_t, NT_DIMS, 1), 2, 0, None)
            yield 16 * LW[seg[0] % 4]
            cuts = list(range(0, n, QCH[seg[0]])) or [0]
            m = [None, None]
            for r0, r1 in zip(cuts, cuts[1:] + [n + 64]):
                for e, w in enumerate((w_a, w_b)):
                    m[e] = park(dot(self.keys(r0, r1), w, NT_DIMS, 1), e, r0, m[e])
                    if r1 == n + 64 and e == 1:
                        m_a = jnp.maximum(m[0], jnp.where(lane >= 64, m_t, NEG))
                        m_b = jnp.maximum(m[1], jnp.where(lane < 64, m_t, NEG))
                        m_a = jnp.broadcast_to(jnp.max(m_a, axis=0, keepdims=True), (8, 128))
                        m_b = jnp.broadcast_to(jnp.max(m_b, axis=0, keepdims=True), (8, 128))
                        slot[1, 448:456, :] = m_a
                        slot[1, 456:464, :] = m_b
                        slot[1, 464:472, :] = jnp.where(lane < 64, m_b, m_a)
                    yield (r1 - r0) // 4 * LW[seg[0] % 4]

    def attend(gi, g, parity, add_mem, pr, j, slot, need_values):
        def prob(e, r0, n, which):
            m2 = tile_rows(slot[1, 448 + 8 * which:456 + 8 * which, :], 16)
            return [jnp.exp2(slot[e, r:r + 16, :] - m2) for r in range(r0, r0 + n, 16)]

        res = [None, None]
        order = [(0, j), (1, j)] + [(e, kt) for e in range(2) for kt in range(j)]
        for n, (e, kt) in enumerate(order):
            need_values(kt)
            if n == 0:
                p_t = prob(0, 448, 64, 2)
            if kt < j:
                p = prob(e, 128 * kt, 128, e)
            else:
                mine = lanes(16) >= 64 if e == 0 else lanes(16) < 64
                p = prob(e, 128 * kt, 64, e) + [jnp.where(mine, t, 0.0) for t in p_t]
            t = dot(_bf(vhead.bitcast(U32)[gi, kt, 5 * pr + 2 * e]),
                    jnp.concatenate(p, axis=0).astype(BF16), kind=2)
            res[e] = t if res[e] is None else res[e] + t
            if n < len(order) - 1:
                yield 8 * AW[seg[0]]
        r_a = res[0]
        r_b = pltpu.roll(res[1], 64, 1)
        keep = 1.0 - gtab[g]
        keep_a = jnp.broadcast_to(keep[2 * pr:2 * pr + 1], (8, 128))
        keep_b = jnp.broadcast_to(keep[2 * pr + 1:2 * pr + 2], (8, 128))
        o_a = r_a[0:24] * tile_rows(keep_a / r_a[24:32], 24)
        o_b = r_b[0:24] * tile_rows(keep_b / r_b[24:32], 24)
        o = jnp.concatenate(
            [o_a[0:16], jnp.where(sub < 4, o_a[16:24], o_b[0:8]), o_b[8:24]], axis=0)
        if add_mem:
            o = o + opart[gi, j, 40 * pr:40 * pr + 40, :]
        if pr == 0:
            opart[gi, j, 0:40, :] = o
        else:
            o = jnp.concatenate([opart[gi, j, 0:40, :], o], axis=0)
            ots[parity, j, rows(g, 80), :] = o.astype(BF16)
        yield 8 * AW[seg[0]]

    def v_proj(s, i, groups, have):
        for j in range(4):
            acc = None
            for c in range(NT):
                t = dot(_bf(wvt[c, i, 0:80, :]), _bf(xb[c, rows(4 * s + j, 64), :]), NT_DIMS)
                acc = t if acc is None else acc + t
                if c == NT - 1:
                    for gi in range(2):
                        groups[gi].park_values(j, acc[80 * gi:80 * gi + 80])
                    have.append(j)
                yield 40

    def chain(*gens):
        for g in gens:
            yield from g

    def units(s):
        return [(gi, pr, j) for gi in range(2) for pr in range(2)
                for j in (range(4) if (gi, pr) == (1, 1) else ORDER[s] if gi + pr else range(4))]

    def cost(j):
        return (48 + 64 * j) * LW[seg[0] % 4], (16 + 16 * j) * AW[seg[0]]

    def carried(u, g, parity):
        gi, pr, j = units(0)[u]
        return attend(gi, g, parity, True, pr, j, slots[u % NSLOT], lambda kt: None), cost(j)[1]

    def segment_step(s, i):
        seg[0] = s
        parts = {}
        if s < NSEG - 1:
            parts["qk"] = (qk_proj(s + 1, i, True, s + 1 < NSEG - 1), 1600)
        if s > 0:
            parts["out"] = (out_proj(s - 1, i), 800)
        if FORWARD[s]:
            parts["fwd"] = (fwd_fft(i, FORWARD[s]), 512 * len(FORWARD[s]))
        if INVERSE[s]:
            parts["inv"] = (inverse(INVERSE[s], (2 * i, 2 * i + 1)), 256 * len(INVERSE[s]))
        names = (("qk", "inv", "out", "fwd"), ("qk", "inv", "fwd", "out"),
                 ("inv", "fwd", "qk", "out"), ("qk", "inv", "out", "fwd"))[FILL_ORDER[s]]
        fill = _Paced([parts[n] for n in names if n in parts], sequential=FILL_ORDER[s] < 3)
        side = []
        if SPECTRUM[s]:
            side.append((spectra(SPECTRUM[s], [4 * i + a for a in range(4)]),
                         4 * SPEC_COST * len(SPECTRUM[s])))
        for c in SPLIT[s]:
            side += [(split_h(i, c), 144), (split_kv(i, c), 704)]
        side = _Paced(side, sequential=True)
        current.clear()
        recent[0] = None
        for _ in range(HEAD[s]):
            fill.step()
        if s > 0:
            untranspose(s - 1, i)
        vt = []
        groups = [Group(s, 2 * i + gi, gi) for gi in range(2)]
        reads = [grp.mem_read() for grp in groups if s > 0]
        updates = [grp.mem_update() for grp in groups if s < NSEG - 1]
        first = _Paced([(chain(*reads[:1], v_proj(s, i, groups, vt), *reads[1:], *updates),
                         800 + 96 * (len(reads) + len(updates)))])
        total = first.total + fill.total
        held = 96 * (s > 0) + 159

        def need_values(kt):
            while len(vt) <= kt:
                first.step()

        def pad(fraction, u):
            target = total * fraction / (1 + TAIL[s])
            early = min(target, held if u < DEPTH else first.total)
            first.advance(early / first.total)
            fill.advance((target - early) / fill.total)
            goal = fraction * SIDE_SPEED[s]
            if side.live and side.done < goal * side.total and recent[0] is not None:
                pace(jnp.minimum(i, 3))
                side.advance(goal)

        todo = units(s)
        whole = sum(sum(cost(j)) for _, _, j in todo)
        done = 0
        for u, (gi, pr, j) in enumerate(todo):
            streams = [(groups[gi].logits(pr, j, slots[u % NSLOT]), cost(j)[0])]
            v = u - DEPTH
            if v < 0:
                streams.append(carried(v + len(todo), (2 * i + 7) & 7,
                                       jnp.where(i > 0, s % 2, 1 - s % 2)))
            else:
                gi, pr, j = todo[v]
                while s > 0 and j not in groups[gi].have_mem:
                    first.step()
                streams.append((attend(gi, 2 * i + gi, s % 2, s > 0, pr, j, slots[v % NSLOT],
                                       need_values), cost(j)[1]))
            att = _Paced(streams[::-1], sequential=u == len(todo) - 1)
            while att.live:
                att.step()
                pad((done + att.done) / whole, u)
            done += att.total
        first.finish()
        fill.finish()
        side.finish()

    def split_h(i, c):
        current.clear()
        current["h"] = True
        for t in range(4):
            ht[c, 64 * t:64 * t + 64, :] = _u32(
                _bf(hb[4 * i + t, 64 * c:64 * c + 64, :]).T)
            yield 4
        for q in range(2):
            for j in range(8):
                wa = ht[c, pl.ds(128 * q + j, 8, stride=8), :]
                wb = ht[c, pl.ds(128 * q + 64 + j, 8, stride=8), :]
                hp[c][2 * j, rows(2 * i + q, 8), :] = _pack2(_lo(wa), _lo(wb))
                hp[c][2 * j + 1, rows(2 * i + q, 8), :] = _pack2(_hi(wa), _hi(wb))
                if j % 2:
                    yield 16

    def split_kv(i, c):
        current.clear()
        current["k"] = True
        taps = [wtab[c, j] for j in range(KS)]
        for q in range(2):
            blk = 2 * i + q
            base = [blk * 128 + 64 * e for e in range(2)]
            hist = []
            for e in range(2):
                w2 = kb[c, pl.ds(base[e] + 30, 8, stride=8), :]
                w1 = kb[c, pl.ds(base[e] + 31, 8, stride=8), :]
                hist.append([_hi(w2), _lo(w1), _hi(w1)])
            for j in range(8):
                kv = [[None, None], [None, None]]
                for e in range(2):
                    kw = kb[c, pl.ds(base[e] + 32 + j, 8, stride=8), :]
                    vw = vb[c, pl.ds(base[e] + j, 8, stride=8), :]
                    kp = hist[e] + [_lo(kw), _hi(kw)]
                    for half, part in enumerate((_lo, _hi)):
                        acc = kp[3 + half] * taps[0]
                        for d in range(1, KS):
                            acc = acc + kp[3 + half - d] * taps[d]
                        kv[half][e] = acc * part(vw)
                        kvf[c][2 * j + half, rows(2 * blk + e, 8), :] = kv[half][e]
                    hist[e] = kp[2:]
                    if e == 0:
                        yield 22
                for half in range(2):
                    xp[c][2 * j + half, rows(blk, 8), :] = _pack2(*kv[half])
                yield 22

    def fwd_fft(i, cs):
        for c in cs:
            for src, dst in ((hp[c], th[c]), (xp[c], tx[c])):
                g = [dot(_bf(fwd[4 * a + i]), _bf(src[4 * a + i])) for a in range(4)]
                for r in range(0, 2 * N1, 16):
                    z = _radix4(*[(g[a][r:r + 8], g[a][r + 8:r + 16]) for a in range(4)], 1)
                    for cc in range(4):
                        dst[r // 16, i, cc, 0] = z[cc][0]
                        dst[r // 16, i, cc, 1] = z[cc][1]
                yield 256

    def spectrum(c, m, slot):
        current.clear()
        current["t"] = c
        for cc in range(4):
            zh = _radix4_tw(*[(th[c][m, b, cc, 0], th[c][m, b, cc, 1]) for b in range(4)], 1, cc)
            yield 17
            zx = _radix4_tw(*[(tx[c][m, b, cc, 0], tx[c][m, b, cc, 1]) for b in range(4)], 1, cc)
            yield 17
            y = [(x[0] * h[0] - x[1] * h[1], x[0] * h[1] + x[1] * h[0]) for x, h in zip(zx, zh)]
            yield 17
            u = _radix4(*y, -1)
            for b in range(4):
                ub[slot, b, cc, 0] = u[b][0]
                ub[slot, b, cc, 1] = u[b][1]
            yield 17
        if SPEC_V[seg[0]]:
            return

        yield from spectrum_end(c, m, slot)

    def spectrum_end(c, m, slot):
        for b in range(4):
            z = _radix4_tw(*[(ub[slot, b, cc, 0], ub[slot, b, cc, 1]) for cc in range(4)], -1, b)
            for a in range(4):
                yb[c][4 * a + b, rows(m, 8), :] = _pack2(*z[a])
            yield 17

    SPEC_COST = 17 * 20

    def spectra(cs, ms, slot0=0):
        prev = None
        for slot, (c, m) in enumerate(((c, m) for c in cs for m in ms), slot0):
            yield from spectrum(c, m, slot)
            if SPEC_V[seg[0]] and prev is not None:
                yield from spectrum_end(*prev)
            prev = (c, m, slot)
        if SPEC_V[seg[0]]:
            yield from spectrum_end(*prev)

    def inverse(cs, jps):
        for c in cs:
            for jp in jps:
                w = qb[c, pl.ds(jp, N1, stride=8), :]
                res = []
                for e, part in enumerate((_lo, _hi)):
                    n2 = 2 * jp + e
                    y = dot(_bf(inv[n2, 0]), _bf(yb[c][n2, 0:64, :]))
                    yield 32
                    y = y + dot(_bf(inv[n2, 1]), _bf(yb[c][n2, 64:128, :]))
                    res.append(part(w) * (y + kvf[c][n2] * tile_rows(wtab[c, KS], N1)))
                    if e == 0:
                        yield 32
                outa[c][pl.ds(jp, N1, stride=8), :] = _pack2(*res)
                yield 32

    start(cp_first, cp_x0, cp_w1)
    sem_zero[0] = 0
    kk = lax.broadcasted_iota(jnp.int32, (64, 128), 0)
    ll = lax.broadcasted_iota(jnp.int32, (64, 128), 1)
    cmask[0] = jnp.where(kk <= ll, 0.0, NEG)
    cmask[1] = jnp.where((ll < 64) | (kk <= ll - 64), 0.0, NEG)
    cmask[2] = jnp.where(kk <= (ll & 63), 0.0, NEG)
    for r in range(11):
        row = sub + 8 * r
        hr = sum((row >= a * DH).astype(jnp.int32) for a in range(1, 4)) if r < 10 else row - 80
        bmask[r] = jnp.left_shift(1, hr)
    for gi in range(2):
        for j in range(4):
            vall[gi, j, 80:88, :] = jnp.ones((8, 128), F32)
    for c in range(NT):
        kb[c, 24:32, :] = jnp.zeros((8, 128), U32)
    for u in range(16 - DEPTH, 16):
        slots[u % NSLOT][...] = jnp.zeros((2, 512, 128), F32)
    vhead[1] = jnp.ones(vhead.shape[1:], BF16)
    opart[1] = jnp.zeros(opart.shape[1:], F32)
    with jax.named_scope("prologue"):
        wait(cp_first)
        start(cp_w2, cp_wv, cp_step[0])
        first_proj(0, (0, 1))
        wait(cp_x0)
        first_proj(0, (2, 3))
        wait(cp_w1)
        for n in range(*W_STAGES[1]):
            first_proj(n)
        wait(cp_w2)
        first_proj(W_STAGES[2][0])
        wait(cp_wv)
        start(cp_step[1])
        taps_t = shift_ref[...].astype(F32)
        skip = ssmd_ref[...].astype(F32)
        for c in range(NT):
            for j in range(KS):
                wtab[c, j] = jnp.broadcast_to(taps_t[j:j + 1, 128 * c:128 * c + 128], (8, 128))
            wtab[c, KS] = jnp.broadcast_to(skip[c:c + 1], (8, 128))
        gates = jax.nn.sigmoid(beta_ref[...].astype(F32))
        gcol = jnp.broadcast_to(gates, (8, H)).T
        gcol = jnp.broadcast_to(gcol[:, 0:1], (H, 128))
        for g in range(8):
            gtab[g] = jnp.concatenate([gcol[4 * g:4 * g + 4]] * 2, axis=0)
        for n in range(NT):
            for c in range(NT):
                wt = _u32(_bf(wvb[n, 64 * c:64 * c + 64, :]).T)
                for r in range(0, 64, 16):
                    step, r0 = divmod(64 * n + r, 80)
                    wvt[c, step, r0:r0 + 16, :] = wt[r:r + 16]
        for n in range(W_STAGES[2][0] + 1, NT):
            first_proj(n)

    def segment(s):
        def body(i, carry):
            if s == 0:
                for j in range(4):
                    @pl.when(i == j)
                    def _():
                        wait(cp_step[j])
                        start(*((cp_step[2],), (cp_step[3],), (cp_seg1,), (cp_seg2,))[j])
            segment_step(s, i)
            if s > 0:
                start(out_b(4 * (s - 1) + i))
            return carry

        with jax.named_scope(f"seg{s}"):
            lax.fori_loop(0, 4, body, 0)

    segment(0)
    wait(cp_seg1)
    segment(1)
    wait(cp_seg2)
    segment(2)
    segment(3)
    start(*[cp_oa[c] for c in INVERSE[3]])
    with jax.named_scope("epilogue"):
        seg[0] = 4
        current.clear()
        recent[0] = None
        last = NT - 1
        rest_tiles = [c for c in range(last) if c not in INVERSE[3]]
        side = _Paced([(spectra((last,), range(16)), 16 * SPEC_COST)])
        span = 1024 * len(rest_tiles) + 800 * MID
        done = 0

        def run(streams):
            nonlocal done
            work = _Paced(streams)
            while work.live:
                before = work.done
                work.step()
                done += work.done - before
                if side.live and side.done < done / span * side.total and recent[0] is not None:
                    pace(sem_zero[0])
                    side.advance(done / span)

        for c in rest_tiles:
            streams = [(inverse((c,), range(8)), 1024)]
            if c == rest_tiles[0]:
                tail = [carried(u, 7, 1) for u in range(16 - DEPTH, 16)]
                streams.append((chain(*[g for g, _ in tail]), sum(w for _, w in tail)))
            run(streams)
            if c == rest_tiles[0]:
                for i in range(4):
                    untranspose(3, i, i)
            start(cp_oa[c])
        for i in range(4):
            if i == MID:
                side.finish()
                run([(inverse((last,), range(8)), 1024)])
                start(cp_oa[last])
            run([(out_proj(3, i, i), 800)])
    wait(*cp_oa, all_of_b)


@jax.jit
def pallas_concat_heads__ssm_conv_h3__memory_aug_infini_attn__prompt_kernel(
    A_q: jax.Array,
    A_k: jax.Array,
    A_v: jax.Array,
    A_shift_k: jax.Array,
    A_ssm_k: jax.Array,
    A_ssm_D: jax.Array,
    B_x: jax.Array,
    B_wq: jax.Array,
    B_wk: jax.Array,
    B_wv: jax.Array,
    B_wo: jax.Array,
    B_beta: jax.Array,
):
    hbm = pl.BlockSpec(memory_space=pltpu.HBM)
    seg_tiles = pltpu.VMEM((NT, L, 128), BF16)
    weight = pltpu.VMEM((NT, D // 2, 128), U32)
    scratch = [
        pltpu.VMEM((NT, S // 2, 128), U32),
        weight, weight, weight, weight,
        pltpu.VMEM((NT, 4, 96, 128), U32),
        pltpu.VMEM((S // 128 + 1, D // 2, 128), U32),
        pltpu.VMEM((NT, 256 + 32, 128), U32),
        pltpu.VMEM((NT + 1, S // 2 + 64, 128), U32),
        pltpu.VMEM((NT, S // 2 + 32, 128), U32),
        pltpu.VMEM((NT, S // 2 + 32, 128), U32),
        pltpu.VMEM((N2, N1, 128), U32),
        pltpu.VMEM((N2, 2, N1 // 2, 128), U32),
        pltpu.VMEM((17, 4, 4, 2, 8, 128), F32),
        pltpu.VMEM((NT, S, 128), BF16),
        pltpu.VMEM((NT, 8, 8, 128), F32),
        pltpu.VMEM((8, 8, 128), F32),
        pltpu.VMEM((3, 64, 128), F32),
        seg_tiles, seg_tiles, seg_tiles, seg_tiles,
        seg_tiles, seg_tiles, seg_tiles, seg_tiles,
        pltpu.VMEM((2, 4, D, 128), BF16),
        pltpu.VMEM((8, 96, 128), F32),
        pltpu.VMEM((2, 4, 8, 128), U32),
        pltpu.VMEM((4, 8, 128), jnp.int32),
        pltpu.VMEM((12, 8, 128), jnp.int32),
        pltpu.VMEM((2, L // 2, 128), U32),
        pltpu.VMEM((2, 4, 88, 128), F32),
        pltpu.VMEM((2, 4, 8, 32, 128), BF16),
        pltpu.VMEM((2, 4, 80, 128), F32),
        pltpu.VMEM((4, NT, 64, 128), U32),
        pltpu.SMEM((1,), jnp.int32),
        pltpu.SemaphoreType.DMA((5,)),
    ]
    scratch += [pltpu.VMEM((N2, N1 // 2, 128), U32)] * (2 * NT)
    scratch += [pltpu.VMEM((N1 // 8 + 1, 4, 4, 2, 8, 128), F32)] * (2 * NT)
    scratch += [pltpu.VMEM((N2, N1, 128), U32)] * NT
    scratch += [pltpu.VMEM((N2, N1, 128), F32)] * NT
    scratch += [pltpu.VMEM((S // 2 + 32, 128), U32)] * NT
    scratch += [pltpu.VMEM((2, 512, 128), F32)] * NSLOT
    scratch += [
        pltpu.VMEM((KS, D), BF16),
        pltpu.VMEM((NT, 128), BF16),
        pltpu.VMEM((1, H), BF16),
    ]
    return pl.pallas_call(
        _kernel,
        out_shape=jax.ShapeDtypeStruct((1, S, 2 * D), BF16),
        in_specs=[hbm] * 14,
        out_specs=hbm,
        scratch_shapes=scratch,
        compiler_params=pltpu.CompilerParams(vmem_limit_bytes=110 * 1024 * 1024),
        name="h3_infini",
    )(A_q, A_k, A_v, A_shift_k.T, A_ssm_k, A_ssm_D.reshape(NT, 128), B_x, B_wq, B_wk, B_wv, B_wo,
      B_beta.reshape(1, H), _FWD, _INV)
```

```python
import math

import jax
import jax.numpy as jnp
import numpy as np
from jax import lax
from jax.experimental import pallas as pl
from jax.experimental.pallas import tpu as pltpu

S = 2048
D = 640
NT = D // 128
H = 32
DH = D // H
NSEG = 4
L = S // NSEG
KS = 4
N1, N2 = 128, 16

F32 = jnp.float32
BF16 = jnp.bfloat16
U32 = jnp.uint32
NN_DIMS = (((1,), (0,)), ((), ()))
NT_DIMS = (((1,), (1,)), ((), ()))
NEG = -1e30
LOG2E = 1.4426950408889634


def _pack_rows(a):
    u = a.astype(np.float32).astype(BF16).view(np.uint16).astype(np.uint32)
    return u[..., 0::2, :] | (u[..., 1::2, :] << 16)


def _dft_tables():
    k1 = np.arange(N1)
    fwd = np.zeros((N2, 2 * N1, N1), np.float64)
    inv = np.zeros((N2, N1, 2 * N1), np.float64)
    kappa = np.arange(N1)
    n1_in = 16 * (kappa // 16) + 8 * (kappa % 2) + (kappa % 16) // 2
    row_re = 16 * (k1 // 8) + k1 % 8
    for n2 in range(N2):
        ang = 2.0 * np.pi * np.outer(k1 + 0.25, N2 * n1_in + n2) / S
        fwd[n2, row_re] = np.cos(ang)
        fwd[n2, row_re + 8] = np.sin(ang)
        ang = 2.0 * np.pi * np.outer(N2 * np.arange(N1) + n2, k1 + 0.25) / S
        inv[n2][:, 2 * k1] = np.cos(ang) / S
        inv[n2][:, 2 * k1 + 1] = np.sin(ang) / S
    inv = inv.reshape(N2, N1, 2, N1).transpose(0, 2, 1, 3)
    return _pack_rows(fwd), _pack_rows(inv)


_FWD, _INV = _dft_tables()


def _dot(a, b, dims=NN_DIMS):
    return lax.dot_general(a, b, dims, preferred_element_type=F32)


def _u32(x):
    return pltpu.bitcast(x, U32)


def _bf(x):
    return pltpu.bitcast(x, BF16)


def _u32_word(x):
    return lax.bitcast_convert_type(x, U32)


def _pack2(a, b):
    return pltpu.pack_elementwise([a, b], packed_dtype=BF16).astype(U32)


def _lo(w):
    return pltpu.unpack_elementwise(w, index=0, packed_dtype=BF16, unpacked_dtype=F32)


def _hi(w):
    return pltpu.unpack_elementwise(w, index=1, packed_dtype=BF16, unpacked_dtype=F32)


def _radix4(x0, x1, x2, x3, sign):
    ar, ai = x0[0] + x2[0], x0[1] + x2[1]
    br, bi = x0[0] - x2[0], x0[1] - x2[1]
    cr, ci = x1[0] + x3[0], x1[1] + x3[1]
    dr, di = x1[0] - x3[0], x1[1] - x3[1]
    y0 = (ar + cr, ai + ci)
    y2 = (ar - cr, ai - ci)
    yp = (br - di, bi + dr)
    ym = (br + di, bi - dr)
    return (y0, yp, y2, ym) if sign > 0 else (y0, ym, y2, yp)


def _twiddle(x, e, sign):
    xr, xi = x
    if e == 0:
        return x
    if e == 4:
        return (-xi, xr) if sign > 0 else (xi, -xr)
    r = math.sqrt(0.5)
    if e == 2:
        return ((xr - xi) * r, (xr + xi) * r) if sign > 0 else ((xr + xi) * r, (xi - xr) * r)
    if e == 6:
        return ((xr + xi) * -r, (xr - xi) * r) if sign > 0 else ((xi - xr) * r, (xr + xi) * -r)
    c, s = math.cos(math.pi * e / 8), sign * math.sin(math.pi * e / 8)
    return (xr * c - xi * s, xr * s + xi * c)


def _radix4_tw(x0, x1, x2, x3, sign, b):
    if b != 2:
        return _radix4(x0, _twiddle(x1, b, sign), _twiddle(x2, 2 * b, sign),
                       _twiddle(x3, 3 * b, sign), sign)
    x1, x3 = _twiddle(x1, 2, sign), _twiddle(x3, 6, sign)
    if sign > 0:
        ar, ai = x0[0] - x2[1], x0[1] + x2[0]
        br, bi = x0[0] + x2[1], x0[1] - x2[0]
    else:
        ar, ai = x0[0] + x2[1], x0[1] - x2[0]
        br, bi = x0[0] - x2[1], x0[1] + x2[0]
    cr, ci = x1[0] + x3[0], x1[1] + x3[1]
    dr, di = x1[0] - x3[0], x1[1] - x3[1]
    y0 = (ar + cr, ai + ci)
    y2 = (ar - cr, ai - ci)
    yp = (br - di, bi + dr)
    ym = (br + di, bi - dr)
    return (y0, yp, y2, ym) if sign > 0 else (y0, ym, y2, yp)


class _Paced:
    def __init__(self, streams, sequential=False):
        self.live = [[g, total, 0] for g, total in streams if total]
        self.total = sum(total for _, total in streams)
        self.done = 0
        self.sequential = sequential

    def step(self):
        cur = self.live[0] if self.sequential else min(self.live, key=lambda e: e[2] / e[1])
        cost = next(cur[0], None)
        if cost is None:
            self.live.remove(cur)
        else:
            cur[2] += cost
            self.done += cost

    def advance(self, fraction):
        while self.live and self.done < fraction * self.total:
            self.step()

    def finish(self):
        self.advance(math.inf)


SPLIT = ((0, 1, 2), (3, 4), (), ())
FORWARD = ((), (0, 1), (2, 3, 4), ())
SPECTRUM = ((), (), (0, 1), (2, 3))
INVERSE = ((), (), (), (0, 1))
DEPTH = 3
NSLOT = 4
ORDER = ((1, 3, 0, 2), (3, 2, 1, 0), (0, 2, 1, 3), (0, 1, 2, 3))
TAIL = (-0.03, -0.03, 0.02, -0.03)
LW = (1.0, 1.0, 1.0, 1.0)
AW = (4.0, 2.0, 4.0, 2.0, 3.0)
QCH = (128, 256, 128, 128)
HEAD = (4, 6, 6, 6)
FILL_ORDER = (0, 1, 1, 2)
PACE_ON = (3, 3, 7, 7, 7)
SIDE_SPEED = (1.03, 1.0, 1.03, 1.0)
MID = 3
PACE_ALL = (3, 2, 2, 3, 0)
SPEC_V = (0, 0, 0, 0, 1)
W_STAGES = ((0, 1), (1, 3), (3, 5))


def _kernel(aq_hbm, ak_hbm, av_hbm, shift_hbm, h_hbm, ssmd_hbm, x_hbm, wq_hbm, wk_hbm,
            wv_hbm, wo_hbm, beta_hbm, fwd_hbm, inv_hbm, out_hbm,
            xb, wqb, wkb, wvb, wob, wvt, hb, ht, kb, vb, qb, fwd, inv,
            ub, outb, wtab, gtab, cmask,
            q0, q1, k0, k1, pq0, pq1, pk0, pk1, ots, mst,
            hmask, hsel, bmask, kwin, vall, vhead, opart, onat, sem_zero, sems, *rest):
    xp, hp, tx, th, yb, kvf, outa = (rest[NT * k:NT * k + NT] for k in range(7))
    slots = rest[7 * NT:7 * NT + NSLOT]
    shift_ref, ssmd_ref, beta_ref = rest[7 * NT + NSLOT:]
    qs, ks, pqs, pks = (q0, q1), (k0, k1), (pq0, pq1), (pk0, pk1)

    def copy(src, dst, sem):
        return [lambda: pltpu.make_async_copy(src, dst, sems.at[sem])]

    def tiles(src, dst, sem, r0, n, ts=range(NT), off=0):
        src = src.bitcast(U32)
        lead = (0,) * (len(src.shape) - 2)
        return [cp for t in ts for cp in copy(
            src.at[lead + (pl.ds(r0 // 2, n // 2), pl.ds(128 * t, 128))],
            dst.at[t, pl.ds(off + r0 // 2, n // 2), :], sem)]

    def conv_inputs(cs, r0, n, sem):
        return (tiles(h_hbm, hb, sem, 128 * cs[0], 128 * len(cs), range(r0 // 128, (r0 + n) // 128))
                + tiles(ak_hbm, kb, sem, r0, n, cs, off=32) + tiles(av_hbm, vb, sem, r0, n, cs))

    def w_stage(k, sem):
        return (tiles(wq_hbm, wqb, sem, 0, D, range(*W_STAGES[k]))
                + tiles(wk_hbm, wkb, sem, 0, D, range(*W_STAGES[k])))

    cp_first = w_stage(0, 0) + tiles(x_hbm, xb, 0, 0, 256)
    cp_x0 = tiles(x_hbm, xb, 1, 256, 256)
    cp_w1, cp_w2 = w_stage(1, 2), w_stage(2, 3)
    cp_wv = (tiles(wv_hbm, wvb, 0, 0, D) + copy(shift_hbm, shift_ref, 0)
             + copy(ssmd_hbm, ssmd_ref, 0) + copy(beta_hbm, beta_ref, 0))
    cp_step = [tiles(x_hbm, xb, sem, L + 128 * i, 128) + conv_inputs(SPLIT[0], L * i, L, sem)
               for i, sem in enumerate((4, 0, 1, 2))]
    cp_seg1 = (tiles(wo_hbm, wob, 3, 0, D) + tiles(x_hbm, xb, 3, 2 * L, L)
               + copy(fwd_hbm, fwd, 3) + conv_inputs(SPLIT[1], 0, S, 3))
    cp_seg2 = (tiles(x_hbm, xb, 4, 3 * L, L) + copy(inv_hbm, inv, 4)
               + tiles(aq_hbm, qb, 4, 0, S))
    cp_oa = [copy(outa[c].at[pl.ds(0, S // 2), :],
                  out_hbm.bitcast(U32).at[0, :, pl.ds(128 * c, 128)], 0) for c in range(NT)]

    def out_b(tile, ns=range(NT)):
        at = pl.ds(128 * tile if isinstance(tile, int) else pl.multiple_of(128 * tile, 128), 128)
        return [cp for n in ns for cp in copy(
            outb.at[n, at, :], out_hbm.at[0, at, pl.ds(D + 128 * n, 128)], 1)]

    all_of_b = copy(outb, outb, 1)

    def start(*groups):
        for g in groups:
            for cp in g:
                cp().start()

    def wait(*groups):
        for g in groups:
            for cp in g:
                cp().wait()

    def rows(i, n):
        return pl.ds(pl.multiple_of(i * n, n), n) if not isinstance(i, int) else pl.ds(i * n, n)

    lane = lax.broadcasted_iota(jnp.int32, (8, 128), 1)
    sub = lax.broadcasted_iota(jnp.int32, (8, 128), 0)

    def lanes(n):
        return lax.broadcasted_iota(jnp.int32, (n, 128), 1)

    recent = [None]
    seg = [0]

    def dot(a, b, dims=NN_DIMS, kind=4):
        out = _dot(a, b, dims)
        if kind & PACE_ON[seg[0]]:
            recent[0] = out
        return out

    current = {}

    def pace(zero):
        v = recent[0][-8:]
        recent[0] = None
        if "h" in current:
            hb[S // 128, rows(zero, 8), :] = _u32_word(v)
        if "k" in current:
            kb[NT, rows(zero, 8), :] = _u32_word(v)
        if "t" in current:
            th[current["t"]][N1 // 8, zero, 0, 0] = v
            if PACE_ALL[seg[0]] & 1:
                tx[current["t"]][N1 // 8, zero, 0, 0] = v
            if PACE_ALL[seg[0]] & 2:
                ub[16, zero, 0, 0] = v

    def qk_proj(s, i, want_pq, want_pk):
        p = s % 2
        tok = rows(4 * s + i, 64)
        for w_ref, dst, fdst, want, scale in (
                (wqb, qs[p], pqs[p], want_pq, DH ** -0.5 * LOG2E),
                (wkb, ks[p], pks[p], want_pk, None)):
            for n in range(NT):
                t = None
                for c in range(NT):
                    part = dot(_bf(xb[c, tok, :]), _bf(w_ref[n, 64 * c:64 * c + 64, :]))
                    t = part if t is None else t + part
                    if c < NT - 1:
                        yield 32
                dst[n, rows(i, 128), :] = (t if scale is None else t * scale).astype(BF16)
                if want:
                    fdst[n, rows(i, 128), :] = jnp.where(t > 0, t + 1.0, jnp.exp(t)).astype(BF16)
                yield 32

    def first_proj(n, js=range(4)):
        for w_ref, dst, scale in ((wqb, qs[0], DH ** -0.5 * LOG2E), (wkb, ks[0], None)):
            for j in js:
                t = None
                for c in range(NT):
                    part = dot(_bf(xb[c, rows(j, 64), :]), _bf(w_ref[n, 64 * c:64 * c + 64, :]))
                    t = part if t is None else t + part
                dst[n, rows(j, 128), :] = (t if scale is None else t * scale).astype(BF16)
                if scale is None:
                    pks[0][n, rows(j, 128), :] = jnp.where(t > 0, t + 1.0, jnp.exp(t)).astype(BF16)

    def untranspose(s, i, slot=0):
        ot = ots.bitcast(U32)
        for c in range(NT):
            onat[slot, c] = _u32(_bf(ot[s % 2, i, 64 * c:64 * c + 64, :]).T)

    def out_proj(s, i, slot=0):
        for n in range(NT):
            t = None
            for c in range(NT):
                part = dot(_bf(onat[slot, c]), _bf(wob[n, 64 * c:64 * c + 64, :]))
                t = part if t is None else t + part
                if c < NT - 1:
                    yield 32
            outb[n, rows(4 * s + i, 128), :] = t.astype(BF16)
            if s == NSEG - 1:
                start(out_b(4 * s + i, (n,)))
            yield 32

    def tile_rows(r, n):
        return jnp.broadcast_to(r[None], (n // 8, 8, 128)).reshape(n, 128)

    class Group:
        def __init__(self, s, g, gi):
            self.s, self.g, self.gi = s, g, gi
            self.t0 = (80 * g) // 128
            self.off = 80 * g - 128 * self.t0
            self.t1 = jnp.minimum(self.t0 + 1, NT - 1)
            rel = (lane - self.off) & 127
            head = sum((rel >= a * DH).astype(jnp.int32) for a in range(1, 5))
            for a in range(4):
                hmask[gi, a] = jnp.where(head == a, np.uint32(0xFFFFFFFF), np.uint32(0))
            hsel[gi] = jnp.left_shift(1, head)
            self.have_keys, self.have_mem = set(), set()

        def window(self, ref, j, r0=0, n=64):
            ref = ref.bitcast(U32)
            at = pl.ds(64 * j + r0, n)
            return jnp.where(lanes(n) >= self.off, ref[self.t0, at, :], ref[self.t1, at, :])

        def keys(self, r0, r1):
            out = []
            for r in range(r0, r1, 64):
                at = pl.ds(r // 2, 32)
                if r in self.have_keys:
                    out.append(kwin[self.gi, at, :])
                else:
                    self.have_keys.add(r)
                    out.append(self.window(ks[self.s % 2], 0, r // 2, 32))
                    kwin[self.gi, at, :] = out[-1]
            return _bf(jnp.concatenate(out, axis=0))

        def park_values(self, j, v80):
            if self.s < NSEG - 1:
                vall[self.gi, j, 0:80, :] = v80
            ones8 = jnp.ones((8, 128), F32)
            for pr in range(2):
                for e in range(2):
                    r0 = 40 * pr + 16 * e
                    vhead[self.gi, j, r0 // 8] = jnp.concatenate(
                        [v80[r0:r0 + 24], ones8], axis=0).astype(BF16)

        def mem_read(self):
            for j in range(4):
                r = dot(mst[self.g, 0:88, :], _bf(self.window(pqs[self.s % 2], j)), NT_DIMS)
                coef = gtab[self.g, 0] / (r[80:88] + 1e-6)
                cb = [jnp.broadcast_to(coef[a:a + 1], (8, 128)) for a in range(4)]
                for pr in range(2):
                    ca, cc = cb[2 * pr], cb[2 * pr + 1]
                    for e, scale in enumerate((ca, ca, jnp.where(sub < 4, ca, cc), cc, cc)):
                        r0 = 40 * pr + 8 * e
                        opart[self.gi, j, r0:r0 + 8, :] = r[r0:r0 + 8] * scale
                self.have_mem.add(j)
                yield 24

        def mem_update(self):
            acc = None
            for j in range(4):
                t = dot(vall[self.gi, j], _bf(self.window(pks[self.s % 2], j)))
                acc = t if acc is None else acc + t
                if j < 3:
                    yield 24
            for r in range(11):
                new = jnp.where(bmask[r] & hsel[self.gi] != 0, acc[8 * r:8 * r + 8], 0.0)
                at = pl.ds(8 * r, 8)
                mst[self.g, at, :] = new if self.s == 0 else mst[self.g, at, :] + new
            yield 24

        def logits(self, pr, j, slot):
            qw = self.window(qs[self.s % 2], j)
            qa = qw & tile_rows(hmask[self.gi, 2 * pr], 64)
            qh = qw & tile_rows(hmask[self.gi, 2 * pr + 1], 64)
            w_a = _bf(qa)
            w_b = _bf(jnp.concatenate([qh[32:64], qh[0:32]], axis=0))
            w_t = _bf(jnp.concatenate([qh[32:64], qa[32:64]], axis=0))
            n = 128 * j

            def park(t, e, r0, m):
                for r in range(0, t.shape[0], 8):
                    v = t[r:r + 8]
                    if e == 2:
                        v = v + cmask[2, r:r + 8, :]
                    elif r0 + r >= n:
                        v = v + cmask[e, r0 + r - n:r0 + r - n + 8, :]
                    slot[e % 2, 448 * (e // 2) + r0 + r:448 * (e // 2) + r0 + r + 8, :] = v
                    m = v if m is None else jnp.maximum(m, v)
                return m

            m_t = park(dot(self.keys(n + 64, n + 128), w_t, NT_DIMS, 1), 2, 0, None)
            yield 16 * LW[seg[0] % 4]
            cuts = list(range(0, n, QCH[seg[0]])) or [0]
            m = [None, None]
            for r0, r1 in zip(cuts, cuts[1:] + [n + 64]):
                for e, w in enumerate((w_a, w_b)):
                    m[e] = park(dot(self.keys(r0, r1), w, NT_DIMS, 1), e, r0, m[e])
                    if r1 == n + 64 and e == 1:
                        m_a = jnp.maximum(m[0], jnp.where(lane >= 64, m_t, NEG))
                        m_b = jnp.maximum(m[1], jnp.where(lane < 64, m_t, NEG))
                        m_a = jnp.broadcast_to(jnp.max(m_a, axis=0, keepdims=True), (8, 128))
                        m_b = jnp.broadcast_to(jnp.max(m_b, axis=0, keepdims=True), (8, 128))
                        slot[1, 448:456, :] = m_a
                        slot[1, 456:464, :] = m_b
                        slot[1, 464:472, :] = jnp.where(lane < 64, m_b, m_a)
                    yield (r1 - r0) // 4 * LW[seg[0] % 4]

    def attend(gi, g, parity, add_mem, pr, j, slot, need_values):
        def prob(e, r0, n, which):
            m2 = tile_rows(slot[1, 448 + 8 * which:456 + 8 * which, :], 16)
            return [jnp.exp2(slot[e, r:r + 16, :] - m2) for r in range(r0, r0 + n, 16)]

        res = [None, None]
        order = [(0, j), (1, j)] + [(e, kt) for e in range(2) for kt in range(j)]
        for n, (e, kt) in enumerate(order):
            need_values(kt)
            if n == 0:
                p_t = prob(0, 448, 64, 2)
            if kt < j:
                p = prob(e, 128 * kt, 128, e)
            else:
                mine = lanes(16) >= 64 if e == 0 else lanes(16) < 64
                p = prob(e, 128 * kt, 64, e) + [jnp.where(mine, t, 0.0) for t in p_t]
            t = dot(_bf(vhead.bitcast(U32)[gi, kt, 5 * pr + 2 * e]),
                    jnp.concatenate(p, axis=0).astype(BF16), kind=2)
            res[e] = t if res[e] is None else res[e] + t
            if n < len(order) - 1:
                yield 8 * AW[seg[0]]
        r_a = res[0]
        r_b = pltpu.roll(res[1], 64, 1)
        keep = 1.0 - gtab[g, 0]
        keep_a = jnp.broadcast_to(keep[2 * pr:2 * pr + 1], (8, 128))
        keep_b = jnp.broadcast_to(keep[2 * pr + 1:2 * pr + 2], (8, 128))
        o_a = r_a[0:24] * tile_rows(keep_a / r_a[24:32], 24)
        o_b = r_b[0:24] * tile_rows(keep_b / r_b[24:32], 24)
        o = jnp.concatenate(
            [o_a[0:16], jnp.where(sub < 4, o_a[16:24], o_b[0:8]), o_b[8:24]], axis=0)
        if add_mem:
            o = o + opart[gi, j, 40 * pr:40 * pr + 40, :]
        if pr == 0:
            opart[gi, j, 0:40, :] = o
        else:
            o = jnp.concatenate([opart[gi, j, 0:40, :], o], axis=0)
            ots[parity, j, rows(g, 80), :] = o.astype(BF16)
        yield 8 * AW[seg[0]]

    def v_proj(s, i, groups, have):
        for j in range(4):
            acc = None
            for c in range(NT):
                t = dot(_bf(wvt[c, i, 0:80, :]), _bf(xb[c, rows(4 * s + j, 64), :]), NT_DIMS)
                acc = t if acc is None else acc + t
                if c == NT - 1:
                    for gi in range(2):
                        groups[gi].park_values(j, acc[80 * gi:80 * gi + 80])
                    have.append(j)
                yield 40

    def chain(*gens):
        for g in gens:
            yield from g

    def units(s):
        return [(gi, pr, j) for gi in range(2) for pr in range(2)
                for j in (range(4) if (gi, pr) == (1, 1) else ORDER[s] if gi + pr else range(4))]

    def cost(j):
        return (48 + 64 * j) * LW[seg[0] % 4], (16 + 16 * j) * AW[seg[0]]

    def carried(u, g, parity):
        gi, pr, j = units(0)[u]
        return attend(gi, g, parity, True, pr, j, slots[u % NSLOT], lambda kt: None), cost(j)[1]

    def segment_step(s, i):
        seg[0] = s
        parts = {}
        if s < NSEG - 1:
            parts["qk"] = (qk_proj(s + 1, i, True, s + 1 < NSEG - 1), 1600)
        if s > 0:
            parts["out"] = (out_proj(s - 1, i), 800)
        if FORWARD[s]:
            parts["fwd"] = (fwd_fft(i, FORWARD[s]), 512 * len(FORWARD[s]))
        if INVERSE[s]:
            parts["inv"] = (inverse(INVERSE[s], (2 * i, 2 * i + 1)), 256 * len(INVERSE[s]))
        names = (("qk", "inv", "out", "fwd"), ("qk", "inv", "fwd", "out"),
                 ("inv", "fwd", "qk", "out"), ("qk", "inv", "out", "fwd"))[FILL_ORDER[s]]
        fill = _Paced([parts[n] for n in names if n in parts], sequential=FILL_ORDER[s] < 3)
        side = []
        if SPECTRUM[s]:
            side.append((spectra(SPECTRUM[s], [4 * i + a for a in range(4)]),
                         4 * SPEC_COST * len(SPECTRUM[s])))
        for c in SPLIT[s]:
            side += [(split_h(i, c), 144), (split_kv(i, c), 704)]
        side = _Paced(side, sequential=True)
        current.clear()
        recent[0] = None
        for _ in range(HEAD[s]):
            fill.step()
        if s > 0:
            untranspose(s - 1, i)
        vt = []
        groups = [Group(s, 2 * i + gi, gi) for gi in range(2)]
        reads = [grp.mem_read() for grp in groups if s > 0]
        updates = [grp.mem_update() for grp in groups if s < NSEG - 1]
        first = _Paced([(chain(*reads[:1], v_proj(s, i, groups, vt), *reads[1:], *updates),
                         800 + 96 * (len(reads) + len(updates)))])
        total = first.total + fill.total
        held = 96 * (s > 0) + 159

        def need_values(kt):
            while len(vt) <= kt:
                first.step()

        def pad(fraction, u):
            target = total * fraction / (1 + TAIL[s])
            early = min(target, held if u < DEPTH else first.total)
            first.advance(early / first.total)
            fill.advance((target - early) / fill.total)
            goal = fraction * SIDE_SPEED[s]
            if side.live and side.done < goal * side.total and recent[0] is not None:
                pace(jnp.minimum(i, 3))
                side.advance(goal)

        todo = units(s)
        whole = sum(sum(cost(j)) for _, _, j in todo)
        done = 0
        for u, (gi, pr, j) in enumerate(todo):
            streams = [(groups[gi].logits(pr, j, slots[u % NSLOT]), cost(j)[0])]
            v = u - DEPTH
            if v < 0:
                streams.append(carried(v + len(todo), (2 * i + 7) & 7,
                                       jnp.where(i > 0, s % 2, 1 - s % 2)))
            else:
                gi, pr, j = todo[v]
                while s > 0 and j not in groups[gi].have_mem:
                    first.step()
                streams.append((attend(gi, 2 * i + gi, s % 2, s > 0, pr, j, slots[v % NSLOT],
                                       need_values), cost(j)[1]))
            att = _Paced(streams[::-1], sequential=u == len(todo) - 1)
            while att.live:
                att.step()
                pad((done + att.done) / whole, u)
            done += att.total
        first.finish()
        fill.finish()
        side.finish()

    def split_h(i, c):
        current.clear()
        current["h"] = True
        for t in range(4):
            ht[c, 64 * t:64 * t + 64, :] = _u32(
                _bf(hb[4 * i + t, 64 * c:64 * c + 64, :]).T)
            yield 4
        for q in range(2):
            for j in range(8):
                wa = ht[c, pl.ds(128 * q + j, 8, stride=8), :]
                wb = ht[c, pl.ds(128 * q + 64 + j, 8, stride=8), :]
                hp[c][2 * j, rows(2 * i + q, 8), :] = _pack2(_lo(wa), _lo(wb))
                hp[c][2 * j + 1, rows(2 * i + q, 8), :] = _pack2(_hi(wa), _hi(wb))
                if j % 2:
                    yield 16

    def split_kv(i, c):
        current.clear()
        current["k"] = True
        taps = [wtab[c, j] for j in range(KS)]
        for q in range(2):
            blk = 2 * i + q
            base = [blk * 128 + 64 * e for e in range(2)]
            hist = []
            for e in range(2):
                w2 = kb[c, pl.ds(base[e] + 30, 8, stride=8), :]
                w1 = kb[c, pl.ds(base[e] + 31, 8, stride=8), :]
                hist.append([_hi(w2), _lo(w1), _hi(w1)])
            for j in range(8):
                kv = [[None, None], [None, None]]
                for e in range(2):
                    kw = kb[c, pl.ds(base[e] + 32 + j, 8, stride=8), :]
                    vw = vb[c, pl.ds(base[e] + j, 8, stride=8), :]
                    kp = hist[e] + [_lo(kw), _hi(kw)]
                    for half, part in enumerate((_lo, _hi)):
                        acc = kp[3 + half] * taps[0]
                        for d in range(1, KS):
                            acc = acc + kp[3 + half - d] * taps[d]
                        kv[half][e] = acc * part(vw)
                        kvf[c][2 * j + half, rows(2 * blk + e, 8), :] = kv[half][e]
                    hist[e] = kp[2:]
                    if e == 0:
                        yield 22
                for half in range(2):
                    xp[c][2 * j + half, rows(blk, 8), :] = _pack2(*kv[half])
                yield 22

    def fwd_fft(i, cs):
        for c in cs:
            for src, dst in ((hp[c], th[c]), (xp[c], tx[c])):
                g = [dot(_bf(fwd[4 * a + i]), _bf(src[4 * a + i])) for a in range(4)]
                for r in range(0, 2 * N1, 16):
                    z = _radix4(*[(g[a][r:r + 8], g[a][r + 8:r + 16]) for a in range(4)], 1)
                    for cc in range(4):
                        dst[r // 16, i, cc, 0] = z[cc][0]
                        dst[r // 16, i, cc, 1] = z[cc][1]
                yield 256

    def spectrum(c, m, slot):
        current.clear()
        current["t"] = c
        for cc in range(4):
            zh = _radix4_tw(*[(th[c][m, b, cc, 0], th[c][m, b, cc, 1]) for b in range(4)], 1, cc)
            yield 17
            zx = _radix4_tw(*[(tx[c][m, b, cc, 0], tx[c][m, b, cc, 1]) for b in range(4)], 1, cc)
            yield 17
            y = [(x[0] * h[0] - x[1] * h[1], x[0] * h[1] + x[1] * h[0]) for x, h in zip(zx, zh)]
            yield 17
            u = _radix4(*y, -1)
            for b in range(4):
                ub[slot, b, cc, 0] = u[b][0]
                ub[slot, b, cc, 1] = u[b][1]
            yield 17
        if SPEC_V[seg[0]]:
            return

        yield from spectrum_end(c, m, slot)

    def spectrum_end(c, m, slot):
        for b in range(4):
            z = _radix4_tw(*[(ub[slot, b, cc, 0], ub[slot, b, cc, 1]) for cc in range(4)], -1, b)
            for a in range(4):
                yb[c][4 * a + b, rows(m, 8), :] = _pack2(*z[a])
            yield 17

    SPEC_COST = 17 * 20

    def spectra(cs, ms, slot0=0):
        prev = None
        for slot, (c, m) in enumerate(((c, m) for c in cs for m in ms), slot0):
            yield from spectrum(c, m, slot)
            if SPEC_V[seg[0]] and prev is not None:
                yield from spectrum_end(*prev)
            prev = (c, m, slot)
        if SPEC_V[seg[0]]:
            yield from spectrum_end(*prev)

    def inverse(cs, jps):
        for c in cs:
            for jp in jps:
                w = qb[c, pl.ds(jp, N1, stride=8), :]
                res = []
                for e, part in enumerate((_lo, _hi)):
                    n2 = 2 * jp + e
                    y = dot(_bf(inv[n2, 0]), _bf(yb[c][n2, 0:64, :]))
                    yield 32
                    y = y + dot(_bf(inv[n2, 1]), _bf(yb[c][n2, 64:128, :]))
                    res.append(part(w) * (y + kvf[c][n2] * tile_rows(wtab[c, KS], N1)))
                    if e == 0:
                        yield 32
                outa[c][pl.ds(jp, N1, stride=8), :] = _pack2(*res)
                yield 32

    start(cp_first, cp_x0, cp_w1)
    sem_zero[0] = 0
    kk = lax.broadcasted_iota(jnp.int32, (64, 128), 0)
    ll = lax.broadcasted_iota(jnp.int32, (64, 128), 1)
    cmask[0] = jnp.where(kk <= ll, 0.0, NEG)
    cmask[1] = jnp.where((ll < 64) | (kk <= ll - 64), 0.0, NEG)
    cmask[2] = jnp.where(kk <= (ll & 63), 0.0, NEG)
    for r in range(11):
        row = sub + 8 * r
        hr = sum((row >= a * DH).astype(jnp.int32) for a in range(1, 4)) if r < 10 else row - 80
        bmask[r] = jnp.left_shift(1, hr)
    for gi in range(2):
        for j in range(4):
            vall[gi, j, 80:88, :] = jnp.ones((8, 128), F32)
    for c in range(NT):
        kb[c, 24:32, :] = jnp.zeros((8, 128), U32)
    for u in range(16 - DEPTH, 16):
        slots[u % NSLOT][...] = jnp.zeros((2, 512, 128), F32)
    vhead[1] = jnp.ones(vhead.shape[1:], BF16)
    opart[1] = jnp.zeros(opart.shape[1:], F32)
    with jax.named_scope("prologue"):
        wait(cp_first)
        start(cp_w2, cp_wv, cp_step[0])
        first_proj(0, (0, 1))
        wait(cp_x0)
        first_proj(0, (2, 3))
        wait(cp_w1)
        for n in range(*W_STAGES[1]):
            first_proj(n)
        wait(cp_w2)
        first_proj(W_STAGES[2][0])
        wait(cp_wv)
        start(cp_step[1])
        taps_t = shift_ref[...].astype(F32)
        skip = ssmd_ref[...].astype(F32)
        for c in range(NT):
            for j in range(KS):
                wtab[c, j] = jnp.broadcast_to(taps_t[j:j + 1, 128 * c:128 * c + 128], (8, 128))
            wtab[c, KS] = jnp.broadcast_to(skip[c:c + 1], (8, 128))
        gates = jax.nn.sigmoid(beta_ref[...].astype(F32))
        gcol = jnp.broadcast_to(gates, (8, H)).T
        gcol = jnp.broadcast_to(gcol[:, 0:1], (H, 128))
        for g in range(8):
            gtab[g, 0] = jnp.concatenate([gcol[4 * g:4 * g + 4]] * 2, axis=0)
        for n in range(NT):
            for c in range(NT):
                wt = _u32(_bf(wvb[n, 64 * c:64 * c + 64, :]).T)
                for r in range(0, 64, 16):
                    step, r0 = divmod(64 * n + r, 80)
                    wvt[c, step, r0:r0 + 16, :] = wt[r:r + 16]
        for n in range(W_STAGES[2][0] + 1, NT):
            first_proj(n)

    def segment(s):
        def body(i, carry):
            if s == 0:
                for j in range(4):
                    @pl.when(i == j)
                    def _():
                        wait(cp_step[j])
                        start(*((cp_step[2],), (cp_step[3],), (cp_seg1,), (cp_seg2,))[j])
            segment_step(s, i)
            if s > 0:
                start(out_b(4 * (s - 1) + i))
            return carry

        with jax.named_scope(f"seg{s}"):
            lax.fori_loop(0, 4, body, 0)

    segment(0)
    wait(cp_seg1)
    segment(1)
    wait(cp_seg2)
    segment(2)
    segment(3)
    start(*[cp_oa[c] for c in INVERSE[3]])
    with jax.named_scope("epilogue"):
        seg[0] = 4
        current.clear()
        recent[0] = None
        last = NT - 1
        rest_tiles = [c for c in range(last) if c not in INVERSE[3]]
        side = _Paced([(spectra((last,), range(16)), 16 * SPEC_COST)])
        span = 1024 * len(rest_tiles) + 800 * MID
        done = 0

        def run(streams):
            nonlocal done
            work = _Paced(streams)
            while work.live:
                before = work.done
                work.step()
                done += work.done - before
                if side.live and side.done < done / span * side.total and recent[0] is not None:
                    pace(sem_zero[0])
                    side.advance(done / span)

        for c in rest_tiles:
            streams = [(inverse((c,), range(8)), 1024)]
            if c == rest_tiles[0]:
                tail = [carried(u, 7, 1) for u in range(16 - DEPTH, 16)]
                streams.append((chain(*[g for g, _ in tail]), sum(w for _, w in tail)))
            run(streams)
            if c == rest_tiles[0]:
                for i in range(4):
                    untranspose(3, i, i)
            start(cp_oa[c])
        for i in range(4):
            if i == MID:
                side.finish()
                run([(inverse((last,), range(8)), 1024)])
                start(cp_oa[last])
            run([(out_proj(3, i, i), 800)])
    wait(*cp_oa, all_of_b)


@jax.jit
def pallas_concat_heads__ssm_conv_h3__memory_aug_infini_attn__prompt_kernel(
    A_q: jax.Array,
    A_k: jax.Array,
    A_v: jax.Array,
    A_shift_k: jax.Array,
    A_ssm_k: jax.Array,
    A_ssm_D: jax.Array,
    B_x: jax.Array,
    B_wq: jax.Array,
    B_wk: jax.Array,
    B_wv: jax.Array,
    B_wo: jax.Array,
    B_beta: jax.Array,
):
    hbm = pl.BlockSpec(memory_space=pltpu.HBM)
    seg_tiles = pltpu.VMEM((NT, L, 128), BF16)
    weight = pltpu.VMEM((NT, D // 2, 128), U32)
    scratch = [
        pltpu.VMEM((NT, S // 2, 128), U32),
        weight, weight, weight, weight,
        pltpu.VMEM((NT, 4, 96, 128), U32),
        pltpu.VMEM((S // 128 + 1, D // 2, 128), U32),
        pltpu.VMEM((NT, 256 + 32, 128), U32),
        pltpu.VMEM((NT + 1, S // 2 + 64, 128), U32),
        pltpu.VMEM((NT, S // 2 + 32, 128), U32),
        pltpu.VMEM((NT, S // 2 + 32, 128), U32),
        pltpu.VMEM((N2, N1, 128), U32),
        pltpu.VMEM((N2, 2, N1 // 2, 128), U32),
        pltpu.VMEM((17, 4, 4, 2, 8, 128), F32),
        pltpu.VMEM((NT, S, 128), BF16),
        pltpu.VMEM((NT, 8, 8, 128), F32),
        pltpu.VMEM((8, 4, 8, 128), F32),
        pltpu.VMEM((3, 64, 128), F32),
        seg_tiles, seg_tiles, seg_tiles, seg_tiles,
        seg_tiles, seg_tiles, seg_tiles, seg_tiles,
        pltpu.VMEM((2, 4, D, 128), BF16),
        pltpu.VMEM((8, 96, 128), F32),
        pltpu.VMEM((2, 4, 8, 128), U32),
        pltpu.VMEM((4, 8, 128), jnp.int32),
        pltpu.VMEM((12, 8, 128), jnp.int32),
        pltpu.VMEM((2, L // 2, 128), U32),
        pltpu.VMEM((2, 4, 88, 128), F32),
        pltpu.VMEM((2, 4, 8, 32, 128), BF16),
        pltpu.VMEM((2, 4, 80, 128), F32),
        pltpu.VMEM((4, NT, 64, 128), U32),
        pltpu.SMEM((1,), jnp.int32),
        pltpu.SemaphoreType.DMA((5,)),
    ]
    scratch += [pltpu.VMEM((N2, N1 // 2, 128), U32)] * (2 * NT)
    scratch += [pltpu.VMEM((N1 // 8 + 1, 4, 4, 2, 8, 128), F32)] * (2 * NT)
    scratch += [pltpu.VMEM((N2, N1, 128), U32)] * NT
    scratch += [pltpu.VMEM((N2, N1, 128), F32)] * NT
    scratch += [pltpu.VMEM((S // 2 + 32, 128), U32)] * NT
    scratch += [pltpu.VMEM((2, 512, 128), F32)] * NSLOT
    scratch += [
        pltpu.VMEM((KS, D), BF16),
        pltpu.VMEM((NT, 128), BF16),
        pltpu.VMEM((1, H), BF16),
    ]
    return pl.pallas_call(
        _kernel,
        out_shape=jax.ShapeDtypeStruct((1, S, 2 * D), BF16),
        in_specs=[hbm] * 14,
        out_specs=hbm,
        scratch_shapes=scratch,
        compiler_params=pltpu.CompilerParams(vmem_limit_bytes=110 * 1024 * 1024),
        name="h3_infini",
    )(A_q, A_k, A_v, A_shift_k.T, A_ssm_k, A_ssm_D.reshape(NT, 128), B_x, B_wq, B_wk, B_wv, B_wo,
      B_beta.reshape(1, H), _FWD, _INV)
```

```python
import math

import jax
import jax.numpy as jnp
import numpy as np
from jax import lax
from jax.experimental import pallas as pl
from jax.experimental.pallas import tpu as pltpu

S = 2048
D = 640
NT = D // 128
H = 32
DH = D // H
NSEG = 4
L = S // NSEG
KS = 4
N1, N2 = 128, 16

F32 = jnp.float32
BF16 = jnp.bfloat16
U32 = jnp.uint32
NN_DIMS = (((1,), (0,)), ((), ()))
NT_DIMS = (((1,), (1,)), ((), ()))
NEG = -1e30
LOG2E = 1.4426950408889634


def _pack_rows(a):
    u = a.astype(np.float32).astype(BF16).view(np.uint16).astype(np.uint32)
    return u[..., 0::2, :] | (u[..., 1::2, :] << 16)


def _dft_tables():
    k1 = np.arange(N1)
    fwd = np.zeros((N2, 2 * N1, N1), np.float64)
    inv = np.zeros((N2, N1, 2 * N1), np.float64)
    kappa = np.arange(N1)
    n1_in = 16 * (kappa // 16) + 8 * (kappa % 2) + (kappa % 16) // 2
    row_re = 16 * (k1 // 8) + k1 % 8
    for n2 in range(N2):
        ang = 2.0 * np.pi * np.outer(k1 + 0.25, N2 * n1_in + n2) / S
        fwd[n2, row_re] = np.cos(ang)
        fwd[n2, row_re + 8] = np.sin(ang)
        ang = 2.0 * np.pi * np.outer(N2 * np.arange(N1) + n2, k1 + 0.25) / S
        inv[n2][:, 2 * k1] = np.cos(ang) / S
        inv[n2][:, 2 * k1 + 1] = np.sin(ang) / S
    inv = inv.reshape(N2, N1, 2, N1).transpose(0, 2, 1, 3)
    return _pack_rows(fwd), _pack_rows(inv)


_FWD, _INV = _dft_tables()


def _dot(a, b, dims=NN_DIMS):
    return lax.dot_general(a, b, dims, preferred_element_type=F32)


def _u32(x):
    return pltpu.bitcast(x, U32)


def _bf(x):
    return pltpu.bitcast(x, BF16)


def _u32_word(x):
    return lax.bitcast_convert_type(x, U32)


def _pack2(a, b):
    return pltpu.pack_elementwise([a, b], packed_dtype=BF16).astype(U32)


def _lo(w):
    return pltpu.unpack_elementwise(w, index=0, packed_dtype=BF16, unpacked_dtype=F32)


def _hi(w):
    return pltpu.unpack_elementwise(w, index=1, packed_dtype=BF16, unpacked_dtype=F32)


def _radix4(x0, x1, x2, x3, sign):
    ar, ai = x0[0] + x2[0], x0[1] + x2[1]
    br, bi = x0[0] - x2[0], x0[1] - x2[1]
    cr, ci = x1[0] + x3[0], x1[1] + x3[1]
    dr, di = x1[0] - x3[0], x1[1] - x3[1]
    y0 = (ar + cr, ai + ci)
    y2 = (ar - cr, ai - ci)
    yp = (br - di, bi + dr)
    ym = (br + di, bi - dr)
    return (y0, yp, y2, ym) if sign > 0 else (y0, ym, y2, yp)


def _twiddle(x, e, sign):
    xr, xi = x
    if e == 0:
        return x
    if e == 4:
        return (-xi, xr) if sign > 0 else (xi, -xr)
    r = math.sqrt(0.5)
    if e == 2:
        return ((xr - xi) * r, (xr + xi) * r) if sign > 0 else ((xr + xi) * r, (xi - xr) * r)
    if e == 6:
        return ((xr + xi) * -r, (xr - xi) * r) if sign > 0 else ((xi - xr) * r, (xr + xi) * -r)
    c, s = math.cos(math.pi * e / 8), sign * math.sin(math.pi * e / 8)
    return (xr * c - xi * s, xr * s + xi * c)


def _radix4_tw(x0, x1, x2, x3, sign, b):
    if b != 2:
        return _radix4(x0, _twiddle(x1, b, sign), _twiddle(x2, 2 * b, sign),
                       _twiddle(x3, 3 * b, sign), sign)
    x1, x3 = _twiddle(x1, 2, sign), _twiddle(x3, 6, sign)
    if sign > 0:
        ar, ai = x0[0] - x2[1], x0[1] + x2[0]
        br, bi = x0[0] + x2[1], x0[1] - x2[0]
    else:
        ar, ai = x0[0] + x2[1], x0[1] - x2[0]
        br, bi = x0[0] - x2[1], x0[1] + x2[0]
    cr, ci = x1[0] + x3[0], x1[1] + x3[1]
    dr, di = x1[0] - x3[0], x1[1] - x3[1]
    y0 = (ar + cr, ai + ci)
    y2 = (ar - cr, ai - ci)
    yp = (br - di, bi + dr)
    ym = (br + di, bi - dr)
    return (y0, yp, y2, ym) if sign > 0 else (y0, ym, y2, yp)


class _Paced:
    def __init__(self, streams, sequential=False):
        self.live = [[g, total, 0] for g, total in streams if total]
        self.total = sum(total for _, total in streams)
        self.done = 0
        self.sequential = sequential

    def step(self):
        cur = self.live[0] if self.sequential else min(self.live, key=lambda e: e[2] / e[1])
        cost = next(cur[0], None)
        if cost is None:
            self.live.remove(cur)
        else:
            cur[2] += cost
            self.done += cost

    def advance(self, fraction):
        while self.live and self.done < fraction * self.total:
            self.step()

    def finish(self):
        self.advance(math.inf)


SPLIT = ((0, 1, 2), (3, 4), (), ())
FORWARD = ((), (0, 1), (2, 3, 4), ())
SPECTRUM = ((), (), (0, 1), (2, 3))
INVERSE = ((), (), (), (0, 1))
W_STAGES = ((0, 1), (1, 3), (3, 5))
DEPTH = 3
NSLOT = 4
ORDER = ((1, 3, 0, 2), (3, 2, 1, 0), (0, 2, 1, 3), (0, 1, 2, 3))
TAIL = (-0.03, 0.02, 0.02, -0.03)
QCH = (128, 256, 192, 128)
HEAD = (4, 4, 6, 6)
FILL_ORDER = (0, 1, 1, 0)
SIDE_SPEED = (1.03, 1.0, 1.0, 1.0, 1.0)
AW = (4.0, 2.0, 4.0, 2.0, 3.0)
PACE_ON = (3, 3, 7, 7, 7)
PACE_ALL = (3, 2, 2, 2, 0)
SPEC_V = (0, 0, 0, 0, 1)
MID = 15


def _kernel(aq_hbm, ak_hbm, av_hbm, shift_hbm, h_hbm, ssmd_hbm, x_hbm, wq_hbm, wk_hbm,
            wv_hbm, wo_hbm, beta_hbm, fwd_hbm, inv_hbm, out_hbm,
            xb, wqb, wkb, wvb, wob, wvt, hb, ht, kb, vb, qb, fwd, inv,
            ub, outb, wtab, gtab, cmask,
            q0, q1, k0, k1, pq0, pq1, pk0, pk1, ots, mst,
            hmask, hsel, bmask, kwin, vall, vhead, opart, onat, zero_ref, sems, *rest):
    xp, hp, tx, th, yb, kvf, outa = (rest[NT * k:NT * k + NT] for k in range(7))
    slots = rest[7 * NT:7 * NT + NSLOT]
    shift_ref, ssmd_ref, beta_ref = rest[7 * NT + NSLOT:]
    qs, ks, pqs, pks = (q0, q1), (k0, k1), (pq0, pq1), (pk0, pk1)

    def copy(src, dst, sem):
        return [lambda: pltpu.make_async_copy(src, dst, sems.at[sem])]

    def tiles(src, dst, sem, r0, n, ts=range(NT), off=0):
        src = src.bitcast(U32)
        lead = (0,) * (len(src.shape) - 2)
        return [cp for t in ts for cp in copy(
            src.at[lead + (pl.ds(r0 // 2, n // 2), pl.ds(128 * t, 128))],
            dst.at[t, pl.ds(off + r0 // 2, n // 2), :], sem)]

    def conv_inputs(cs, r0, n, sem):
        return (tiles(h_hbm, hb, sem, 128 * cs[0], 128 * len(cs), range(r0 // 128, (r0 + n) // 128))
                + tiles(ak_hbm, kb, sem, r0, n, cs, off=32) + tiles(av_hbm, vb, sem, r0, n, cs))

    def w_stage(k, sem):
        return (tiles(wq_hbm, wqb, sem, 0, D, range(*W_STAGES[k]))
                + tiles(wk_hbm, wkb, sem, 0, D, range(*W_STAGES[k])))

    cp_first = w_stage(0, 0) + tiles(x_hbm, xb, 0, 0, 256)
    cp_x0 = tiles(x_hbm, xb, 1, 256, 256)
    cp_w1, cp_w2 = w_stage(1, 2), w_stage(2, 3)
    cp_wv = (tiles(wv_hbm, wvb, 0, 0, D) + copy(shift_hbm, shift_ref, 0)
             + copy(ssmd_hbm, ssmd_ref, 0) + copy(beta_hbm, beta_ref, 0))
    cp_step = [tiles(x_hbm, xb, sem, L + 128 * i, 128) + conv_inputs(SPLIT[0], L * i, L, sem)
               for i, sem in enumerate((4, 0, 1, 2))]
    cp_seg1 = (tiles(wo_hbm, wob, 3, 0, D) + tiles(x_hbm, xb, 3, 2 * L, L)
               + copy(fwd_hbm, fwd, 3) + conv_inputs(SPLIT[1], 0, S, 3))
    cp_seg2 = (tiles(x_hbm, xb, 4, 3 * L, L) + copy(inv_hbm, inv, 4)
               + tiles(aq_hbm, qb, 4, 0, S))
    cp_oa = [copy(outa[c].at[pl.ds(0, S // 2), :],
                  out_hbm.bitcast(U32).at[0, :, pl.ds(128 * c, 128)], 0) for c in range(NT)]

    def out_b(tile, ns=range(NT)):
        at = pl.ds(128 * tile if isinstance(tile, int) else pl.multiple_of(128 * tile, 128), 128)
        return [cp for n in ns for cp in copy(
            outb.at[n, at, :], out_hbm.at[0, at, pl.ds(D + 128 * n, 128)], 1)]

    all_of_b = copy(outb, outb, 1)

    def start(*groups):
        for g in groups:
            for cp in g:
                cp().start()

    def wait(*groups):
        for g in groups:
            for cp in g:
                cp().wait()

    def rows(i, n):
        return pl.ds(pl.multiple_of(i * n, n), n) if not isinstance(i, int) else pl.ds(i * n, n)

    lane = lax.broadcasted_iota(jnp.int32, (8, 128), 1)
    sub = lax.broadcasted_iota(jnp.int32, (8, 128), 0)

    def lanes(n):
        return lax.broadcasted_iota(jnp.int32, (n, 128), 1)

    recent = [None]
    seg = [0]

    def dot(a, b, dims=NN_DIMS, kind=4):
        out = _dot(a, b, dims)
        if kind & PACE_ON[seg[0]]:
            recent[0] = out
        return out

    current = {}

    def pace(zero):
        v = recent[0][-8:]
        recent[0] = None
        if "h" in current:
            hb[S // 128, rows(zero, 8), :] = _u32_word(v)
        if "k" in current:
            kb[NT, rows(zero, 8), :] = _u32_word(v)
        if "t" in current:
            th[current["t"]][N1 // 8, zero, 0, 0] = v
            if PACE_ALL[seg[0]] & 1:
                tx[current["t"]][N1 // 8, zero, 0, 0] = v
            if PACE_ALL[seg[0]] & 2:
                ub[16, zero, 0, 0] = v

    def qk_proj(s, i, want_pq, want_pk):
        p = s % 2
        tok = rows(4 * s + i, 64)
        for w_ref, dst, fdst, want, scale in (
                (wqb, qs[p], pqs[p], want_pq, DH ** -0.5 * LOG2E),
                (wkb, ks[p], pks[p], want_pk, None)):
            for n in range(NT):
                t = None
                for c in range(NT):
                    part = dot(_bf(xb[c, tok, :]), _bf(w_ref[n, 64 * c:64 * c + 64, :]))
                    t = part if t is None else t + part
                    if c < NT - 1:
                        yield 32
                dst[n, rows(i, 128), :] = (t if scale is None else t * scale).astype(BF16)
                if want:
                    fdst[n, rows(i, 128), :] = jnp.where(t > 0, t + 1.0, jnp.exp(t)).astype(BF16)
                yield 32

    def first_proj(n, js=range(4)):
        for w_ref, dst, scale in ((wqb, qs[0], DH ** -0.5 * LOG2E), (wkb, ks[0], None)):
            for j in js:
                t = None
                for c in range(NT):
                    part = dot(_bf(xb[c, rows(j, 64), :]), _bf(w_ref[n, 64 * c:64 * c + 64, :]))
                    t = part if t is None else t + part
                dst[n, rows(j, 128), :] = (t if scale is None else t * scale).astype(BF16)
                if scale is None:
                    pks[0][n, rows(j, 128), :] = jnp.where(t > 0, t + 1.0, jnp.exp(t)).astype(BF16)

    def untranspose(s, i, slot=0):
        ot = ots.bitcast(U32)
        for c in range(NT):
            onat[slot, c] = _u32(_bf(ot[s % 2, i, 64 * c:64 * c + 64, :]).T)

    def out_proj(s, i, slot=0):
        for n in range(NT):
            t = None
            for c in range(NT):
                part = dot(_bf(onat[slot, c]), _bf(wob[n, 64 * c:64 * c + 64, :]))
                t = part if t is None else t + part
                if c < NT - 1:
                    yield 32
            outb[n, rows(4 * s + i, 128), :] = t.astype(BF16)
            if s == NSEG - 1:
                start(out_b(4 * s + i, (n,)))
            yield 32

    def tile_rows(r, n):
        return jnp.broadcast_to(r[None], (n // 8, 8, 128)).reshape(n, 128)

    class Group:
        def __init__(self, s, g, gi):
            self.s, self.g, self.gi = s, g, gi
            self.t0 = (80 * g) // 128
            self.off = 80 * g - 128 * self.t0
            self.t1 = jnp.minimum(self.t0 + 1, NT - 1)
            rel = (lane - self.off) & 127
            head = sum((rel >= a * DH).astype(jnp.int32) for a in range(1, 5))
            for a in range(4):
                hmask[gi, a] = jnp.where(head == a, np.uint32(0xFFFFFFFF), np.uint32(0))
            hsel[gi] = jnp.left_shift(1, head)
            self.have_keys, self.have_mem = set(), set()

        def window(self, ref, j, r0=0, n=64):
            ref = ref.bitcast(U32)
            at = pl.ds(64 * j + r0, n)
            return jnp.where(lanes(n) >= self.off, ref[self.t0, at, :], ref[self.t1, at, :])

        def keys(self, r0, r1):
            out = []
            for r in range(r0, r1, 64):
                at = pl.ds(r // 2, 32)
                if r in self.have_keys:
                    out.append(kwin[self.gi, at, :])
                else:
                    self.have_keys.add(r)
                    out.append(self.window(ks[self.s % 2], 0, r // 2, 32))
                    kwin[self.gi, at, :] = out[-1]
            return _bf(jnp.concatenate(out, axis=0))

        def park_values(self, j, v80):
            if self.s < NSEG - 1:
                vall[self.gi, j, 0:80, :] = v80
            ones8 = jnp.ones((8, 128), F32)
            for pr in range(2):
                for e in range(2):
                    r0 = 40 * pr + 16 * e
                    vhead[self.gi, j, r0 // 8] = jnp.concatenate(
                        [v80[r0:r0 + 24], ones8], axis=0).astype(BF16)

        def mem_read(self):
            for j in range(4):
                r = dot(mst[self.g, 0:88, :], _bf(self.window(pqs[self.s % 2], j)), NT_DIMS)
                coef = gtab[self.g, 0] / (r[80:88] + 1e-6)
                cb = [jnp.broadcast_to(coef[a:a + 1], (8, 128)) for a in range(4)]
                for pr in range(2):
                    ca, cc = cb[2 * pr], cb[2 * pr + 1]
                    for e, scale in enumerate((ca, ca, jnp.where(sub < 4, ca, cc), cc, cc)):
                        r0 = 40 * pr + 8 * e
                        opart[self.gi, j, r0:r0 + 8, :] = r[r0:r0 + 8] * scale
                self.have_mem.add(j)
                yield 24

        def mem_update(self):
            acc = None
            for j in range(4):
                t = dot(vall[self.gi, j], _bf(self.window(pks[self.s % 2], j)))
                acc = t if acc is None else acc + t
                if j < 3:
                    yield 24
            for r in range(11):
                new = jnp.where(bmask[r] & hsel[self.gi] != 0, acc[8 * r:8 * r + 8], 0.0)
                at = pl.ds(8 * r, 8)
                mst[self.g, at, :] = new if self.s == 0 else mst[self.g, at, :] + new
            yield 24

        def logits(self, pr, j, slot):
            qw = self.window(qs[self.s % 2], j)
            qa = qw & tile_rows(hmask[self.gi, 2 * pr], 64)
            qh = qw & tile_rows(hmask[self.gi, 2 * pr + 1], 64)
            w_a = _bf(qa)
            w_b = _bf(jnp.concatenate([qh[32:64], qh[0:32]], axis=0))
            w_t = _bf(jnp.concatenate([qh[32:64], qa[32:64]], axis=0))
            n = 128 * j

            def park(t, e, r0, m):
                for r in range(0, t.shape[0], 8):
                    v = t[r:r + 8]
                    if e == 2:
                        v = v + cmask[2, r:r + 8, :]
                    elif r0 + r >= n:
                        v = v + cmask[e, r0 + r - n:r0 + r - n + 8, :]
                    slot[e % 2, 448 * (e // 2) + r0 + r:448 * (e // 2) + r0 + r + 8, :] = v
                    m = v if m is None else jnp.maximum(m, v)
                return m

            m_t = park(dot(self.keys(n + 64, n + 128), w_t, NT_DIMS, 1), 2, 0, None)
            yield 16
            cuts = list(range(0, n, QCH[seg[0]])) or [0]
            m = [None, None]
            for r0, r1 in zip(cuts, cuts[1:] + [n + 64]):
                for e, w in enumerate((w_a, w_b)):
                    m[e] = park(dot(self.keys(r0, r1), w, NT_DIMS, 1), e, r0, m[e])
                    if r1 == n + 64 and e == 1:
                        m_a = jnp.maximum(m[0], jnp.where(lane >= 64, m_t, NEG))
                        m_b = jnp.maximum(m[1], jnp.where(lane < 64, m_t, NEG))
                        m_a = jnp.broadcast_to(jnp.max(m_a, axis=0, keepdims=True), (8, 128))
                        m_b = jnp.broadcast_to(jnp.max(m_b, axis=0, keepdims=True), (8, 128))
                        slot[1, 448:456, :] = m_a
                        slot[1, 456:464, :] = m_b
                        slot[1, 464:472, :] = jnp.where(lane < 64, m_b, m_a)
                    yield (r1 - r0) // 4

    def attend(gi, g, parity, add_mem, pr, j, slot, need_values):
        def prob(e, r0, n, which):
            m2 = tile_rows(slot[1, 448 + 8 * which:456 + 8 * which, :], 16)
            return [jnp.exp2(slot[e, r:r + 16, :] - m2) for r in range(r0, r0 + n, 16)]

        res = [None, None]
        order = [(0, j), (1, j)] + [(e, kt) for e in range(2) for kt in range(j)]
        for n, (e, kt) in enumerate(order):
            need_values(kt)
            if n == 0:
                p_t = prob(0, 448, 64, 2)
            if kt < j:
                p = prob(e, 128 * kt, 128, e)
            else:
                mine = lanes(16) >= 64 if e == 0 else lanes(16) < 64
                p = prob(e, 128 * kt, 64, e) + [jnp.where(mine, t, 0.0) for t in p_t]
            t = dot(_bf(vhead.bitcast(U32)[gi, kt, 5 * pr + 2 * e]),
                    jnp.concatenate(p, axis=0).astype(BF16), kind=2)
            res[e] = t if res[e] is None else res[e] + t
            if n < len(order) - 1:
                yield 8 * AW[seg[0]]
        r_a = res[0]
        r_b = pltpu.roll(res[1], 64, 1)
        keep = 1.0 - gtab[g, 0]
        keep_a = jnp.broadcast_to(keep[2 * pr:2 * pr + 1], (8, 128))
        keep_b = jnp.broadcast_to(keep[2 * pr + 1:2 * pr + 2], (8, 128))
        o_a = r_a[0:24] * tile_rows(keep_a / r_a[24:32], 24)
        o_b = r_b[0:24] * tile_rows(keep_b / r_b[24:32], 24)
        o = jnp.concatenate(
            [o_a[0:16], jnp.where(sub < 4, o_a[16:24], o_b[0:8]), o_b[8:24]], axis=0)
        if add_mem:
            o = o + opart[gi, j, 40 * pr:40 * pr + 40, :]
        if pr == 0:
            opart[gi, j, 0:40, :] = o
        else:
            o = jnp.concatenate([opart[gi, j, 0:40, :], o], axis=0)
            ots[parity, j, rows(g, 80), :] = o.astype(BF16)
        yield 8 * AW[seg[0]]

    def v_proj(s, i, groups, have):
        for j in range(4):
            acc = None
            for c in range(NT):
                t = dot(_bf(wvt[c, i, 0:80, :]), _bf(xb[c, rows(4 * s + j, 64), :]), NT_DIMS)
                acc = t if acc is None else acc + t
                if c == NT - 1:
                    for gi in range(2):
                        groups[gi].park_values(j, acc[80 * gi:80 * gi + 80])
                    have.append(j)
                yield 40

    def chain(*gens):
        for g in gens:
            yield from g

    def units(s):
        return [(gi, pr, j) for gi in range(2) for pr in range(2)
                for j in (range(4) if (gi, pr) == (1, 1) else ORDER[s] if gi + pr else range(4))]

    def cost(j):
        return 48 + 64 * j, (16 + 16 * j) * AW[seg[0]]

    def carried(u, g, parity):
        gi, pr, j = units(0)[u]
        return attend(gi, g, parity, True, pr, j, slots[u % NSLOT], lambda kt: None), cost(j)[1]

    def segment_step(s, i):
        seg[0] = s
        parts = {}
        if s < NSEG - 1:
            parts["qk"] = (qk_proj(s + 1, i, True, s + 1 < NSEG - 1), 1600)
        if s > 0:
            parts["out"] = (out_proj(s - 1, i), 800)
        if FORWARD[s]:
            parts["fwd"] = (fwd_fft(i, FORWARD[s]), 512 * len(FORWARD[s]))
        if INVERSE[s]:
            parts["inv"] = (inverse(INVERSE[s], (2 * i, 2 * i + 1)), 256 * len(INVERSE[s]))
        names = (("qk", "inv", "out", "fwd"), ("qk", "inv", "fwd", "out"),
                 ("inv", "fwd", "qk", "out"), ("qk", "inv", "out", "fwd"))[FILL_ORDER[s]]
        fill = _Paced([parts[n] for n in names if n in parts], sequential=FILL_ORDER[s] < 3)
        side = []
        if SPECTRUM[s]:
            side.append((spectra(SPECTRUM[s], [4 * i + a for a in range(4)]),
                         4 * SPEC_COST * len(SPECTRUM[s])))
        for c in SPLIT[s]:
            side += [(split_h(i, c), 144), (split_kv(i, c), 704)]
        side = _Paced(side, sequential=True)
        current.clear()
        recent[0] = None
        for _ in range(HEAD[s]):
            fill.step()
        if s > 0:
            untranspose(s - 1, i)
        vt = []
        groups = [Group(s, 2 * i + gi, gi) for gi in range(2)]
        reads = [grp.mem_read() for grp in groups if s > 0]
        updates = [grp.mem_update() for grp in groups if s < NSEG - 1]
        first = _Paced([(chain(*reads[:1], v_proj(s, i, groups, vt), *reads[1:], *updates),
                         800 + 96 * (len(reads) + len(updates)))])
        total = first.total + fill.total
        held = 96 * (s > 0) + 159

        def need_values(kt):
            while len(vt) <= kt:
                first.step()

        def pad(fraction, u):
            target = total * fraction / (1 + TAIL[s])
            early = min(target, held if u < DEPTH else first.total)
            first.advance(early / first.total)
            fill.advance((target - early) / fill.total)
            goal = fraction * SIDE_SPEED[s]
            if side.live and side.done < goal * side.total and recent[0] is not None:
                pace(jnp.minimum(i, 3))
                side.advance(goal)

        todo = units(s)
        whole = sum(sum(cost(j)) for _, _, j in todo)
        done = 0
        for u, (gi, pr, j) in enumerate(todo):
            streams = [(groups[gi].logits(pr, j, slots[u % NSLOT]), cost(j)[0])]
            v = u - DEPTH
            if v < 0:
                streams.append(carried(v + len(todo), (2 * i + 7) & 7,
                                       jnp.where(i > 0, s % 2, 1 - s % 2)))
            else:
                gi, pr, j = todo[v]
                while s > 0 and j not in groups[gi].have_mem:
                    first.step()
                streams.append((attend(gi, 2 * i + gi, s % 2, s > 0, pr, j, slots[v % NSLOT],
                                       need_values), cost(j)[1]))
            att = _Paced(streams[::-1], sequential=u == len(todo) - 1)
            while att.live:
                att.step()
                pad((done + att.done) / whole, u)
            done += att.total
        first.finish()
        fill.finish()
        side.finish()

    def split_h(i, c):
        current.clear()
        current["h"] = True
        for t in range(4):
            ht[c, 64 * t:64 * t + 64, :] = _u32(
                _bf(hb[4 * i + t, 64 * c:64 * c + 64, :]).T)
            yield 4
        for q in range(2):
            for j in range(8):
                wa = ht[c, pl.ds(128 * q + j, 8, stride=8), :]
                wb = ht[c, pl.ds(128 * q + 64 + j, 8, stride=8), :]
                hp[c][2 * j, rows(2 * i + q, 8), :] = _pack2(_lo(wa), _lo(wb))
                hp[c][2 * j + 1, rows(2 * i + q, 8), :] = _pack2(_hi(wa), _hi(wb))
                if j % 2:
                    yield 16

    def split_kv(i, c):
        current.clear()
        current["k"] = True
        taps = [wtab[c, j] for j in range(KS)]
        for q in range(2):
            blk = 2 * i + q
            base = [blk * 128 + 64 * e for e in range(2)]
            hist = []
            for e in range(2):
                w2 = kb[c, pl.ds(base[e] + 30, 8, stride=8), :]
                w1 = kb[c, pl.ds(base[e] + 31, 8, stride=8), :]
                hist.append([_hi(w2), _lo(w1), _hi(w1)])
            for j in range(8):
                kv = [[None, None], [None, None]]
                for e in range(2):
                    kw = kb[c, pl.ds(base[e] + 32 + j, 8, stride=8), :]
                    vw = vb[c, pl.ds(base[e] + j, 8, stride=8), :]
                    kp = hist[e] + [_lo(kw), _hi(kw)]
                    for half, part in enumerate((_lo, _hi)):
                        acc = kp[3 + half] * taps[0]
                        for d in range(1, KS):
                            acc = acc + kp[3 + half - d] * taps[d]
                        kv[half][e] = acc * part(vw)
                        kvf[c][2 * j + half, rows(2 * blk + e, 8), :] = kv[half][e]
                    hist[e] = kp[2:]
                    if e == 0:
                        yield 22
                for half in range(2):
                    xp[c][2 * j + half, rows(blk, 8), :] = _pack2(*kv[half])
                yield 22

    def fwd_fft(i, cs):
        for c in cs:
            for src, dst in ((hp[c], th[c]), (xp[c], tx[c])):
                g = [dot(_bf(fwd[4 * a + i]), _bf(src[4 * a + i])) for a in range(4)]
                for r in range(0, 2 * N1, 16):
                    z = _radix4(*[(g[a][r:r + 8], g[a][r + 8:r + 16]) for a in range(4)], 1)
                    for cc in range(4):
                        dst[r // 16, i, cc, 0] = z[cc][0]
                        dst[r // 16, i, cc, 1] = z[cc][1]
                yield 256

    def spectrum(c, m, slot):
        current.clear()
        current["t"] = c
        for cc in range(4):
            zh = _radix4_tw(*[(th[c][m, b, cc, 0], th[c][m, b, cc, 1]) for b in range(4)], 1, cc)
            yield 17
            zx = _radix4_tw(*[(tx[c][m, b, cc, 0], tx[c][m, b, cc, 1]) for b in range(4)], 1, cc)
            yield 17
            y = [(x[0] * h[0] - x[1] * h[1], x[0] * h[1] + x[1] * h[0]) for x, h in zip(zx, zh)]
            yield 17
            u = _radix4(*y, -1)
            for b in range(4):
                ub[slot, b, cc, 0] = u[b][0]
                ub[slot, b, cc, 1] = u[b][1]
            yield 17
        if SPEC_V[seg[0]]:
            return

        yield from spectrum_end(c, m, slot)

    def spectrum_end(c, m, slot):
        for b in range(4):
            z = _radix4_tw(*[(ub[slot, b, cc, 0], ub[slot, b, cc, 1]) for cc in range(4)], -1, b)
            for a in range(4):
                yb[c][4 * a + b, rows(m, 8), :] = _pack2(*z[a])
            yield 17

    SPEC_COST = 17 * 20

    def spectra(cs, ms, slot0=0):
        prev = None
        for slot, (c, m) in enumerate(((c, m) for c in cs for m in ms), slot0):
            yield from spectrum(c, m, slot)
            if SPEC_V[seg[0]] and prev is not None:
                yield from spectrum_end(*prev)
            prev = (c, m, slot)
        if SPEC_V[seg[0]]:
            yield from spectrum_end(*prev)

    def inverse(cs, jps):
        for c in cs:
            for jp in jps:
                w = qb[c, pl.ds(jp, N1, stride=8), :]
                res = []
                for e, part in enumerate((_lo, _hi)):
                    n2 = 2 * jp + e
                    y = dot(_bf(inv[n2, 0]), _bf(yb[c][n2, 0:64, :]))
                    yield 32
                    y = y + dot(_bf(inv[n2, 1]), _bf(yb[c][n2, 64:128, :]))
                    res.append(part(w) * (y + kvf[c][n2] * tile_rows(wtab[c, KS], N1)))
                    if e == 0:
                        yield 32
                outa[c][pl.ds(jp, N1, stride=8), :] = _pack2(*res)
                yield 32

    start(cp_first, cp_x0, cp_w1)
    zero_ref[0] = 0
    kk = lax.broadcasted_iota(jnp.int32, (64, 128), 0)
    ll = lax.broadcasted_iota(jnp.int32, (64, 128), 1)
    cmask[0] = jnp.where(kk <= ll, 0.0, NEG)
    cmask[1] = jnp.where((ll < 64) | (kk <= ll - 64), 0.0, NEG)
    cmask[2] = jnp.where(kk <= (ll & 63), 0.0, NEG)
    for r in range(11):
        row = sub + 8 * r
        hr = sum((row >= a * DH).astype(jnp.int32) for a in range(1, 4)) if r < 10 else row - 80
        bmask[r] = jnp.left_shift(1, hr)
    for gi in range(2):
        for j in range(4):
            vall[gi, j, 80:88, :] = jnp.ones((8, 128), F32)
    for c in range(NT):
        kb[c, 24:32, :] = jnp.zeros((8, 128), U32)
    for u in range(16 - DEPTH, 16):
        slots[u % NSLOT][...] = jnp.zeros((2, 512, 128), F32)
    vhead[1] = jnp.ones(vhead.shape[1:], BF16)
    opart[1] = jnp.zeros(opart.shape[1:], F32)
    wait(cp_first)
    start(cp_w2, cp_wv, cp_step[0])
    first_proj(0, (0, 1))
    wait(cp_x0)
    first_proj(0, (2, 3))
    wait(cp_w1)
    for n in range(*W_STAGES[1]):
        first_proj(n)
    wait(cp_w2)
    first_proj(W_STAGES[2][0])
    wait(cp_wv)
    start(cp_step[1])
    taps_t = shift_ref[...].astype(F32)
    skip = ssmd_ref[...].astype(F32)
    for c in range(NT):
        for j in range(KS):
            wtab[c, j] = jnp.broadcast_to(taps_t[j:j + 1, 128 * c:128 * c + 128], (8, 128))
        wtab[c, KS] = jnp.broadcast_to(skip[c:c + 1], (8, 128))
    gates = jax.nn.sigmoid(beta_ref[...].astype(F32))
    gcol = jnp.broadcast_to(gates, (8, H)).T
    gcol = jnp.broadcast_to(gcol[:, 0:1], (H, 128))
    for g in range(8):
        gtab[g, 0] = jnp.concatenate([gcol[4 * g:4 * g + 4]] * 2, axis=0)
    for n in range(NT):
        for c in range(NT):
            wt = _u32(_bf(wvb[n, 64 * c:64 * c + 64, :]).T)
            for r in range(0, 64, 16):
                step, r0 = divmod(64 * n + r, 80)
                wvt[c, step, r0:r0 + 16, :] = wt[r:r + 16]
    for n in range(W_STAGES[2][0] + 1, NT):
        first_proj(n)

    def segment(s):
        def body(i, carry):
            if s == 0:
                for j in range(4):
                    @pl.when(i == j)
                    def _():
                        wait(cp_step[j])
                        start(*((cp_step[2],), (cp_step[3],), (cp_seg1,), (cp_seg2,))[j])
            segment_step(s, i)
            if s > 0:
                start(out_b(4 * (s - 1) + i))
            return carry

        lax.fori_loop(0, 4, body, 0)

    segment(0)
    wait(cp_seg1)
    segment(1)
    wait(cp_seg2)
    segment(2)
    segment(3)
    start(*[cp_oa[c] for c in INVERSE[3]])
    seg[0] = 4
    current.clear()
    recent[0] = None
    last = NT - 1
    rest_tiles = [c for c in range(last) if c not in INVERSE[3]]
    side = _Paced([(spectra((last,), range(16)), 16 * SPEC_COST)])
    span = (1024 * len(rest_tiles) + 160 * MID) / SIDE_SPEED[4]
    done = 0

    def run(streams):
        nonlocal done
        work = _Paced(streams)
        while work.live:
            before = work.done
            work.step()
            done += work.done - before
            if side.live and side.done < done / span * side.total and recent[0] is not None:
                pace(zero_ref[0])
                side.advance(done / span)

    for c in rest_tiles:
        streams = [(inverse((c,), range(8)), 1024)]
        if c == rest_tiles[0]:
            tail = [carried(u, 7, 1) for u in range(16 - DEPTH, 16)]
            streams.append((chain(*[g for g, _ in tail]), sum(w for _, w in tail)))
        run(streams)
        if c == rest_tiles[0]:
            for i in range(4):
                untranspose(3, i, i)
        start(cp_oa[c])
    proj = _Paced([(chain(*[out_proj(3, i, i) for i in range(4)]), 3200)])

    def part(cost):
        goal = proj.done + cost
        while proj.live and proj.done < goal:
            before = proj.done
            proj.step()
            yield proj.done - before

    run([(part(160 * MID), 160 * MID)])
    side.finish()
    run([(inverse((last,), range(8)), 1024)])
    start(cp_oa[last])
    proj.finish()
    wait(*cp_oa, all_of_b)


@jax.jit
def pallas_concat_heads__ssm_conv_h3__memory_aug_infini_attn__prompt_kernel(
    A_q: jax.Array,
    A_k: jax.Array,
    A_v: jax.Array,
    A_shift_k: jax.Array,
    A_ssm_k: jax.Array,
    A_ssm_D: jax.Array,
    B_x: jax.Array,
    B_wq: jax.Array,
    B_wk: jax.Array,
    B_wv: jax.Array,
    B_wo: jax.Array,
    B_beta: jax.Array,
):
    hbm = pl.BlockSpec(memory_space=pltpu.HBM)
    seg_tiles = pltpu.VMEM((NT, L, 128), BF16)
    weight = pltpu.VMEM((NT, D // 2, 128), U32)
    scratch = [
        pltpu.VMEM((NT, S // 2, 128), U32),
        weight, weight, weight, weight,
        pltpu.VMEM((NT, 4, 96, 128), U32),
        pltpu.VMEM((S // 128 + 1, D // 2, 128), U32),
        pltpu.VMEM((NT, 256 + 32, 128), U32),
        pltpu.VMEM((NT + 1, S // 2 + 64, 128), U32),
        pltpu.VMEM((NT, S // 2 + 32, 128), U32),
        pltpu.VMEM((NT, S // 2 + 32, 128), U32),
        pltpu.VMEM((N2, N1, 128), U32),
        pltpu.VMEM((N2, 2, N1 // 2, 128), U32),
        pltpu.VMEM((17, 4, 4, 2, 8, 128), F32),
        pltpu.VMEM((NT, S, 128), BF16),
        pltpu.VMEM((NT, 8, 8, 128), F32),
        pltpu.VMEM((8, 4, 8, 128), F32),
        pltpu.VMEM((3, 64, 128), F32),
        seg_tiles, seg_tiles, seg_tiles, seg_tiles,
        seg_tiles, seg_tiles, seg_tiles, seg_tiles,
        pltpu.VMEM((2, 4, D, 128), BF16),
        pltpu.VMEM((8, 96, 128), F32),
        pltpu.VMEM((2, 4, 8, 128), U32),
        pltpu.VMEM((4, 8, 128), jnp.int32),
        pltpu.VMEM((12, 8, 128), jnp.int32),
        pltpu.VMEM((2, L // 2, 128), U32),
        pltpu.VMEM((2, 4, 88, 128), F32),
        pltpu.VMEM((2, 4, 8, 32, 128), BF16),
        pltpu.VMEM((2, 4, 80, 128), F32),
        pltpu.VMEM((4, NT, 64, 128), U32),
        pltpu.SMEM((1,), jnp.int32),
        pltpu.SemaphoreType.DMA((5,)),
    ]
    scratch += [pltpu.VMEM((N2, N1 // 2, 128), U32)] * (2 * NT)
    scratch += [pltpu.VMEM((N1 // 8 + 1, 4, 4, 2, 8, 128), F32)] * (2 * NT)
    scratch += [pltpu.VMEM((N2, N1, 128), U32)] * NT
    scratch += [pltpu.VMEM((N2, N1, 128), F32)] * NT
    scratch += [pltpu.VMEM((S // 2 + 32, 128), U32)] * NT
    scratch += [pltpu.VMEM((2, 512, 128), F32)] * NSLOT
    scratch += [
        pltpu.VMEM((KS, D), BF16),
        pltpu.VMEM((NT, 128), BF16),
        pltpu.VMEM((1, H), BF16),
    ]
    return pl.pallas_call(
        _kernel,
        out_shape=jax.ShapeDtypeStruct((1, S, 2 * D), BF16),
        in_specs=[hbm] * 14,
        out_specs=hbm,
        scratch_shapes=scratch,
        compiler_params=pltpu.CompilerParams(vmem_limit_bytes=110 * 1024 * 1024),
        name="h3_infini",
    )(A_q, A_k, A_v, A_shift_k.T, A_ssm_k, A_ssm_D.reshape(NT, 128), B_x, B_wq, B_wk, B_wv, B_wo,
      B_beta.reshape(1, H), _FWD, _INV)
```

```python
import math

import jax
import jax.numpy as jnp
import numpy as np
from jax import lax
from jax.experimental import pallas as pl
from jax.experimental.pallas import tpu as pltpu

S = 2048
D = 640
NT = D // 128
H = 32
DH = D // H
NSEG = 4
L = S // NSEG
KS = 4
N1, N2 = 128, 16

F32 = jnp.float32
BF16 = jnp.bfloat16
U32 = jnp.uint32
NN_DIMS = (((1,), (0,)), ((), ()))
NT_DIMS = (((1,), (1,)), ((), ()))
NEG = -1e30
LOG2E = 1.4426950408889634


def _pack_rows(a):
    u = a.astype(np.float32).astype(BF16).view(np.uint16).astype(np.uint32)
    return u[..., 0::2, :] | (u[..., 1::2, :] << 16)


def _dft_tables():
    k1 = np.arange(N1)
    fwd = np.zeros((N2, 2 * N1, N1), np.float64)
    inv = np.zeros((N2, N1, 2 * N1), np.float64)
    kappa = np.arange(N1)
    n1_in = 16 * (kappa // 16) + 8 * (kappa % 2) + (kappa % 16) // 2
    row_re = 16 * (k1 // 8) + k1 % 8
    for n2 in range(N2):
        ang = 2.0 * np.pi * np.outer(k1 + 0.25, N2 * n1_in + n2) / S
        fwd[n2, row_re] = np.cos(ang)
        fwd[n2, row_re + 8] = np.sin(ang)
        ang = 2.0 * np.pi * np.outer(N2 * np.arange(N1) + n2, k1 + 0.25) / S
        inv[n2][:, 2 * k1] = np.cos(ang) / S
        inv[n2][:, 2 * k1 + 1] = np.sin(ang) / S
    inv = inv.reshape(N2, N1, 2, N1).transpose(0, 2, 1, 3)
    return _pack_rows(fwd), _pack_rows(inv)


_FWD, _INV = _dft_tables()


def _dot(a, b, dims=NN_DIMS):
    return lax.dot_general(a, b, dims, preferred_element_type=F32)


def _u32(x):
    return pltpu.bitcast(x, U32)


def _bf(x):
    return pltpu.bitcast(x, BF16)


def _u32_word(x):
    return lax.bitcast_convert_type(x, U32)


def _pack2(a, b):
    return pltpu.pack_elementwise([a, b], packed_dtype=BF16).astype(U32)


def _lo(w):
    return pltpu.unpack_elementwise(w, index=0, packed_dtype=BF16, unpacked_dtype=F32)


def _hi(w):
    return pltpu.unpack_elementwise(w, index=1, packed_dtype=BF16, unpacked_dtype=F32)


def _radix4(x0, x1, x2, x3, sign):
    ar, ai = x0[0] + x2[0], x0[1] + x2[1]
    br, bi = x0[0] - x2[0], x0[1] - x2[1]
    cr, ci = x1[0] + x3[0], x1[1] + x3[1]
    dr, di = x1[0] - x3[0], x1[1] - x3[1]
    y0 = (ar + cr, ai + ci)
    y2 = (ar - cr, ai - ci)
    yp = (br - di, bi + dr)
    ym = (br + di, bi - dr)
    return (y0, yp, y2, ym) if sign > 0 else (y0, ym, y2, yp)


def _twiddle(x, e, sign):
    xr, xi = x
    if e == 0:
        return x
    if e == 4:
        return (-xi, xr) if sign > 0 else (xi, -xr)
    r = math.sqrt(0.5)
    if e == 2:
        return ((xr - xi) * r, (xr + xi) * r) if sign > 0 else ((xr + xi) * r, (xi - xr) * r)
    if e == 6:
        return ((xr + xi) * -r, (xr - xi) * r) if sign > 0 else ((xi - xr) * r, (xr + xi) * -r)
    c, s = math.cos(math.pi * e / 8), sign * math.sin(math.pi * e / 8)
    return (xr * c - xi * s, xr * s + xi * c)


def _radix4_tw(x0, x1, x2, x3, sign, b):
    if b != 2:
        return _radix4(x0, _twiddle(x1, b, sign), _twiddle(x2, 2 * b, sign),
                       _twiddle(x3, 3 * b, sign), sign)
    x1, x3 = _twiddle(x1, 2, sign), _twiddle(x3, 6, sign)
    if sign > 0:
        ar, ai = x0[0] - x2[1], x0[1] + x2[0]
        br, bi = x0[0] + x2[1], x0[1] - x2[0]
    else:
        ar, ai = x0[0] + x2[1], x0[1] - x2[0]
        br, bi = x0[0] - x2[1], x0[1] + x2[0]
    cr, ci = x1[0] + x3[0], x1[1] + x3[1]
    dr, di = x1[0] - x3[0], x1[1] - x3[1]
    y0 = (ar + cr, ai + ci)
    y2 = (ar - cr, ai - ci)
    yp = (br - di, bi + dr)
    ym = (br + di, bi - dr)
    return (y0, yp, y2, ym) if sign > 0 else (y0, ym, y2, yp)


class _Paced:
    def __init__(self, streams, sequential=False):
        self.live = [[g, total, 0] for g, total in streams if total]
        self.total = sum(total for _, total in streams)
        self.done = 0
        self.sequential = sequential

    def step(self):
        cur = self.live[0] if self.sequential else min(self.live, key=lambda e: e[2] / e[1])
        cost = next(cur[0], None)
        if cost is None:
            self.live.remove(cur)
        else:
            cur[2] += cost
            self.done += cost

    def advance(self, fraction):
        while self.live and self.done < fraction * self.total:
            self.step()

    def finish(self):
        self.advance(math.inf)


SPLIT = ((0, 1, 2), (3, 4), (), ())
FORWARD = ((), (0, 1), (2, 3, 4), ())
SPECTRUM = ((), (), (0, 1), (2, 3))
INVERSE = ((), (), (), (0, 1))
W_STAGES = ((0, 1), (1, 3), (3, 5))
DEPTH = 3
NSLOT = 4
ORDER = ((1, 3, 0, 2), (3, 2, 1, 0), (0, 2, 1, 3), (0, 1, 2, 3))
TAIL = (-0.03, 0.02, 0.02, -0.03)
QCH = (128, 192, 192, 128)
HEAD = (8, 2, 6, 6)
FILL_ORDER = (0, 1, 1, 0)
SIDE_SPEED = (1.015, 1.08, 1.0, 1.0, 1.0)
AW = (4.0, 2.0, 4.0, 2.0, 3.0)
PACE_ON = (3, 3, 7, 7, 7)
PACE_ALL = (3, 2, 2, 2, 0)
SPEC_V = (0, 0, 0, 0, 1)
MID = 15


def _kernel(aq_hbm, ak_hbm, av_hbm, shift_hbm, h_hbm, ssmd_hbm, x_hbm, wq_hbm, wk_hbm,
            wv_hbm, wo_hbm, beta_hbm, fwd_hbm, inv_hbm, out_hbm,
            xb, wqb, wkb, wvb, wob, wvt, hb, ht, kb, vb, qb, fwd, inv,
            ub, outb, wtab, gtab, cmask,
            q0, q1, k0, k1, pq0, pq1, pk0, pk1, ots, mst,
            hmask, hsel, bmask, kwin, vall, vhead, opart, onat, zero_ref, sems, *rest):
    xp, hp, tx, th, yb, kvf, outa = (rest[NT * k:NT * k + NT] for k in range(7))
    slots = rest[7 * NT:7 * NT + NSLOT]
    shift_ref, ssmd_ref, beta_ref = rest[7 * NT + NSLOT:]
    qs, ks, pqs, pks = (q0, q1), (k0, k1), (pq0, pq1), (pk0, pk1)

    def copy(src, dst, sem):
        return [lambda: pltpu.make_async_copy(src, dst, sems.at[sem])]

    def tiles(src, dst, sem, r0, n, ts=range(NT), off=0):
        src = src.bitcast(U32)
        lead = (0,) * (len(src.shape) - 2)
        return [cp for t in ts for cp in copy(
            src.at[lead + (pl.ds(r0 // 2, n // 2), pl.ds(128 * t, 128))],
            dst.at[t, pl.ds(off + r0 // 2, n // 2), :], sem)]

    def conv_inputs(cs, r0, n, sem):
        return (tiles(h_hbm, hb, sem, 128 * cs[0], 128 * len(cs), range(r0 // 128, (r0 + n) // 128))
                + tiles(ak_hbm, kb, sem, r0, n, cs, off=32) + tiles(av_hbm, vb, sem, r0, n, cs))

    def w_stage(k, sem):
        return (tiles(wq_hbm, wqb, sem, 0, D, range(*W_STAGES[k]))
                + tiles(wk_hbm, wkb, sem, 0, D, range(*W_STAGES[k])))

    cp_first = w_stage(0, 0) + tiles(x_hbm, xb, 0, 0, 256)
    cp_x0 = tiles(x_hbm, xb, 1, 256, 256)
    cp_w1, cp_w2 = w_stage(1, 2), w_stage(2, 3)
    cp_wv = (tiles(wv_hbm, wvb, 0, 0, D) + copy(shift_hbm, shift_ref, 0)
             + copy(ssmd_hbm, ssmd_ref, 0) + copy(beta_hbm, beta_ref, 0))
    cp_step = [tiles(x_hbm, xb, sem, L + 128 * i, 128) + conv_inputs(SPLIT[0], L * i, L, sem)
               for i, sem in enumerate((4, 0, 1, 2))]
    cp_seg1 = (tiles(wo_hbm, wob, 3, 0, D) + tiles(x_hbm, xb, 3, 2 * L, L)
               + copy(fwd_hbm, fwd, 3) + conv_inputs(SPLIT[1], 0, S, 3))
    cp_seg2 = (tiles(x_hbm, xb, 4, 3 * L, L) + copy(inv_hbm, inv, 4)
               + tiles(aq_hbm, qb, 4, 0, S))
    cp_oa = [copy(outa[c].at[pl.ds(0, S // 2), :],
                  out_hbm.bitcast(U32).at[0, :, pl.ds(128 * c, 128)], 0) for c in range(NT)]

    def out_b(tile, ns=range(NT)):
        at = pl.ds(128 * tile if isinstance(tile, int) else pl.multiple_of(128 * tile, 128), 128)
        return [cp for n in ns for cp in copy(
            outb.at[n, at, :], out_hbm.at[0, at, pl.ds(D + 128 * n, 128)], 1)]

    all_of_b = copy(outb, outb, 1)

    def start(*groups):
        for g in groups:
            for cp in g:
                cp().start()

    def wait(*groups):
        for g in groups:
            for cp in g:
                cp().wait()

    def rows(i, n):
        return pl.ds(pl.multiple_of(i * n, n), n) if not isinstance(i, int) else pl.ds(i * n, n)

    lane = lax.broadcasted_iota(jnp.int32, (8, 128), 1)
    sub = lax.broadcasted_iota(jnp.int32, (8, 128), 0)

    def lanes(n):
        return lax.broadcasted_iota(jnp.int32, (n, 128), 1)

    recent = [None]
    seg = [0]

    def dot(a, b, dims=NN_DIMS, kind=4):
        out = _dot(a, b, dims)
        if kind & PACE_ON[seg[0]]:
            recent[0] = out
        return out

    current = {}

    def pace(zero):
        v = recent[0][-8:]
        recent[0] = None
        if "h" in current:
            hb[S // 128, rows(zero, 8), :] = _u32_word(v)
        if "k" in current:
            kb[NT, rows(zero, 8), :] = _u32_word(v)
        if "t" in current:
            th[current["t"]][N1 // 8, zero, 0, 0] = v
            if PACE_ALL[seg[0]] & 1:
                tx[current["t"]][N1 // 8, zero, 0, 0] = v
            if PACE_ALL[seg[0]] & 2:
                ub[16, zero, 0, 0] = v

    def qk_proj(s, i, want_pq, want_pk):
        p = s % 2
        tok = rows(4 * s + i, 64)
        for w_ref, dst, fdst, want, scale in (
                (wqb, qs[p], pqs[p], want_pq, DH ** -0.5 * LOG2E),
                (wkb, ks[p], pks[p], want_pk, None)):
            for n in range(NT):
                t = None
                for c in range(NT):
                    part = dot(_bf(xb[c, tok, :]), _bf(w_ref[n, 64 * c:64 * c + 64, :]))
                    t = part if t is None else t + part
                    if c < NT - 1:
                        yield 32
                dst[n, rows(i, 128), :] = (t if scale is None else t * scale).astype(BF16)
                if want:
                    fdst[n, rows(i, 128), :] = jnp.where(t > 0, t + 1.0, jnp.exp(t)).astype(BF16)
                yield 32

    def first_proj(n, js=range(4)):
        for w_ref, dst, scale in ((wkb, ks[0], None), (wqb, qs[0], DH ** -0.5 * LOG2E)):
            for j in js:
                t = None
                for c in range(NT):
                    part = dot(_bf(xb[c, rows(j, 64), :]), _bf(w_ref[n, 64 * c:64 * c + 64, :]))
                    t = part if t is None else t + part
                dst[n, rows(j, 128), :] = (t if scale is None else t * scale).astype(BF16)
                if scale is None:
                    pks[0][n, rows(j, 128), :] = jnp.where(t > 0, t + 1.0, jnp.exp(t)).astype(BF16)

    def untranspose(s, i, slot=0):
        ot = ots.bitcast(U32)
        for c in range(NT):
            onat[slot, c] = _u32(_bf(ot[s % 2, i, 64 * c:64 * c + 64, :]).T)

    def out_proj(s, i, slot=0):
        for n in range(NT):
            t = None
            for c in range(NT):
                part = dot(_bf(onat[slot, c]), _bf(wob[n, 64 * c:64 * c + 64, :]))
                t = part if t is None else t + part
                if c < NT - 1:
                    yield 32
            outb[n, rows(4 * s + i, 128), :] = t.astype(BF16)
            start(out_b(4 * s + i, (n,)))
            yield 32

    def tile_rows(r, n):
        return jnp.broadcast_to(r[None], (n // 8, 8, 128)).reshape(n, 128)

    class Group:
        def __init__(self, s, g, gi):
            self.s, self.g, self.gi = s, g, gi
            self.t0 = (80 * g) // 128
            self.off = 80 * g - 128 * self.t0
            self.t1 = jnp.minimum(self.t0 + 1, NT - 1)
            rel = (lane - self.off) & 127
            head = sum((rel >= a * DH).astype(jnp.int32) for a in range(1, 5))
            for a in range(4):
                hmask[gi, a] = jnp.where(head == a, np.uint32(0xFFFFFFFF), np.uint32(0))
            hsel[gi] = jnp.left_shift(1, head)
            self.have_keys, self.have_mem = set(), set()

        def window(self, ref, j, r0=0, n=64):
            ref = ref.bitcast(U32)
            at = pl.ds(64 * j + r0, n)
            return jnp.where(lanes(n) >= self.off, ref[self.t0, at, :], ref[self.t1, at, :])

        def keys(self, r0, r1):
            out = []
            for r in range(r0, r1, 64):
                at = pl.ds(r // 2, 32)
                if r in self.have_keys:
                    out.append(kwin[self.gi, at, :])
                else:
                    self.have_keys.add(r)
                    out.append(self.window(ks[self.s % 2], 0, r // 2, 32))
                    kwin[self.gi, at, :] = out[-1]
            return _bf(jnp.concatenate(out, axis=0))

        def park_values(self, j, v80):
            if self.s < NSEG - 1:
                vall[self.gi, j, 0:80, :] = v80
            ones8 = jnp.ones((8, 128), F32)
            for pr in range(2):
                for e in range(2):
                    r0 = 40 * pr + 16 * e
                    vhead[self.gi, j, r0 // 8] = jnp.concatenate(
                        [v80[r0:r0 + 24], ones8], axis=0).astype(BF16)

        def mem_read(self):
            for j in range(4):
                r = dot(mst[self.g, 0:88, :], _bf(self.window(pqs[self.s % 2], j)), NT_DIMS)
                coef = gtab[self.g, 0] / (r[80:88] + 1e-6)
                cb = [jnp.broadcast_to(coef[a:a + 1], (8, 128)) for a in range(4)]
                for pr in range(2):
                    ca, cc = cb[2 * pr], cb[2 * pr + 1]
                    for e, scale in enumerate((ca, ca, jnp.where(sub < 4, ca, cc), cc, cc)):
                        r0 = 40 * pr + 8 * e
                        opart[self.gi, j, r0:r0 + 8, :] = r[r0:r0 + 8] * scale
                self.have_mem.add(j)
                yield 24

        def mem_update(self):
            acc = None
            for j in range(4):
                t = dot(vall[self.gi, j], _bf(self.window(pks[self.s % 2], j)))
                acc = t if acc is None else acc + t
                if j < 3:
                    yield 24
            for r in range(11):
                new = jnp.where(bmask[r] & hsel[self.gi] != 0, acc[8 * r:8 * r + 8], 0.0)
                at = pl.ds(8 * r, 8)
                mst[self.g, at, :] = new if self.s == 0 else mst[self.g, at, :] + new
            yield 24

        def logits(self, pr, j, slot):
            qw = self.window(qs[self.s % 2], j)
            qa = qw & tile_rows(hmask[self.gi, 2 * pr], 64)
            qh = qw & tile_rows(hmask[self.gi, 2 * pr + 1], 64)
            w_a = _bf(qa)
            w_b = _bf(jnp.concatenate([qh[32:64], qh[0:32]], axis=0))
            w_t = _bf(jnp.concatenate([qh[32:64], qa[32:64]], axis=0))
            n = 128 * j

            def park(t, e, r0, m):
                for r in range(0, t.shape[0], 8):
                    v = t[r:r + 8]
                    if e == 2:
                        v = v + cmask[2, r:r + 8, :]
                    elif r0 + r >= n:
                        v = v + cmask[e, r0 + r - n:r0 + r - n + 8, :]
                    slot[e % 2, 448 * (e // 2) + r0 + r:448 * (e // 2) + r0 + r + 8, :] = v
                    m = v if m is None else jnp.maximum(m, v)
                return m

            m_t = park(dot(self.keys(n + 64, n + 128), w_t, NT_DIMS, 1), 2, 0, None)
            yield 16
            cuts = list(range(0, n, QCH[seg[0]])) or [0]
            m = [None, None]
            for r0, r1 in zip(cuts, cuts[1:] + [n + 64]):
                for e, w in enumerate((w_a, w_b)):
                    m[e] = park(dot(self.keys(r0, r1), w, NT_DIMS, 1), e, r0, m[e])
                    if r1 == n + 64 and e == 1:
                        m_a = jnp.maximum(m[0], jnp.where(lane >= 64, m_t, NEG))
                        m_b = jnp.maximum(m[1], jnp.where(lane < 64, m_t, NEG))
                        m_a = jnp.broadcast_to(jnp.max(m_a, axis=0, keepdims=True), (8, 128))
                        m_b = jnp.broadcast_to(jnp.max(m_b, axis=0, keepdims=True), (8, 128))
                        slot[1, 448:456, :] = m_a
                        slot[1, 456:464, :] = m_b
                        slot[1, 464:472, :] = jnp.where(lane < 64, m_b, m_a)
                    yield (r1 - r0) // 4

    def attend(gi, g, parity, add_mem, pr, j, slot, need_values):
        def prob(e, r0, n, which):
            m2 = tile_rows(slot[1, 448 + 8 * which:456 + 8 * which, :], 16)
            return [jnp.exp2(slot[e, r:r + 16, :] - m2) for r in range(r0, r0 + n, 16)]

        res = [None, None]
        order = [(0, j), (1, j)] + [(e, kt) for e in range(2) for kt in range(j)]
        for n, (e, kt) in enumerate(order):
            need_values(kt)
            if n == 0:
                p_t = prob(0, 448, 64, 2)
            if kt < j:
                p = prob(e, 128 * kt, 128, e)
            else:
                mine = lanes(16) >= 64 if e == 0 else lanes(16) < 64
                p = prob(e, 128 * kt, 64, e) + [jnp.where(mine, t, 0.0) for t in p_t]
            t = dot(_bf(vhead.bitcast(U32)[gi, kt, 5 * pr + 2 * e]),
                    jnp.concatenate(p, axis=0).astype(BF16), kind=2)
            res[e] = t if res[e] is None else res[e] + t
            if n < len(order) - 1:
                yield 8 * AW[seg[0]]
        r_a = res[0]
        r_b = pltpu.roll(res[1], 64, 1)
        keep = 1.0 - gtab[g, 0]
        keep_a = jnp.broadcast_to(keep[2 * pr:2 * pr + 1], (8, 128))
        keep_b = jnp.broadcast_to(keep[2 * pr + 1:2 * pr + 2], (8, 128))
        o_a = r_a[0:24] * tile_rows(keep_a / r_a[24:32], 24)
        o_b = r_b[0:24] * tile_rows(keep_b / r_b[24:32], 24)
        o = jnp.concatenate(
            [o_a[0:16], jnp.where(sub < 4, o_a[16:24], o_b[0:8]), o_b[8:24]], axis=0)
        if add_mem:
            o = o + opart[gi, j, 40 * pr:40 * pr + 40, :]
        if pr == 0:
            opart[gi, j, 0:40, :] = o
        else:
            o = jnp.concatenate([opart[gi, j, 0:40, :], o], axis=0)
            ots[parity, j, rows(g, 80), :] = o.astype(BF16)
        yield 8 * AW[seg[0]]

    def v_proj(s, i, groups, have):
        for j in range(4):
            acc = None
            for c in range(NT):
                t = dot(_bf(wvt[c, i, 0:80, :]), _bf(xb[c, rows(4 * s + j, 64), :]), NT_DIMS)
                acc = t if acc is None else acc + t
                if c == NT - 1:
                    for gi in range(2):
                        groups[gi].park_values(j, acc[80 * gi:80 * gi + 80])
                    have.append(j)
                yield 40

    def chain(*gens):
        for g in gens:
            yield from g

    def units(s):
        return [(gi, pr, j) for gi in range(2) for pr in range(2)
                for j in (range(4) if (gi, pr) == (1, 1) else ORDER[s] if gi + pr else range(4))]

    def cost(j):
        return 48 + 64 * j, (16 + 16 * j) * AW[seg[0]]

    def carried(u, g, parity):
        gi, pr, j = units(0)[u]
        return attend(gi, g, parity, True, pr, j, slots[u % NSLOT], lambda kt: None), cost(j)[1]

    def segment_step(s, i):
        seg[0] = s
        parts = {}
        if s < NSEG - 1:
            parts["qk"] = (qk_proj(s + 1, i, True, s + 1 < NSEG - 1), 1600)
        if s > 0:
            parts["out"] = (out_proj(s - 1, i), 800)
        if FORWARD[s]:
            parts["fwd"] = (fwd_fft(i, FORWARD[s]), 512 * len(FORWARD[s]))
        if INVERSE[s]:
            parts["inv"] = (inverse(INVERSE[s], (2 * i, 2 * i + 1)), 256 * len(INVERSE[s]))
        names = (("qk", "inv", "out", "fwd"), ("qk", "inv", "fwd", "out"),
                 ("inv", "fwd", "qk", "out"), ("qk", "inv", "out", "fwd"))[FILL_ORDER[s]]
        fill = _Paced([parts[n] for n in names if n in parts], sequential=FILL_ORDER[s] < 3)
        side = []
        if SPECTRUM[s]:
            side.append((spectra(SPECTRUM[s], [4 * i + a for a in range(4)]),
                         4 * SPEC_COST * len(SPECTRUM[s])))
        for c in SPLIT[s]:
            side += [(split_h(i, c), 144), (split_kv(i, c), 704)]
        side = _Paced(side, sequential=True)
        current.clear()
        recent[0] = None
        for _ in range(HEAD[s]):
            fill.step()
        if s > 0:
            untranspose(s - 1, i)
        vt = []
        groups = [Group(s, 2 * i + gi, gi) for gi in range(2)]
        reads = [grp.mem_read() for grp in groups if s > 0]
        updates = [grp.mem_update() for grp in groups if s < NSEG - 1]
        first = _Paced([(chain(*reads[:1], v_proj(s, i, groups, vt), *reads[1:], *updates),
                         800 + 96 * (len(reads) + len(updates)))])
        total = first.total + fill.total
        held = 96 * (s > 0) + 159

        def need_values(kt):
            while len(vt) <= kt:
                first.step()

        def pad(fraction, u):
            target = total * fraction / (1 + TAIL[s])
            early = min(target, held if u < DEPTH else first.total)
            first.advance(early / first.total)
            fill.advance((target - early) / fill.total)
            goal = fraction * SIDE_SPEED[s]
            if side.live and side.done < goal * side.total and recent[0] is not None:
                pace(jnp.minimum(i, 3))
                side.advance(goal)

        todo = units(s)
        whole = sum(sum(cost(j)) for _, _, j in todo)
        done = 0
        for u, (gi, pr, j) in enumerate(todo):
            streams = [(groups[gi].logits(pr, j, slots[u % NSLOT]), cost(j)[0])]
            v = u - DEPTH
            if v < 0:
                streams.append(carried(v + len(todo), (2 * i + 7) & 7,
                                       jnp.where(i > 0, s % 2, 1 - s % 2)))
            else:
                gi, pr, j = todo[v]
                while s > 0 and j not in groups[gi].have_mem:
                    first.step()
                streams.append((attend(gi, 2 * i + gi, s % 2, s > 0, pr, j, slots[v % NSLOT],
                                       need_values), cost(j)[1]))
            att = _Paced(streams[::-1], sequential=u == len(todo) - 1)
            while att.live:
                att.step()
                pad((done + att.done) / whole, u)
            done += att.total
        first.finish()
        fill.finish()
        side.finish()

    def split_h(i, c):
        current.clear()
        current["h"] = True
        for t in range(4):
            ht[c, 64 * t:64 * t + 64, :] = _u32(
                _bf(hb[4 * i + t, 64 * c:64 * c + 64, :]).T)
            yield 4
        for q in range(2):
            for j in range(8):
                wa = ht[c, pl.ds(128 * q + j, 8, stride=8), :]
                wb = ht[c, pl.ds(128 * q + 64 + j, 8, stride=8), :]
                hp[c][2 * j, rows(2 * i + q, 8), :] = _pack2(_lo(wa), _lo(wb))
                hp[c][2 * j + 1, rows(2 * i + q, 8), :] = _pack2(_hi(wa), _hi(wb))
                if j % 2:
                    yield 16

    def split_kv(i, c):
        current.clear()
        current["k"] = True
        taps = [wtab[c, j] for j in range(KS)]
        for q in range(2):
            blk = 2 * i + q
            base = [blk * 128 + 64 * e for e in range(2)]
            hist = []
            for e in range(2):
                w2 = kb[c, pl.ds(base[e] + 30, 8, stride=8), :]
                w1 = kb[c, pl.ds(base[e] + 31, 8, stride=8), :]
                hist.append([_hi(w2), _lo(w1), _hi(w1)])
            for j in range(8):
                kv = [[None, None], [None, None]]
                for e in range(2):
                    kw = kb[c, pl.ds(base[e] + 32 + j, 8, stride=8), :]
                    vw = vb[c, pl.ds(base[e] + j, 8, stride=8), :]
                    kp = hist[e] + [_lo(kw), _hi(kw)]
                    for half, part in enumerate((_lo, _hi)):
                        acc = kp[3 + half] * taps[0]
                        for d in range(1, KS):
                            acc = acc + kp[3 + half - d] * taps[d]
                        kv[half][e] = acc * part(vw)
                        kvf[c][2 * j + half, rows(2 * blk + e, 8), :] = kv[half][e]
                    hist[e] = kp[2:]
                    if e == 0:
                        yield 22
                for half in range(2):
                    xp[c][2 * j + half, rows(blk, 8), :] = _pack2(*kv[half])
                yield 22

    def fwd_fft(i, cs):
        for c in cs:
            for src, dst in ((hp[c], th[c]), (xp[c], tx[c])):
                g = [dot(_bf(fwd[4 * a + i]), _bf(src[4 * a + i])) for a in range(4)]
                for r in range(0, 2 * N1, 16):
                    z = _radix4(*[(g[a][r:r + 8], g[a][r + 8:r + 16]) for a in range(4)], 1)
                    for cc in range(4):
                        dst[r // 16, i, cc, 0] = z[cc][0]
                        dst[r // 16, i, cc, 1] = z[cc][1]
                yield 256

    def spectrum(c, m, slot):
        current.clear()
        current["t"] = c
        for cc in range(4):
            zh = _radix4_tw(*[(th[c][m, b, cc, 0], th[c][m, b, cc, 1]) for b in range(4)], 1, cc)
            yield 17
            zx = _radix4_tw(*[(tx[c][m, b, cc, 0], tx[c][m, b, cc, 1]) for b in range(4)], 1, cc)
            yield 17
            y = [(x[0] * h[0] - x[1] * h[1], x[0] * h[1] + x[1] * h[0]) for x, h in zip(zx, zh)]
            yield 17
            u = _radix4(*y, -1)
            for b in range(4):
                ub[slot, b, cc, 0] = u[b][0]
                ub[slot, b, cc, 1] = u[b][1]
            yield 17
        if SPEC_V[seg[0]]:
            return

        yield from spectrum_end(c, m, slot)

    def spectrum_end(c, m, slot):
        for b in range(4):
            z = _radix4_tw(*[(ub[slot, b, cc, 0], ub[slot, b, cc, 1]) for cc in range(4)], -1, b)
            for a in range(4):
                yb[c][4 * a + b, rows(m, 8), :] = _pack2(*z[a])
            yield 17

    SPEC_COST = 17 * 20

    def spectra(cs, ms, slot0=0):
        prev = None
        for slot, (c, m) in enumerate(((c, m) for c in cs for m in ms), slot0):
            yield from spectrum(c, m, slot)
            if SPEC_V[seg[0]] and prev is not None:
                yield from spectrum_end(*prev)
            prev = (c, m, slot)
        if SPEC_V[seg[0]]:
            yield from spectrum_end(*prev)

    def inverse(cs, jps):
        for c in cs:
            for jp in jps:
                w = qb[c, pl.ds(jp, N1, stride=8), :]
                res = []
                for e, part in enumerate((_lo, _hi)):
                    n2 = 2 * jp + e
                    y = dot(_bf(inv[n2, 0]), _bf(yb[c][n2, 0:64, :]))
                    yield 32
                    y = y + dot(_bf(inv[n2, 1]), _bf(yb[c][n2, 64:128, :]))
                    res.append(part(w) * (y + kvf[c][n2] * tile_rows(wtab[c, KS], N1)))
                    if e == 0:
                        yield 32
                outa[c][pl.ds(jp, N1, stride=8), :] = _pack2(*res)
                yield 32

    start(cp_first, cp_x0, cp_w1)
    zero_ref[0] = 0
    kk = lax.broadcasted_iota(jnp.int32, (64, 128), 0)
    ll = lax.broadcasted_iota(jnp.int32, (64, 128), 1)
    cmask[0] = jnp.where(kk <= ll, 0.0, NEG)
    cmask[1] = jnp.where((ll < 64) | (kk <= ll - 64), 0.0, NEG)
    cmask[2] = jnp.where(kk <= (ll & 63), 0.0, NEG)
    for r in range(11):
        row = sub + 8 * r
        hr = sum((row >= a * DH).astype(jnp.int32) for a in range(1, 4)) if r < 10 else row - 80
        bmask[r] = jnp.left_shift(1, hr)
    for gi in range(2):
        for j in range(4):
            vall[gi, j, 80:88, :] = jnp.ones((8, 128), F32)
    for c in range(NT):
        kb[c, 24:32, :] = jnp.zeros((8, 128), U32)
    for u in range(16 - DEPTH, 16):
        slots[u % NSLOT][...] = jnp.zeros((2, 512, 128), F32)
    vhead[1] = jnp.ones(vhead.shape[1:], BF16)
    opart[1] = jnp.zeros(opart.shape[1:], F32)
    wait(cp_first)
    start(cp_w2, cp_wv, cp_step[0])
    first_proj(0, (0, 1))
    wait(cp_x0)
    first_proj(0, (2, 3))
    wait(cp_w1)
    for n in range(*W_STAGES[1]):
        first_proj(n)
    wait(cp_w2)
    first_proj(W_STAGES[2][0])
    wait(cp_wv)
    start(cp_step[1])
    taps_t = shift_ref[...].astype(F32)
    skip = ssmd_ref[...].astype(F32)
    for c in range(NT):
        for j in range(KS):
            wtab[c, j] = jnp.broadcast_to(taps_t[j:j + 1, 128 * c:128 * c + 128], (8, 128))
        wtab[c, KS] = jnp.broadcast_to(skip[c:c + 1], (8, 128))
    gates = jax.nn.sigmoid(beta_ref[...].astype(F32))
    gcol = jnp.broadcast_to(gates, (8, H)).T
    gcol = jnp.broadcast_to(gcol[:, 0:1], (H, 128))
    for g in range(8):
        gtab[g, 0] = jnp.concatenate([gcol[4 * g:4 * g + 4]] * 2, axis=0)
    for n in range(NT):
        for c in range(NT):
            wt = _u32(_bf(wvb[n, 64 * c:64 * c + 64, :]).T)
            for r in range(0, 64, 16):
                step, r0 = divmod(64 * n + r, 80)
                wvt[c, step, r0:r0 + 16, :] = wt[r:r + 16]
    for n in range(W_STAGES[2][0] + 1, NT):
        first_proj(n)

    def segment(s):
        def body(i, carry):
            if s == 0:
                for j in range(4):
                    @pl.when(i == j)
                    def _():
                        wait(cp_step[j])
                        start(*((cp_step[2],), (cp_step[3],), (cp_seg1,), (cp_seg2,))[j])
            segment_step(s, i)
            return carry

        lax.fori_loop(0, 4, body, 0)

    segment(0)
    wait(cp_seg1)
    segment(1)
    wait(cp_seg2)
    segment(2)
    segment(3)
    start(*[cp_oa[c] for c in INVERSE[3]])
    seg[0] = 4
    current.clear()
    recent[0] = None
    last = NT - 1
    rest_tiles = [c for c in range(last) if c not in INVERSE[3]]
    side = _Paced([(spectra((last,), range(16)), 16 * SPEC_COST)])
    span = (1024 * len(rest_tiles) + 160 * MID) / SIDE_SPEED[4]
    done = 0

    def run(streams):
        nonlocal done
        work = _Paced(streams)
        while work.live:
            before = work.done
            work.step()
            done += work.done - before
            if side.live and side.done < done / span * side.total and recent[0] is not None:
                pace(zero_ref[0])
                side.advance(done / span)

    for c in rest_tiles:
        streams = [(inverse((c,), range(8)), 1024)]
        if c == rest_tiles[0]:
            tail = [carried(u, 7, 1) for u in range(16 - DEPTH, 16)]
            streams.append((chain(*[g for g, _ in tail]), sum(w for _, w in tail)))
        run(streams)
        if c == rest_tiles[0]:
            for i in range(4):
                untranspose(3, i, i)
        start(cp_oa[c])
    proj = _Paced([(chain(*[out_proj(3, i, i) for i in range(4)]), 3200)])

    def part(cost):
        goal = proj.done + cost
        while proj.live and proj.done < goal:
            before = proj.done
            proj.step()
            yield proj.done - before

    run([(part(160 * MID), 160 * MID)])
    side.finish()
    run([(inverse((last,), range(8)), 1024)])
    start(cp_oa[last])
    proj.finish()
    wait(*cp_oa, all_of_b)


@jax.jit
def pallas_concat_heads__ssm_conv_h3__memory_aug_infini_attn__prompt_kernel(
    A_q: jax.Array,
    A_k: jax.Array,
    A_v: jax.Array,
    A_shift_k: jax.Array,
    A_ssm_k: jax.Array,
    A_ssm_D: jax.Array,
    B_x: jax.Array,
    B_wq: jax.Array,
    B_wk: jax.Array,
    B_wv: jax.Array,
    B_wo: jax.Array,
    B_beta: jax.Array,
):
    hbm = pl.BlockSpec(memory_space=pltpu.HBM)
    seg_tiles = pltpu.VMEM((NT, L, 128), BF16)
    weight = pltpu.VMEM((NT, D // 2, 128), U32)
    scratch = [
        pltpu.VMEM((NT, S // 2, 128), U32),
        weight, weight, weight, weight,
        pltpu.VMEM((NT, 4, 96, 128), U32),
        pltpu.VMEM((S // 128 + 1, D // 2, 128), U32),
        pltpu.VMEM((NT, 256 + 32, 128), U32),
        pltpu.VMEM((NT + 1, S // 2 + 64, 128), U32),
        pltpu.VMEM((NT, S // 2 + 32, 128), U32),
        pltpu.VMEM((NT, S // 2 + 32, 128), U32),
        pltpu.VMEM((N2, N1, 128), U32),
        pltpu.VMEM((N2, 2, N1 // 2, 128), U32),
        pltpu.VMEM((17, 4, 4, 2, 8, 128), F32),
        pltpu.VMEM((NT, S, 128), BF16),
        pltpu.VMEM((NT, 8, 8, 128), F32),
        pltpu.VMEM((8, 4, 8, 128), F32),
        pltpu.VMEM((3, 64, 128), F32),
        seg_tiles, seg_tiles, seg_tiles, seg_tiles,
        seg_tiles, seg_tiles, seg_tiles, seg_tiles,
        pltpu.VMEM((2, 4, D, 128), BF16),
        pltpu.VMEM((8, 96, 128), F32),
        pltpu.VMEM((2, 4, 8, 128), U32),
        pltpu.VMEM((4, 8, 128), jnp.int32),
        pltpu.VMEM((12, 8, 128), jnp.int32),
        pltpu.VMEM((2, L // 2, 128), U32),
        pltpu.VMEM((2, 4, 88, 128), F32),
        pltpu.VMEM((2, 4, 8, 32, 128), BF16),
        pltpu.VMEM((2, 4, 80, 128), F32),
        pltpu.VMEM((4, NT, 64, 128), U32),
        pltpu.SMEM((1,), jnp.int32),
        pltpu.SemaphoreType.DMA((5,)),
    ]
    scratch += [pltpu.VMEM((N2, N1 // 2, 128), U32)] * (2 * NT)
    scratch += [pltpu.VMEM((N1 // 8 + 1, 4, 4, 2, 8, 128), F32)] * (2 * NT)
    scratch += [pltpu.VMEM((N2, N1, 128), U32)] * NT
    scratch += [pltpu.VMEM((N2, N1, 128), F32)] * NT
    scratch += [pltpu.VMEM((S // 2 + 32, 128), U32)] * NT
    scratch += [pltpu.VMEM((2, 512, 128), F32)] * NSLOT
    scratch += [
        pltpu.VMEM((KS, D), BF16),
        pltpu.VMEM((NT, 128), BF16),
        pltpu.VMEM((1, H), BF16),
    ]
    return pl.pallas_call(
        _kernel,
        out_shape=jax.ShapeDtypeStruct((1, S, 2 * D), BF16),
        in_specs=[hbm] * 14,
        out_specs=hbm,
        scratch_shapes=scratch,
        compiler_params=pltpu.CompilerParams(vmem_limit_bytes=110 * 1024 * 1024),
        name="h3_infini",
    )(A_q, A_k, A_v, A_shift_k.T, A_ssm_k, A_ssm_D.reshape(NT, 128), B_x, B_wq, B_wk, B_wv, B_wo,
      B_beta.reshape(1, H), _FWD, _INV)
```

```python
import math

import jax
import jax.numpy as jnp
import numpy as np
from jax import lax
from jax.experimental import pallas as pl
from jax.experimental.pallas import tpu as pltpu

S = 2048
D = 640
NT = D // 128
H = 32
DH = D // H
NSEG = 4
L = S // NSEG
KS = 4
N1, N2 = 128, 16

F32 = jnp.float32
BF16 = jnp.bfloat16
U32 = jnp.uint32
NN_DIMS = (((1,), (0,)), ((), ()))
NT_DIMS = (((1,), (1,)), ((), ()))
NEG = -1e30
LOG2E = 1.4426950408889634


def _pack_rows(a):
    u = a.astype(np.float32).astype(BF16).view(np.uint16).astype(np.uint32)
    return u[..., 0::2, :] | (u[..., 1::2, :] << 16)


def _dft_tables():
    k1 = np.arange(N1)
    fwd = np.zeros((N2, 2 * N1, N1), np.float64)
    inv = np.zeros((N2, N1, 2 * N1), np.float64)
    kappa = np.arange(N1)
    n1_in = 16 * (kappa // 16) + 8 * (kappa % 2) + (kappa % 16) // 2
    row_re = 16 * (k1 // 8) + k1 % 8
    for n2 in range(N2):
        ang = 2.0 * np.pi * np.outer(k1 + 0.25, N2 * n1_in + n2) / S
        fwd[n2, row_re] = np.cos(ang)
        fwd[n2, row_re + 8] = np.sin(ang)
        ang = 2.0 * np.pi * np.outer(N2 * np.arange(N1) + n2, k1 + 0.25) / S
        inv[n2][:, 2 * k1] = np.cos(ang) / S
        inv[n2][:, 2 * k1 + 1] = np.sin(ang) / S
    inv = inv.reshape(N2, N1, 2, N1).transpose(0, 2, 1, 3)
    return _pack_rows(fwd), _pack_rows(inv)


_FWD, _INV = _dft_tables()


def _dot(a, b, dims=NN_DIMS):
    return lax.dot_general(a, b, dims, preferred_element_type=F32)


def _u32(x):
    return pltpu.bitcast(x, U32)


def _bf(x):
    return pltpu.bitcast(x, BF16)


def _u32_word(x):
    return lax.bitcast_convert_type(x, U32)


def _pack2(a, b):
    return pltpu.pack_elementwise([a, b], packed_dtype=BF16).astype(U32)


def _lo(w):
    return pltpu.unpack_elementwise(w, index=0, packed_dtype=BF16, unpacked_dtype=F32)


def _hi(w):
    return pltpu.unpack_elementwise(w, index=1, packed_dtype=BF16, unpacked_dtype=F32)


def _radix4(x0, x1, x2, x3, sign):
    ar, ai = x0[0] + x2[0], x0[1] + x2[1]
    br, bi = x0[0] - x2[0], x0[1] - x2[1]
    cr, ci = x1[0] + x3[0], x1[1] + x3[1]
    dr, di = x1[0] - x3[0], x1[1] - x3[1]
    y0 = (ar + cr, ai + ci)
    y2 = (ar - cr, ai - ci)
    yp = (br - di, bi + dr)
    ym = (br + di, bi - dr)
    return (y0, yp, y2, ym) if sign > 0 else (y0, ym, y2, yp)


def _twiddle(x, e, sign):
    xr, xi = x
    if e == 0:
        return x
    r = math.sqrt(0.5)
    if e == 2:
        return ((xr - xi) * r, (xr + xi) * r) if sign > 0 else ((xr + xi) * r, (xi - xr) * r)
    if e == 6:
        return ((xr + xi) * -r, (xr - xi) * r) if sign > 0 else ((xi - xr) * r, (xr + xi) * -r)
    c, s = math.cos(math.pi * e / 8), sign * math.sin(math.pi * e / 8)
    return (xr * c - xi * s, xr * s + xi * c)


def _radix4_tw(x0, x1, x2, x3, sign, b):
    if b != 2:
        return _radix4(x0, _twiddle(x1, b, sign), _twiddle(x2, 2 * b, sign),
                       _twiddle(x3, 3 * b, sign), sign)
    x1, x3 = _twiddle(x1, 2, sign), _twiddle(x3, 6, sign)
    if sign > 0:
        ar, ai = x0[0] - x2[1], x0[1] + x2[0]
        br, bi = x0[0] + x2[1], x0[1] - x2[0]
    else:
        ar, ai = x0[0] + x2[1], x0[1] - x2[0]
        br, bi = x0[0] - x2[1], x0[1] + x2[0]
    cr, ci = x1[0] + x3[0], x1[1] + x3[1]
    dr, di = x1[0] - x3[0], x1[1] - x3[1]
    y0 = (ar + cr, ai + ci)
    y2 = (ar - cr, ai - ci)
    yp = (br - di, bi + dr)
    ym = (br + di, bi - dr)
    return (y0, yp, y2, ym) if sign > 0 else (y0, ym, y2, yp)


class _Paced:
    def __init__(self, streams, sequential=False):
        self.live = [[g, total, 0] for g, total in streams if total]
        self.total = sum(total for _, total in streams)
        self.done = 0
        self.sequential = sequential

    def step(self):
        cur = self.live[0] if self.sequential else min(self.live, key=lambda e: e[2] / e[1])
        cost = next(cur[0], None)
        if cost is None:
            self.live.remove(cur)
        else:
            cur[2] += cost
            self.done += cost

    def advance(self, fraction):
        while self.live and self.done < fraction * self.total:
            self.step()

    def finish(self):
        self.advance(math.inf)


SPLIT = ((0, 1, 2), (3, 4), (), ())
FORWARD = ((), (0, 1), (2, 3, 4), ())
SPECTRUM = ((), (), (0, 1), (2, 3))
INVERSE = ((), (), (), (0, 1))
W_STAGES = ((0, 1), (1, 3), (3, 5))
DEPTH = 3
NSLOT = 4
ORDER = ((1, 3, 0, 2), (3, 2, 1, 0), (0, 2, 1, 3), (0, 1, 2, 3))
TAIL = (-0.03, 0.02, 0.02, -0.03)
QCH = (128, 192, 192, 128)
HEAD = (8, 2, 6, 6)
FILL_ORDER = (0, 1, 1, 0)
SIDE_SPEED = (1.015, 1.08, 1.0, 1.0, 1.0)
AW = (4.0, 2.0, 4.0, 2.0, 3.0)
PACE_ON = (3, 3, 7, 7, 7)
PACE_ALL = (3, 2, 2, 2, 0)
SPEC_V = (0, 0, 0, 0, 1)
MID = 15


def _kernel(aq_hbm, ak_hbm, av_hbm, shift_hbm, h_hbm, ssmd_hbm, x_hbm, wq_hbm, wk_hbm,
            wv_hbm, wo_hbm, beta_hbm, fwd_hbm, inv_hbm, out_hbm,
            xb, wqb, wkb, wvb, wob, wvt, hb, ht, kb, vb, qb, fwd, inv,
            ub, outb, wtab, gtab, cmask,
            q0, q1, k0, k1, pq0, pq1, pk0, pk1, ots, mst,
            hmask, hsel, bmask, kwin, vall, vhead, opart, onat, zero_ref, sems, *rest):
    xp, hp, tx, th, yb, kvf, outa = (rest[NT * k:NT * k + NT] for k in range(7))
    slots = rest[7 * NT:7 * NT + NSLOT]
    shift_ref, ssmd_ref, beta_ref = rest[7 * NT + NSLOT:]
    qs, ks, pqs, pks = (q0, q1), (k0, k1), (pq0, pq1), (pk0, pk1)

    def copy(src, dst, sem):
        return [lambda: pltpu.make_async_copy(src, dst, sems.at[sem])]

    def tiles(src, dst, sem, r0, n, ts=range(NT), off=0):
        src = src.bitcast(U32)
        lead = (0,) * (len(src.shape) - 2)
        return [cp for t in ts for cp in copy(
            src.at[lead + (pl.ds(r0 // 2, n // 2), pl.ds(128 * t, 128))],
            dst.at[t, pl.ds(off + r0 // 2, n // 2), :], sem)]

    def conv_inputs(cs, r0, n, sem):
        return (tiles(h_hbm, hb, sem, 128 * cs[0], 128 * len(cs), range(r0 // 128, (r0 + n) // 128))
                + tiles(ak_hbm, kb, sem, r0, n, cs, off=32) + tiles(av_hbm, vb, sem, r0, n, cs))

    def w_stage(k, sem):
        return (tiles(wq_hbm, wqb, sem, 0, D, range(*W_STAGES[k]))
                + tiles(wk_hbm, wkb, sem, 0, D, range(*W_STAGES[k])))

    cp_first = w_stage(0, 0) + tiles(x_hbm, xb, 0, 0, 256)
    cp_x0 = tiles(x_hbm, xb, 1, 256, 256)
    cp_w1, cp_w2 = w_stage(1, 2), w_stage(2, 3)
    cp_wv = (tiles(wv_hbm, wvb, 0, 0, D) + copy(shift_hbm, shift_ref, 0)
             + copy(ssmd_hbm, ssmd_ref, 0) + copy(beta_hbm, beta_ref, 0))
    cp_step = [tiles(x_hbm, xb, sem, L + 128 * i, 128) + conv_inputs(SPLIT[0], L * i, L, sem)
               for i, sem in enumerate((4, 0, 1, 2))]
    cp_seg1 = (tiles(wo_hbm, wob, 3, 0, D) + tiles(x_hbm, xb, 3, 2 * L, L)
               + copy(fwd_hbm, fwd, 3) + conv_inputs(SPLIT[1], 0, S, 3))
    cp_seg2 = (tiles(x_hbm, xb, 4, 3 * L, L) + copy(inv_hbm, inv, 4)
               + tiles(aq_hbm, qb, 4, 0, S))
    cp_oa = [copy(outa[c].at[pl.ds(0, S // 2), :],
                  out_hbm.bitcast(U32).at[0, :, pl.ds(128 * c, 128)], 0) for c in range(NT)]

    def out_b(tile, n):
        at = pl.ds(128 * tile if isinstance(tile, int) else pl.multiple_of(128 * tile, 128), 128)
        return copy(outb.at[n, at, :], out_hbm.at[0, at, pl.ds(D + 128 * n, 128)], 1)

    all_of_b = copy(outb, outb, 1)

    def start(*groups):
        for g in groups:
            for cp in g:
                cp().start()

    def wait(*groups):
        for g in groups:
            for cp in g:
                cp().wait()

    def rows(i, n):
        return pl.ds(pl.multiple_of(i * n, n), n) if not isinstance(i, int) else pl.ds(i * n, n)

    lane = lax.broadcasted_iota(jnp.int32, (8, 128), 1)
    sub = lax.broadcasted_iota(jnp.int32, (8, 128), 0)

    def lanes(n):
        return lax.broadcasted_iota(jnp.int32, (n, 128), 1)

    recent = [None]
    seg = [0]

    def dot(a, b, dims=NN_DIMS, kind=4):
        out = _dot(a, b, dims)
        if kind & PACE_ON[seg[0]]:
            recent[0] = out
        return out

    current = {}

    def pace(zero):
        v = recent[0][-8:]
        recent[0] = None
        if "h" in current:
            hb[S // 128, rows(zero, 8), :] = _u32_word(v)
        if "k" in current:
            kb[NT, rows(zero, 8), :] = _u32_word(v)
        if "t" in current:
            th[current["t"]][N1 // 8, zero, 0, 0] = v
            if PACE_ALL[seg[0]] & 1:
                tx[current["t"]][N1 // 8, zero, 0, 0] = v
            if PACE_ALL[seg[0]] & 2:
                ub[16, zero, 0, 0] = v

    def qk_proj(s, i, want_pq, want_pk):
        p = s % 2
        tok = rows(4 * s + i, 64)
        for w_ref, dst, fdst, want, scale in (
                (wqb, qs[p], pqs[p], want_pq, DH ** -0.5 * LOG2E),
                (wkb, ks[p], pks[p], want_pk, None)):
            for n in range(NT):
                t = None
                for c in range(NT):
                    part = dot(_bf(xb[c, tok, :]), _bf(w_ref[n, 64 * c:64 * c + 64, :]))
                    t = part if t is None else t + part
                    if c < NT - 1:
                        yield 32
                dst[n, rows(i, 128), :] = (t if scale is None else t * scale).astype(BF16)
                if want:
                    fdst[n, rows(i, 128), :] = jnp.where(t > 0, t + 1.0, jnp.exp(t)).astype(BF16)
                yield 32

    def first_proj(n, js=range(4)):
        for w_ref, dst, scale in ((wkb, ks[0], None), (wqb, qs[0], DH ** -0.5 * LOG2E)):
            for j in js:
                t = None
                for c in range(NT):
                    part = dot(_bf(xb[c, rows(j, 64), :]), _bf(w_ref[n, 64 * c:64 * c + 64, :]))
                    t = part if t is None else t + part
                dst[n, rows(j, 128), :] = (t if scale is None else t * scale).astype(BF16)
                if scale is None:
                    pks[0][n, rows(j, 128), :] = jnp.where(t > 0, t + 1.0, jnp.exp(t)).astype(BF16)

    def untranspose(s, i, slot=0):
        ot = ots.bitcast(U32)
        for c in range(NT):
            onat[slot, c] = _u32(_bf(ot[s % 2, i, 64 * c:64 * c + 64, :]).T)

    def out_proj(s, i, slot=0):
        for n in range(NT):
            t = None
            for c in range(NT):
                part = dot(_bf(onat[slot, c]), _bf(wob[n, 64 * c:64 * c + 64, :]))
                t = part if t is None else t + part
                if c < NT - 1:
                    yield 32
            outb[n, rows(4 * s + i, 128), :] = t.astype(BF16)
            start(out_b(4 * s + i, n))
            yield 32

    def tile_rows(r, n):
        return jnp.broadcast_to(r[None], (n // 8, 8, 128)).reshape(n, 128)

    class Group:
        def __init__(self, s, g, gi):
            self.s, self.g, self.gi = s, g, gi
            self.t0 = (80 * g) // 128
            self.off = 80 * g - 128 * self.t0
            self.t1 = jnp.minimum(self.t0 + 1, NT - 1)
            rel = (lane - self.off) & 127
            head = sum((rel >= a * DH).astype(jnp.int32) for a in range(1, 5))
            for a in range(4):
                hmask[gi, a] = jnp.where(head == a, np.uint32(0xFFFFFFFF), np.uint32(0))
            hsel[gi] = jnp.left_shift(1, head)
            self.have_keys, self.have_mem = set(), set()

        def window(self, ref, j, r0=0, n=64):
            ref = ref.bitcast(U32)
            at = pl.ds(64 * j + r0, n)
            return jnp.where(lanes(n) >= self.off, ref[self.t0, at, :], ref[self.t1, at, :])

        def keys(self, r0, r1):
            out = []
            for r in range(r0, r1, 64):
                at = pl.ds(r // 2, 32)
                if r in self.have_keys:
                    out.append(kwin[self.gi, at, :])
                else:
                    self.have_keys.add(r)
                    out.append(self.window(ks[self.s % 2], 0, r // 2, 32))
                    kwin[self.gi, at, :] = out[-1]
            return _bf(jnp.concatenate(out, axis=0))

        def park_values(self, j, v80):
            if self.s < NSEG - 1:
                vall[self.gi, j, 0:80, :] = v80
            ones8 = jnp.ones((8, 128), F32)
            for pr in range(2):
                for e in range(2):
                    r0 = 40 * pr + 16 * e
                    vhead[self.gi, j, r0 // 8] = jnp.concatenate(
                        [v80[r0:r0 + 24], ones8], axis=0).astype(BF16)

        def mem_read(self):
            for j in range(4):
                r = dot(mst[self.g, 0:88, :], _bf(self.window(pqs[self.s % 2], j)), NT_DIMS)
                coef = gtab[self.g, 0] / (r[80:88] + 1e-6)
                cb = [jnp.broadcast_to(coef[a:a + 1], (8, 128)) for a in range(4)]
                for pr in range(2):
                    ca, cc = cb[2 * pr], cb[2 * pr + 1]
                    for e, scale in enumerate((ca, ca, jnp.where(sub < 4, ca, cc), cc, cc)):
                        r0 = 40 * pr + 8 * e
                        opart[self.gi, j, r0:r0 + 8, :] = r[r0:r0 + 8] * scale
                self.have_mem.add(j)
                yield 24

        def mem_update(self):
            acc = None
            for j in range(4):
                t = dot(vall[self.gi, j], _bf(self.window(pks[self.s % 2], j)))
                acc = t if acc is None else acc + t
                if j < 3:
                    yield 24
            for r in range(11):
                new = jnp.where(bmask[r] & hsel[self.gi] != 0, acc[8 * r:8 * r + 8], 0.0)
                at = pl.ds(8 * r, 8)
                mst[self.g, at, :] = new if self.s == 0 else mst[self.g, at, :] + new
            yield 24

        def logits(self, pr, j, slot):
            qw = self.window(qs[self.s % 2], j)
            qa = qw & tile_rows(hmask[self.gi, 2 * pr], 64)
            qh = qw & tile_rows(hmask[self.gi, 2 * pr + 1], 64)
            w_a = _bf(qa)
            w_b = _bf(jnp.concatenate([qh[32:64], qh[0:32]], axis=0))
            w_t = _bf(jnp.concatenate([qh[32:64], qa[32:64]], axis=0))
            n = 128 * j

            def park(t, e, r0, m):
                for r in range(0, t.shape[0], 8):
                    v = t[r:r + 8]
                    if e == 2:
                        v = v + cmask[2, r:r + 8, :]
                    elif r0 + r >= n:
                        v = v + cmask[e, r0 + r - n:r0 + r - n + 8, :]
                    slot[e % 2, 448 * (e // 2) + r0 + r:448 * (e // 2) + r0 + r + 8, :] = v
                    m = v if m is None else jnp.maximum(m, v)
                return m

            m_t = park(dot(self.keys(n + 64, n + 128), w_t, NT_DIMS, 1), 2, 0, None)
            yield 16
            cuts = list(range(0, n, QCH[seg[0]])) or [0]
            m = [None, None]
            for r0, r1 in zip(cuts, cuts[1:] + [n + 64]):
                for e, w in enumerate((w_a, w_b)):
                    m[e] = park(dot(self.keys(r0, r1), w, NT_DIMS, 1), e, r0, m[e])
                    if r1 == n + 64 and e == 1:
                        m_a = jnp.maximum(m[0], jnp.where(lane >= 64, m_t, NEG))
                        m_b = jnp.maximum(m[1], jnp.where(lane < 64, m_t, NEG))
                        m_a = jnp.broadcast_to(jnp.max(m_a, axis=0, keepdims=True), (8, 128))
                        m_b = jnp.broadcast_to(jnp.max(m_b, axis=0, keepdims=True), (8, 128))
                        slot[1, 448:456, :] = m_a
                        slot[1, 456:464, :] = m_b
                        slot[1, 464:472, :] = jnp.where(lane < 64, m_b, m_a)
                    yield (r1 - r0) // 4

    def attend(gi, g, parity, add_mem, pr, j, slot, need_values):
        def prob(e, r0, n, which):
            m2 = tile_rows(slot[1, 448 + 8 * which:456 + 8 * which, :], 16)
            return [jnp.exp2(slot[e, r:r + 16, :] - m2) for r in range(r0, r0 + n, 16)]

        res = [None, None]
        order = [(0, j), (1, j)] + [(e, kt) for e in range(2) for kt in range(j)]
        for n, (e, kt) in enumerate(order):
            need_values(kt)
            if n == 0:
                p_t = prob(0, 448, 64, 2)
            if kt < j:
                p = prob(e, 128 * kt, 128, e)
            else:
                mine = lanes(16) >= 64 if e == 0 else lanes(16) < 64
                p = prob(e, 128 * kt, 64, e) + [jnp.where(mine, t, 0.0) for t in p_t]
            t = dot(_bf(vhead.bitcast(U32)[gi, kt, 5 * pr + 2 * e]),
                    jnp.concatenate(p, axis=0).astype(BF16), kind=2)
            res[e] = t if res[e] is None else res[e] + t
            if n < len(order) - 1:
                yield 8 * AW[seg[0]]
        r_a = res[0]
        r_b = pltpu.roll(res[1], 64, 1)
        keep = 1.0 - gtab[g, 0]
        keep_a = jnp.broadcast_to(keep[2 * pr:2 * pr + 1], (8, 128))
        keep_b = jnp.broadcast_to(keep[2 * pr + 1:2 * pr + 2], (8, 128))
        o_a = r_a[0:24] * tile_rows(keep_a / r_a[24:32], 24)
        o_b = r_b[0:24] * tile_rows(keep_b / r_b[24:32], 24)
        o = jnp.concatenate(
            [o_a[0:16], jnp.where(sub < 4, o_a[16:24], o_b[0:8]), o_b[8:24]], axis=0)
        if add_mem:
            o = o + opart[gi, j, 40 * pr:40 * pr + 40, :]
        if pr == 0:
            opart[gi, j, 0:40, :] = o
        else:
            o = jnp.concatenate([opart[gi, j, 0:40, :], o], axis=0)
            ots[parity, j, rows(g, 80), :] = o.astype(BF16)
        yield 8 * AW[seg[0]]

    def v_proj(s, i, groups, have):
        for j in range(4):
            acc = None
            for c in range(NT):
                t = dot(_bf(wvt[c, i, 0:80, :]), _bf(xb[c, rows(4 * s + j, 64), :]), NT_DIMS)
                acc = t if acc is None else acc + t
                if c == NT - 1:
                    for gi in range(2):
                        groups[gi].park_values(j, acc[80 * gi:80 * gi + 80])
                    have.append(j)
                yield 40

    def chain(*gens):
        for g in gens:
            yield from g

    def units(s):
        return [(gi, pr, j) for gi in range(2) for pr in range(2)
                for j in (range(4) if (gi, pr) == (1, 1) else ORDER[s] if gi + pr else range(4))]

    def cost(j):
        return 48 + 64 * j, (16 + 16 * j) * AW[seg[0]]

    def carried(u, g, parity):
        gi, pr, j = units(0)[u]
        return attend(gi, g, parity, True, pr, j, slots[u % NSLOT], lambda kt: None), cost(j)[1]

    def segment_step(s, i):
        seg[0] = s
        parts = {}
        if s < NSEG - 1:
            parts["qk"] = (qk_proj(s + 1, i, True, s + 1 < NSEG - 1), 1600)
        if s > 0:
            parts["out"] = (out_proj(s - 1, i), 800)
        if FORWARD[s]:
            parts["fwd"] = (fwd_fft(i, FORWARD[s]), 512 * len(FORWARD[s]))
        if INVERSE[s]:
            parts["inv"] = (inverse(INVERSE[s], (2 * i, 2 * i + 1)), 256 * len(INVERSE[s]))
        names = (("qk", "inv", "out", "fwd"), ("qk", "inv", "fwd", "out"),
                 ("inv", "fwd", "qk", "out"), ("qk", "inv", "out", "fwd"))[FILL_ORDER[s]]
        fill = _Paced([parts[n] for n in names if n in parts], sequential=FILL_ORDER[s] < 3)
        side = []
        if SPECTRUM[s]:
            side.append((spectra(SPECTRUM[s], [4 * i + a for a in range(4)]),
                         4 * SPEC_COST * len(SPECTRUM[s])))
        for c in SPLIT[s]:
            side += [(split_h(i, c), 144), (split_kv(i, c), 704)]
        side = _Paced(side, sequential=True)
        current.clear()
        recent[0] = None
        for _ in range(HEAD[s]):
            fill.step()
        if s > 0:
            untranspose(s - 1, i)
        vt = []
        groups = [Group(s, 2 * i + gi, gi) for gi in range(2)]
        reads = [grp.mem_read() for grp in groups if s > 0]
        updates = [grp.mem_update() for grp in groups if s < NSEG - 1]
        first = _Paced([(chain(*reads[:1], v_proj(s, i, groups, vt), *reads[1:], *updates),
                         800 + 96 * (len(reads) + len(updates)))])
        total = first.total + fill.total
        held = 96 * (s > 0) + 159

        def need_values(kt):
            while len(vt) <= kt:
                first.step()

        def pad(fraction, u):
            target = total * fraction / (1 + TAIL[s])
            early = min(target, held if u < DEPTH else first.total)
            first.advance(early / first.total)
            fill.advance((target - early) / fill.total)
            goal = fraction * SIDE_SPEED[s]
            if side.live and side.done < goal * side.total and recent[0] is not None:
                pace(jnp.minimum(i, 3))
                side.advance(goal)

        todo = units(s)
        whole = sum(sum(cost(j)) for _, _, j in todo)
        done = 0
        for u, (gi, pr, j) in enumerate(todo):
            streams = [(groups[gi].logits(pr, j, slots[u % NSLOT]), cost(j)[0])]
            v = u - DEPTH
            if v < 0:
                streams.append(carried(v + len(todo), (2 * i + 7) & 7,
                                       jnp.where(i > 0, s % 2, 1 - s % 2)))
            else:
                gi, pr, j = todo[v]
                while s > 0 and j not in groups[gi].have_mem:
                    first.step()
                streams.append((attend(gi, 2 * i + gi, s % 2, s > 0, pr, j, slots[v % NSLOT],
                                       need_values), cost(j)[1]))
            att = _Paced(streams[::-1], sequential=u == len(todo) - 1)
            while att.live:
                att.step()
                pad((done + att.done) / whole, u)
            done += att.total
        first.finish()
        fill.finish()
        side.finish()

    def split_h(i, c):
        current.clear()
        current["h"] = True
        for t in range(4):
            ht[c, 64 * t:64 * t + 64, :] = _u32(
                _bf(hb[4 * i + t, 64 * c:64 * c + 64, :]).T)
            yield 4
        for q in range(2):
            for j in range(8):
                wa = ht[c, pl.ds(128 * q + j, 8, stride=8), :]
                wb = ht[c, pl.ds(128 * q + 64 + j, 8, stride=8), :]
                hp[c][2 * j, rows(2 * i + q, 8), :] = _pack2(_lo(wa), _lo(wb))
                hp[c][2 * j + 1, rows(2 * i + q, 8), :] = _pack2(_hi(wa), _hi(wb))
                if j % 2:
                    yield 16

    def split_kv(i, c):
        current.clear()
        current["k"] = True
        taps = [wtab[c, j] for j in range(KS)]
        for q in range(2):
            blk = 2 * i + q
            base = [blk * 128 + 64 * e for e in range(2)]
            hist = []
            for e in range(2):
                w2 = kb[c, pl.ds(base[e] + 30, 8, stride=8), :]
                w1 = kb[c, pl.ds(base[e] + 31, 8, stride=8), :]
                hist.append([_hi(w2), _lo(w1), _hi(w1)])
            for j in range(8):
                kv = [[None, None], [None, None]]
                for e in range(2):
                    kw = kb[c, pl.ds(base[e] + 32 + j, 8, stride=8), :]
                    vw = vb[c, pl.ds(base[e] + j, 8, stride=8), :]
                    kp = hist[e] + [_lo(kw), _hi(kw)]
                    for half, part in enumerate((_lo, _hi)):
                        acc = kp[3 + half] * taps[0]
                        for d in range(1, KS):
                            acc = acc + kp[3 + half - d] * taps[d]
                        kv[half][e] = acc * part(vw)
                        kvf[c][2 * j + half, rows(2 * blk + e, 8), :] = kv[half][e]
                    hist[e] = kp[2:]
                    if e == 0:
                        yield 22
                for half in range(2):
                    xp[c][2 * j + half, rows(blk, 8), :] = _pack2(*kv[half])
                yield 22

    def fwd_fft(i, cs):
        for c in cs:
            for src, dst in ((hp[c], th[c]), (xp[c], tx[c])):
                g = [dot(_bf(fwd[4 * a + i]), _bf(src[4 * a + i])) for a in range(4)]
                for r in range(0, 2 * N1, 16):
                    z = _radix4(*[(g[a][r:r + 8], g[a][r + 8:r + 16]) for a in range(4)], 1)
                    for cc in range(4):
                        dst[r // 16, i, cc, 0] = z[cc][0]
                        dst[r // 16, i, cc, 1] = z[cc][1]
                yield 256

    def spectrum(c, m, slot):
        current.clear()
        current["t"] = c
        for cc in range(4):
            zh = _radix4_tw(*[(th[c][m, b, cc, 0], th[c][m, b, cc, 1]) for b in range(4)], 1, cc)
            yield 17
            zx = _radix4_tw(*[(tx[c][m, b, cc, 0], tx[c][m, b, cc, 1]) for b in range(4)], 1, cc)
            yield 17
            y = [(x[0] * h[0] - x[1] * h[1], x[0] * h[1] + x[1] * h[0]) for x, h in zip(zx, zh)]
            yield 17
            u = _radix4(*y, -1)
            for b in range(4):
                ub[slot, b, cc, 0] = u[b][0]
                ub[slot, b, cc, 1] = u[b][1]
            yield 17
        if SPEC_V[seg[0]]:
            return

        yield from spectrum_end(c, m, slot)

    def spectrum_end(c, m, slot):
        for b in range(4):
            z = _radix4_tw(*[(ub[slot, b, cc, 0], ub[slot, b, cc, 1]) for cc in range(4)], -1, b)
            for a in range(4):
                yb[c][4 * a + b, rows(m, 8), :] = _pack2(*z[a])
            yield 17

    SPEC_COST = 17 * 20

    def spectra(cs, ms):
        prev = None
        for slot, (c, m) in enumerate((c, m) for c in cs for m in ms):
            yield from spectrum(c, m, slot)
            if SPEC_V[seg[0]] and prev is not None:
                yield from spectrum_end(*prev)
            prev = (c, m, slot)
        if SPEC_V[seg[0]]:
            yield from spectrum_end(*prev)

    def inverse(cs, jps):
        for c in cs:
            for jp in jps:
                w = qb[c, pl.ds(jp, N1, stride=8), :]
                res = []
                for e, part in enumerate((_lo, _hi)):
                    n2 = 2 * jp + e
                    y = dot(_bf(inv[n2, 0]), _bf(yb[c][n2, 0:64, :]))
                    yield 32
                    y = y + dot(_bf(inv[n2, 1]), _bf(yb[c][n2, 64:128, :]))
                    res.append(part(w) * (y + kvf[c][n2] * tile_rows(wtab[c, KS], N1)))
                    if e == 0:
                        yield 32
                outa[c][pl.ds(jp, N1, stride=8), :] = _pack2(*res)
                yield 32

    start(cp_first, cp_x0, cp_w1)
    zero_ref[0] = 0
    kk = lax.broadcasted_iota(jnp.int32, (64, 128), 0)
    ll = lax.broadcasted_iota(jnp.int32, (64, 128), 1)
    cmask[0] = jnp.where(kk <= ll, 0.0, NEG)
    cmask[1] = jnp.where((ll < 64) | (kk <= ll - 64), 0.0, NEG)
    cmask[2] = jnp.where(kk <= (ll & 63), 0.0, NEG)
    for r in range(11):
        row = sub + 8 * r
        hr = sum((row >= a * DH).astype(jnp.int32) for a in range(1, 4)) if r < 10 else row - 80
        bmask[r] = jnp.left_shift(1, hr)
    for gi in range(2):
        for j in range(4):
            vall[gi, j, 80:88, :] = jnp.ones((8, 128), F32)
    for c in range(NT):
        kb[c, 24:32, :] = jnp.zeros((8, 128), U32)
    for u in range(16 - DEPTH, 16):
        slots[u % NSLOT][...] = jnp.zeros((2, 512, 128), F32)
    vhead[1] = jnp.ones(vhead.shape[1:], BF16)
    opart[1] = jnp.zeros(opart.shape[1:], F32)
    wait(cp_first)
    start(cp_w2, cp_wv, cp_step[0])
    first_proj(0, (0, 1))
    wait(cp_x0)
    first_proj(0, (2, 3))
    wait(cp_w1)
    for n in range(*W_STAGES[1]):
        first_proj(n)
    wait(cp_w2)
    first_proj(W_STAGES[2][0])
    wait(cp_wv)
    start(cp_step[1])
    taps_t = shift_ref[...].astype(F32)
    skip = ssmd_ref[...].astype(F32)
    for c in range(NT):
        for j in range(KS):
            wtab[c, j] = jnp.broadcast_to(taps_t[j:j + 1, 128 * c:128 * c + 128], (8, 128))
        wtab[c, KS] = jnp.broadcast_to(skip[c:c + 1], (8, 128))
    gates = jax.nn.sigmoid(beta_ref[...].astype(F32))
    gcol = jnp.broadcast_to(gates, (8, H)).T
    gcol = jnp.broadcast_to(gcol[:, 0:1], (H, 128))
    for g in range(8):
        gtab[g, 0] = jnp.concatenate([gcol[4 * g:4 * g + 4]] * 2, axis=0)
    for n in range(NT):
        for c in range(NT):
            wt = _u32(_bf(wvb[n, 64 * c:64 * c + 64, :]).T)
            for r in range(0, 64, 16):
                step, r0 = divmod(64 * n + r, 80)
                wvt[c, step, r0:r0 + 16, :] = wt[r:r + 16]
    for n in range(W_STAGES[2][0] + 1, NT):
        first_proj(n)

    def segment(s):
        def body(i, carry):
            if s == 0:
                for j in range(4):
                    @pl.when(i == j)
                    def _():
                        wait(cp_step[j])
                        start(*((cp_step[2],), (cp_step[3],), (cp_seg1,), (cp_seg2,))[j])
            segment_step(s, i)
            return carry

        lax.fori_loop(0, 4, body, 0)

    segment(0)
    wait(cp_seg1)
    segment(1)
    wait(cp_seg2)
    segment(2)
    segment(3)
    start(*[cp_oa[c] for c in INVERSE[3]])
    seg[0] = 4
    current.clear()
    recent[0] = None
    last = NT - 1
    rest_tiles = [c for c in range(last) if c not in INVERSE[3]]
    side = _Paced([(spectra((last,), range(16)), 16 * SPEC_COST)])
    span = (1024 * len(rest_tiles) + 160 * MID) / SIDE_SPEED[4]
    done = 0

    def run(streams):
        nonlocal done
        work = _Paced(streams)
        while work.live:
            before = work.done
            work.step()
            done += work.done - before
            if side.live and side.done < done / span * side.total and recent[0] is not None:
                pace(zero_ref[0])
                side.advance(done / span)

    for c in rest_tiles:
        streams = [(inverse((c,), range(8)), 1024)]
        if c == rest_tiles[0]:
            tail = [carried(u, 7, 1) for u in range(16 - DEPTH, 16)]
            streams.append((chain(*[g for g, _ in tail]), sum(w for _, w in tail)))
        run(streams)
        if c == rest_tiles[0]:
            for i in range(4):
                untranspose(3, i, i)
        start(cp_oa[c])
    proj = _Paced([(chain(*[out_proj(3, i, i) for i in range(4)]), 3200)])

    def part(cost):
        goal = proj.done + cost
        while proj.live and proj.done < goal:
            before = proj.done
            proj.step()
            yield proj.done - before

    run([(part(160 * MID), 160 * MID)])
    side.finish()
    run([(inverse((last,), range(8)), 1024)])
    start(cp_oa[last])
    proj.finish()
    wait(*cp_oa, all_of_b)


@jax.jit
def pallas_concat_heads__ssm_conv_h3__memory_aug_infini_attn__prompt_kernel(
    A_q: jax.Array,
    A_k: jax.Array,
    A_v: jax.Array,
    A_shift_k: jax.Array,
    A_ssm_k: jax.Array,
    A_ssm_D: jax.Array,
    B_x: jax.Array,
    B_wq: jax.Array,
    B_wk: jax.Array,
    B_wv: jax.Array,
    B_wo: jax.Array,
    B_beta: jax.Array,
):
    hbm = pl.BlockSpec(memory_space=pltpu.HBM)
    seg_tiles = pltpu.VMEM((NT, L, 128), BF16)
    weight = pltpu.VMEM((NT, D // 2, 128), U32)
    scratch = [
        pltpu.VMEM((NT, S // 2, 128), U32),
        weight, weight, weight, weight,
        pltpu.VMEM((NT, 4, 96, 128), U32),
        pltpu.VMEM((S // 128 + 1, D // 2, 128), U32),
        pltpu.VMEM((NT, 256 + 32, 128), U32),
        pltpu.VMEM((NT + 1, S // 2 + 64, 128), U32),
        pltpu.VMEM((NT, S // 2 + 32, 128), U32),
        pltpu.VMEM((NT, S // 2 + 32, 128), U32),
        pltpu.VMEM((N2, N1, 128), U32),
        pltpu.VMEM((N2, 2, N1 // 2, 128), U32),
        pltpu.VMEM((17, 4, 4, 2, 8, 128), F32),
        pltpu.VMEM((NT, S, 128), BF16),
        pltpu.VMEM((NT, 8, 8, 128), F32),
        pltpu.VMEM((8, 4, 8, 128), F32),
        pltpu.VMEM((3, 64, 128), F32),
        seg_tiles, seg_tiles, seg_tiles, seg_tiles,
        seg_tiles, seg_tiles, seg_tiles, seg_tiles,
        pltpu.VMEM((2, 4, D, 128), BF16),
        pltpu.VMEM((8, 96, 128), F32),
        pltpu.VMEM((2, 4, 8, 128), U32),
        pltpu.VMEM((4, 8, 128), jnp.int32),
        pltpu.VMEM((12, 8, 128), jnp.int32),
        pltpu.VMEM((2, L // 2, 128), U32),
        pltpu.VMEM((2, 4, 88, 128), F32),
        pltpu.VMEM((2, 4, 8, 32, 128), BF16),
        pltpu.VMEM((2, 4, 80, 128), F32),
        pltpu.VMEM((4, NT, 64, 128), U32),
        pltpu.SMEM((1,), jnp.int32),
        pltpu.SemaphoreType.DMA((5,)),
    ]
    scratch += [pltpu.VMEM((N2, N1 // 2, 128), U32)] * (2 * NT)
    scratch += [pltpu.VMEM((N1 // 8 + 1, 4, 4, 2, 8, 128), F32)] * (2 * NT)
    scratch += [pltpu.VMEM((N2, N1, 128), U32)] * NT
    scratch += [pltpu.VMEM((N2, N1, 128), F32)] * NT
    scratch += [pltpu.VMEM((S // 2 + 32, 128), U32)] * NT
    scratch += [pltpu.VMEM((2, 512, 128), F32)] * NSLOT
    scratch += [
        pltpu.VMEM((KS, D), BF16),
        pltpu.VMEM((NT, 128), BF16),
        pltpu.VMEM((1, H), BF16),
    ]
    return pl.pallas_call(
        _kernel,
        out_shape=jax.ShapeDtypeStruct((1, S, 2 * D), BF16),
        in_specs=[hbm] * 14,
        out_specs=hbm,
        scratch_shapes=scratch,
        compiler_params=pltpu.CompilerParams(vmem_limit_bytes=110 * 1024 * 1024),
        name="h3_infini",
    )(A_q, A_k, A_v, A_shift_k.T, A_ssm_k, A_ssm_D.reshape(NT, 128), B_x, B_wq, B_wk, B_wv, B_wo,
      B_beta.reshape(1, H), _FWD, _INV)
```

```python
import math

import jax
import jax.numpy as jnp
import numpy as np
from jax import lax
from jax.experimental import pallas as pl
from jax.experimental.pallas import tpu as pltpu

S = 2048
D = 640
NT = D // 128
H = 32
DH = D // H
NSEG = 4
L = S // NSEG
KS = 4
N1, N2 = 128, 16

F32 = jnp.float32
BF16 = jnp.bfloat16
U32 = jnp.uint32
NN_DIMS = (((1,), (0,)), ((), ()))
NT_DIMS = (((1,), (1,)), ((), ()))
NEG = -1e30
LOG2E = 1.4426950408889634


def _pack_rows(a):
    u = a.astype(np.float32).astype(BF16).view(np.uint16).astype(np.uint32)
    return u[..., 0::2, :] | (u[..., 1::2, :] << 16)


def _dft_tables():
    k1 = np.arange(N1)
    fwd = np.zeros((N2, 2 * N1, N1), np.float64)
    inv = np.zeros((N2, N1, 2 * N1), np.float64)
    row_re = 16 * (k1 // 8) + k1 % 8
    for n2 in range(N2):
        ang = 2.0 * np.pi * np.outer(k1 + 0.25, N2 * np.arange(N1) + n2) / S
        fwd[n2, row_re] = np.cos(ang)
        fwd[n2, row_re + 8] = np.sin(ang)
        inv[n2] = fwd[n2].T / S
    inv = inv.reshape(N2, N1, 2, N1).transpose(0, 2, 1, 3)
    return _pack_rows(fwd), _pack_rows(inv)


_FWD, _INV = _dft_tables()


def _dot(a, b, dims=NN_DIMS):
    return lax.dot_general(a, b, dims, preferred_element_type=F32)


def _u32(x):
    return pltpu.bitcast(x, U32)


def _bf(x):
    return pltpu.bitcast(x, BF16)


def _u32_word(x):
    return lax.bitcast_convert_type(x, U32)


def _lo(w):
    return lax.bitcast_convert_type(w << 16, F32)


def _hi(w):
    return lax.bitcast_convert_type(w & np.uint32(0xFFFF0000), F32)


def _stack(a, b):
    return jnp.concatenate([a, b], axis=0).astype(BF16)


def _interleave(a, b):
    r = _stack(a, b).astype(F32)
    n = a.shape[0]
    return (_u32_word(r[:n]) >> 16) | _u32_word(r[n:])


def _radix4(x0, x1, x2, x3, sign):
    ar, ai = x0[0] + x2[0], x0[1] + x2[1]
    br, bi = x0[0] - x2[0], x0[1] - x2[1]
    cr, ci = x1[0] + x3[0], x1[1] + x3[1]
    dr, di = x1[0] - x3[0], x1[1] - x3[1]
    y0 = (ar + cr, ai + ci)
    y2 = (ar - cr, ai - ci)
    yp = (br - di, bi + dr)
    ym = (br + di, bi - dr)
    return (y0, yp, y2, ym) if sign > 0 else (y0, ym, y2, yp)


def _twiddle(x, e, sign):
    xr, xi = x
    if e == 0:
        return x
    r = math.sqrt(0.5)
    if e == 2:
        return ((xr - xi) * r, (xr + xi) * r) if sign > 0 else ((xr + xi) * r, (xi - xr) * r)
    if e == 6:
        return ((xr + xi) * -r, (xr - xi) * r) if sign > 0 else ((xi - xr) * r, (xr + xi) * -r)
    c, s = math.cos(math.pi * e / 8), sign * math.sin(math.pi * e / 8)
    return (xr * c - xi * s, xr * s + xi * c)


def _radix4_tw(x0, x1, x2, x3, sign, b):
    if b != 2:
        return _radix4(x0, _twiddle(x1, b, sign), _twiddle(x2, 2 * b, sign),
                       _twiddle(x3, 3 * b, sign), sign)
    x1, x3 = _twiddle(x1, 2, sign), _twiddle(x3, 6, sign)
    if sign > 0:
        ar, ai = x0[0] - x2[1], x0[1] + x2[0]
        br, bi = x0[0] + x2[1], x0[1] - x2[0]
    else:
        ar, ai = x0[0] + x2[1], x0[1] - x2[0]
        br, bi = x0[0] - x2[1], x0[1] + x2[0]
    cr, ci = x1[0] + x3[0], x1[1] + x3[1]
    dr, di = x1[0] - x3[0], x1[1] - x3[1]
    y0 = (ar + cr, ai + ci)
    y2 = (ar - cr, ai - ci)
    yp = (br - di, bi + dr)
    ym = (br + di, bi - dr)
    return (y0, yp, y2, ym) if sign > 0 else (y0, ym, y2, yp)


class _Paced:
    def __init__(self, streams, sequential=False):
        self.live = [[g, total, 0] for g, total in streams if total]
        self.total = sum(total for _, total in streams)
        self.done = 0
        self.sequential = sequential

    def step(self):
        cur = self.live[0] if self.sequential else min(self.live, key=lambda e: e[2] / e[1])
        cost = next(cur[0], None)
        if cost is None:
            self.live.remove(cur)
        else:
            cur[2] += cost
            self.done += cost

    def advance(self, fraction):
        while self.live and self.done < fraction * self.total:
            self.step()

    def finish(self):
        self.advance(math.inf)


SPLIT = ((0, 1, 2), (3, 4), (), ())
FORWARD = ((), (0, 1), (2, 3, 4), ())
SPECTRUM = ((), (), (0, 1), (2, 3))
INVERSE = ((), (), (), (0, 1))
W_STAGES = ((0, 1), (1, 3), (3, 5))
DEPTH = 3
NSLOT = 4
ORDER = ((1, 3, 0, 2), (3, 2, 1, 0), (0, 2, 1, 3), (0, 1, 2, 3))
TAIL = (-0.03, 0.02, 0.02, -0.03)
QCH = (128, 192, 192, 128)
HEAD = (8, 2, 6, 6)
FILL_ORDER = (0, 1, 1, 0)
SIDE_SPEED = (1.015, 1.08, 1.0, 1.0, 1.0)
AW = (4.0, 2.0, 4.0, 2.0, 3.0)
PACE_ON = (3, 3, 7, 7, 7)
PACE_ALL = (3, 2, 2, 2, 0)
SPEC_V = (0, 0, 0, 0, 1)
MID = 15


def _kernel(aq_hbm, ak_hbm, av_hbm, shift_hbm, h_hbm, ssmd_hbm, x_hbm, wq_hbm, wk_hbm,
            wv_hbm, wo_hbm, beta_hbm, fwd_hbm, inv_hbm, out_hbm,
            xb, wqb, wkb, wvb, wob, wvt, hb, ht, kb, vb, qb, fwd, inv,
            ub, outb, wtab, gtab, cmask,
            q0, q1, k0, k1, pq0, pq1, pk0, pk1, ots, mst,
            hmask, hsel, bmask, kwin, vall, vhead, opart, onat, zero_ref, sems, *rest):
    xp, hp, tx, th, yb, kvf, outa = (rest[NT * k:NT * k + NT] for k in range(7))
    slots = rest[7 * NT:7 * NT + NSLOT]
    shift_ref, ssmd_ref, beta_ref = rest[7 * NT + NSLOT:]
    qs, ks, pqs, pks = (q0, q1), (k0, k1), (pq0, pq1), (pk0, pk1)

    def copy(src, dst, sem):
        return [lambda: pltpu.make_async_copy(src, dst, sems.at[sem])]

    def tiles(src, dst, sem, r0, n, ts=range(NT), off=0):
        src = src.bitcast(U32)
        lead = (0,) * (len(src.shape) - 2)
        return [cp for t in ts for cp in copy(
            src.at[lead + (pl.ds(r0 // 2, n // 2), pl.ds(128 * t, 128))],
            dst.at[t, pl.ds(off + r0 // 2, n // 2), :], sem)]

    def conv_inputs(cs, r0, n, sem):
        return (tiles(h_hbm, hb, sem, 128 * cs[0], 128 * len(cs), range(r0 // 128, (r0 + n) // 128))
                + tiles(ak_hbm, kb, sem, r0, n, cs, off=32) + tiles(av_hbm, vb, sem, r0, n, cs))

    def w_stage(k, sem):
        return (tiles(wq_hbm, wqb, sem, 0, D, range(*W_STAGES[k]))
                + tiles(wk_hbm, wkb, sem, 0, D, range(*W_STAGES[k])))

    cp_first = w_stage(0, 0) + tiles(x_hbm, xb, 0, 0, 256)
    cp_x0 = tiles(x_hbm, xb, 1, 256, 256)
    cp_w1, cp_w2 = w_stage(1, 2), w_stage(2, 3)
    cp_wv = (tiles(wv_hbm, wvb, 0, 0, D) + copy(shift_hbm, shift_ref, 0)
             + copy(ssmd_hbm, ssmd_ref, 0) + copy(beta_hbm, beta_ref, 0))
    cp_step = [tiles(x_hbm, xb, sem, L + 128 * i, 128) + conv_inputs(SPLIT[0], L * i, L, sem)
               for i, sem in enumerate((4, 0, 1, 2))]
    cp_seg1 = (tiles(wo_hbm, wob, 3, 0, D) + tiles(x_hbm, xb, 3, 2 * L, L)
               + copy(fwd_hbm, fwd, 3) + conv_inputs(SPLIT[1], 0, S, 3))
    cp_seg2 = (tiles(x_hbm, xb, 4, 3 * L, L) + copy(inv_hbm, inv, 4)
               + tiles(aq_hbm, qb, 4, 0, S))
    cp_oa = [copy(outa[c].at[pl.ds(0, S // 2), :],
                  out_hbm.bitcast(U32).at[0, :, pl.ds(128 * c, 128)], 0) for c in range(NT)]

    def out_b(tile, n):
        at = pl.ds(128 * tile if isinstance(tile, int) else pl.multiple_of(128 * tile, 128), 128)
        return copy(outb.at[n, at, :], out_hbm.at[0, at, pl.ds(D + 128 * n, 128)], 1)

    all_of_b = copy(outb, outb, 1)

    def start(*groups):
        for g in groups:
            for cp in g:
                cp().start()

    def wait(*groups):
        for g in groups:
            for cp in g:
                cp().wait()

    def rows(i, n):
        return pl.ds(pl.multiple_of(i * n, n), n) if not isinstance(i, int) else pl.ds(i * n, n)

    lane = lax.broadcasted_iota(jnp.int32, (8, 128), 1)
    sub = lax.broadcasted_iota(jnp.int32, (8, 128), 0)

    def lanes(n):
        return lax.broadcasted_iota(jnp.int32, (n, 128), 1)

    recent = [None]
    seg = [0]

    def dot(a, b, dims=NN_DIMS, kind=4):
        out = _dot(a, b, dims)
        if kind & PACE_ON[seg[0]]:
            recent[0] = out
        return out

    current = {}

    def pace(zero):
        v = recent[0][-8:]
        recent[0] = None
        if "h" in current:
            hb[S // 128, rows(zero, 8), :] = _u32_word(v)
        if "k" in current:
            kb[NT, rows(zero, 8), :] = _u32_word(v)
        if "t" in current:
            th[current["t"]][N1 // 8, zero, 0, 0] = v
            if PACE_ALL[seg[0]] & 1:
                tx[current["t"]][N1 // 8, zero, 0, 0] = v
            if PACE_ALL[seg[0]] & 2:
                ub[16, zero, 0, 0] = v

    def qk_proj(s, i, want_pq, want_pk):
        p = s % 2
        tok = rows(4 * s + i, 64)
        for w_ref, dst, fdst, want, scale in (
                (wqb, qs[p], pqs[p], want_pq, DH ** -0.5 * LOG2E),
                (wkb, ks[p], pks[p], want_pk, None)):
            for n in range(NT):
                t = None
                for c in range(NT):
                    part = dot(_bf(xb[c, tok, :]), _bf(w_ref[n, 64 * c:64 * c + 64, :]))
                    t = part if t is None else t + part
                    if c < NT - 1:
                        yield 32
                dst[n, rows(i, 128), :] = (t if scale is None else t * scale).astype(BF16)
                if want:
                    fdst[n, rows(i, 128), :] = jnp.where(t > 0, t + 1.0, jnp.exp(t)).astype(BF16)
                yield 32

    def first_proj(n, js=range(4)):
        for w_ref, dst, scale in ((wkb, ks[0], None), (wqb, qs[0], DH ** -0.5 * LOG2E)):
            for j in js:
                t = None
                for c in range(NT):
                    part = dot(_bf(xb[c, rows(j, 64), :]), _bf(w_ref[n, 64 * c:64 * c + 64, :]))
                    t = part if t is None else t + part
                dst[n, rows(j, 128), :] = (t if scale is None else t * scale).astype(BF16)
                if scale is None:
                    pks[0][n, rows(j, 128), :] = jnp.where(t > 0, t + 1.0, jnp.exp(t)).astype(BF16)

    def untranspose(s, i, slot=0):
        ot = ots.bitcast(U32)
        for c in range(NT):
            onat[slot, c] = _u32(_bf(ot[s % 2, i, 64 * c:64 * c + 64, :]).T)

    def out_proj(s, i, slot=0):
        for n in range(NT):
            t = None
            for c in range(NT):
                part = dot(_bf(onat[slot, c]), _bf(wob[n, 64 * c:64 * c + 64, :]))
                t = part if t is None else t + part
                if c < NT - 1:
                    yield 32
            outb[n, rows(4 * s + i, 128), :] = t.astype(BF16)
            start(out_b(4 * s + i, n))
            yield 32

    def tile_rows(r, n):
        return jnp.broadcast_to(r[None], (n // 8, 8, 128)).reshape(n, 128)

    class Group:
        def __init__(self, s, g, gi):
            self.s, self.g, self.gi = s, g, gi
            self.t0 = (80 * g) // 128
            self.off = 80 * g - 128 * self.t0
            self.t1 = jnp.minimum(self.t0 + 1, NT - 1)
            rel = (lane - self.off) & 127
            head = sum((rel >= a * DH).astype(jnp.int32) for a in range(1, 5))
            for a in range(4):
                hmask[gi, a] = jnp.where(head == a, np.uint32(0xFFFFFFFF), np.uint32(0))
            hsel[gi] = jnp.left_shift(1, head)
            self.have_keys, self.have_mem = set(), set()

        def window(self, ref, j, r0=0, n=64):
            ref = ref.bitcast(U32)
            at = pl.ds(64 * j + r0, n)
            return jnp.where(lanes(n) >= self.off, ref[self.t0, at, :], ref[self.t1, at, :])

        def keys(self, r0, r1):
            out = []
            for r in range(r0, r1, 64):
                at = pl.ds(r // 2, 32)
                if r in self.have_keys:
                    out.append(kwin[self.gi, at, :])
                else:
                    self.have_keys.add(r)
                    out.append(self.window(ks[self.s % 2], 0, r // 2, 32))
                    kwin[self.gi, at, :] = out[-1]
            return _bf(jnp.concatenate(out, axis=0))

        def park_values(self, j, v80):
            if self.s < NSEG - 1:
                vall[self.gi, j, 0:80, :] = v80
            ones8 = jnp.ones((8, 128), F32)
            for pr in range(2):
                for e in range(2):
                    r0 = 40 * pr + 16 * e
                    vhead[self.gi, j, r0 // 8] = jnp.concatenate(
                        [v80[r0:r0 + 24], ones8], axis=0).astype(BF16)

        def mem_read(self):
            for j in range(4):
                r = dot(mst[self.g, 0:88, :], _bf(self.window(pqs[self.s % 2], j)), NT_DIMS)
                coef = gtab[self.g, 0] / (r[80:88] + 1e-6)
                cb = [jnp.broadcast_to(coef[a:a + 1], (8, 128)) for a in range(4)]
                for pr in range(2):
                    ca, cc = cb[2 * pr], cb[2 * pr + 1]
                    for e, scale in enumerate((ca, ca, jnp.where(sub < 4, ca, cc), cc, cc)):
                        r0 = 40 * pr + 8 * e
                        opart[self.gi, j, r0:r0 + 8, :] = r[r0:r0 + 8] * scale
                self.have_mem.add(j)
                yield 24

        def mem_update(self):
            acc = None
            for j in range(4):
                t = dot(vall[self.gi, j], _bf(self.window(pks[self.s % 2], j)))
                acc = t if acc is None else acc + t
                if j < 3:
                    yield 24
            for r in range(11):
                new = jnp.where(bmask[r] & hsel[self.gi] != 0, acc[8 * r:8 * r + 8], 0.0)
                at = pl.ds(8 * r, 8)
                mst[self.g, at, :] = new if self.s == 0 else mst[self.g, at, :] + new
            yield 24

        def logits(self, pr, j, slot):
            qw = self.window(qs[self.s % 2], j)
            qa = qw & tile_rows(hmask[self.gi, 2 * pr], 64)
            qh = qw & tile_rows(hmask[self.gi, 2 * pr + 1], 64)
            w_a = _bf(qa)
            w_b = _bf(jnp.concatenate([qh[32:64], qh[0:32]], axis=0))
            w_t = _bf(jnp.concatenate([qh[32:64], qa[32:64]], axis=0))
            n = 128 * j

            def park(t, e, r0, m):
                for r in range(0, t.shape[0], 8):
                    v = t[r:r + 8]
                    if e == 2:
                        v = v + cmask[2, r:r + 8, :]
                    elif r0 + r >= n:
                        v = v + cmask[e, r0 + r - n:r0 + r - n + 8, :]
                    slot[e % 2, 448 * (e // 2) + r0 + r:448 * (e // 2) + r0 + r + 8, :] = v
                    m = v if m is None else jnp.maximum(m, v)
                return m

            m_t = park(dot(self.keys(n + 64, n + 128), w_t, NT_DIMS, 1), 2, 0, None)
            yield 16
            cuts = list(range(0, n, QCH[seg[0]])) or [0]
            m = [None, None]
            for r0, r1 in zip(cuts, cuts[1:] + [n + 64]):
                for e, w in enumerate((w_a, w_b)):
                    m[e] = park(dot(self.keys(r0, r1), w, NT_DIMS, 1), e, r0, m[e])
                    if r1 == n + 64 and e == 1:
                        m_a = jnp.maximum(m[0], jnp.where(lane >= 64, m_t, NEG))
                        m_b = jnp.maximum(m[1], jnp.where(lane < 64, m_t, NEG))
                        m_a = jnp.broadcast_to(jnp.max(m_a, axis=0, keepdims=True), (8, 128))
                        m_b = jnp.broadcast_to(jnp.max(m_b, axis=0, keepdims=True), (8, 128))
                        slot[1, 448:456, :] = m_a
                        slot[1, 456:464, :] = m_b
                        slot[1, 464:472, :] = jnp.where(lane < 64, m_b, m_a)
                    yield (r1 - r0) // 4

    def attend(gi, g, parity, add_mem, pr, j, slot, need_values):
        def prob(e, r0, n, which):
            m2 = tile_rows(slot[1, 448 + 8 * which:456 + 8 * which, :], 16)
            return [jnp.exp2(slot[e, r:r + 16, :] - m2) for r in range(r0, r0 + n, 16)]

        res = [None, None]
        order = [(0, j), (1, j)] + [(e, kt) for e in range(2) for kt in range(j)]
        for n, (e, kt) in enumerate(order):
            need_values(kt)
            if n == 0:
                p_t = prob(0, 448, 64, 2)
            if kt < j:
                p = prob(e, 128 * kt, 128, e)
            else:
                mine = lanes(16) >= 64 if e == 0 else lanes(16) < 64
                p = prob(e, 128 * kt, 64, e) + [jnp.where(mine, t, 0.0) for t in p_t]
            t = dot(_bf(vhead.bitcast(U32)[gi, kt, 5 * pr + 2 * e]),
                    jnp.concatenate(p, axis=0).astype(BF16), kind=2)
            res[e] = t if res[e] is None else res[e] + t
            if n < len(order) - 1:
                yield 8 * AW[seg[0]]
        r_a = res[0]
        r_b = pltpu.roll(res[1], 64, 1)
        keep = 1.0 - gtab[g, 0]
        keep_a = jnp.broadcast_to(keep[2 * pr:2 * pr + 1], (8, 128))
        keep_b = jnp.broadcast_to(keep[2 * pr + 1:2 * pr + 2], (8, 128))
        o_a = r_a[0:24] * tile_rows(keep_a / r_a[24:32], 24)
        o_b = r_b[0:24] * tile_rows(keep_b / r_b[24:32], 24)
        o = jnp.concatenate(
            [o_a[0:16], jnp.where(sub < 4, o_a[16:24], o_b[0:8]), o_b[8:24]], axis=0)
        if add_mem:
            o = o + opart[gi, j, 40 * pr:40 * pr + 40, :]
        if pr == 0:
            opart[gi, j, 0:40, :] = o
        else:
            o = jnp.concatenate([opart[gi, j, 0:40, :], o], axis=0)
            ots[parity, j, rows(g, 80), :] = o.astype(BF16)
        yield 8 * AW[seg[0]]

    def v_proj(s, i, groups, have):
        for j in range(4):
            acc = None
            for c in range(NT):
                t = dot(_bf(wvt[c, i, 0:80, :]), _bf(xb[c, rows(4 * s + j, 64), :]), NT_DIMS)
                acc = t if acc is None else acc + t
                if c == NT - 1:
                    for gi in range(2):
                        groups[gi].park_values(j, acc[80 * gi:80 * gi + 80])
                    have.append(j)
                yield 40

    def chain(*gens):
        for g in gens:
            yield from g

    def units(s):
        return [(gi, pr, j) for gi in range(2) for pr in range(2)
                for j in (range(4) if (gi, pr) == (1, 1) else ORDER[s] if gi + pr else range(4))]

    def cost(j):
        return 48 + 64 * j, (16 + 16 * j) * AW[seg[0]]

    def carried(u, g, parity):
        gi, pr, j = units(0)[u]
        return attend(gi, g, parity, True, pr, j, slots[u % NSLOT], lambda kt: None), cost(j)[1]

    def segment_step(s, i):
        seg[0] = s
        parts = {}
        if s < NSEG - 1:
            parts["qk"] = (qk_proj(s + 1, i, True, s + 1 < NSEG - 1), 1600)
        if s > 0:
            parts["out"] = (out_proj(s - 1, i), 800)
        if FORWARD[s]:
            parts["fwd"] = (fwd_fft(i, FORWARD[s]), 512 * len(FORWARD[s]))
        if INVERSE[s]:
            parts["inv"] = (inverse(INVERSE[s], (2 * i, 2 * i + 1)), 256 * len(INVERSE[s]))
        names = (("qk", "inv", "out", "fwd"), ("qk", "inv", "fwd", "out"),
                 ("inv", "fwd", "qk", "out"), ("qk", "inv", "out", "fwd"))[FILL_ORDER[s]]
        fill = _Paced([parts[n] for n in names if n in parts], sequential=FILL_ORDER[s] < 3)
        side = []
        if SPECTRUM[s]:
            side.append((spectra(SPECTRUM[s], [4 * i + a for a in range(4)]),
                         4 * SPEC_COST * len(SPECTRUM[s])))
        for c in SPLIT[s]:
            side += [(split_h(i, c), 144), (split_kv(i, c), 704)]
        side = _Paced(side, sequential=True)
        current.clear()
        recent[0] = None
        for _ in range(HEAD[s]):
            fill.step()
        if s > 0:
            untranspose(s - 1, i)
        vt = []
        groups = [Group(s, 2 * i + gi, gi) for gi in range(2)]
        reads = [grp.mem_read() for grp in groups if s > 0]
        updates = [grp.mem_update() for grp in groups if s < NSEG - 1]
        first = _Paced([(chain(*reads[:1], v_proj(s, i, groups, vt), *reads[1:], *updates),
                         800 + 96 * (len(reads) + len(updates)))])
        total = first.total + fill.total
        held = 96 * (s > 0) + 159

        def need_values(kt):
            while len(vt) <= kt:
                first.step()

        def pad(fraction, u):
            target = total * fraction / (1 + TAIL[s])
            early = min(target, held if u < DEPTH else first.total)
            first.advance(early / first.total)
            fill.advance((target - early) / fill.total)
            goal = fraction * SIDE_SPEED[s]
            if side.live and side.done < goal * side.total and recent[0] is not None:
                pace(jnp.minimum(i, 3))
                side.advance(goal)

        todo = units(s)
        whole = sum(sum(cost(j)) for _, _, j in todo)
        done = 0
        for u, (gi, pr, j) in enumerate(todo):
            streams = [(groups[gi].logits(pr, j, slots[u % NSLOT]), cost(j)[0])]
            v = u - DEPTH
            if v < 0:
                streams.append(carried(v + len(todo), (2 * i + 7) & 7,
                                       jnp.where(i > 0, s % 2, 1 - s % 2)))
            else:
                gi, pr, j = todo[v]
                while s > 0 and j not in groups[gi].have_mem:
                    first.step()
                streams.append((attend(gi, 2 * i + gi, s % 2, s > 0, pr, j, slots[v % NSLOT],
                                       need_values), cost(j)[1]))
            att = _Paced(streams[::-1], sequential=u == len(todo) - 1)
            while att.live:
                att.step()
                pad((done + att.done) / whole, u)
            done += att.total
        first.finish()
        fill.finish()
        side.finish()

    def split_h(i, c):
        current.clear()
        current["h"] = True
        for t in range(4):
            ht[c, 64 * t:64 * t + 64, :] = _u32(
                _bf(hb[4 * i + t, 64 * c:64 * c + 64, :]).T)
            yield 4
        for q in range(2):
            for j in range(8):
                wa = ht[c, pl.ds(128 * q + j, 8, stride=8), :]
                wb = ht[c, pl.ds(128 * q + 64 + j, 8, stride=8), :]
                hp[c][2 * j, rows(2 * i + q, 16), :] = _stack(_lo(wa), _lo(wb))
                hp[c][2 * j + 1, rows(2 * i + q, 16), :] = _stack(_hi(wa), _hi(wb))
                if j % 2:
                    yield 16

    def split_kv(i, c):
        current.clear()
        current["k"] = True
        taps = [wtab[c, j] for j in range(KS)]
        for q in range(2):
            blk = 2 * i + q
            base = [blk * 128 + 64 * e for e in range(2)]
            hist = []
            for e in range(2):
                w2 = kb[c, pl.ds(base[e] + 30, 8, stride=8), :]
                w1 = kb[c, pl.ds(base[e] + 31, 8, stride=8), :]
                hist.append([_hi(w2), _lo(w1), _hi(w1)])
            for j in range(8):
                kv = [[None, None], [None, None]]
                for e in range(2):
                    kw = kb[c, pl.ds(base[e] + 32 + j, 8, stride=8), :]
                    vw = vb[c, pl.ds(base[e] + j, 8, stride=8), :]
                    kp = hist[e] + [_lo(kw), _hi(kw)]
                    for half, part in enumerate((_lo, _hi)):
                        acc = kp[3 + half] * taps[0]
                        for d in range(1, KS):
                            acc = acc + kp[3 + half - d] * taps[d]
                        kv[half][e] = acc * part(vw)
                        kvf[c][2 * j + half, rows(2 * blk + e, 8), :] = kv[half][e]
                    hist[e] = kp[2:]
                    if e == 0:
                        yield 22
                for half in range(2):
                    xp[c][2 * j + half, rows(blk, 16), :] = _stack(*kv[half])
                yield 22

    def fwd_fft(i, cs):
        for c in cs:
            for src, dst in ((hp[c], th[c]), (xp[c], tx[c])):
                g = [dot(_bf(fwd[4 * a + i]), _bf(src.bitcast(U32)[4 * a + i])) for a in range(4)]
                for r in range(0, 2 * N1, 16):
                    z = _radix4(*[(g[a][r:r + 8], g[a][r + 8:r + 16]) for a in range(4)], 1)
                    for cc in range(4):
                        dst[r // 16, i, cc, 0] = z[cc][0]
                        dst[r // 16, i, cc, 1] = z[cc][1]
                yield 256

    def spectrum(c, m, slot):
        current.clear()
        current["t"] = c
        for cc in range(4):
            zh = _radix4_tw(*[(th[c][m, b, cc, 0], th[c][m, b, cc, 1]) for b in range(4)], 1, cc)
            yield 17
            zx = _radix4_tw(*[(tx[c][m, b, cc, 0], tx[c][m, b, cc, 1]) for b in range(4)], 1, cc)
            yield 17
            y = [(x[0] * h[0] - x[1] * h[1], x[0] * h[1] + x[1] * h[0]) for x, h in zip(zx, zh)]
            yield 17
            u = _radix4(*y, -1)
            for b in range(4):
                ub[slot, b, cc, 0] = u[b][0]
                ub[slot, b, cc, 1] = u[b][1]
            yield 17
        if SPEC_V[seg[0]]:
            return

        yield from spectrum_end(c, m, slot)

    def spectrum_end(c, m, slot):
        for b in range(4):
            z = _radix4_tw(*[(ub[slot, b, cc, 0], ub[slot, b, cc, 1]) for cc in range(4)], -1, b)
            for a in range(4):
                yb[c][4 * a + b, rows(m, 16), :] = _stack(*z[a])
            yield 17

    SPEC_COST = 17 * 20

    def spectra(cs, ms):
        prev = None
        for slot, (c, m) in enumerate((c, m) for c in cs for m in ms):
            yield from spectrum(c, m, slot)
            if SPEC_V[seg[0]] and prev is not None:
                yield from spectrum_end(*prev)
            prev = (c, m, slot)
        if SPEC_V[seg[0]]:
            yield from spectrum_end(*prev)

    def inverse(cs, jps):
        for c in cs:
            for jp in jps:
                w = qb[c, pl.ds(jp, N1, stride=8), :]
                res = []
                for e, part in enumerate((_lo, _hi)):
                    n2 = 2 * jp + e
                    y = dot(_bf(inv[n2, 0]), _bf(yb[c].bitcast(U32)[n2, 0:64, :]))
                    yield 32
                    y = y + dot(_bf(inv[n2, 1]), _bf(yb[c].bitcast(U32)[n2, 64:128, :]))
                    res.append(part(w) * (y + kvf[c][n2] * tile_rows(wtab[c, KS], N1)))
                    if e == 0:
                        yield 32
                outa[c][pl.ds(jp, N1, stride=8), :] = _interleave(*res)
                yield 32

    start(cp_first, cp_x0, cp_w1)
    zero_ref[0] = 0
    kk = lax.broadcasted_iota(jnp.int32, (64, 128), 0)
    ll = lax.broadcasted_iota(jnp.int32, (64, 128), 1)
    cmask[0] = jnp.where(kk <= ll, 0.0, NEG)
    cmask[1] = jnp.where((ll < 64) | (kk <= ll - 64), 0.0, NEG)
    cmask[2] = jnp.where(kk <= (ll & 63), 0.0, NEG)
    for r in range(11):
        row = sub + 8 * r
        hr = sum((row >= a * DH).astype(jnp.int32) for a in range(1, 4)) if r < 10 else row - 80
        bmask[r] = jnp.left_shift(1, hr)
    for gi in range(2):
        for j in range(4):
            vall[gi, j, 80:88, :] = jnp.ones((8, 128), F32)
    for c in range(NT):
        kb[c, 24:32, :] = jnp.zeros((8, 128), U32)
    for u in range(16 - DEPTH, 16):
        slots[u % NSLOT][...] = jnp.zeros((2, 512, 128), F32)
    vhead[1] = jnp.ones(vhead.shape[1:], BF16)
    opart[1] = jnp.zeros(opart.shape[1:], F32)
    wait(cp_first)
    start(cp_w2, cp_wv, cp_step[0])
    first_proj(0, (0, 1))
    wait(cp_x0)
    first_proj(0, (2, 3))
    wait(cp_w1)
    for n in range(*W_STAGES[1]):
        first_proj(n)
    wait(cp_w2)
    first_proj(W_STAGES[2][0])
    wait(cp_wv)
    start(cp_step[1])
    taps_t = shift_ref[...].astype(F32)
    skip = ssmd_ref[...].astype(F32)
    for c in range(NT):
        for j in range(KS):
            wtab[c, j] = jnp.broadcast_to(taps_t[j:j + 1, 128 * c:128 * c + 128], (8, 128))
        wtab[c, KS] = jnp.broadcast_to(skip[c:c + 1], (8, 128))
    gates = jax.nn.sigmoid(beta_ref[...].astype(F32))
    gcol = jnp.broadcast_to(gates, (8, H)).T
    gcol = jnp.broadcast_to(gcol[:, 0:1], (H, 128))
    for g in range(8):
        gtab[g, 0] = jnp.concatenate([gcol[4 * g:4 * g + 4]] * 2, axis=0)
    for n in range(NT):
        for c in range(NT):
            wt = _u32(_bf(wvb[n, 64 * c:64 * c + 64, :]).T)
            for r in range(0, 64, 16):
                step, r0 = divmod(64 * n + r, 80)
                wvt[c, step, r0:r0 + 16, :] = wt[r:r + 16]
    for n in range(W_STAGES[2][0] + 1, NT):
        first_proj(n)

    def segment(s):
        def body(i, carry):
            if s == 0:
                for j in range(4):
                    @pl.when(i == j)
                    def _():
                        wait(cp_step[j])
                        start(*((cp_step[2],), (cp_step[3],), (cp_seg1,), (cp_seg2,))[j])
            segment_step(s, i)
            return carry

        lax.fori_loop(0, 4, body, 0)

    segment(0)
    wait(cp_seg1)
    segment(1)
    wait(cp_seg2)
    segment(2)
    segment(3)
    start(*[cp_oa[c] for c in INVERSE[3]])
    seg[0] = 4
    current.clear()
    recent[0] = None
    last = NT - 1
    rest_tiles = [c for c in range(last) if c not in INVERSE[3]]
    side = _Paced([(spectra((last,), range(16)), 16 * SPEC_COST)])
    span = (1024 * len(rest_tiles) + 160 * MID) / SIDE_SPEED[4]
    done = 0

    def run(streams):
        nonlocal done
        work = _Paced(streams)
        while work.live:
            before = work.done
            work.step()
            done += work.done - before
            if side.live and side.done < done / span * side.total and recent[0] is not None:
                pace(zero_ref[0])
                side.advance(done / span)

    for c in rest_tiles:
        streams = [(inverse((c,), range(8)), 1024)]
        if c == rest_tiles[0]:
            tail = [carried(u, 7, 1) for u in range(16 - DEPTH, 16)]
            streams.append((chain(*[g for g, _ in tail]), sum(w for _, w in tail)))
        run(streams)
        if c == rest_tiles[0]:
            for i in range(4):
                untranspose(3, i, i)
        start(cp_oa[c])
    proj = _Paced([(chain(*[out_proj(3, i, i) for i in range(4)]), 3200)])

    def part(cost):
        goal = proj.done + cost
        while proj.live and proj.done < goal:
            before = proj.done
            proj.step()
            yield proj.done - before

    run([(part(160 * MID), 160 * MID)])
    side.finish()
    run([(inverse((last,), range(8)), 1024)])
    start(cp_oa[last])
    proj.finish()
    wait(*cp_oa, all_of_b)


@jax.jit
def pallas_concat_heads__ssm_conv_h3__memory_aug_infini_attn__prompt_kernel(
    A_q: jax.Array,
    A_k: jax.Array,
    A_v: jax.Array,
    A_shift_k: jax.Array,
    A_ssm_k: jax.Array,
    A_ssm_D: jax.Array,
    B_x: jax.Array,
    B_wq: jax.Array,
    B_wk: jax.Array,
    B_wv: jax.Array,
    B_wo: jax.Array,
    B_beta: jax.Array,
):
    hbm = pl.BlockSpec(memory_space=pltpu.HBM)
    seg_tiles = pltpu.VMEM((NT, L, 128), BF16)
    weight = pltpu.VMEM((NT, D // 2, 128), U32)
    scratch = [
        pltpu.VMEM((NT, S // 2, 128), U32),
        weight, weight, weight, weight,
        pltpu.VMEM((NT, 4, 96, 128), U32),
        pltpu.VMEM((S // 128 + 1, D // 2, 128), U32),
        pltpu.VMEM((NT, 256 + 32, 128), U32),
        pltpu.VMEM((NT + 1, S // 2 + 64, 128), U32),
        pltpu.VMEM((NT, S // 2 + 32, 128), U32),
        pltpu.VMEM((NT, S // 2 + 32, 128), U32),
        pltpu.VMEM((N2, N1, 128), U32),
        pltpu.VMEM((N2, 2, N1 // 2, 128), U32),
        pltpu.VMEM((17, 4, 4, 2, 8, 128), F32),
        pltpu.VMEM((NT, S, 128), BF16),
        pltpu.VMEM((NT, 8, 8, 128), F32),
        pltpu.VMEM((8, 4, 8, 128), F32),
        pltpu.VMEM((3, 64, 128), F32),
        seg_tiles, seg_tiles, seg_tiles, seg_tiles,
        seg_tiles, seg_tiles, seg_tiles, seg_tiles,
        pltpu.VMEM((2, 4, D, 128), BF16),
        pltpu.VMEM((8, 96, 128), F32),
        pltpu.VMEM((2, 4, 8, 128), U32),
        pltpu.VMEM((4, 8, 128), jnp.int32),
        pltpu.VMEM((12, 8, 128), jnp.int32),
        pltpu.VMEM((2, L // 2, 128), U32),
        pltpu.VMEM((2, 4, 88, 128), F32),
        pltpu.VMEM((2, 4, 8, 32, 128), BF16),
        pltpu.VMEM((2, 4, 80, 128), F32),
        pltpu.VMEM((4, NT, 64, 128), U32),
        pltpu.SMEM((1,), jnp.int32),
        pltpu.SemaphoreType.DMA((5,)),
    ]
    scratch += [pltpu.VMEM((N2, N1, 128), BF16)] * (2 * NT)
    scratch += [pltpu.VMEM((N1 // 8 + 1, 4, 4, 2, 8, 128), F32)] * (2 * NT)
    scratch += [pltpu.VMEM((N2, 2 * N1, 128), BF16)] * NT
    scratch += [pltpu.VMEM((N2, N1, 128), F32)] * NT
    scratch += [pltpu.VMEM((S // 2 + 32, 128), U32)] * NT
    scratch += [pltpu.VMEM((2, 512, 128), F32)] * NSLOT
    scratch += [
        pltpu.VMEM((KS, D), BF16),
        pltpu.VMEM((NT, 128), BF16),
        pltpu.VMEM((1, H), BF16),
    ]
    return pl.pallas_call(
        _kernel,
        out_shape=jax.ShapeDtypeStruct((1, S, 2 * D), BF16),
        in_specs=[hbm] * 14,
        out_specs=hbm,
        scratch_shapes=scratch,
        compiler_params=pltpu.CompilerParams(vmem_limit_bytes=110 * 1024 * 1024),
        name="h3_infini",
    )(A_q, A_k, A_v, A_shift_k.T, A_ssm_k, A_ssm_D.reshape(NT, 128), B_x, B_wq, B_wk, B_wv, B_wo,
      B_beta.reshape(1, H), _FWD, _INV)
```

```python
import math

import jax
import jax.numpy as jnp
import numpy as np
from jax import lax
from jax.experimental import pallas as pl
from jax.experimental.pallas import tpu as pltpu

S = 2048
D = 640
NT = D // 128
H = 32
DH = D // H
NSEG = 4
L = S // NSEG
KS = 4
N1, N2 = 128, 16

F32 = jnp.float32
BF16 = jnp.bfloat16
U32 = jnp.uint32
NN_DIMS = (((1,), (0,)), ((), ()))
NT_DIMS = (((1,), (1,)), ((), ()))
NEG = -1e30
LOG2E = 1.4426950408889634


def _pack_rows(a):
    u = a.astype(np.float32).astype(BF16).view(np.uint16).astype(np.uint32)
    return u[..., 0::2, :] | (u[..., 1::2, :] << 16)


def _dft_tables():
    k1 = np.arange(N1)
    fwd = np.zeros((N2, 2 * N1, N1), np.float64)
    inv = np.zeros((N2, N1, 2 * N1), np.float64)
    row_re = 16 * (k1 // 8) + k1 % 8
    for n2 in range(N2):
        ang = 2.0 * np.pi * np.outer(k1 + 0.25, N2 * np.arange(N1) + n2) / S
        fwd[n2, row_re] = np.cos(ang)
        fwd[n2, row_re + 8] = np.sin(ang)
        inv[n2] = fwd[n2].T / S
    inv = inv.reshape(N2, N1, 2, N1).transpose(0, 2, 1, 3)
    return _pack_rows(fwd), _pack_rows(inv)


_FWD, _INV = _dft_tables()


def _dot(a, b, dims=NN_DIMS):
    return lax.dot_general(a, b, dims, preferred_element_type=F32)


def _u32(x):
    return pltpu.bitcast(x, U32)


def _bf(x):
    return pltpu.bitcast(x, BF16)


def _u32_word(x):
    return lax.bitcast_convert_type(x, U32)


def _lo(w):
    return lax.bitcast_convert_type(w << 16, F32)


def _hi(w):
    return lax.bitcast_convert_type(w & np.uint32(0xFFFF0000), F32)


def _stack(a, b):
    return jnp.concatenate([a, b], axis=0).astype(BF16)


def _interleave(a, b):
    r = _stack(a, b).astype(F32)
    n = a.shape[0]
    return (_u32_word(r[:n]) >> 16) | _u32_word(r[n:])


def _radix4(x0, x1, x2, x3, sign):
    ar, ai = x0[0] + x2[0], x0[1] + x2[1]
    br, bi = x0[0] - x2[0], x0[1] - x2[1]
    cr, ci = x1[0] + x3[0], x1[1] + x3[1]
    dr, di = x1[0] - x3[0], x1[1] - x3[1]
    y0 = (ar + cr, ai + ci)
    y2 = (ar - cr, ai - ci)
    yp = (br - di, bi + dr)
    ym = (br + di, bi - dr)
    return (y0, yp, y2, ym) if sign > 0 else (y0, ym, y2, yp)


def _twiddle(x, e, sign):
    xr, xi = x
    if e == 0:
        return x
    r = math.sqrt(0.5)
    if e == 2:
        return ((xr - xi) * r, (xr + xi) * r) if sign > 0 else ((xr + xi) * r, (xi - xr) * r)
    if e == 6:
        return ((xr + xi) * -r, (xr - xi) * r) if sign > 0 else ((xi - xr) * r, (xr + xi) * -r)
    c, s = math.cos(math.pi * e / 8), sign * math.sin(math.pi * e / 8)
    return (xr * c - xi * s, xr * s + xi * c)


def _radix4_tw(x0, x1, x2, x3, sign, b):
    if b != 2:
        return _radix4(x0, _twiddle(x1, b, sign), _twiddle(x2, 2 * b, sign),
                       _twiddle(x3, 3 * b, sign), sign)
    x1, x3 = _twiddle(x1, 2, sign), _twiddle(x3, 6, sign)
    if sign > 0:
        ar, ai = x0[0] - x2[1], x0[1] + x2[0]
        br, bi = x0[0] + x2[1], x0[1] - x2[0]
    else:
        ar, ai = x0[0] + x2[1], x0[1] - x2[0]
        br, bi = x0[0] - x2[1], x0[1] + x2[0]
    cr, ci = x1[0] + x3[0], x1[1] + x3[1]
    dr, di = x1[0] - x3[0], x1[1] - x3[1]
    y0 = (ar + cr, ai + ci)
    y2 = (ar - cr, ai - ci)
    yp = (br - di, bi + dr)
    ym = (br + di, bi - dr)
    return (y0, yp, y2, ym) if sign > 0 else (y0, ym, y2, yp)


class _Paced:
    def __init__(self, streams, sequential=False):
        self.live = [[g, total, 0] for g, total in streams if total]
        self.total = sum(total for _, total in streams)
        self.done = 0
        self.sequential = sequential

    def step(self):
        cur = self.live[0] if self.sequential else min(self.live, key=lambda e: e[2] / e[1])
        cost = next(cur[0], None)
        if cost is None:
            self.live.remove(cur)
        else:
            cur[2] += cost
            self.done += cost

    def advance(self, fraction):
        while self.live and self.done < fraction * self.total:
            self.step()

    def finish(self):
        self.advance(math.inf)


SPLIT = ((0, 1, 2), (3, 4), (), ())
FORWARD = ((), (0, 1), (2, 3, 4), ())
SPECTRUM = ((), (), (0, 1), (2, 3))
INVERSE = ((), (), (), (0, 1))
W_STAGES = ((0, 1), (1, 2), (2, 5))
DEPTH = 3
NSLOT = 4
ORDER = ((1, 3, 0, 2), (1, 3, 0, 2), (0, 2, 1, 3), (0, 1, 2, 3))
TAIL = (-0.03, 0.02, -0.015, -0.03)
QCH = (128, 192, 192, 128)
HEAD = (8, 6, 6, 6)
FILL_ORDER = (0, 0, 1, 0)
SIDE_SPEED = (1.015, 1.0, 1.0, 1.0, 1.0)
AW = (4.0, 1.75, 1.75, 2.0, 3.0)
PACE_ON = (3, 3, 7, 7, 7)
PACE_ALL = (3, 3, 2, 2, 0)
SPEC_V = (0, 0, 0, 0, 1)
MID = 15


def _kernel(aq_hbm, ak_hbm, av_hbm, shift_hbm, h_hbm, ssmd_hbm, x_hbm, wq_hbm, wk_hbm,
            wv_hbm, wo_hbm, beta_hbm, fwd_hbm, inv_hbm, out_hbm,
            xb, wqb, wkb, wvb, wob, wvt, hb, ht, kb, vb, qb, fwd, inv,
            ub, outb, wtab, gtab, cmask,
            q0, q1, k0, k1, pq0, pq1, pk0, pk1, ots, mst,
            hmask, hsel, bmask, kwin, vall, vhead, opart, onat, zero_ref, sems, *rest):
    xp, hp, tx, th, yb, kvf, outa = (rest[NT * k:NT * k + NT] for k in range(7))
    slots = rest[7 * NT:7 * NT + NSLOT]
    shift_ref, ssmd_ref, beta_ref = rest[7 * NT + NSLOT:]
    qs, ks, pqs, pks = (q0, q1), (k0, k1), (pq0, pq1), (pk0, pk1)

    def copy(src, dst, sem):
        return [lambda: pltpu.make_async_copy(src, dst, sems.at[sem])]

    def tiles(src, dst, sem, r0, n, ts=range(NT), off=0):
        src = src.bitcast(U32)
        lead = (0,) * (len(src.shape) - 2)
        return [cp for t in ts for cp in copy(
            src.at[lead + (pl.ds(r0 // 2, n // 2), pl.ds(128 * t, 128))],
            dst.at[t, pl.ds(off + r0 // 2, n // 2), :], sem)]

    def conv_inputs(cs, r0, n, sem):
        return (tiles(h_hbm, hb, sem, 128 * cs[0], 128 * len(cs), range(r0 // 128, (r0 + n) // 128))
                + tiles(ak_hbm, kb, sem, r0, n, cs, off=32) + tiles(av_hbm, vb, sem, r0, n, cs))

    def w_stage(k, sem):
        return (tiles(wq_hbm, wqb, sem, 0, D, range(*W_STAGES[k]))
                + tiles(wk_hbm, wkb, sem, 0, D, range(*W_STAGES[k])))

    cp_first = w_stage(0, 0) + tiles(x_hbm, xb, 0, 0, 256)
    cp_x0 = tiles(x_hbm, xb, 1, 256, 256)
    cp_w1, cp_w2 = w_stage(1, 2), w_stage(2, 3)
    cp_wv = (tiles(wv_hbm, wvb, 0, 0, D) + copy(shift_hbm, shift_ref, 0)
             + copy(ssmd_hbm, ssmd_ref, 0) + copy(beta_hbm, beta_ref, 0))
    cp_step = [tiles(x_hbm, xb, sem, L + 128 * i, 128) + conv_inputs(SPLIT[0], L * i, L, sem)
               for i, sem in enumerate((4, 0, 1, 2))]
    cp_seg1 = (tiles(wo_hbm, wob, 3, 0, D) + tiles(x_hbm, xb, 3, 2 * L, L)
               + copy(fwd_hbm, fwd, 3) + conv_inputs(SPLIT[1], 0, S, 3))
    cp_seg2 = (tiles(x_hbm, xb, 4, 3 * L, L) + copy(inv_hbm, inv, 4)
               + tiles(aq_hbm, qb, 4, 0, S))
    cp_oa = [copy(outa[c].at[pl.ds(0, S // 2), :],
                  out_hbm.bitcast(U32).at[0, :, pl.ds(128 * c, 128)], 0) for c in range(NT)]

    def out_b(tile, n):
        at = pl.ds(128 * tile if isinstance(tile, int) else pl.multiple_of(128 * tile, 128), 128)
        return copy(outb.at[n, at, :], out_hbm.at[0, at, pl.ds(D + 128 * n, 128)], 1)

    all_of_b = copy(outb, outb, 1)

    def start(*groups):
        for g in groups:
            for cp in g:
                cp().start()

    def wait(*groups):
        for g in groups:
            for cp in g:
                cp().wait()

    def rows(i, n):
        return pl.ds(pl.multiple_of(i * n, n), n) if not isinstance(i, int) else pl.ds(i * n, n)

    lane = lax.broadcasted_iota(jnp.int32, (8, 128), 1)
    sub = lax.broadcasted_iota(jnp.int32, (8, 128), 0)

    def lanes(n):
        return lax.broadcasted_iota(jnp.int32, (n, 128), 1)

    recent = [None]
    seg = [0]

    def dot(a, b, dims=NN_DIMS, kind=4):
        out = _dot(a, b, dims)
        if kind & PACE_ON[seg[0]]:
            recent[0] = out
        return out

    current = {}

    def pace(zero):
        v = recent[0][-8:]
        recent[0] = None
        if "h" in current:
            hb[S // 128, rows(zero, 8), :] = _u32_word(v)
        if "k" in current:
            kb[NT, rows(zero, 8), :] = _u32_word(v)
        if "t" in current:
            th[current["t"]][N1 // 8, zero, 0, 0] = v
            if PACE_ALL[seg[0]] & 1:
                tx[current["t"]][N1 // 8, zero, 0, 0] = v
            if PACE_ALL[seg[0]] & 2:
                ub[16, zero, 0, 0] = v

    def qk_proj(s, i, want_pq, want_pk):
        p = s % 2
        tok = rows(4 * s + i, 64)
        for w_ref, dst, fdst, want, scale in (
                (wqb, qs[p], pqs[p], want_pq, DH ** -0.5 * LOG2E),
                (wkb, ks[p], pks[p], want_pk, None)):
            for n in range(NT):
                t = None
                for c in range(NT):
                    part = dot(_bf(xb[c, tok, :]), _bf(w_ref[n, 64 * c:64 * c + 64, :]))
                    t = part if t is None else t + part
                    if c < NT - 1:
                        yield 32
                dst[n, rows(i, 128), :] = (t if scale is None else t * scale).astype(BF16)
                if want:
                    fdst[n, rows(i, 128), :] = jnp.where(t > 0, t + 1.0, jnp.exp(t)).astype(BF16)
                yield 32

    def first_proj(n, js=range(4)):
        for w_ref, dst, scale in ((wkb, ks[0], None), (wqb, qs[0], DH ** -0.5 * LOG2E)):
            for j in js:
                t = None
                for c in range(NT):
                    part = dot(_bf(xb[c, rows(j, 64), :]), _bf(w_ref[n, 64 * c:64 * c + 64, :]))
                    t = part if t is None else t + part
                dst[n, rows(j, 128), :] = (t if scale is None else t * scale).astype(BF16)
                if scale is None:
                    pks[0][n, rows(j, 128), :] = jnp.where(t > 0, t + 1.0, jnp.exp(t)).astype(BF16)

    untransposed = set()

    def untranspose(s, i, slot=0):
        ot = ots.bitcast(U32)
        for c in range(NT):
            onat[slot, c] = _u32(_bf(ot[s % 2, i, 64 * c:64 * c + 64, :]).T)
        untransposed.add((s, slot))

    def out_proj(s, i, slot=0):
        assert (s, slot) in untransposed
        for n in range(NT):
            t = None
            for c in range(NT):
                part = dot(_bf(onat[slot, c]), _bf(wob[n, 64 * c:64 * c + 64, :]))
                t = part if t is None else t + part
                if c < NT - 1:
                    yield 32
            outb[n, rows(4 * s + i, 128), :] = t.astype(BF16)
            start(out_b(4 * s + i, n))
            yield 32

    def tile_rows(r, n):
        return jnp.broadcast_to(r[None], (n // 8, 8, 128)).reshape(n, 128)

    carrying = [False]

    class Group:
        def __init__(self, s, g, gi):
            self.s, self.g, self.gi = s, g, gi
            self.t0 = (80 * g) // 128
            self.off = 80 * g - 128 * self.t0
            self.t1 = jnp.minimum(self.t0 + 1, NT - 1)
            rel = (lane - self.off) & 127
            head = sum((rel >= a * DH).astype(jnp.int32) for a in range(1, 5))
            for a in range(4):
                hmask[gi, a] = jnp.where(head == a, np.uint32(0xFFFFFFFF), np.uint32(0))
            hsel[gi] = jnp.left_shift(1, head)
            self.have_keys, self.have_mem = set(), set()

        def window(self, ref, j, r0=0, n=64):
            ref = ref.bitcast(U32)
            at = pl.ds(64 * j + r0, n)
            return jnp.where(lanes(n) >= self.off, ref[self.t0, at, :], ref[self.t1, at, :])

        def keys(self, r0, r1):
            out = []
            for r in range(r0, r1, 64):
                at = pl.ds(r // 2, 32)
                if r in self.have_keys:
                    out.append(kwin[self.gi, at, :])
                else:
                    self.have_keys.add(r)
                    out.append(self.window(ks[self.s % 2], 0, r // 2, 32))
                    kwin[self.gi, at, :] = out[-1]
            return _bf(jnp.concatenate(out, axis=0))

        def park_values(self, j, v80):
            assert not carrying[0]
            if self.s < NSEG - 1:
                vall[self.gi, j, 0:80, :] = v80
            ones8 = jnp.ones((8, 128), F32)
            for pr in range(2):
                for e in range(2):
                    r0 = 40 * pr + 16 * e
                    vhead[self.gi, j, r0 // 8] = jnp.concatenate(
                        [v80[r0:r0 + 24], ones8], axis=0).astype(BF16)

        def mem_read(self):
            for j in range(4):
                assert not (carrying[0] and self.gi == 1)
                r = dot(mst[self.g, 0:88, :], _bf(self.window(pqs[self.s % 2], j)), NT_DIMS)
                coef = gtab[self.g, 0] / (r[80:88] + 1e-6)
                cb = [jnp.broadcast_to(coef[a:a + 1], (8, 128)) for a in range(4)]
                for pr in range(2):
                    ca, cc = cb[2 * pr], cb[2 * pr + 1]
                    for e, scale in enumerate((ca, ca, jnp.where(sub < 4, ca, cc), cc, cc)):
                        r0 = 40 * pr + 8 * e
                        opart[self.gi, j, r0:r0 + 8, :] = r[r0:r0 + 8] * scale
                self.have_mem.add(j)
                yield 24

        def mem_update(self):
            acc = None
            for j in range(4):
                t = dot(vall[self.gi, j], _bf(self.window(pks[self.s % 2], j)))
                acc = t if acc is None else acc + t
                if j < 3:
                    yield 24
            for r in range(11):
                new = jnp.where(bmask[r] & hsel[self.gi] != 0, acc[8 * r:8 * r + 8], 0.0)
                at = pl.ds(8 * r, 8)
                mst[self.g, at, :] = new if self.s == 0 else mst[self.g, at, :] + new
            yield 24

        def logits(self, pr, j, slot):
            qw = self.window(qs[self.s % 2], j)
            qa = qw & tile_rows(hmask[self.gi, 2 * pr], 64)
            qh = qw & tile_rows(hmask[self.gi, 2 * pr + 1], 64)
            w_a = _bf(qa)
            w_b = _bf(jnp.concatenate([qh[32:64], qh[0:32]], axis=0))
            w_t = _bf(jnp.concatenate([qh[32:64], qa[32:64]], axis=0))
            n = 128 * j

            def park(t, e, r0, m):
                for r in range(0, t.shape[0], 8):
                    v = t[r:r + 8]
                    if e == 2:
                        v = v + cmask[2, r:r + 8, :]
                    elif r0 + r >= n:
                        v = v + cmask[e, r0 + r - n:r0 + r - n + 8, :]
                    slot[e % 2, 448 * (e // 2) + r0 + r:448 * (e // 2) + r0 + r + 8, :] = v
                    m = v if m is None else jnp.maximum(m, v)
                return m

            m_t = park(dot(self.keys(n + 64, n + 128), w_t, NT_DIMS, 1), 2, 0, None)
            yield 16
            cuts = list(range(0, n, QCH[seg[0]])) or [0]
            m = [None, None]
            for r0, r1 in zip(cuts, cuts[1:] + [n + 64]):
                for e, w in enumerate((w_a, w_b)):
                    m[e] = park(dot(self.keys(r0, r1), w, NT_DIMS, 1), e, r0, m[e])
                    if r1 == n + 64 and e == 1:
                        m_a = jnp.maximum(m[0], jnp.where(lane >= 64, m_t, NEG))
                        m_b = jnp.maximum(m[1], jnp.where(lane < 64, m_t, NEG))
                        m_a = jnp.broadcast_to(jnp.max(m_a, axis=0, keepdims=True), (8, 128))
                        m_b = jnp.broadcast_to(jnp.max(m_b, axis=0, keepdims=True), (8, 128))
                        slot[1, 448:456, :] = m_a
                        slot[1, 456:464, :] = m_b
                        slot[1, 464:472, :] = jnp.where(lane < 64, m_b, m_a)
                    yield (r1 - r0) // 4

    def attend(gi, g, parity, add_mem, pr, j, slot, need_values):
        def prob(e, r0, n, which):
            m2 = tile_rows(slot[1, 448 + 8 * which:456 + 8 * which, :], 16)
            return [jnp.exp2(slot[e, r:r + 16, :] - m2) for r in range(r0, r0 + n, 16)]

        res = [None, None]
        order = [(0, j), (1, j)] + [(e, kt) for e in range(2) for kt in range(j)]
        for n, (e, kt) in enumerate(order):
            need_values(kt)
            if n == 0:
                p_t = prob(0, 448, 64, 2)
            if kt < j:
                p = prob(e, 128 * kt, 128, e)
            else:
                mine = lanes(16) >= 64 if e == 0 else lanes(16) < 64
                p = prob(e, 128 * kt, 64, e) + [jnp.where(mine, t, 0.0) for t in p_t]
            t = dot(_bf(vhead.bitcast(U32)[gi, kt, 5 * pr + 2 * e]),
                    jnp.concatenate(p, axis=0).astype(BF16), kind=2)
            res[e] = t if res[e] is None else res[e] + t
            if n < len(order) - 1:
                yield 8 * AW[seg[0]]
        r_a = res[0]
        r_b = pltpu.roll(res[1], 64, 1)
        keep = 1.0 - gtab[g, 0]
        keep_a = jnp.broadcast_to(keep[2 * pr:2 * pr + 1], (8, 128))
        keep_b = jnp.broadcast_to(keep[2 * pr + 1:2 * pr + 2], (8, 128))
        o_a = r_a[0:24] * tile_rows(keep_a / r_a[24:32], 24)
        o_b = r_b[0:24] * tile_rows(keep_b / r_b[24:32], 24)
        o = jnp.concatenate(
            [o_a[0:16], jnp.where(sub < 4, o_a[16:24], o_b[0:8]), o_b[8:24]], axis=0)
        if add_mem:
            o = o + opart[gi, j, 40 * pr:40 * pr + 40, :]
        if pr == 0:
            opart[gi, j, 0:40, :] = o
        else:
            o = jnp.concatenate([opart[gi, j, 0:40, :], o], axis=0)
            ots[parity, j, rows(g, 80), :] = o.astype(BF16)
        yield 8 * AW[seg[0]]

    def v_proj(s, i, groups, have):
        for j in range(4):
            acc = None
            for c in range(NT):
                t = dot(_bf(wvt[c, i, 0:80, :]), _bf(xb[c, rows(4 * s + j, 64), :]), NT_DIMS)
                acc = t if acc is None else acc + t
                if c == NT - 1:
                    for gi in range(2):
                        groups[gi].park_values(j, acc[80 * gi:80 * gi + 80])
                    have.append(j)
                yield 40

    def chain(*gens):
        for g in gens:
            yield from g

    def units(s):
        return [(gi, pr, j) for gi in range(2) for pr in range(2)
                for j in (range(4) if (gi, pr) == (1, 1) else ORDER[s] if gi + pr else range(4))]

    def cost(j):
        return 48 + 64 * j, (16 + 16 * j) * AW[seg[0]]

    def carried(u, g, parity):
        gi, pr, j = units(0)[u]
        return attend(gi, g, parity, True, pr, j, slots[u % NSLOT], lambda kt: None), cost(j)[1]

    def segment_step(s, i):
        seg[0] = s
        parts = {}
        if s < NSEG - 1:
            parts["qk"] = (qk_proj(s + 1, i, True, s + 1 < NSEG - 1), 1600)
        if s > 0:
            parts["out"] = (out_proj(s - 1, i), 800)
        if FORWARD[s]:
            parts["fwd"] = (fwd_fft(i, FORWARD[s]), 512 * len(FORWARD[s]))
        if INVERSE[s]:
            parts["inv"] = (inverse(INVERSE[s], (2 * i, 2 * i + 1)), 256 * len(INVERSE[s]))
        names = (("qk", "inv", "out", "fwd"), ("qk", "inv", "fwd", "out"),
                 ("inv", "fwd", "qk", "out"))[FILL_ORDER[s]]
        fill = _Paced([parts[n] for n in names if n in parts], sequential=True)
        side = []
        if SPECTRUM[s]:
            side.append((spectra(SPECTRUM[s], [4 * i + a for a in range(4)]),
                         4 * SPEC_COST * len(SPECTRUM[s])))
        for c in SPLIT[s]:
            side += [(split_h(i, c), 144), (split_kv(i, c), 704)]
        side = _Paced(side, sequential=True)
        current.clear()
        recent[0] = None
        for _ in range(HEAD[s]):
            fill.step()
        if s > 0:
            untranspose(s - 1, i)
        vt = []
        groups = [Group(s, 2 * i + gi, gi) for gi in range(2)]
        reads = [grp.mem_read() for grp in groups if s > 0]
        updates = [grp.mem_update() for grp in groups if s < NSEG - 1]
        first = _Paced([(chain(*reads[:1], v_proj(s, i, groups, vt), *reads[1:], *updates),
                         800 + 96 * (len(reads) + len(updates)))])
        total = first.total + fill.total
        held = 96 * (s > 0) + 159

        def need_values(kt):
            while len(vt) <= kt:
                first.step()

        def pad(fraction, u):
            target = total * fraction / (1 + TAIL[s])
            early = min(target, held if u < DEPTH else first.total)
            first.advance(early / first.total)
            fill.advance((target - early) / fill.total)
            goal = fraction * SIDE_SPEED[s]
            if side.live and side.done < goal * side.total and recent[0] is not None:
                pace(jnp.minimum(i, 3))
                side.advance(goal)

        todo = units(s)
        whole = sum(sum(cost(j)) for _, _, j in todo)
        done = 0
        for u, (gi, pr, j) in enumerate(todo):
            carrying[0] = u < DEPTH
            streams = [(groups[gi].logits(pr, j, slots[u % NSLOT]), cost(j)[0])]
            v = u - DEPTH
            if v < 0:
                streams.append(carried(v + len(todo), (2 * i + 7) & 7,
                                       jnp.where(i > 0, s % 2, 1 - s % 2)))
            else:
                gi, pr, j = todo[v]
                while s > 0 and j not in groups[gi].have_mem:
                    first.step()
                streams.append((attend(gi, 2 * i + gi, s % 2, s > 0, pr, j, slots[v % NSLOT],
                                       need_values), cost(j)[1]))
            att = _Paced(streams[::-1], sequential=u == len(todo) - 1)
            while att.live:
                att.step()
                pad((done + att.done) / whole, u)
            done += att.total
        first.finish()
        fill.finish()
        side.finish()

    def split_h(i, c):
        current.clear()
        current["h"] = True
        for t in range(4):
            ht[c, 64 * t:64 * t + 64, :] = _u32(
                _bf(hb[4 * i + t, 64 * c:64 * c + 64, :]).T)
            yield 4
        for q in range(2):
            for j in range(8):
                wa = ht[c, pl.ds(128 * q + j, 8, stride=8), :]
                wb = ht[c, pl.ds(128 * q + 64 + j, 8, stride=8), :]
                hp[c][2 * j, rows(2 * i + q, 16), :] = _stack(_lo(wa), _lo(wb))
                hp[c][2 * j + 1, rows(2 * i + q, 16), :] = _stack(_hi(wa), _hi(wb))
                if j % 2:
                    yield 16

    def split_kv(i, c):
        current.clear()
        current["k"] = True
        taps = [wtab[c, j] for j in range(KS)]
        for q in range(2):
            blk = 2 * i + q
            base = [blk * 128 + 64 * e for e in range(2)]
            hist = []
            for e in range(2):
                w2 = kb[c, pl.ds(base[e] + 30, 8, stride=8), :]
                w1 = kb[c, pl.ds(base[e] + 31, 8, stride=8), :]
                hist.append([_hi(w2), _lo(w1), _hi(w1)])
            for j in range(8):
                kv = [[None, None], [None, None]]
                for e in range(2):
                    kw = kb[c, pl.ds(base[e] + 32 + j, 8, stride=8), :]
                    vw = vb[c, pl.ds(base[e] + j, 8, stride=8), :]
                    kp = hist[e] + [_lo(kw), _hi(kw)]
                    for half, part in enumerate((_lo, _hi)):
                        acc = kp[3 + half] * taps[0]
                        for d in range(1, KS):
                            acc = acc + kp[3 + half - d] * taps[d]
                        kv[half][e] = acc * part(vw)
                        kvf[c][2 * j + half, rows(2 * blk + e, 8), :] = kv[half][e]
                    hist[e] = kp[2:]
                    if e == 0:
                        yield 22
                for half in range(2):
                    xp[c][2 * j + half, rows(blk, 16), :] = _stack(*kv[half])
                yield 22

    def fwd_fft(i, cs):
        for c in cs:
            for src, dst in ((hp[c], th[c]), (xp[c], tx[c])):
                g = [dot(_bf(fwd[4 * a + i]), _bf(src.bitcast(U32)[4 * a + i])) for a in range(4)]
                for r in range(0, 2 * N1, 16):
                    z = _radix4(*[(g[a][r:r + 8], g[a][r + 8:r + 16]) for a in range(4)], 1)
                    for cc in range(4):
                        dst[r // 16, i, cc, 0] = z[cc][0]
                        dst[r // 16, i, cc, 1] = z[cc][1]
                yield 256

    def spectrum(c, m, slot):
        current.clear()
        current["t"] = c
        for cc in range(4):
            zh = _radix4_tw(*[(th[c][m, b, cc, 0], th[c][m, b, cc, 1]) for b in range(4)], 1, cc)
            yield 17
            zx = _radix4_tw(*[(tx[c][m, b, cc, 0], tx[c][m, b, cc, 1]) for b in range(4)], 1, cc)
            yield 17
            y = [(x[0] * h[0] - x[1] * h[1], x[0] * h[1] + x[1] * h[0]) for x, h in zip(zx, zh)]
            yield 17
            u = _radix4(*y, -1)
            for b in range(4):
                ub[slot, b, cc, 0] = u[b][0]
                ub[slot, b, cc, 1] = u[b][1]
            yield 17
        if SPEC_V[seg[0]]:
            return

        yield from spectrum_end(c, m, slot)

    def spectrum_end(c, m, slot):
        for b in range(4):
            z = _radix4_tw(*[(ub[slot, b, cc, 0], ub[slot, b, cc, 1]) for cc in range(4)], -1, b)
            for a in range(4):
                yb[c][4 * a + b, rows(m, 16), :] = _stack(*z[a])
            yield 17

    SPEC_COST = 17 * 20

    def spectra(cs, ms):
        prev = None
        for slot, (c, m) in enumerate((c, m) for c in cs for m in ms):
            yield from spectrum(c, m, slot)
            if SPEC_V[seg[0]] and prev is not None:
                yield from spectrum_end(*prev)
            prev = (c, m, slot)
        if SPEC_V[seg[0]]:
            yield from spectrum_end(*prev)

    def inverse(cs, jps):
        for c in cs:
            for jp in jps:
                w = qb[c, pl.ds(jp, N1, stride=8), :]
                res = []
                for e, part in enumerate((_lo, _hi)):
                    n2 = 2 * jp + e
                    y = dot(_bf(inv[n2, 0]), _bf(yb[c].bitcast(U32)[n2, 0:64, :]))
                    yield 32
                    y = y + dot(_bf(inv[n2, 1]), _bf(yb[c].bitcast(U32)[n2, 64:128, :]))
                    res.append(part(w) * (y + kvf[c][n2] * tile_rows(wtab[c, KS], N1)))
                    if e == 0:
                        yield 32
                outa[c][pl.ds(jp, N1, stride=8), :] = _interleave(*res)
                yield 32

    start(cp_first, cp_x0, cp_w1)
    zero_ref[0] = 0
    kk = lax.broadcasted_iota(jnp.int32, (64, 128), 0)
    ll = lax.broadcasted_iota(jnp.int32, (64, 128), 1)
    cmask[0] = jnp.where(kk <= ll, 0.0, NEG)
    cmask[1] = jnp.where((ll < 64) | (kk <= ll - 64), 0.0, NEG)
    cmask[2] = jnp.where(kk <= (ll & 63), 0.0, NEG)
    for r in range(11):
        row = sub + 8 * r
        hr = sum((row >= a * DH).astype(jnp.int32) for a in range(1, 4)) if r < 10 else row - 80
        bmask[r] = jnp.left_shift(1, hr)
    for gi in range(2):
        for j in range(4):
            vall[gi, j, 80:88, :] = jnp.ones((8, 128), F32)
    for c in range(NT):
        kb[c, 24:32, :] = jnp.zeros((8, 128), U32)
    for u in range(16 - DEPTH, 16):
        slots[u % NSLOT][...] = jnp.zeros((2, 512, 128), F32)
    vhead[1] = jnp.ones(vhead.shape[1:], BF16)
    opart[1] = jnp.zeros(opart.shape[1:], F32)
    wait(cp_first)
    start(cp_w2, cp_wv, cp_step[0])
    first_proj(0, (0, 1))
    wait(cp_x0)
    first_proj(0, (2, 3))
    wait(cp_w1)
    for n in range(*W_STAGES[1]):
        first_proj(n)
    wait(cp_w2)
    for n in range(W_STAGES[2][0], NT - 1):
        first_proj(n)
    wait(cp_wv)
    start(cp_step[1])
    taps_t = shift_ref[...].astype(F32)
    skip = ssmd_ref[...].astype(F32)
    for c in range(NT):
        for j in range(KS):
            wtab[c, j] = jnp.broadcast_to(taps_t[j:j + 1, 128 * c:128 * c + 128], (8, 128))
        wtab[c, KS] = jnp.broadcast_to(skip[c:c + 1], (8, 128))
    gates = jax.nn.sigmoid(beta_ref[...].astype(F32))
    gcol = jnp.broadcast_to(gates, (8, H)).T
    gcol = jnp.broadcast_to(gcol[:, 0:1], (H, 128))
    for g in range(8):
        gtab[g, 0] = jnp.concatenate([gcol[4 * g:4 * g + 4]] * 2, axis=0)
    for n in range(NT):
        for c in range(NT):
            wt = _u32(_bf(wvb[n, 64 * c:64 * c + 64, :]).T)
            for r in range(0, 64, 16):
                step, r0 = divmod(64 * n + r, 80)
                wvt[c, step, r0:r0 + 16, :] = wt[r:r + 16]
    first_proj(NT - 1)

    def segment(s):
        def body(i, carry):
            if s == 0:
                for j in range(4):
                    @pl.when(i == j)
                    def _():
                        wait(cp_step[j])
                        start(*((cp_step[2],), (cp_step[3],), (cp_seg1,), (cp_seg2,))[j])
            segment_step(s, i)
            return carry

        lax.fori_loop(0, 4, body, 0)

    segment(0)
    wait(cp_seg1)
    segment(1)
    wait(cp_seg2)
    segment(2)
    segment(3)
    start(*[cp_oa[c] for c in INVERSE[3]])
    seg[0] = 4
    current.clear()
    recent[0] = None
    last = NT - 1
    rest_tiles = [c for c in range(last) if c not in INVERSE[3]]
    side = _Paced([(spectra((last,), range(16)), 16 * SPEC_COST)])
    span = (1024 * len(rest_tiles) + 160 * MID) / SIDE_SPEED[4]
    done = 0

    def run(streams):
        nonlocal done
        work = _Paced(streams)
        while work.live:
            before = work.done
            work.step()
            done += work.done - before
            if side.live and side.done < done / span * side.total and recent[0] is not None:
                pace(zero_ref[0])
                side.advance(done / span)

    for c in rest_tiles:
        streams = [(inverse((c,), range(8)), 1024)]
        if c == rest_tiles[0]:
            tail = [carried(u, 7, 1) for u in range(16 - DEPTH, 16)]
            streams.append((chain(*[g for g, _ in tail]), sum(w for _, w in tail)))
        run(streams)
        if c == rest_tiles[0]:
            for i in range(4):
                untranspose(3, i, i)
        start(cp_oa[c])
    proj = _Paced([(chain(*[out_proj(3, i, i) for i in range(4)]), 3200)])

    def part(cost):
        goal = proj.done + cost
        while proj.live and proj.done < goal:
            before = proj.done
            proj.step()
            yield proj.done - before

    run([(part(160 * MID), 160 * MID)])
    side.finish()
    run([(inverse((last,), range(8)), 1024)])
    start(cp_oa[last])
    proj.finish()
    wait(*cp_oa, all_of_b)


@jax.jit
def pallas_concat_heads__ssm_conv_h3__memory_aug_infini_attn__prompt_kernel(
    A_q: jax.Array,
    A_k: jax.Array,
    A_v: jax.Array,
    A_shift_k: jax.Array,
    A_ssm_k: jax.Array,
    A_ssm_D: jax.Array,
    B_x: jax.Array,
    B_wq: jax.Array,
    B_wk: jax.Array,
    B_wv: jax.Array,
    B_wo: jax.Array,
    B_beta: jax.Array,
):
    hbm = pl.BlockSpec(memory_space=pltpu.HBM)
    seg_tiles = pltpu.VMEM((NT, L, 128), BF16)
    weight = pltpu.VMEM((NT, D // 2, 128), U32)
    scratch = [
        pltpu.VMEM((NT, S // 2, 128), U32),
        weight, weight, weight, weight,
        pltpu.VMEM((NT, 4, 96, 128), U32),
        pltpu.VMEM((S // 128 + 1, D // 2, 128), U32),
        pltpu.VMEM((NT, 256 + 32, 128), U32),
        pltpu.VMEM((NT + 1, S // 2 + 64, 128), U32),
        pltpu.VMEM((NT, S // 2 + 32, 128), U32),
        pltpu.VMEM((NT, S // 2 + 32, 128), U32),
        pltpu.VMEM((N2, N1, 128), U32),
        pltpu.VMEM((N2, 2, N1 // 2, 128), U32),
        pltpu.VMEM((17, 4, 4, 2, 8, 128), F32),
        pltpu.VMEM((NT, S, 128), BF16),
        pltpu.VMEM((NT, 8, 8, 128), F32),
        pltpu.VMEM((8, 4, 8, 128), F32),
        pltpu.VMEM((3, 64, 128), F32),
        seg_tiles, seg_tiles, seg_tiles, seg_tiles,
        seg_tiles, seg_tiles, seg_tiles, seg_tiles,
        pltpu.VMEM((2, 4, D, 128), BF16),
        pltpu.VMEM((8, 96, 128), F32),
        pltpu.VMEM((2, 4, 8, 128), U32),
        pltpu.VMEM((4, 8, 128), jnp.int32),
        pltpu.VMEM((12, 8, 128), jnp.int32),
        pltpu.VMEM((2, L // 2, 128), U32),
        pltpu.VMEM((2, 4, 88, 128), F32),
        pltpu.VMEM((2, 4, 8, 32, 128), BF16),
        pltpu.VMEM((2, 4, 80, 128), F32),
        pltpu.VMEM((4, NT, 64, 128), U32),
        pltpu.SMEM((1,), jnp.int32),
        pltpu.SemaphoreType.DMA((5,)),
    ]
    scratch += [pltpu.VMEM((N2, N1, 128), BF16)] * (2 * NT)
    scratch += [pltpu.VMEM((N1 // 8 + 1, 4, 4, 2, 8, 128), F32)] * (2 * NT)
    scratch += [pltpu.VMEM((N2, 2 * N1, 128), BF16)] * NT
    scratch += [pltpu.VMEM((N2, N1, 128), F32)] * NT
    scratch += [pltpu.VMEM((S // 2 + 32, 128), U32)] * NT
    scratch += [pltpu.VMEM((2, 512, 128), F32)] * NSLOT
    scratch += [
        pltpu.VMEM((KS, D), BF16),
        pltpu.VMEM((NT, 128), BF16),
        pltpu.VMEM((1, H), BF16),
    ]
    return pl.pallas_call(
        _kernel,
        out_shape=jax.ShapeDtypeStruct((1, S, 2 * D), BF16),
        in_specs=[hbm] * 14,
        out_specs=hbm,
        scratch_shapes=scratch,
        compiler_params=pltpu.CompilerParams(vmem_limit_bytes=110 * 1024 * 1024),
        name="h3_infini",
    )(A_q, A_k, A_v, A_shift_k.T, A_ssm_k, A_ssm_D.reshape(NT, 128), B_x, B_wq, B_wk, B_wv, B_wo,
      B_beta.reshape(1, H), _FWD, _INV)
```
